```python
import jax
import jax.numpy as jnp

def _softmax(x, axis=-1):
    return jax.nn.softmax(x, axis=axis)
def _gelu(x):
    return jax.nn.gelu(x, approximate=True)
def _silu(x):
    return jax.nn.silu(x)
def _sigmoid(x):
    return jax.nn.sigmoid(x)
def _layernorm(x, axis=-1, eps=1e-5):
    m = jnp.mean(x, axis=axis, keepdims=True)
    v = jnp.var(x, axis=axis, keepdims=True)
    return (x - m) / jnp.sqrt(v + eps)
def _scatter_add(tgt, idx, src, axis=0):
    return tgt.at[idx].add(src)
def _segment_sum(src, seg, n):
    return jax.ops.segment_sum(src, seg, n)
class _Rng:
    def __init__(self, key):
        self._k = key
    def _next(self):
        self._k, sub = jax.random.split(self._k)
        return sub
    def normal(self, shape):
        return jax.random.normal(self._next(), shape, dtype=jnp.bfloat16)
    def randint(self, lo, hi, shape):
        return jax.random.randint(self._next(), shape, lo, hi, dtype=jnp.int32)
    def uniform(self, shape, lo=0.0, hi=1.0):
        return jax.random.uniform(self._next(), shape, jnp.bfloat16, lo, hi)
    def permutation(self, n):
        return jax.random.permutation(self._next(), n)


kernel_name = 'concat_heads__sliding_local_dilated__compressed_kv_cla__prompt'

def setup_inputs():
    _rng = _Rng(jax.random.key(int.from_bytes(__import__("os").urandom(4), "little")))
    _w = (lambda a: (lambda t: t.astype(jnp.bfloat16) if jnp.issubdtype(t.dtype, jnp.floating) else t)(jnp.asarray(a)))
    def _A_setup():
        B, S, D = 1, 2048, 1024
        return {
            "x": _w((lambda *s: _rng.normal(s) * 0.05)(B, S, D)),
            "wqkv": _w((lambda *s: _rng.normal(s) * 0.05)(D, 3 * D)),
            "wo": _w((lambda *s: _rng.normal(s) * 0.05)(D, D)),
        }
    _A_in = _A_setup()

    def _B_setup():
        B, H, Sq, Sk, D, M = 1, 32, 2048, 2048, 128, 1024
        Dc = 4 * D
        return {
            "x": _w((lambda *s: _rng.normal(s) * 0.05)(B, Sq, M)),
            "c_kv": _w((lambda *s: _rng.normal(s) * 0.05)(B, Sk, Dc)),
            "w_q": _w((lambda *s: _rng.normal(s) * 0.05)(M, H, D) * (M ** -0.5)),
            "w_uk": _w((lambda *s: _rng.normal(s) * 0.05)(Dc, H, D) * (Dc ** -0.5)),
            "w_uv": _w((lambda *s: _rng.normal(s) * 0.05)(Dc, H, D) * (Dc ** -0.5)),
            "w_o": _w((lambda *s: _rng.normal(s) * 0.05)(H, D, M) * ((H * D) ** -0.5)),
        }
    _B_in = _B_setup()

    return {
        "A_x": _A_in["x"],
        "A_wqkv": _A_in["wqkv"],
        "A_wo": _A_in["wo"],
        "B_x": _B_in["x"],
        "B_c_kv": _B_in["c_kv"],
        "B_w_q": _B_in["w_q"],
        "B_w_uk": _B_in["w_uk"],
        "B_w_uv": _B_in["w_uv"],
        "B_w_o": _B_in["w_o"],
    }

def reference(A_x, A_wqkv, A_wo, B_x, B_c_kv, B_w_q, B_w_uk, B_w_uv, B_w_o):
    def _A_ref(x, wqkv, wo):
        B, S, D = x.shape
        H = 32; Dh = D // H
        W, dil = 8, 2
        qkv = (lambda x, *d: x.transpose(*d))((x @ wqkv).reshape(B, S, 3, H, Dh), 2, 0, 3, 1, 4)
        q, k, v = qkv[0], qkv[1], qkv[2]
        scale = Dh ** -0.5
        pos = jnp.arange(S)
        off = jnp.arange(W) * dil
        idx = pos[:, None] - off[None, :]
        mask = idx >= 0
        idx_c = jnp.where(mask, idx, 0).reshape(-1)
        kg = k[:, :, idx_c, :].reshape(B, H, S, W, Dh)
        vg = v[:, :, idx_c, :].reshape(B, H, S, W, Dh)
        logits = jnp.einsum("bhsd,bhswd->bhsw", q, kg) * scale
        logits = jnp.where(mask[None, None, :, :], logits, -1e9)
        attn = _softmax(logits, axis=-1)
        o = jnp.einsum("bhsw,bhswd->bhsd", attn, vg)
        return (lambda x, *d: x.transpose(*d))(o, 0, 2, 1, 3).reshape(B, S, D) @ wo

    def _B_ref(x, c_kv, w_q, w_uk, w_uv, w_o):
        B, Sq, M = x.shape[0], x.shape[1], x.shape[2]
        Sk = c_kv.shape[1]
        H, D = w_q.shape[1], w_q.shape[2]
        q = jnp.einsum("bqm,mhd->bhqd", x, w_q)
        k = jnp.einsum("bkc,chd->bhkd", c_kv, w_uk)
        v = jnp.einsum("bkc,chd->bhkd", c_kv, w_uv)
        scores = jnp.einsum("bhqd,bhkd->bhqk", q, k) * (D ** -0.5)
        off = Sk - Sq
        qi = jnp.arange(Sq)[:, None]
        kj = jnp.arange(Sk)[None, :]
        cmask = kj <= (qi + off)
        scores = jnp.where(cmask[None, None], scores, -1e9)
        p = _softmax(scores, axis=-1)
        ctx = jnp.einsum("bhqk,bhkd->bhqd", p, v)
        return jnp.einsum("bhqd,hdm->bqm", ctx, w_o)

    a = _A_ref(A_x, A_wqkv, A_wo)
    b = _B_ref(B_x, B_c_kv, B_w_q, B_w_uk, B_w_uv, B_w_o)
    return jnp.concatenate([a, b], axis=-1)
```

```python
import functools
import math

import jax
import jax.numpy as jnp
from jax import lax
import jax.experimental.pallas as pl
import jax.experimental.pallas.tpu as pltpu

F32 = jnp.float32
BF16 = jnp.bfloat16
U32 = jnp.uint32
I32 = jnp.int32
LANES = 128
NT_DIMS = (((1,), (1,)), ((), ()))
LOG2E = math.log2(math.e)
MASKED = -1e9

S = 2048
DA = 1024
HA, DHA = 32, 32
WIN, DIL = 8, 2
HALO = 32
MB = 1024
HB, DB = 32, 128
DC = 512


def _quad(x):
    h = len(x) // 2
    return ([r[:h] for r in x[:h]], [r[h:] for r in x[:h]],
            [r[:h] for r in x[h:]], [r[h:] for r in x[h:]])


def _add(x, y):
    return [[a + b for a, b in zip(rx, ry)] for rx, ry in zip(x, y)]


def _sub(x, y):
    return [[a - b for a, b in zip(rx, ry)] for rx, ry in zip(x, y)]


def s_lhs(a):
    if len(a) == 1:
        return [a[0][0]]
    a11, a12, a21, a22 = _quad(a)
    parts = [_add(a11, a22), _add(a21, a22), a11, a22, _add(a11, a12), _sub(a21, a11), _sub(a12, a22)]
    return [z for p in parts for z in s_lhs(p)]


def s_rhs(b):
    if len(b) == 1:
        return [b[0][0]]
    b11, b12, b21, b22 = _quad(b)
    parts = [_add(b11, b22), b11, _sub(b12, b22), _sub(b21, b11), b22, _add(b11, b12), _add(b21, b22)]
    return [z for p in parts for z in s_rhs(p)]


LHS_TERMS = (((1, 0, 0), (1, 1, 1)), ((1, 1, 0), (1, 1, 1)), ((1, 0, 0),), ((1, 1, 1),),
             ((1, 0, 0), (1, 0, 1)), ((1, 1, 0), (-1, 0, 0)), ((1, 0, 1), (-1, 1, 1)))
RHS_TERMS = (((1, 0, 0), (1, 1, 1)), ((1, 0, 0),), ((1, 0, 1), (-1, 1, 1)), ((1, 1, 0), (-1, 0, 0)),
             ((1, 1, 1),), ((1, 0, 0), (1, 0, 1)), ((1, 1, 0), (1, 1, 1)))


def s_mul(prod, level, emit, base=0):
    if level == 0:
        emit(0, 0, prod(base))
        yield
        return
    n = 2 ** (level - 1)
    step = 7 ** (level - 1)

    def m(i):
        out = [[None] * n for _ in range(n)]

        def keep(a, b, v):
            out[a][b] = v

        yield from s_mul(prod, level - 1, keep, base + (i - 1) * step)
        return out

    def put(x, oi, oj):
        for a in range(n):
            for b in range(n):
                emit(oi * n + a, oj * n + b, x[a][b])

    m2 = yield from m(2)
    m4 = yield from m(4)
    put(_add(m2, m4), 1, 0)
    m1 = yield from m(1)
    c11 = _add(m1, m4)
    c22 = _sub(m1, m2)
    m7 = yield from m(7)
    c11 = _add(c11, m7)
    m5 = yield from m(5)
    put(_sub(c11, m5), 0, 0)
    m3 = yield from m(3)
    put(_add(m3, m5), 0, 1)
    c22 = _add(c22, m3)
    m6 = yield from m(6)
    put(_add(c22, m6), 1, 1)


def _drain(gen):
    for _ in gen:
        pass


def _chain(*gens):
    for g in gens:
        yield from g


def _weigh(gen, w):
    for _ in gen:
        yield w


def _interleave(*streams):
    gens = [s[0] for s in streams]
    total = [s[1] for s in streams]
    span = [s[2:] if len(s) > 2 else (0.0, 1.0) for s in streams]
    done = [0.0] * len(gens)
    live = list(range(len(gens)))
    while live:
        i = min(live, key=lambda k: span[k][0] + (span[k][1] - span[k][0]) * done[k] / total[k])
        try:
            w = next(gens[i])
            done[i] += 1 if w is None else w
        except StopIteration:
            live.remove(i)


def _split(u):
    return pltpu.bitcast(u << 16, F32), pltpu.bitcast(u & jnp.uint32(0xFFFF0000), F32)


def _join(lo, hi):
    return pltpu.bitcast(pltpu.pack_elementwise([lo, hi], packed_dtype=BF16), U32)


def _join_shuffled(v):
    r, c = v.shape
    v4 = v.reshape(r // 16, 2, 8, c)
    return _join(v4[:, 0].reshape(r // 2, c), v4[:, 1].reshape(r // 2, c))


def _unshuffle(pos):
    return (pos & ~15) + ((pos & 15) >> 1) + 8 * (pos & 1)


def _half(u):
    return pltpu.bitcast(u, BF16)


def _cat(xs, axis):
    return xs[0] if len(xs) == 1 else jnp.concatenate(xs, axis=axis)


def _ds(start, size):
    if isinstance(start, int):
        return pl.ds(start, size)
    return pl.ds(pl.multiple_of(start, min(size, 16)), size)


def _when(cond, fn):
    if isinstance(cond, bool):
        if cond:
            fn()
    else:
        pl.when(cond)(fn)


def _loop(n, body, unroll=1):
    if n == unroll:
        for i in range(n):
            body(i)
        return

    def trip(t, _):
        for u in range(unroll):
            body(t * unroll + u)

    lax.fori_loop(0, n // unroll, trip, None)


class _Pacer:
    def __init__(self, words, lag=1):
        self.lag = lag
        self.words = words | 1
        self.marks = []

    def mark(self, v):
        self.marks.append(pltpu.bitcast(v[:, 0:LANES], U32))
        return v

    def hold(self, x, lag=None):
        lag = lag or self.lag
        if len(self.marks) < lag:
            return x
        rows = x.shape[0]
        never = jnp.concatenate([self.words] * (rows // 8), axis=0) == 0
        return pltpu.bitcast(jnp.where(never, self.marks[-lag][0:rows], pltpu.bitcast(x, U32)), x.dtype)


class _NoPacer:
    def mark(self, v):
        return v

    def hold(self, x, lag=None):
        return x


def build(LA=2, LAO=2, LB=2, LO=2, ra=256, ukv=1, uo=1, uh=1, up=1,
          seq_mode="mid", att_mode="d1", kgrp=2, name="fused", dbg=(), flags=None,
          sp_att=(0., .8), sp_ro=(.05, .4), sp_prep=(.05, .5), zrows=16,
          sp_local=(0., .95), sp_prepa=(.1, .95), kv_first=False, pace4=True, pace6=True, pacea=True,
          pacelo=True, wlo=6, wsm=0, fly6=True, lag4=1, lag6=3, laga=2, mix6=True, hk=8, hv=4, o_pos=0, unroll6=2, elag=5, marks='qp', sp_lb=(.05, .9), pace1=True, bx_at=0, u1=2, sp_s1=(0., .8), att5=('d2', 4, 0, 'qp'), pace5=False):
    nA, pA = 2 ** LA, 7 ** LA
    nAO, pAO = 2 ** LAO, 7 ** LAO
    nB, pB = 2 ** LB, 7 ** LB
    nO, pO = 2 ** LO, 7 ** LO
    assert LB >= 1
    gh = nB
    ngrp = HB // gh
    ppg = gh // 2
    nblk = S // ra
    kq = DA // nA
    mq = S // nB
    crow = mq // gh

    def recip(l):
        r = pltpu.reciprocal(l, approx=True)
        return r * (2.0 - l * r)

    def strassen_pairs(load, n, side, store, pacer):
        h = n // 2
        combine = s_lhs if side is LHS_TERMS else s_rhs
        for top, terms in enumerate(side):
            halves = [None, None]
            for sign, qi, qj in terms:
                blocks = [[load(qi * h + i, qj * h + j, pacer.hold) for j in range(h)] for i in range(h)]
                for e in range(2):
                    quad = [[blk[e] for blk in row] for row in blocks]
                    halves[e] = quad if halves[e] is None else (_add if sign > 0 else _sub)(halves[e], quad)
            parts = [combine(x) for x in halves]
            for p in range(len(parts[0])):
                store(top * len(parts[0]) + p, _join(parts[0][p], parts[1][p]))
            yield

    def kernel(ax_hbm, wqkv_hbm, awo_hbm, bx_hbm, c_hbm, wq_hbm, wuk_hbm, wuv_hbm, bwo_hbm,
               out_hbm, x_raw, w_raw, awo_raw, ctx, stage, ro_w, sem_out, sem_a):

        def out_copy(slot, row0, col0):
            return pltpu.make_async_copy(
                stage.at[slot], out_hbm.at[_ds(row0, ra), pl.ds(col0, DA)], sem_out.at[slot])

        kq_o = (HB * DB) // nO // 2
        tpo = 8 // nO

        def ro_rows(p, ct, r0, rows):
            return pl.ds((p * tpo + ct) * kq_o + r0, rows)

        def attend_b(c_raw, bwo_raw, lx, lc, rq0, rk0, rv0, rq1, rk1, rv1,
                     qs0, ks0, vs0, qs1, ks1, vs1, sq0, sk0, sv0, sq1, sk1, sv1, sem_in, sem_g):
            rsets = ((rq0, rk0, rv0), (rq1, rk1, rv1))
            qkv = ((qs0, ks0, vs0), (qs1, ks1, vs1))
            staged = ((sq0, sk0, sv0), (sq1, sk1, sv1))

            def weight_copies(par, grp, w):
                words = (wq_hbm, wuk_hbm, wuv_hbm)[w].bitcast(U32)
                n = words.shape[0]
                return [pltpu.make_async_copy(
                    words.at[:, (HB // 2) * parity + grp * ppg + pr],
                    staged[par][w].at[pl.ds((2 * pr + parity) * n, n)], sem_g.at[3 * par + w])
                    for pr in range(ppg) for parity in range(2)]

            def group_copies(par, grp):
                return [c for w in range(3) for c in weight_copies(par, grp, w)]

            def act_copies(src, dst, part, sem):
                return [pltpu.make_async_copy(src.at[_ds(i * mq + part * crow, crow)],
                                              dst.at[_ds(i * mq + part * crow, crow)], sem) for i in range(nB)]

            def c_copies(part):
                return act_copies(c_hbm, c_raw, part, sem_in.at[part])

            c_bx = [pltpu.make_async_copy(bx_hbm, bwo_raw.at[pl.ds(0, S)], sem_in.at[gh])]

            def wo_copies(grp):
                rows = 2 * kq_o // ngrp
                return [pltpu.make_async_copy(bwo_hbm.at[_ds(i * 2 * kq_o + grp * rows, rows)],
                                              bwo_raw.at[_ds(i * 2 * kq_o + grp * rows, rows)], sem_in.at[gh + 1])
                        for i in range(nO)]

            def prep_r(par, w, part, pacer):
                src, dst = staged[par][w], rsets[par][w]
                width = (MB, DC, DC)[w] // 2
                kb = width // nB
                rows = kb // gh
                for s in range(0, rows, 8):
                    r = part * rows + s

                    def load(i, j, hold):
                        return [_split(hold(src[_ds((2 * (j // 2) + e) * width + i * kb + r, 8), :]))[j % 2]
                                for e in range(2)]

                    def store(p, words):
                        dst[p, _ds(r, 8), :] = words

                    yield from strassen_pairs(load, nB, RHS_TERMS, store, pacer)

            def n_prep_r(w):
                return (MB, DC, DC)[w] // nB // gh // 16 * 7

            def prep_group(par, part, pacer):
                return _chain(*[prep_r(par, w, part, pacer) for w in range(3)])

            n_prep = sum(n_prep_r(w) for w in range(3))

            c_a = ([pltpu.make_async_copy(ax_hbm.at[:, pl.ds(j * LANES, LANES)], x_raw.at[j], sem_a) for j in range(8)]
                   + [pltpu.make_async_copy(awo_hbm.at[:, pl.ds(j * LANES, LANES)], awo_raw.at[j], sem_a) for j in range(8)]
                   + [pltpu.make_async_copy(wqkv_hbm, w_raw, sem_a)])

            def prep_lhs(tile, dst, width, part, pacer):
                kb = width // nB
                for t in range(kb // LANES):
                    for s in range(0, crow, 16):
                        r = part * crow + s

                        def load(i, j, hold):
                            return _split(hold(pltpu.bitcast(tile(j * (kb // LANES) + t, _ds(i * mq + r, 16)), U32)))

                        def store(p, words):
                            dst[p, t, _ds(r // 2, 8), :] = words

                        yield from strassen_pairs(load, nB, LHS_TERMS, store, pacer)

            def n_prep_lhs(width):
                return width // nB // LANES * (crow // 16) * 7

            def project(par, w, part, pacer):
                lhs_ref, ktiles = (lx, 8 // nB) if w == 0 else (lc, 4 // nB)
                w_ref, dst = rsets[par][w], qkv[par][w]
                r0 = part * crow

                def prod(p):
                    a = _cat([_half(lhs_ref[p, t, _ds(r0 // 2, crow // 2), :]) for t in range(ktiles)], 1)
                    return pacer.mark(jnp.dot(a, _half(w_ref[p]), preferred_element_type=F32))

                def emit(i, j, v):
                    if w == 0:
                        dst[j, _ds(i * mq + r0, crow), :] = (v * (DB ** -0.5 * LOG2E)).astype(BF16)
                    else:
                        dst[j, _ds((i * mq + r0) // 2, crow // 2), :] = _join_shuffled(v)

                return _weigh(s_mul(prod, LB, emit), ktiles)

            n_proj = pB * (16 // nB)
            bq = LANES
            nb = S // bq

            def attention(par, hl, head, pacer, att_mode, kgrp, elag, marks):
                qs, ks, vs = qkv[par]
                tri = (lax.broadcasted_iota(I32, (bq, bq), 0)
                       >= _unshuffle(lax.broadcasted_iota(I32, (bq, bq), 1)))

                def qk(i):
                    q = qs[hl, i * bq:(i + 1) * bq, :]
                    tiles = []
                    mx = None
                    for c0 in range(0, i + 1, kgrp):
                        n = min(kgrp, i + 1 - c0)
                        k = _half(ks[hl, c0 * bq // 2:(c0 + n) * bq // 2, :])
                        s = lax.dot_general(q, k, NT_DIMS, preferred_element_type=F32)
                        if 'q' in marks:
                            pacer.mark(s)
                        for c in range(n):
                            t = s[:, c * bq:(c + 1) * bq]
                            if c0 + c == i:
                                t = jnp.where(tri, t, MASKED * LOG2E)
                            tiles.append(t)
                            mx = t if mx is None else jnp.maximum(mx, t)
                        yield n
                    return tiles, jnp.max(mx, axis=1, keepdims=True)

                def softmax(tiles, m):
                    ps = [jnp.exp2(s - m) for s in tiles]
                    l = jnp.sum(functools.reduce(jnp.add, ps), axis=1, keepdims=True)
                    return ps, l

                def pv(i, ps, l):
                    o = None
                    for c0 in range(0, i + 1, kgrp):
                        n = min(kgrp, i + 1 - c0)
                        v = _half(vs[hl, c0 * bq // 2:(c0 + n) * bq // 2, :])
                        t = jnp.dot(_cat(ps[c0:c0 + n], 1).astype(BF16), v, preferred_element_type=F32)
                        o = t if o is None else o + t
                        yield n
                    ctx[head, i * bq:(i + 1) * bq, :] = (o * recip(l)).astype(BF16)

                def soft_pv(i, tiles, m):
                    o = l = None
                    m = jnp.broadcast_to(m, (bq, bq))
                    for c0 in range(0, i + 1, kgrp):
                        n = min(kgrp, i + 1 - c0)
                        mc = pacer.hold(m, elag) if elag else m
                        ps = [jnp.exp2(s - mc) for s in tiles[c0:c0 + n]]
                        for p in ps:
                            l = p if l is None else l + p
                        v = _half(vs[hl, c0 * bq // 2:(c0 + n) * bq // 2, :])
                        t = jnp.dot(_cat(ps, 1).astype(BF16), v, preferred_element_type=F32)
                        if 'p' in marks:
                            pacer.mark(t)
                        o = t if o is None else o + t
                        yield n
                    l = jnp.sum(l, axis=1, keepdims=True)
                    ctx[head, i * bq:(i + 1) * bq, :] = (o * recip(l)).astype(BF16)

                if seq_mode == "mid":
                    seq = list(range(0, nb, 2)) + list(range(1, nb, 2))[::-1]
                elif seq_mode == "alt":
                    seq = [x for pr in zip(range(nb // 2), range(nb - 1, nb // 2 - 1, -1)) for x in pr]
                elif seq_mode == "down":
                    seq = list(range(nb))[::-1]
                elif seq_mode == "up":
                    seq = list(range(nb))
                s, p = {}, {}
                s[0] = yield from qk(seq[0])
                for n in range(nb + 1):
                    if n + 1 < nb:
                        s[n + 1] = yield from qk(seq[n + 1])
                    if att_mode == "d1":
                        if n < nb:
                            yield from soft_pv(seq[n], *s[n])
                        continue
                    if att_mode == "d1b":
                        if n >= 1:
                            yield from soft_pv(seq[n - 1], *s[n - 1])
                        continue
                    if n < nb:
                        p[n] = softmax(*s[n])
                    if n >= 1:
                        yield from pv(seq[n - 1], *p[n - 1])

            n_att = nb * (nb + 1)
            orow = (HB * DB) // nO // HB

            def prep_ro(head, pacer):
                for ct in range(tpo):
                    for s in range(0, orow, 16):
                        r = head * orow + s

                        def load(i, j, hold):
                            c0 = (j * tpo + ct) * LANES
                            return _split(hold(pltpu.bitcast(bwo_raw[_ds(i * 2 * kq_o + r, 16), c0:c0 + LANES], U32)))

                        def store(p, words):
                            ro_w[_ds((p * tpo + ct) * kq_o + r // 2, 8), :] = words

                        yield from strassen_pairs(load, nO, RHS_TERMS, store, pacer)

            n_prep_ro = tpo * (orow // 16) * 7

            def head_step(par, g, hl, main):
                if 'p4' not in dbg and 'p5' not in dbg:
                    @pl.when(hl == 0)
                    def _():
                        for c in wo_copies(g):
                            c.wait()
                        for c in wo_copies(g + 1) if main else c_a:
                            c.start()

                if main and 'p4' not in dbg:
                    @pl.when((hl == 0) & (g + 2 < ngrp))
                    def _():
                        for c in group_copies(par, g + 2):
                            c.wait()

                    @pl.when((hl == 0) & (g + 3 < ngrp))
                    def _():
                        for c in group_copies(1 - par, g + 3):
                            c.start()

                pacer = _Pacer(lc[0, 0, 0:8, :], lag4)
                pacer2 = pacer if (pace4 if main else pace5) else _NoPacer()
                parts = [(attention(par, hl, g * gh + hl, pacer, *((att_mode, kgrp, elag, marks) if main else att5)), n_att, *(sp_att if main else (0., 1.)))]
                if main:
                    parts.append((_chain(*[project(1 - par, w, hl, pacer) for w in range(3)]), n_proj))
                if 'noro' not in dbg:
                    parts.append((prep_ro(g * gh + hl, pacer2), n_prep_ro, *sp_ro))
                if main and 'noprep' not in dbg:
                    parts.append((prep_group(par, hl, pacer2), n_prep, *sp_prep))
                _interleave(*parts)

            if 'p4' in dbg or 'p5' in dbg:
                o32 = out_hbm.bitcast(U32)
                for r in (lx.at[0, 0], lc.at[0, 0], rq1.at[0], rk1.at[0], rv1.at[0], ks0.at[0], vs0.at[0], sq0, sk0, sv0):
                    pltpu.sync_copy(o32.at[pl.ds(0, 8), pl.ds(0, LANES)], r.at[pl.ds(0, 8)])
                pltpu.sync_copy(out_hbm.at[pl.ds(0, 16), pl.ds(0, LANES)], qs0.at[0, pl.ds(0, 16)])
                pltpu.sync_copy(bwo_hbm.at[pl.ds(0, 16)], bwo_raw.at[pl.ds(0, 16)])
                with jax.named_scope('P4_dbg'):
                    _loop(16, lambda t: head_step(0, t // gh, t % gh, 'p4' in dbg), uh)
                for r in (ctx, qs1):
                    pltpu.sync_copy(r.at[0, pl.ds(0, 16)], out_hbm.at[pl.ds(0, 16), pl.ds(0, LANES)])
                for r in (ro_w, ks1.at[0], vs1.at[0], rq0.at[0], rk0.at[0], rv0.at[0]):
                    pltpu.sync_copy(r.at[pl.ds(0, 8)], o32.at[pl.ds(0, 8), pl.ds(0, LANES)])
                return

            def c_tile(t, rows):
                return c_raw[rows, t * LANES:(t + 1) * LANES]

            def x_tile(t, rows):
                return bwo_raw[rows, t * LANES:(t + 1) * LANES]

            first = c_copies(0) + weight_copies(0, 0, 1) + weight_copies(0, 0, 2)
            with jax.named_scope('S0'):
                for c in first:
                    c.start()
                for c in first:
                    c.wait()
                for part in range(1, gh):
                    for c in c_copies(part):
                        c.start()
                _drain(prep_lhs(c_tile, lc, DC, 0, _NoPacer()))
                _loop(gh, lambda part: _drain(prep_r(0, 1, part, _NoPacer())))

            def first_k(part):
                pacer = _Pacer(rk0[0, 0:8, :])
                rest, n = [prep_r(0, 2, part, pacer)], n_prep_r(2)
                if part + 1 < gh:
                    for c in c_copies(part + 1):
                        c.wait()
                    rest.insert(0, prep_lhs(c_tile, lc, DC, part + 1, pacer))
                    n += n_prep_lhs(DC)
                if part == bx_at:
                    for c in c_bx + weight_copies(0, 0, 0):
                        c.start()
                _interleave((project(0, 1, part, pacer), n_proj // 4), (_chain(*rest), n, 0.05, 0.95))

            with jax.named_scope('S1k'):
                _loop(gh, first_k, gh)
            with jax.named_scope('S1v'):
                _loop(u1, lambda part: _drain(project(0, 2, part, _NoPacer())), u1)
                for c in c_bx + weight_copies(0, 0, 0):
                    c.wait()
                for c in group_copies(1, 1):
                    c.start()
                pacer = _Pacer(rk0[0, 0:8, :])
                _interleave((_chain(*[project(0, 2, part, pacer) for part in range(u1, gh)]), n_proj // 4 * (gh - u1)),
                            (_chain(*[prep_r(0, 0, part, pacer) for part in range(gh)],
                                    *[prep_lhs(x_tile, lx, MB, part, pacer) for part in range(gh)]),
                             gh * (n_prep_r(0) + n_prep_lhs(MB)), *sp_s1))
            with jax.named_scope('S1b'):
                for c in group_copies(1, 1):
                    c.wait()
                for c in group_copies(0, 2) + wo_copies(0):
                    c.start()

            def first_q(part):
                pacer = _Pacer(rk0[0, 0:8, :])
                _interleave((project(0, 0, part, pacer), n_proj // 2), (prep_group(1, part, pacer), n_prep, 0.05, 0.95))

            with jax.named_scope('S2'):
                _loop(gh, first_q, up)

            def two_groups(t, _):
                _loop(gh, lambda hl: head_step(0, 2 * t, hl, True), uh)

                @pl.when(t < ngrp // 2 - 1)
                def _():
                    _loop(gh, lambda hl: head_step(1, 2 * t + 1, hl, True), uh)

            with jax.named_scope('P4_main'):
                lax.fori_loop(0, ngrp // 2, two_groups, None)
            with jax.named_scope('P5_tail'):
                _loop(gh, lambda hl: head_step(1, ngrp - 1, hl, False), uh)
            for c in c_a:
                c.wait()

        if 'noB' not in dbg:
            pl.run_scoped(
                attend_b,
                pltpu.VMEM((S, DC), BF16),
                pltpu.VMEM((HB * DB, MB), BF16),
                pltpu.VMEM((pB, 8 // nB, mq // 2, LANES), U32),
                pltpu.VMEM((pB, 4 // nB, mq // 2, LANES), U32),
                *[pltpu.VMEM((pB, w // nB // 2, LANES), U32) for w in (MB, DC, DC) * 2],
                *[t for _ in range(2) for t in (pltpu.VMEM((gh, S, LANES), BF16),
                                                pltpu.VMEM((gh, S // 2, LANES), U32),
                                                pltpu.VMEM((gh, S // 2, LANES), U32))],
                *[pltpu.VMEM((ppg * w, LANES), U32) for w in (MB, DC, DC) * 2],
                pltpu.SemaphoreType.DMA((gh + 2,)),
                pltpu.SemaphoreType.DMA((6,)),
            )

        def finish(rq_w, rk_w, rv_w, rao_w, la):
            ra_w = (rq_w, rk_w, rv_w)
            wrows = kq // nblk
            tpa, tpao = 8 // nA, 8 // nAO
            grp_rows = 16 * nA
            assert nA == nAO

            def permuted_rows(t, r0, pacer):
                lane = lax.broadcasted_iota(I32, (8, LANES), 1)
                s, ch, a = lane >> 5, (lane & 31) >> 2, lane & 3
                head = _unshuffle(lane & 31)
                g1 = []
                for j in range(8):
                    c0 = t * DA + j * LANES
                    u = pacer.hold(pltpu.bitcast(w_raw[_ds(r0, 16), c0:c0 + LANES], I32))
                    g1.append(jnp.take_along_axis(u, a * 32 + 4 * ((ch - j) & 7) + s, axis=1))
                v = [g1[(0 - i) % 8] for i in range(8)]
                for bit in (1, 2, 4):
                    v = [jnp.where((ch & bit) != 0, v[(i - bit) % 8], v[i]) for i in range(8)]
                return [pltpu.bitcast(jnp.take_along_axis(
                    v[i], s * 32 + (((head >> 2) + i) & 7) * 4 + (head & 3), axis=1), U32) for i in range(8)]

            def prep_w(blk, t, pacer):
                for s in range(0, wrows, 16):
                    tiles = []
                    for i in range(nA):
                        tiles.append(permuted_rows(t, i * kq + blk * wrows + s, pacer))
                        yield
                    for ct in range(tpa):
                        def store(p, words):
                            ra_w[t][p, ct, _ds((blk * wrows + s) // 2, 8), :] = words

                        yield from strassen_pairs(lambda i, j, hold: _split(hold(tiles[i][j * tpa + ct])), nA, RHS_TERMS, store, pacer)

            n_prep_w = (wrows // 16) * (nA + tpa * 7)

            def prep_la(blk, pacer):
                for c in range(ra // grp_rows):
                    for t in range(tpa):
                        def load(i, j, hold):
                            words = x_raw.at[j * tpa + t].bitcast(U32).at[_ds(blk * (ra // 2), ra // 2)]
                            w0 = (c * grp_rows + 32 * (i // 2)) // 2
                            return [_split(hold(words[pl.ds(w0 + e, 8, stride=2), :]))[i % 2] for e in range(2)]

                        def store(p, words):
                            la[p, t, _ds((blk * (ra // nA) + 16 * c) // 2, 8), :] = words

                        yield from strassen_pairs(load, nA, LHS_TERMS, store, pacer)

            n_prep_la = (ra // grp_rows) * tpa * 7

            def prep_wo(blk, pacer):
                dpq = 16 // nAO
                per = nblk // tpao
                ct = blk // per
                n = 2 * dpq // per
                assert per in (2, 4) and n in (2, 4)
                for dp in range(dpq):
                    if per == 4 and dp % 2:
                        continue
                    h0 = 16 * (blk % 2)
                    dd = dp + ((blk // 2) % 2 if per == 4 else 0)
                    src = {}
                    for i in range(nAO):
                        for j in range(nAO):
                            words = awo_raw.at[j * tpao + ct].bitcast(U32).at[pl.ds(pl.multiple_of(h0 * 16, 256), 256)]
                            for e in range(2):
                                u = words[pl.ds(8 * e * 16 + i * dpq + dp, 8, stride=16), :]
                                if per == 4:
                                    u = jnp.where((blk // 2) % 2 == 1,
                                                  words[pl.ds(8 * e * 16 + i * dpq + dp + 1, 8, stride=16), :], u)
                                src[i, j, e] = pacer.hold(u)
                        yield
                    for half in range(2):
                        def store(p, words):
                            rao_w[p, ct, _ds(((2 * dd + half) * HA + h0) // 2, 8), :] = words

                        yield from strassen_pairs(lambda i, j, hold: [_split(hold(src[i, j, e]))[half] for e in range(2)],
                                                  nAO, RHS_TERMS, store, pacer)

            n_prep_wo = (2 * (16 // nAO) * tpao // nblk) * (nAO + 2 * 7)

            def project_b(lb0, lb1):
                rq = ra // nO
                hq = HB // nO
                lb = (lb0, lb1)

                def prep_lb(blk, dst, pacer):
                    for h in range(hq):
                        for r in range(0, rq, 16):
                            def load(a, j, hold):
                                return _split(hold(pltpu.bitcast(ctx[j * hq + h, _ds(blk * ra + a * rq + r, 16), :], U32)))

                            def store(p, words):
                                dst[p, h, r // 2:r // 2 + 8, :] = words

                            yield from strassen_pairs(load, nO, LHS_TERMS, store, pacer)

                n_prep_lb = hq * (rq // 16) * 7

                def out_b(i, par):
                    _when(i >= 2, lambda: out_copy(par, 0, DA).wait())
                    pacer = _Pacer(ro_w[0:8, :], lag6) if pace6 else _NoPacer()

                    if fly6:
                        blocks = [[_cat([ctx[j * hq + h, _ds(i * ra + a * rq, rq), :] for h in range(hq)], 1).astype(F32)
                                   for j in range(nO)] for a in range(nO)]
                        lhs = [v.astype(BF16) for v in s_lhs(blocks)]

                    def prod(p):
                        x = lhs[p] if fly6 else _cat([_half(lb[par][p, h]) for h in range(hq)], 1)
                        w = _cat([_half(ro_w[ro_rows(p, ct, 0, kq_o), :]) for ct in range(tpo)], 1)
                        return pacer.mark(jnp.dot(x, w, preferred_element_type=F32))

                    def emit(a, j, v):
                        stage[par, a * rq:(a + 1) * rq, j * tpo * LANES:(j + 1) * tpo * LANES] = v.astype(BF16)

                    nxt = min(i + 1, nblk - 1) if isinstance(i, int) else jnp.minimum(i + 1, nblk - 1)
                    parts = [(s_mul(prod, LO, emit), pO)]
                    if not fly6:
                        parts.append((prep_lb(nxt, lb[1 - par], pacer), n_prep_lb, *sp_lb))
                    if 'noprepa' not in dbg:
                        if mix6:
                            parts += [(prep_w(i, t, pacer), n_prep_w, *sp_prepa) for t in range(3)]
                            parts += [(prep_la(i, pacer), n_prep_la, *sp_prepa), (prep_wo(i, pacer), n_prep_wo, *sp_prepa)]
                        else:
                            parts.append((_chain(*[prep_w(i, t, pacer) for t in range(3)], prep_la(i, pacer), prep_wo(i, pacer)),
                                          3 * n_prep_w + n_prep_la + n_prep_wo, *sp_prepa))
                    _interleave(*parts)
                    out_copy(par, i * ra, DA).start()

                if not fly6:
                    _drain(prep_lb(0, lb0, _NoPacer()))
                with jax.named_scope('P6_out'):
                    if unroll6 == 2:
                        lax.fori_loop(0, nblk // 2, lambda t, _: (out_b(2 * t, 0), out_b(2 * t + 1, 1))[0], None)
                    else:
                        lax.fori_loop(0, nblk, lambda t, _: out_b(t, t % 2), None)

            def branch_a(lo, qa, ka, va):
                def proj_a(t, blk, pacer):
                    rq = ra // nA
                    dst, row0 = ((qa, (blk % 2) * (ra // 2)), (ka, blk * (ra // 2) + HALO), (va, blk * (ra // 2) + HALO))[t]

                    def prod(p):
                        x = _cat([_half(la[p, k, _ds(blk * rq // 2, rq // 2), :]) for k in range(tpa)], 1)
                        w = _cat([_half(ra_w[t][p, ct]) for ct in range(tpa)], 1)
                        return pacer.mark(jnp.dot(x, w, preferred_element_type=F32))

                    def emit(i, j, v):
                        for ct in range(tpa):
                            for c in range(rq // 16):
                                dst[2 * (j * tpa + ct) + i % 2, _ds(row0 + c * (grp_rows // 2) + 16 * (i // 2), 16), :] = (
                                    v[16 * c:16 * (c + 1), ct * LANES:(ct + 1) * LANES])

                    return s_mul(prod, LA, emit)

                def local_attn(blk, pacer):
                    row0, slot = blk * (ra // 2), blk % 2
                    o = {}
                    for r in range(0, ra // 2, 8):
                        for par in range(2):
                            pos = row0 + r + lax.broadcasted_iota(I32, (8, LANES), 0)
                            q = [qa[2 * j + par, _ds(slot * (ra // 2) + r, 8), :] for j in range(8)]
                            logits = []
                            for w in range(WIN):
                                acc = None
                                for j in range(8):
                                    k = ka[2 * j + par, pl.ds(row0 + r + HALO - w, 8), :]
                                    t = q[j] * (pacer.hold(k) if j % hk == 0 else k)
                                    acc = t if acc is None else acc + t
                                acc = acc + pltpu.roll(acc, 64, 1)
                                acc = acc + pltpu.roll(acc, 32, 1)
                                acc = acc * (DHA ** -0.5 * LOG2E)
                                if r < w:
                                    acc = jnp.where(pos >= w, acc, MASKED * LOG2E)
                                logits.append(acc)
                                yield
                            m = functools.reduce(jnp.maximum, logits)
                            e = [jnp.exp2(l - m) for l in logits]
                            inv = recip(functools.reduce(jnp.add, e))
                            e = [x * inv for x in e]
                            for j in range(8):
                                acc = None
                                for w in range(WIN):
                                    v = va[2 * j + par, pl.ds(row0 + r + HALO - w, 8), :]
                                    t = e[w] * (pacer.hold(v) if w % hv == 0 else v)
                                    acc = t if acc is None else acc + t
                                o[r, par, j] = acc
                                yield
                        if (2 * r + 16) % grp_rows == 0:
                            c = 2 * r // grp_rows
                            for t in range(tpao):
                                def load(i, j, hold):
                                    return [hold(o[c * (grp_rows // 2) + 8 * i, par, j * tpao + t]) for par in range(2)]

                                def store(p, words):
                                    lo[slot * pAO + p, t, 8 * c:8 * (c + 1), :] = words

                                yield from _weigh(strassen_pairs(load, nAO, LHS_TERMS, store, pacer if pacelo else _NoPacer()), wlo)

                n_local = (16 + wsm) * (ra // 8) + tpao * (ra // grp_rows) * 7 * wlo

                def out_a(blk, pacer):
                    rq = ra // nAO
                    slot = blk % 2

                    def prod(p):
                        x = _cat([_half(lo[slot * pAO + p, k]) for k in range(tpao)], 1)
                        w = _cat([_half(rao_w[p, ct]) for ct in range(tpao)], 1)
                        return pacer.mark(jnp.dot(x, w, preferred_element_type=F32))

                    def emit(i, j, v):
                        for c in range(rq // 16):
                            r = c * grp_rows + 16 * i
                            stage[slot, r:r + 16, j * tpao * LANES:(j + 1) * tpao * LANES] = (
                                v[16 * c:16 * (c + 1)].astype(BF16))

                    return s_mul(prod, LAO, emit)

                def a_step(i, project=True, attend=True, final=True):
                    if final:
                        out_copy((i - 1) % 2, 0, 0).wait()
                    pacer = _Pacer(rk_w[0, 0, 0:8, :], laga) if pacea else _NoPacer()
                    mm = [proj_a(t, i + 1, pacer) for t in (1, 2, 0)] if project else []
                    if final:
                        mm.insert(min(o_pos, len(mm)), out_a(i - 1, pacer))
                    parts = [(_chain(*mm), (3 * pA if project else 0) + (pAO if final else 0))]
                    if attend:
                        parts.append((local_attn(i, pacer), n_local, *sp_local))
                    _interleave(*parts)
                    if final:
                        out_copy((i - 1) % 2, (i - 1) * ra, 0).start()

                o32 = out_hbm.bitcast(U32)
                if 'pa' in dbg:
                    for r in (la.at[0, 0], rq_w.at[0, 0], rk_w.at[0, 0], rv_w.at[0, 0], rao_w.at[0, 0], lo.at[0, 0]):
                        pltpu.sync_copy(o32.at[pl.ds(0, 8), pl.ds(0, LANES)], r.at[pl.ds(0, 8)])
                    for r in (qa, ka, va):
                        pltpu.sync_copy(out_hbm.bitcast(F32).at[pl.ds(0, 8), pl.ds(0, LANES)], r.at[0, pl.ds(0, 8)])
                    out_copy(0, 0, 0).start()
                    out_copy(1, 0, 0).start()
                    with jax.named_scope('PA_dbg'):
                        _loop(nblk - 2, lambda t: a_step(t + 1), ukv)
                    out_copy(0, 0, 0).wait()
                    out_copy(1, 0, 0).wait()
                    for r in (qa, ka, va):
                        pltpu.sync_copy(r.at[0, pl.ds(0, 8)], out_hbm.bitcast(F32).at[pl.ds(0, 8), pl.ds(0, LANES)])
                    pltpu.sync_copy(lo.at[0, 0, pl.ds(0, 8)], o32.at[pl.ds(0, 8), pl.ds(0, LANES)])
                    return
                zeros = jnp.zeros((HALO, LANES), F32)
                for j in range(16):
                    ka[j, 0:HALO, :] = zeros
                    va[j, 0:HALO, :] = zeros
                with jax.named_scope('PA0'):
                    a_step(-1, attend=False, final=False)
                with jax.named_scope('PA1'):
                    a_step(0, final=False)
                with jax.named_scope('PA2'):
                    _loop(nblk - 2, lambda t: a_step(t + 1), ukv)
                with jax.named_scope('PA3'):
                    a_step(nblk - 1, project=False)
                with jax.named_scope('PA4'):
                    a_step(nblk, project=False, attend=False)
                out_copy(0, 0, 0).wait()
                out_copy(1, 0, 0).wait()


            if 'noP6' not in dbg:
                if 'p6' in dbg:
                    o32 = out_hbm.bitcast(U32)
                    pltpu.sync_copy(o32.at[pl.ds(0, 8), pl.ds(0, LANES)], ro_w.at[pl.ds(0, 8)])
                    pltpu.sync_copy(out_hbm.at[pl.ds(0, 16), pl.ds(0, LANES)], ctx.at[0, pl.ds(0, 16)])
                    pltpu.sync_copy(out_hbm.at[pl.ds(0, 16), pl.ds(0, LANES)], x_raw.at[0, pl.ds(0, 16)])
                    pltpu.sync_copy(out_hbm.at[pl.ds(0, 16), pl.ds(0, LANES)], awo_raw.at[0, pl.ds(0, 16)])
                    pltpu.sync_copy(wqkv_hbm.at[pl.ds(0, 16)], w_raw.at[pl.ds(0, 16)])
                pl.run_scoped(project_b, *[pltpu.VMEM((pO, HB // nO, ra // nO // 2, LANES), U32) for _ in range(2)])
            if 'p6' in dbg:
                out_copy(0, 0, 0).wait()
                out_copy(1, 0, 0).wait()
                for r in (la.at[0, 0], rq_w.at[0, 0], rk_w.at[0, 0], rv_w.at[0, 0], rao_w.at[0, 0]):
                    pltpu.sync_copy(r.at[pl.ds(0, 8)], o32.at[pl.ds(0, 8), pl.ds(0, LANES)])
                return
            pl.run_scoped(
                branch_a,
                pltpu.VMEM((2 * pAO, 8 // nAO, ra // nAO // 2, LANES), U32),
                pltpu.VMEM((16, ra, LANES), F32),
                pltpu.VMEM((16, HALO + S // 2, LANES), F32),
                pltpu.VMEM((16, HALO + S // 2, LANES), F32),
            )

        if 'noA' not in dbg:
            pl.run_scoped(
                finish,
                *[pltpu.VMEM((pA, 8 // nA, kq // 2, LANES), U32) for _ in range(3)],
                pltpu.VMEM((pAO, 8 // nAO, DA // nAO // 2, LANES), U32),
                pltpu.VMEM((pA, 8 // nA, S // nA // 2, LANES), U32),
            )

    def run(A_x, A_wqkv, A_wo, B_x, B_c_kv, B_w_q, B_w_uk, B_w_uv, B_w_o):
        any_spec = pl.BlockSpec(memory_space=pl.ANY)
        out = pl.pallas_call(
            kernel,
            in_specs=[any_spec] * 9,
            out_specs=any_spec,
            out_shape=jax.ShapeDtypeStruct((S, DA + MB), BF16),
            scratch_shapes=[
                pltpu.VMEM((8, S, LANES), BF16),
                pltpu.VMEM((DA, 3 * DA), BF16),
                pltpu.VMEM((8, DA, LANES), BF16),
                pltpu.VMEM((HB, S, LANES), BF16),
                pltpu.VMEM((2, ra, DA), BF16),
                pltpu.VMEM((pO * (8 // nO) * (HB * DB // nO // 2) + zrows, LANES), U32),
                pltpu.SemaphoreType.DMA((2,)),
                pltpu.SemaphoreType.DMA(()),
            ],
            compiler_params=pltpu.CompilerParams(vmem_limit_bytes=127 * 2 ** 20, flags=flags),
            name=name,
        )(A_x.reshape(S, DA), A_wqkv, A_wo, B_x.reshape(S, MB), B_c_kv.reshape(S, DC),
          B_w_q.reshape(MB // 2, 2 * HB, DB), B_w_uk.reshape(DC // 2, 2 * HB, DB),
          B_w_uv.reshape(DC // 2, 2 * HB, DB), B_w_o.reshape(HB * DB, MB))
        return out.reshape(1, S, DA + MB)

    return run


_run = build()


@jax.jit
def pallas_concat_heads__sliding_local_dilated__compressed_kv_cla__prompt_kernel(A_x, A_wqkv, A_wo, B_x, B_c_kv, B_w_q, B_w_uk, B_w_uv, B_w_o):
    return _run(A_x, A_wqkv, A_wo, B_x, B_c_kv, B_w_q, B_w_uk, B_w_uv, B_w_o)
```

```python
import functools
import math

import jax
import jax.numpy as jnp
from jax import lax
import jax.experimental.pallas as pl
import jax.experimental.pallas.tpu as pltpu

F32 = jnp.float32
BF16 = jnp.bfloat16
U32 = jnp.uint32
I32 = jnp.int32
LANES = 128
NT_DIMS = (((1,), (1,)), ((), ()))
LOG2E = math.log2(math.e)
MASKED = -1e9

S = 2048
DA = 1024
HA, DHA = 32, 32
WIN, DIL = 8, 2
HALO = 32
MB = 1024
HB, DB = 32, 128
DC = 512


def _quad(x):
    h = len(x) // 2
    return ([r[:h] for r in x[:h]], [r[h:] for r in x[:h]],
            [r[:h] for r in x[h:]], [r[h:] for r in x[h:]])


def _add(x, y):
    return [[a + b for a, b in zip(rx, ry)] for rx, ry in zip(x, y)]


def _sub(x, y):
    return [[a - b for a, b in zip(rx, ry)] for rx, ry in zip(x, y)]


def s_lhs(a):
    if len(a) == 1:
        return [a[0][0]]
    a11, a12, a21, a22 = _quad(a)
    parts = [_add(a11, a22), _add(a21, a22), a11, a22, _add(a11, a12), _sub(a21, a11), _sub(a12, a22)]
    return [z for p in parts for z in s_lhs(p)]


def s_rhs(b):
    if len(b) == 1:
        return [b[0][0]]
    b11, b12, b21, b22 = _quad(b)
    parts = [_add(b11, b22), b11, _sub(b12, b22), _sub(b21, b11), b22, _add(b11, b12), _add(b21, b22)]
    return [z for p in parts for z in s_rhs(p)]


LHS_TERMS = (((1, 0, 0), (1, 1, 1)), ((1, 1, 0), (1, 1, 1)), ((1, 0, 0),), ((1, 1, 1),),
             ((1, 0, 0), (1, 0, 1)), ((1, 1, 0), (-1, 0, 0)), ((1, 0, 1), (-1, 1, 1)))
RHS_TERMS = (((1, 0, 0), (1, 1, 1)), ((1, 0, 0),), ((1, 0, 1), (-1, 1, 1)), ((1, 1, 0), (-1, 0, 0)),
             ((1, 1, 1),), ((1, 0, 0), (1, 0, 1)), ((1, 1, 0), (1, 1, 1)))


TOP_ORDER = (1, 3, 0, 6, 4, 2, 5)


def s_mul(prod, level, emit, base=0):
    if level == 0:
        emit(0, 0, prod(base))
        yield
        return
    n = 2 ** (level - 1)
    step = 7 ** (level - 1)

    def m(i):
        out = [[None] * n for _ in range(n)]

        def keep(a, b, v):
            out[a][b] = v

        yield from s_mul(prod, level - 1, keep, base + (i - 1) * step)
        return out

    def put(x, oi, oj):
        for a in range(n):
            for b in range(n):
                emit(oi * n + a, oj * n + b, x[a][b])

    m2 = yield from m(2)
    m4 = yield from m(4)
    put(_add(m2, m4), 1, 0)
    m1 = yield from m(1)
    c11 = _add(m1, m4)
    c22 = _sub(m1, m2)
    m7 = yield from m(7)
    c11 = _add(c11, m7)
    m5 = yield from m(5)
    put(_sub(c11, m5), 0, 0)
    m3 = yield from m(3)
    put(_add(m3, m5), 0, 1)
    c22 = _add(c22, m3)
    m6 = yield from m(6)
    put(_add(c22, m6), 1, 1)


def _drain(gen):
    for _ in gen:
        pass


def _chain(*gens):
    for g in gens:
        yield from g


def _weigh(gen, w):
    for _ in gen:
        yield w


def _interleave(*streams):
    gens = [s[0] for s in streams]
    total = [s[1] for s in streams]
    span = [s[2:] if len(s) > 2 else (0.0, 1.0) for s in streams]
    done = [0.0] * len(gens)
    live = list(range(len(gens)))
    while live:
        i = min(live, key=lambda k: span[k][0] + (span[k][1] - span[k][0]) * done[k] / total[k])
        try:
            w = next(gens[i])
            done[i] += 1 if w is None else w
        except StopIteration:
            live.remove(i)


def _split(u):
    return pltpu.bitcast(u << 16, F32), pltpu.bitcast(u & jnp.uint32(0xFFFF0000), F32)


def _join(lo, hi):
    return pltpu.bitcast(pltpu.pack_elementwise([lo, hi], packed_dtype=BF16), U32)


def _join_shuffled(v):
    r, c = v.shape
    v4 = v.reshape(r // 16, 2, 8, c)
    return _join(v4[:, 0].reshape(r // 2, c), v4[:, 1].reshape(r // 2, c))


def _split_shuffled(u):
    lo, hi = _split(u)
    r, c = u.shape
    return jnp.stack([lo.reshape(r // 8, 8, c), hi.reshape(r // 8, 8, c)], axis=1).reshape(2 * r, c)


def _unshuffle(pos):
    return (pos & ~15) + ((pos & 15) >> 1) + 8 * (pos & 1)


def _half(u):
    return pltpu.bitcast(u, BF16)


def _cat(xs, axis):
    return xs[0] if len(xs) == 1 else jnp.concatenate(xs, axis=axis)


def _ds(start, size):
    if isinstance(start, int):
        return pl.ds(start, size)
    return pl.ds(pl.multiple_of(start, min(size, 16)), size)


def _when(cond, fn):
    if isinstance(cond, bool):
        if cond:
            fn()
    else:
        pl.when(cond)(fn)


def _loop(n, body, unroll=1):
    if n == unroll:
        for i in range(n):
            body(i)
        return

    def trip(t, _):
        for u in range(unroll):
            body(t * unroll + u)

    lax.fori_loop(0, n // unroll, trip, None)


class _Pacer:
    def __init__(self, words, lag=1):
        self.lag = lag
        self.words = words | 1
        self.marks = []

    def mark(self, v):
        self.marks.append(pltpu.bitcast(v[:, 0:LANES], U32))
        return v

    def hold(self, x, lag=None):
        lag = lag or self.lag
        if len(self.marks) < lag:
            return x
        rows = x.shape[0]
        never = jnp.concatenate([self.words] * (rows // 8), axis=0) == 0
        return pltpu.bitcast(jnp.where(never, self.marks[-lag][0:rows], pltpu.bitcast(x, U32)), x.dtype)


class _LagView:
    def __init__(self, pacer, lag):
        self.pacer, self.lag = pacer, lag

    def hold(self, x):
        return self.pacer.hold(x, self.lag)


class _NoPacer:
    def mark(self, v):
        return v

    def hold(self, x, lag=None):
        return x


def build(LA=2, LAO=2, LB=2, LO=2, ra=256, ro=256, lmode='top', lrows=16, pacel=True, lagl=1, lend=.84, gsub=4, wperm=.4, hold2=False, hm=True, hr=False, hq0=True, pace3=True, lag3=0, two_stage=2, ukv=1, uo=1, uh=1, up=1,
          seq_mode="mid", att_mode="d1", kgrp=1, name="fused", dbg=(), flags=None,
          sp_att=(0., .8), sp_ro=(.3, .6), sp_prep=(.03, .95), zrows=0, vstat=1,
          sp_local=(.04, .96), sp_prepa=(.02, .95), kv_first=False, pace4=True, pace6=True, pacea=True,
          pacelo=True, wlo=6, wsm=4, fly6=True, lag4=1, lag6=1, laga=3, mix6=True, hk=4, hv=4, o_pos=0, unroll6=2, elag=6, marks='qp', sp_lb=(.05, .9), pace1=True, bx_at=0, u1=2, wv_first=True, wv_at=0, lag1=1, lagk=1, pacek=False, sp_k=(.05, .95), sp_s1=(.03, .95), att5=('d1b', 2, 3, 'qp'), pace5=True):
    nA, pA = 2 ** LA, 7 ** LA
    nAO, pAO = 2 ** LAO, 7 ** LAO
    nB, pB = 2 ** LB, 7 ** LB
    nO, pO = 2 ** LO, 7 ** LO
    assert LB >= 1
    gh = nB
    ngrp = HB // gh
    ppg = gh // 2
    nblk = S // ra
    kq = DA // nA
    mq = S // nB
    crow = mq // gh

    def recip(l):
        r = pltpu.reciprocal(l, approx=True)
        return r * (2.0 - l * r)

    def strassen_pairs(load, n, side, store, pacer):
        h = n // 2
        combine = s_lhs if side is LHS_TERMS else s_rhs
        for top, terms in enumerate(side):
            halves = [None, None]
            for sign, qi, qj in terms:
                blocks = [[load(qi * h + i, qj * h + j, pacer.hold) for j in range(h)] for i in range(h)]
                for e in range(2):
                    quad = [[blk[e] for blk in row] for row in blocks]
                    halves[e] = quad if halves[e] is None else (_add if sign > 0 else _sub)(halves[e], quad)
            parts = [combine(x) for x in halves]
            for p in range(len(parts[0])):
                store(top * len(parts[0]) + p, _join(parts[0][p], parts[1][p]))
            yield

    def kernel(ax_hbm, wqkv_hbm, awo_hbm, bx_hbm, c_hbm, wq_hbm, wuk_hbm, wuv_hbm, bwo_hbm,
               out_hbm, x_raw, w_raw, awo_raw, wp, ctx, stage, ro_w, sem_out, sem_a):

        def out_copy(slot, row0, col0, rows=ra):
            return pltpu.make_async_copy(
                stage.at[slot, pl.ds(0, rows)], out_hbm.at[_ds(row0, rows), pl.ds(col0, DA)], sem_out.at[slot])

        kq_o = (HB * DB) // nO // 2
        tpo = 8 // nO

        def ro_rows(p, ct, r0, rows):
            return pl.ds((p * tpo + ct) * kq_o + r0, rows)

        wrows = kq // nblk

        def permuted_rows(t, r0, pacer):
            lane = lax.broadcasted_iota(I32, (8, LANES), 1)
            s, ch, a = lane >> 5, (lane & 31) >> 2, lane & 3
            head = _unshuffle(lane & 31)
            g1 = []
            for j in range(8):
                c0 = t * DA + j * LANES
                u = pacer.hold(pltpu.bitcast(w_raw[_ds(r0, 16), c0:c0 + LANES], I32))
                g1.append(jnp.take_along_axis(u, a * 32 + 4 * ((ch - j) & 7) + s, axis=1))
                if j % gsub == gsub - 1:
                    yield wperm
            v = [g1[(0 - i) % 8] for i in range(8)]
            for bit in (1, 2, 4):
                v = [jnp.where((ch & bit) != 0, v[(i - bit) % 8], v[i]) for i in range(8)]
            out = []
            for i in range(8):
                u = pacer.hold(v[i]) if hold2 else v[i]
                out.append(pltpu.bitcast(jnp.take_along_axis(
                    u, s * 32 + (((head >> 2) + i) & 7) * 4 + (head & 3), axis=1), U32))
                if i % gsub == gsub - 1:
                    yield wperm
            return out

        def wp_rows(blk, t, i, s, c):
            return _ds((((t * nA + i) * (wrows // 16) + s // 16) * 8 + c) * 8, 8)

        def permute_w(blk, t, pacer, quarters=range(nA)):
            for s in range(0, wrows, 16):
                for i in quarters:
                    tiles = yield from permuted_rows(t, i * kq + (blk % nblk) * wrows + s, pacer)
                    for c in range(8):
                        wp[wp_rows(blk, t, i, s, c), :] = tiles[c]

        n_perm_w = (wrows // 16) * nA * 2 * (8 // gsub) * wperm

        def attend_b(c_raw, bwo_raw, lx, lc, rq0, rk0, rv0, rq1, rk1, rv1,
                     qs0, ks0, vs0, qs1, ks1, vs1, sq0, sk0, sv0, sq1, sk1, sv1, sem_in, sem_g):
            rsets = ((rq0, rk0, rv0), (rq1, rk1, rv1))
            qkv = ((qs0, ks0, vs0), (qs1, ks1, vs1))
            staged = ((sq0, sk0, sv0), (sq1, sk1, sv1))

            def weight_copies(par, grp, w):
                words = (wq_hbm, wuk_hbm, wuv_hbm)[w].bitcast(U32)
                n = words.shape[0]
                return [pltpu.make_async_copy(
                    words.at[:, (HB // 2) * parity + grp * ppg + pr],
                    staged[par][w].at[pl.ds((2 * pr + parity) * n, n)], sem_g.at[3 * par + w])
                    for pr in range(ppg) for parity in range(2)]

            def group_copies(par, grp):
                return [c for w in range(3) for c in weight_copies(par, grp, w)]

            def act_copies(src, dst, part, sem):
                return [pltpu.make_async_copy(src.at[_ds(i * mq + part * crow, crow)],
                                              dst.at[_ds(i * mq + part * crow, crow)], sem) for i in range(nB)]

            def c_copies(part):
                return act_copies(c_hbm, c_raw, part, sem_in.at[part])

            c_bx = [pltpu.make_async_copy(bx_hbm, bwo_raw.at[pl.ds(0, S)], sem_in.at[gh])]

            def wo_copies(grp):
                rows = 2 * kq_o // ngrp
                return [pltpu.make_async_copy(bwo_hbm.at[_ds(i * 2 * kq_o + grp * rows, rows)],
                                              bwo_raw.at[_ds(i * 2 * kq_o + grp * rows, rows)], sem_in.at[gh + 1])
                        for i in range(nO)]

            def prep_r(par, w, part, pacer):
                src, dst = staged[par][w], rsets[par][w]
                width = (MB, DC, DC)[w] // 2
                kb = width // nB
                rows = kb // gh
                for s in range(0, rows, 8):
                    r = part * rows + s

                    def load(i, j, hold):
                        return [_split(hold(src[_ds((2 * (j // 2) + e) * width + i * kb + r, 8), :]))[j % 2]
                                for e in range(2)]

                    def store(p, words):
                        dst[p, _ds(r, 8), :] = words

                    yield from strassen_pairs(load, nB, RHS_TERMS, store, pacer)

            def n_prep_r(w):
                return (MB, DC, DC)[w] // nB // gh // 16 * 7

            def prep_group(par, part, pacer):
                return _chain(*[prep_r(par, w, part, pacer) for w in range(3)])

            n_prep = sum(n_prep_r(w) for w in range(3))

            c_a = ([pltpu.make_async_copy(ax_hbm.at[:, pl.ds(j * LANES, LANES)], x_raw.at[j], sem_a) for j in range(8)]
                   + [pltpu.make_async_copy(awo_hbm.at[:, pl.ds(j * LANES, LANES)], awo_raw.at[j], sem_a) for j in range(8)]
                   + [pltpu.make_async_copy(wqkv_hbm, w_raw, sem_a)])

            def prep_lhs(tile, dst, width, part, pacer):
                kb = width // nB
                for t in range(kb // LANES):
                    for s in range(0, crow, 16):
                        r = part * crow + s

                        def load(i, j, hold):
                            return _split(hold(pltpu.bitcast(tile(j * (kb // LANES) + t, _ds(i * mq + r, 16)), U32)))

                        def store(p, words):
                            dst[p, t, _ds(r // 2, 8), :] = words

                        yield from strassen_pairs(load, nB, LHS_TERMS, store, pacer)

            def n_prep_lhs(width):
                return width // nB // LANES * (crow // 16) * 7

            def project(par, w, part, pacer):
                lhs_ref, ktiles = (lx, 8 // nB) if w == 0 else (lc, 4 // nB)
                w_ref, dst = rsets[par][w], qkv[par][w]
                r0 = part * crow

                def prod(p):
                    a = _cat([_half(lhs_ref[p, t, _ds(r0 // 2, crow // 2), :]) for t in range(ktiles)], 1)
                    return pacer.mark(jnp.dot(a, _half(w_ref[p]), preferred_element_type=F32))

                def emit(i, j, v):
                    if w == 0:
                        dst[j, _ds(i * mq + r0, crow), :] = (v * (DB ** -0.5 * LOG2E)).astype(BF16)
                    else:
                        dst[j, _ds((i * mq + r0) // 2, crow // 2), :] = _join_shuffled(v)

                return _weigh(s_mul(prod, LB, emit), ktiles)

            n_proj = pB * (16 // nB)
            bq = LANES
            nb = S // bq

            def attention(par, hl, head, pacer, att_mode, kgrp, elag, marks):
                qs, ks, vs = qkv[par]
                tri = (lax.broadcasted_iota(I32, (bq, bq), 0)
                       >= _unshuffle(lax.broadcasted_iota(I32, (bq, bq), 1)))

                def qk(i):
                    q = qs[hl, i * bq:(i + 1) * bq, :]
                    tiles = []
                    mx = None
                    for c0 in range(0, i + 1, kgrp):
                        n = min(kgrp, i + 1 - c0)
                        k = _half(ks[hl, c0 * bq // 2:(c0 + n) * bq // 2, :])
                        s = lax.dot_general(q, k, NT_DIMS, preferred_element_type=F32)
                        if 'q' in marks:
                            pacer.mark(s)
                        for c in range(n):
                            t = s[:, c * bq:(c + 1) * bq]
                            if c0 + c == i:
                                t = jnp.where(tri, t, MASKED * LOG2E)
                            tiles.append(t)
                            mx = t if mx is None else jnp.maximum(mx, t)
                        yield n
                    return tiles, jnp.max(mx, axis=1, keepdims=True)

                def softmax(tiles, m):
                    ps = [jnp.exp2(s - m) for s in tiles]
                    l = jnp.sum(functools.reduce(jnp.add, ps), axis=1, keepdims=True)
                    return ps, l

                def pv(i, ps, l):
                    o = None
                    for c0 in range(0, i + 1, kgrp):
                        n = min(kgrp, i + 1 - c0)
                        v = _half(vs[hl, c0 * bq // 2:(c0 + n) * bq // 2, :])
                        t = jnp.dot(_cat(ps[c0:c0 + n], 1).astype(BF16), v, preferred_element_type=F32)
                        o = t if o is None else o + t
                        yield n
                    ctx[head, i * bq // 2:(i + 1) * bq // 2, :] = _join_shuffled(o * recip(l))

                def soft_pv(i, tiles, m):
                    o = l = None
                    m = jnp.broadcast_to(m, (bq, bq))
                    for c0 in range(0, i + 1, kgrp):
                        n = min(kgrp, i + 1 - c0)
                        mc = pacer.hold(m, elag) if elag else m
                        ps = [jnp.exp2(s - mc) for s in tiles[c0:c0 + n]]
                        for p in ps:
                            l = p if l is None else l + p
                        v = _half(vs[hl, c0 * bq // 2:(c0 + n) * bq // 2, :])
                        t = jnp.dot(_cat(ps, 1).astype(BF16), v, preferred_element_type=F32)
                        if 'p' in marks:
                            pacer.mark(t)
                        o = t if o is None else o + t
                        yield n
                    l = jnp.sum(l, axis=1, keepdims=True)
                    ctx[head, i * bq // 2:(i + 1) * bq // 2, :] = _join_shuffled(o * recip(l))

                if seq_mode == "mid":
                    seq = list(range(0, nb, 2)) + list(range(1, nb, 2))[::-1]
                elif seq_mode == "alt":
                    seq = [x for pr in zip(range(nb // 2), range(nb - 1, nb // 2 - 1, -1)) for x in pr]
                elif seq_mode == "down":
                    seq = list(range(nb))[::-1]
                elif seq_mode == "up":
                    seq = list(range(nb))
                s, p = {}, {}
                s[0] = yield from qk(seq[0])
                for n in range(nb + 1):
                    if n + 1 < nb:
                        s[n + 1] = yield from qk(seq[n + 1])
                    if att_mode == "d1":
                        if n < nb:
                            yield from soft_pv(seq[n], *s[n])
                        continue
                    if att_mode == "d1b":
                        if n >= 1:
                            yield from soft_pv(seq[n - 1], *s[n - 1])
                        continue
                    if n < nb:
                        p[n] = softmax(*s[n])
                    if n >= 1:
                        yield from pv(seq[n - 1], *p[n - 1])

            n_att = nb * (nb + 1)
            orow = (HB * DB) // nO // HB

            def prep_ro(head, pacer):
                for ct in range(tpo):
                    for s in range(0, orow, 16):
                        r = head * orow + s

                        def load(i, j, hold):
                            c0 = (j * tpo + ct) * LANES
                            return _split(hold(pltpu.bitcast(bwo_raw[_ds(i * 2 * kq_o + r, 16), c0:c0 + LANES], U32)))

                        def store(p, words):
                            ro_w[_ds((p * tpo + ct) * kq_o + r // 2, 8), :] = words

                        yield from strassen_pairs(load, nO, RHS_TERMS, store, pacer)

            n_prep_ro = tpo * (orow // 16) * 7

            def head_step(par, g, hl, main):
                if 'p4' not in dbg and 'p5' not in dbg:
                    @pl.when(hl == 0)
                    def _():
                        for c in wo_copies(g):
                            c.wait()
                        if main:
                            for c in wo_copies(g + 1):
                                c.start()
                        else:
                            for c in c_a:
                                c.wait()

                    if main and par == 0:
                        @pl.when((hl == 0) & (g == ngrp - 2))
                        def _():
                            for c in c_a:
                                c.start()

                if main and 'p4' not in dbg:
                    @pl.when((hl == 0) & (g + 2 < ngrp))
                    def _():
                        for c in group_copies(par, g + 2):
                            c.wait()

                    @pl.when((hl == 0) & (g + 3 < ngrp))
                    def _():
                        for c in group_copies(1 - par, g + 3):
                            c.start()

                pacer = _Pacer(lc[0, 0, 0:8, :], lag4)
                pacer2 = pacer if (pace4 if main else pace5) else _NoPacer()
                parts = [(attention(par, hl, g * gh + hl, pacer, *((att_mode, kgrp, elag, marks) if main else att5)), n_att, *(sp_att if main else (0., 1.)))]
                if main:
                    parts.append((_chain(*[project(1 - par, w, hl, pacer) for w in range(3)]), n_proj))
                if 'noro' not in dbg:
                    parts.append((prep_ro(g * gh + hl, pacer2), n_prep_ro, *sp_ro))
                if not main:
                    assert gh == nA
                    parts.append((_chain(*[permute_w(0, t, pacer, [hl]) for t in range(3)]), 3 * n_perm_w / nA, .1, .8))
                if main and 'noprep' not in dbg:
                    parts.append((prep_group(par, hl, pacer2), n_prep, *sp_prep))
                _interleave(*parts)

            if 'p4' in dbg or 'p5' in dbg:
                o32 = out_hbm.bitcast(U32)
                for r in (lx.at[0, 0], lc.at[0, 0], rq1.at[0], rk1.at[0], rv1.at[0], ks0.at[0], vs0.at[0], sq0, sk0, sv0):
                    pltpu.sync_copy(o32.at[pl.ds(0, 8), pl.ds(0, LANES)], r.at[pl.ds(0, 8)])
                pltpu.sync_copy(out_hbm.at[pl.ds(0, 16), pl.ds(0, LANES)], qs0.at[0, pl.ds(0, 16)])
                pltpu.sync_copy(bwo_hbm.at[pl.ds(0, 16)], bwo_raw.at[pl.ds(0, 16)])
                pltpu.sync_copy(wqkv_hbm.at[pl.ds(0, 16)], w_raw.at[pl.ds(0, 16)])
                with jax.named_scope('P4_dbg'):
                    _loop(16, lambda t: head_step(0, t // gh, t % gh, 'p4' in dbg), uh)
                for r in (qs1,):
                    pltpu.sync_copy(r.at[0, pl.ds(0, 16)], out_hbm.at[pl.ds(0, 16), pl.ds(0, LANES)])
                for r in (wp, ctx.at[0], ro_w, ks1.at[0], vs1.at[0], rq0.at[0], rk0.at[0], rv0.at[0]):
                    pltpu.sync_copy(r.at[pl.ds(0, 8)], o32.at[pl.ds(0, 8), pl.ds(0, LANES)])
                return

            def c_tile(t, rows):
                return c_raw[rows, t * LANES:(t + 1) * LANES]

            def x_tile(t, rows):
                return bwo_raw[rows, t * LANES:(t + 1) * LANES]

            first = c_copies(0) + weight_copies(0, 0, 1)
            with jax.named_scope('S0'):
                for c in first:
                    c.start()
                for c in first:
                    c.wait()
                for c in [c for p in range(1, gh) for c in c_copies(p)] + weight_copies(0, 0, 2):
                    c.start()
                _drain(prep_lhs(c_tile, lc, DC, 0, _NoPacer()))
                _loop(gh, lambda part: _drain(prep_r(0, 1, part, _NoPacer())))
                for c in c_bx + weight_copies(0, 0, 0):
                    c.start()

            def first_k(part):
                if part + 1 < gh:
                    for c in c_copies(part + 1):
                        c.wait()
                    rest = (prep_lhs(c_tile, lc, DC, part + 1, _NoPacer()), n_prep_lhs(DC))
                else:
                    for c in weight_copies(0, 0, 2):
                        c.wait()
                    rest = (_chain(*[prep_r(0, 2, u, _NoPacer()) for u in range(gh)]), gh * n_prep_r(2))
                _interleave((project(0, 1, part, _NoPacer()), n_proj // 4), rest)

            with jax.named_scope('S1k'):
                _loop(gh, first_k, gh)
            with jax.named_scope('S1v'):
                _loop(gh - 1 - vstat, lambda part: _drain(project(0, 2, part, _NoPacer())))
                for part in range(gh - 1 - vstat, gh - 1):
                    _drain(project(0, 2, part, _NoPacer()))
            with jax.named_scope('S1b'):
                for c in c_bx + weight_copies(0, 0, 0):
                    c.wait()
                for c in group_copies(1, 1):
                    c.start()
                _interleave((project(0, 2, gh - 1, _NoPacer()), n_proj // 4),
                            (_chain(*[prep_r(0, 0, u, _NoPacer()) for u in range(gh)],
                                    prep_lhs(x_tile, lx, MB, 0, _NoPacer())), gh * n_prep_r(0) + n_prep_lhs(MB)))
            with jax.named_scope('S2a'):
                _interleave((project(0, 0, 0, _NoPacer()), n_proj // 2),
                            (_chain(*[prep_lhs(x_tile, lx, MB, u, _NoPacer()) for u in range(1, gh)]),
                             (gh - 1) * n_prep_lhs(MB)))
                for c in group_copies(1, 1):
                    c.wait()
                for c in group_copies(0, 2) + wo_copies(0):
                    c.start()
                _drain(prep_group(1, 0, _NoPacer()))

            def first_q(part):
                pacer = _Pacer(rk0[0, 0:8, :])
                _interleave((project(0, 0, part, pacer), n_proj // 2), (prep_group(1, part, pacer), n_prep, .05, .95))

            with jax.named_scope('S2'):
                _loop(gh - 1, lambda u: first_q(u + 1))

            if 'start' in dbg:
                for c in group_copies(0, 2) + wo_copies(0):
                    c.wait()
                o32 = out_hbm.bitcast(U32)
                for r in (qs0,):
                    pltpu.sync_copy(r.at[0, pl.ds(0, 16)], out_hbm.at[pl.ds(0, 16), pl.ds(0, LANES)])
                for r in (ks0.at[0], vs0.at[0], rq1.at[0], rk1.at[0], rv1.at[0]):
                    pltpu.sync_copy(r.at[pl.ds(0, 8)], o32.at[pl.ds(0, 8), pl.ds(0, LANES)])
                return

            def two_groups(t, _):
                _loop(gh, lambda hl: head_step(0, 2 * t, hl, True), uh)

                @pl.when(t < ngrp // 2 - 1)
                def _():
                    _loop(gh, lambda hl: head_step(1, 2 * t + 1, hl, True), uh)

            with jax.named_scope('P4_main'):
                lax.fori_loop(0, ngrp // 2, two_groups, None)
            with jax.named_scope('P5_tail'):
                _loop(gh, lambda hl: head_step(1, ngrp - 1, hl, False), uh)

        if 'noB' not in dbg:
            pl.run_scoped(
                attend_b,
                pltpu.VMEM((S, DC), BF16),
                pltpu.VMEM((HB * DB, MB), BF16),
                pltpu.VMEM((pB, 8 // nB, mq // 2, LANES), U32),
                pltpu.VMEM((pB, 4 // nB, mq // 2, LANES), U32),
                *[pltpu.VMEM((pB, w // nB // 2, LANES), U32) for w in (MB, DC, DC) * 2],
                *[t for _ in range(2) for t in (pltpu.VMEM((gh, S, LANES), BF16),
                                                pltpu.VMEM((gh, S // 2, LANES), U32),
                                                pltpu.VMEM((gh, S // 2, LANES), U32))],
                *[pltpu.VMEM((ppg * w, LANES), U32) for w in (MB, DC, DC) * 2],
                pltpu.SemaphoreType.DMA((gh + 2,)),
                pltpu.SemaphoreType.DMA((6,)),
            )

        def finish(rq_w, rk_w, rv_w, rao_w, la):
            ra_w = (rq_w, rk_w, rv_w)
            tpa, tpao = 8 // nA, 8 // nAO
            grp_rows = 16 * nA
            assert nA == nAO

            def prep_w(blk, t, pacer):
                for s in range(0, wrows, 16):
                    if not two_stage:
                        tiles = []
                        for i in range(nA):
                            tiles.append((yield from permuted_rows(t, i * kq + blk * wrows + s, pacer)))
                    for ct in range(tpa):
                        def load(i, j, hold):
                            if two_stage:
                                return _split(hold(wp[wp_rows(blk, t, i, s, j * tpa + ct), :]))
                            return _split(hold(tiles[i][j * tpa + ct]))

                        def store(p, words):
                            ra_w[t][p, ct, _ds((blk * wrows + s) // 2, 8), :] = words

                        yield from strassen_pairs(load, nA, RHS_TERMS, store, pacer)

            n_prep_w = (wrows // 16) * tpa * 7 + (0 if two_stage else n_perm_w)

            def prep_la(blk, pacer):
                for c in range(ra // grp_rows):
                    for t in range(tpa):
                        def load(i, j, hold):
                            words = x_raw.at[j * tpa + t].bitcast(U32).at[_ds(blk * (ra // 2), ra // 2)]
                            w0 = (c * grp_rows + 32 * (i // 2)) // 2
                            return [_split(hold(words[pl.ds(w0 + e, 8, stride=2), :]))[i % 2] for e in range(2)]

                        def store(p, words):
                            la[p, t, _ds((blk * (ra // nA) + 16 * c) // 2, 8), :] = words

                        yield from strassen_pairs(load, nA, LHS_TERMS, store, pacer)

            n_prep_la = (ra // grp_rows) * tpa * 7

            def prep_wo(blk, pacer):
                dpq = 16 // nAO
                per = nblk // tpao
                ct = blk // per
                n = 2 * dpq // per
                assert per in (2, 4) and n in (2, 4)
                for dp in range(dpq):
                    if per == 4 and dp % 2:
                        continue
                    h0 = 16 * (blk % 2)
                    dd = dp + ((blk // 2) % 2 if per == 4 else 0)
                    src = {}
                    for i in range(nAO):
                        for j in range(nAO):
                            words = awo_raw.at[j * tpao + ct].bitcast(U32).at[pl.ds(pl.multiple_of(h0 * 16, 256), 256)]
                            for e in range(2):
                                u = words[pl.ds(8 * e * 16 + i * dpq + dp, 8, stride=16), :]
                                if per == 4:
                                    u = jnp.where((blk // 2) % 2 == 1,
                                                  words[pl.ds(8 * e * 16 + i * dpq + dp + 1, 8, stride=16), :], u)
                                src[i, j, e] = pacer.hold(u)
                        yield
                    for half in range(2):
                        def store(p, words):
                            rao_w[p, ct, _ds(((2 * dd + half) * HA + h0) // 2, 8), :] = words

                        yield from strassen_pairs(lambda i, j, hold: [_split(hold(src[i, j, e]))[half] for e in range(2)],
                                                  nAO, RHS_TERMS, store, pacer)

            n_prep_wo = (2 * (16 // nAO) * tpao // nblk) * (nAO + 2 * 7)

            def out_b(i):
                rq = ro // nO
                hq = HB // nO
                slot = i % 2
                _when(i >= 2, lambda: out_copy(slot, 0, DA, ro).wait())
                pacer = _Pacer(ro_w[0:8, :], lag6) if pace6 else _NoPacer()
                lhs = {}

                def make_lhs(top):
                    h2 = nO // 2
                    for h in range(hq):
                        for r in range(0, rq, lrows):
                            quad = None
                            for sign, qi, qj in LHS_TERMS[top]:
                                part = [[_split_shuffled(lpacer.hold(ctx[
                                    (qj * h2 + j) * hq + h, _ds((i * ro + (qi * h2 + a) * rq + r) // 2, lrows // 2), :]))
                                    for j in range(h2)] for a in range(h2)]
                                quad = part if quad is None else (_add if sign > 0 else _sub)(quad, part)
                            for p, v in enumerate(s_lhs(quad)):
                                lhs.setdefault(top * (pO // 7) + p, {}).setdefault(h, []).append(v)
                            yield

                lpacer = _LagView(pacer, lagl) if pacel else _NoPacer()
                if lmode == "all":
                    blocks = [[_cat([_split_shuffled(ctx[j * hq + h, _ds((i * ro + a * rq) // 2, rq // 2), :])
                                     for h in range(hq)], 1) for j in range(nO)] for a in range(nO)]
                    lhs_all = [v.astype(BF16) for v in s_lhs(blocks)]
                else:
                    _drain(make_lhs(TOP_ORDER[0]))

                def prod(p):
                    w = _cat([_half(ro_w[ro_rows(p, ct, 0, kq_o), :]) for ct in range(tpo)], 1)
                    if lmode == "all":
                        x = lhs_all[p]
                    else:
                        x = _cat([_cat(lhs[p][h], 0) for h in range(hq)], 1).astype(BF16)
                    return pacer.mark(jnp.dot(x, w, preferred_element_type=F32))

                def emit(a, j, v):
                    stage[slot, a * rq:(a + 1) * rq, j * tpo * LANES:(j + 1) * tpo * LANES] = v.astype(BF16)

                parts = [(s_mul(prod, LO, emit), pO)]
                if lmode != "all":
                    parts.append((_chain(*[make_lhs(t) for t in TOP_ORDER[1:]]), 6 * hq * (rq // lrows), 0., lend))
                if 'noprepa' not in dbg:
                    blks = [i * (ro // ra) + u for u in range(ro // ra)]
                    n = len(blks)
                    more = [(_chain(prep_w(i, t, pacer), permute_w(i + 1, t, pacer)), n_prep_w + n_perm_w)
                            for t in range(3)]
                    if 'nola' not in dbg:
                        more.append((_chain(*[prep_la(b, pacer) for b in blks]), n * n_prep_la))
                    if 'nowo' not in dbg:
                        more.append((_chain(*[prep_wo(b, pacer) for b in blks]), n * n_prep_wo))
                    if mix6:
                        parts += [(*m, *sp_prepa) for m in more]
                    else:
                        parts.append((_chain(*[m[0] for m in more]), sum(m[1] for m in more), *sp_prepa))
                _interleave(*parts)
                out_copy(slot, i * ro, DA, ro).start()

            def branch_a(lo, qa, ka, va):
                def proj_a(t, blk, pacer):
                    rq = ra // nA
                    dst, row0 = ((qa, (blk % 2) * (ra // 2)), (ka, blk * (ra // 2) + HALO), (va, blk * (ra // 2) + HALO))[t]

                    def prod(p):
                        x = _cat([_half(la[p, k, _ds(blk * rq // 2, rq // 2), :]) for k in range(tpa)], 1)
                        w = _cat([_half(ra_w[t][p, ct]) for ct in range(tpa)], 1)
                        return pacer.mark(jnp.dot(x, w, preferred_element_type=F32))

                    def emit(i, j, v):
                        for ct in range(tpa):
                            for c in range(rq // 16):
                                dst[2 * (j * tpa + ct) + i % 2, _ds(row0 + c * (grp_rows // 2) + 16 * (i // 2), 16), :] = (
                                    v[16 * c:16 * (c + 1), ct * LANES:(ct + 1) * LANES])

                    return s_mul(prod, LA, emit)

                def local_attn(blk, pacer, chain):
                    row0, slot = blk * (ra // 2), blk % 2
                    o = {}
                    for r in range(0, ra // 2, 8):
                        for par in range(2):
                            pos = row0 + r + lax.broadcasted_iota(I32, (8, LANES), 0)
                            q = [qa[2 * j + par, _ds(slot * (ra // 2) + r, 8), :] for j in range(8)]
                            if hq0:
                                q = [chain.hold(pacer.hold(x)) for x in q]
                            logits = []
                            for w in range(WIN):
                                acc = None
                                for j in range(8):
                                    k = ka[2 * j + par, pl.ds(row0 + r + HALO - w, 8), :]
                                    t = q[j] * (pacer.hold(k) if j % hk == 0 else k)
                                    acc = t if acc is None else acc + t
                                if hr:
                                    acc = pacer.hold(acc)
                                acc = acc + pltpu.roll(acc, 64, 1)
                                acc = acc + pltpu.roll(acc, 32, 1)
                                acc = acc * (DHA ** -0.5 * LOG2E)
                                if r < w:
                                    acc = jnp.where(pos >= w, acc, MASKED * LOG2E)
                                logits.append(acc)
                                yield
                            m = functools.reduce(jnp.maximum, logits)
                            if hm:
                                m = pacer.hold(m)
                            e = [jnp.exp2(l - m) for l in logits]
                            inv = recip(functools.reduce(jnp.add, e))
                            e = [x * inv for x in e]
                            yield wsm
                            for j in range(8):
                                acc = None
                                for w in range(WIN):
                                    v = va[2 * j + par, pl.ds(row0 + r + HALO - w, 8), :]
                                    t = e[w] * (pacer.hold(v) if w % hv == 0 else v)
                                    acc = t if acc is None else acc + t
                                o[r, par, j] = acc
                                yield
                            chain.mark(acc)
                        if (2 * r + 16) % grp_rows == 0:
                            c = 2 * r // grp_rows
                            for t in range(tpao):
                                def load(i, j, hold):
                                    return [hold(o[c * (grp_rows // 2) + 8 * i, par, j * tpao + t]) for par in range(2)]

                                def store(p, words):
                                    lo[slot * pAO + p, t, 8 * c:8 * (c + 1), :] = words

                                yield from _weigh(strassen_pairs(load, nAO, LHS_TERMS, store,
                                                                 pacer if pacelo else _NoPacer()), wlo)

                n_local = (16 + wsm) * (ra // 8) + tpao * (ra // grp_rows) * 7 * wlo

                def out_a(blk, pacer):
                    rq = ra // nAO
                    slot = blk % 2

                    def prod(p):
                        x = _cat([_half(lo[slot * pAO + p, k]) for k in range(tpao)], 1)
                        w = _cat([_half(rao_w[p, ct]) for ct in range(tpao)], 1)
                        return pacer.mark(jnp.dot(x, w, preferred_element_type=F32))

                    def emit(i, j, v):
                        for c in range(rq // 16):
                            r = c * grp_rows + 16 * i
                            stage[slot, r:r + 16, j * tpao * LANES:(j + 1) * tpao * LANES] = (
                                v[16 * c:16 * (c + 1)].astype(BF16))

                    return s_mul(prod, LAO, emit)

                def a_step(i, project=True, attend=True, final=True):
                    if final:
                        _when(i >= 3, lambda: out_copy((i - 1) % 2, 0, 0).wait())
                    pacer = _Pacer(rk_w[0, 0, 0:8, :], laga if project else 8) if (pacea if project else pace3) else _NoPacer()
                    mm = [proj_a(t, i + 1, pacer) for t in (1, 2, 0)] if project else []
                    if final:
                        mm.insert(min(o_pos, len(mm)), out_a(i - 1, pacer))
                    parts = [(_chain(*mm), (3 * pA if project else 0) + (pAO if final else 0))]
                    if attend:
                        chain = _NoPacer() if project or not lag3 else _Pacer(rk_w[0, 0, 0:8, :], lag3)
                        parts.append((local_attn(i, pacer, chain), n_local, *sp_local))
                    _interleave(*parts)
                    if final:
                        out_copy((i - 1) % 2, (i - 1) * ra, 0).start()

                o32 = out_hbm.bitcast(U32)
                if 'pa' in dbg:
                    for r in (la.at[0, 0], rq_w.at[0, 0], rk_w.at[0, 0], rv_w.at[0, 0], rao_w.at[0, 0], lo.at[0, 0]):
                        pltpu.sync_copy(o32.at[pl.ds(0, 8), pl.ds(0, LANES)], r.at[pl.ds(0, 8)])
                    for r in (qa, ka, va):
                        pltpu.sync_copy(out_hbm.bitcast(F32).at[pl.ds(0, 8), pl.ds(0, LANES)], r.at[0, pl.ds(0, 8)])
                    with jax.named_scope('PA_dbg'):
                        if 'pa3' in dbg:
                            _loop(nblk - 2, lambda t: a_step(t + 1, project=False))
                        elif 'pa1' in dbg:
                            _loop(nblk - 2, lambda t: a_step(t + 1, final=False))
                        else:
                            _loop(nblk - 2, lambda t: a_step(t + 1), ukv)
                    out_copy(0, 0, 0).wait()
                    out_copy(1, 0, 0).wait()
                    for r in (qa, ka, va):
                        pltpu.sync_copy(r.at[0, pl.ds(0, 8)], out_hbm.bitcast(F32).at[pl.ds(0, 8), pl.ds(0, LANES)])
                    pltpu.sync_copy(lo.at[0, 0, pl.ds(0, 8)], o32.at[pl.ds(0, 8), pl.ds(0, LANES)])
                    return
                zeros = jnp.zeros((HALO, LANES), F32)
                for j in range(16):
                    ka[j, 0:HALO, :] = zeros
                    va[j, 0:HALO, :] = zeros
                with jax.named_scope('PA0'):
                    a_step(-1, attend=False, final=False)
                with jax.named_scope('PA1'):
                    a_step(0, final=False)
                with jax.named_scope('PA2'):
                    _loop(nblk - 2, lambda t: a_step(t + 1), ukv)
                with jax.named_scope('PA3'):
                    a_step(nblk - 1, project=False)
                with jax.named_scope('PA4'):
                    a_step(nblk, project=False, attend=False)
                out_copy(0, 0, 0).wait()
                out_copy(1, 0, 0).wait()


            if 'noP6' not in dbg:
                if 'p6' in dbg:
                    o32 = out_hbm.bitcast(U32)
                    pltpu.sync_copy(o32.at[pl.ds(0, 8), pl.ds(0, LANES)], ro_w.at[pl.ds(0, 8)])
                    pltpu.sync_copy(o32.at[pl.ds(0, 8), pl.ds(0, LANES)], ctx.at[0, pl.ds(0, 8)])
                    pltpu.sync_copy(out_hbm.at[pl.ds(0, 16), pl.ds(0, LANES)], x_raw.at[0, pl.ds(0, 16)])
                    pltpu.sync_copy(out_hbm.at[pl.ds(0, 16), pl.ds(0, LANES)], awo_raw.at[0, pl.ds(0, 16)])
                    pltpu.sync_copy(wqkv_hbm.at[pl.ds(0, 16)], w_raw.at[pl.ds(0, 16)])
                with jax.named_scope('P6_out'):
                    _loop(S // ro, out_b, uo)
                for slot in range(2):
                    out_copy(slot, 0, DA, ro).wait()
            if 'p6' in dbg:
                for r in (la.at[0, 0], rq_w.at[0, 0], rk_w.at[0, 0], rv_w.at[0, 0], rao_w.at[0, 0]):
                    pltpu.sync_copy(r.at[pl.ds(0, 8)], o32.at[pl.ds(0, 8), pl.ds(0, LANES)])
                return
            pl.run_scoped(
                branch_a,
                pltpu.VMEM((2 * pAO, 8 // nAO, ra // nAO // 2, LANES), U32),
                pltpu.VMEM((16, ra, LANES), F32),
                pltpu.VMEM((16, HALO + S // 2, LANES), F32),
                pltpu.VMEM((16, HALO + S // 2, LANES), F32),
            )

        if 'noA' not in dbg:
            pl.run_scoped(
                finish,
                *[pltpu.VMEM((pA, 8 // nA, kq // 2, LANES), U32) for _ in range(3)],
                pltpu.VMEM((pAO, 8 // nAO, DA // nAO // 2, LANES), U32),
                pltpu.VMEM((pA, 8 // nA, S // nA // 2, LANES), U32),
            )

    def run(A_x, A_wqkv, A_wo, B_x, B_c_kv, B_w_q, B_w_uk, B_w_uv, B_w_o):
        any_spec = pl.BlockSpec(memory_space=pl.ANY)
        out = pl.pallas_call(
            kernel,
            in_specs=[any_spec] * 9,
            out_specs=any_spec,
            out_shape=jax.ShapeDtypeStruct((S, DA + MB), BF16),
            scratch_shapes=[
                pltpu.VMEM((8, S, LANES), BF16),
                pltpu.VMEM((DA, 3 * DA), BF16),
                pltpu.VMEM((8, DA, LANES), BF16),
                pltpu.VMEM((3 * nA * (kq // nblk // 16) * 64, LANES), U32),
                pltpu.VMEM((HB, S // 2, LANES), U32),
                pltpu.VMEM((2, max(ra, ro), DA), BF16),
                pltpu.VMEM((pO * (8 // nO) * (HB * DB // nO // 2) + zrows, LANES), U32),
                pltpu.SemaphoreType.DMA((2,)),
                pltpu.SemaphoreType.DMA(()),
            ],
            compiler_params=pltpu.CompilerParams(vmem_limit_bytes=127 * 2 ** 20, flags=flags),
            name=name,
        )(A_x.reshape(S, DA), A_wqkv, A_wo, B_x.reshape(S, MB), B_c_kv.reshape(S, DC),
          B_w_q.reshape(MB // 2, 2 * HB, DB), B_w_uk.reshape(DC // 2, 2 * HB, DB),
          B_w_uv.reshape(DC // 2, 2 * HB, DB), B_w_o.reshape(HB * DB, MB))
        return out.reshape(1, S, DA + MB)

    return run


_run = build()


@jax.jit
def pallas_concat_heads__sliding_local_dilated__compressed_kv_cla__prompt_kernel(A_x, A_wqkv, A_wo, B_x, B_c_kv, B_w_q, B_w_uk, B_w_uv, B_w_o):
    return _run(A_x, A_wqkv, A_wo, B_x, B_c_kv, B_w_q, B_w_uk, B_w_uv, B_w_o)
```

```python
import functools
import math

import jax
import jax.numpy as jnp
from jax import lax
import jax.experimental.pallas as pl
import jax.experimental.pallas.tpu as pltpu

F32 = jnp.float32
BF16 = jnp.bfloat16
U32 = jnp.uint32
I32 = jnp.int32
LANES = 128
NT_DIMS = (((1,), (1,)), ((), ()))
LOG2E = math.log2(math.e)
MASKED = -1e9

SEQ = 2048
DA = 1024
HA, DHA = 32, 32
WIN = 8
HALO = 32
MB = 1024
HB, DB = 32, 128
DC = 512

LEVELS = 2
NS = 2 ** LEVELS
NP = 7 ** LEVELS
GROUP = NS
NGROUP = HB // GROUP
MQ = SEQ // NS
PART = MQ // GROUP
ROWS = 256
NBLK = SEQ // ROWS
KQ = DA // NS
TPB = KQ // LANES
KO = HB * DB // NS
WROWS = KQ // NBLK
TILE = LANES
NTILE = SEQ // TILE


LHS_TERMS = (((1, 0, 0), (1, 1, 1)), ((1, 1, 0), (1, 1, 1)), ((1, 0, 0),), ((1, 1, 1),),
             ((1, 0, 0), (1, 0, 1)), ((1, 1, 0), (-1, 0, 0)), ((1, 0, 1), (-1, 1, 1)))
RHS_TERMS = (((1, 0, 0), (1, 1, 1)), ((1, 0, 0),), ((1, 0, 1), (-1, 1, 1)), ((1, 1, 0), (-1, 0, 0)),
             ((1, 1, 1),), ((1, 0, 0), (1, 0, 1)), ((1, 1, 0), (1, 1, 1)))
TOP_ORDER = (1, 3, 0, 6, 4, 2, 5)


def _add(x, y):
    return [[a + b for a, b in zip(rx, ry)] for rx, ry in zip(x, y)]


def _sub(x, y):
    return [[a - b for a, b in zip(rx, ry)] for rx, ry in zip(x, y)]


def _operand(terms, quadrant):
    total = None
    for sign, i, j in terms:
        q = quadrant(i, j)
        total = q if total is None else (_add if sign > 0 else _sub)(total, q)
    return total


def _operands(side, blocks):
    half = len(blocks) // 2
    if half == 0:
        return [blocks[0][0]]

    def quadrant(i, j):
        return [row[j * half:(j + 1) * half] for row in blocks[i * half:(i + 1) * half]]

    return [x for terms in side for x in _operands(side, _operand(terms, quadrant))]


def _multiply(product, emit, level=LEVELS, base=0):
    if level == 0:
        emit(0, 0, product(base))
        yield
        return
    n = 2 ** (level - 1)

    def m(i):
        out = [[None] * n for _ in range(n)]

        def keep(a, b, v):
            out[a][b] = v

        yield from _multiply(product, keep, level - 1, base + (i - 1) * 7 ** (level - 1))
        return out

    def put(x, oi, oj):
        for a in range(n):
            for b in range(n):
                emit(oi * n + a, oj * n + b, x[a][b])

    m2 = yield from m(2)
    m4 = yield from m(4)
    put(_add(m2, m4), 1, 0)
    m1 = yield from m(1)
    c11 = _add(m1, m4)
    c22 = _sub(m1, m2)
    m7 = yield from m(7)
    c11 = _add(c11, m7)
    m5 = yield from m(5)
    put(_sub(c11, m5), 0, 0)
    m3 = yield from m(3)
    put(_add(m3, m5), 0, 1)
    c22 = _add(c22, m3)
    m6 = yield from m(6)
    put(_add(c22, m6), 1, 1)


def _build_operands(side, load, store, hold):
    half = NS // 2
    for top, terms in enumerate(side):
        loaded = {(i, j): [[load(i * half + a, j * half + b, hold) for b in range(half)] for a in range(half)]
                  for _, i, j in terms}
        lo, hi = (_operands(side, _operand(terms, lambda i, j: [[x[e] for x in row] for row in loaded[i, j]]))
                  for e in range(2))
        for p in range(NP // 7):
            store(top * (NP // 7) + p, _join(lo[p], hi[p]))
        yield


def _split(words):
    return pltpu.bitcast(words << 16, F32), pltpu.bitcast(words & jnp.uint32(0xFFFF0000), F32)


def _join(lo, hi):
    return pltpu.bitcast(pltpu.pack_elementwise([lo, hi], packed_dtype=BF16), U32)


def _join_shuffled(v):
    r, c = v.shape
    v = v.reshape(r // 16, 2, 8, c)
    return _join(v[:, 0].reshape(r // 2, c), v[:, 1].reshape(r // 2, c))


def _split_shuffled(words):
    lo, hi = _split(words)
    r, c = words.shape
    return jnp.stack([lo.reshape(r // 8, 8, c), hi.reshape(r // 8, 8, c)], axis=1).reshape(2 * r, c)


def _unshuffle(pos):
    return (pos & ~15) + ((pos & 15) >> 1) + 8 * (pos & 1)


def _matrix(words):
    return pltpu.bitcast(words, BF16)


def _cat(xs, axis):
    return xs[0] if len(xs) == 1 else jnp.concatenate(xs, axis=axis)


def _ds(start, size):
    if isinstance(start, int):
        return pl.ds(start, size)
    return pl.ds(pl.multiple_of(start, min(size, 16)), size)


def _shifted(ref, step, steps, n):
    return ref.at[_ds(step * n, ref.shape[0] - (steps - 1) * n)]


def _when(cond, fn):
    if isinstance(cond, bool):
        if cond:
            fn()
    else:
        pl.when(cond)(fn)


def _loop(n, body):
    lax.fori_loop(0, n, lambda i, carry: body(i), None)


def _start(copies):
    for c in copies:
        c.start()


def _wait(copies):
    for c in copies:
        c.wait()


def _run(steps):
    for _ in steps:
        pass


def _chain(*streams):
    for steps in streams:
        yield from steps


def _weigh(steps, weight):
    for _ in steps:
        yield weight


def _interleave(*streams):
    spans = [s[2:] if len(s) > 2 else (0.0, 1.0) for s in streams]
    done = [0.0] * len(streams)
    live = list(range(len(streams)))
    while live:
        i = min(live, key=lambda k: spans[k][0] + (spans[k][1] - spans[k][0]) * done[k] / streams[k][1])
        try:
            weight = next(streams[i][0])
            done[i] += 1 if weight is None else weight
        except StopIteration:
            live.remove(i)


class _Pacer:
    def __init__(self, words):
        self.odd = words | 1
        self.marks = []

    def mark(self, v):
        self.marks.append(pltpu.bitcast(v[:, 0:LANES], U32))
        return v

    def after(self, lag):
        def hold(x):
            if len(self.marks) < lag:
                return x
            rows = x.shape[0]
            never = jnp.concatenate([self.odd] * (rows // 8), axis=0) == 0
            return pltpu.bitcast(jnp.where(never, self.marks[-lag][0:rows], pltpu.bitcast(x, U32)), x.dtype)

        return hold


def _same(x):
    return x


def _reciprocal(x):
    r = pltpu.reciprocal(x, approx=True)
    return r * (2.0 - x * r)


def build(name="fused_attention", dbg=(),
          head=dict(order=(2, 6, 10, 14, 15, 13, 12, 11, 9, 8, 7, 5, 4, 3, 1, 0), qk=4, pv=1, lag=6),
          tail=dict(order=(0, 2, 4, 6, 8, 10, 12, 14, 15, 13, 11, 9, 7, 5, 3, 1), qk=2, pv=2, lag=3),
          sp_att=(0., .8), sp_wo=(.05, .4), sp_w=(.03, .95), lag4=1,
          sp_lhs=(0., .84), sp_a=(.02, .95), w_shuffle=.4, lag6=1, lagl=1,
          a_main=(3, (.09, .99)), a_first=(2, (.06, .98)), a_last=(4, (0., .96)), w_lo=6, w_soft=4,
          a_order=(2, 1, 0), v_static=0):

    def kernel(ax_hbm, wqkv_hbm, awo_hbm, bx_hbm, c_hbm, wq_hbm, wuk_hbm, wuv_hbm, bwo_hbm, out_hbm,
               ax_raw, wqkv_raw, awo_raw, c_raw, bwo_raw,
               lx, lc, rq0, rq1, rk0, rk1, rv0, rv1, qs0, qs1, ks0, ks1, vs0, vs1,
               sq0, sq1, sk0, sk1, sv0, sv1, ctx, ro, wp, lo, qa, stage,
               sem_c, sem_x, sem_wo, sem_w, sem_a, sem_out):

        def out_copy(slot, row0, col0):
            return pltpu.make_async_copy(
                stage.at[slot], out_hbm.at[_ds(row0, ROWS), pl.ds(col0, DA)], sem_out.at[slot])

        def touch(*refs):
            for r in refs:
                while len(r.shape) > 2:
                    r = r.at[0]
                if r.dtype == BF16:
                    pltpu.sync_copy(r.at[pl.ds(0, 16), pl.ds(0, LANES)], out_hbm.at[pl.ds(0, 16), pl.ds(0, LANES)])
                    pltpu.sync_copy(out_hbm.at[pl.ds(0, 16), pl.ds(0, LANES)], r.at[pl.ds(0, 16), pl.ds(0, LANES)])
                else:
                    o = out_hbm.bitcast(r.dtype).at[pl.ds(0, 8), pl.ds(0, LANES)]
                    pltpu.sync_copy(r.at[pl.ds(0, 8)], o)
                    pltpu.sync_copy(o, r.at[pl.ds(0, 8)])

        a_inputs = ([pltpu.make_async_copy(ax_hbm.at[:, pl.ds(j * LANES, LANES)], ax_raw.at[j], sem_a)
                     for j in range(DA // LANES)]
                    + [pltpu.make_async_copy(awo_hbm.at[:, pl.ds(j * LANES, LANES)], awo_raw.at[j], sem_a)
                       for j in range(DA // LANES)]
                    + [pltpu.make_async_copy(wqkv_hbm, wqkv_raw, sem_a)])

        def wp_rows(t, i, s, c):
            return _ds((((t * NS + i) * (WROWS // 16) + s // 16) * 8 + c) * 8, 8)

        def shuffle_columns(blk, t, hold, quarters=range(NS)):
            lane = lax.broadcasted_iota(I32, (8, LANES), 1)
            slot, chunk, low = lane >> 5, (lane & 31) >> 2, lane & 3
            head_of = _unshuffle(lane & 31)
            for s in range(0, WROWS, 16):
                for i in quarters:
                    rows = _ds(i * KQ + (blk % NBLK) * WROWS + s, 16)
                    moved = []
                    for j in range(8):
                        c0 = t * DA + j * LANES
                        u = hold(pltpu.bitcast(wqkv_raw[rows, c0:c0 + LANES], I32))
                        moved.append(jnp.take_along_axis(u, low * 32 + 4 * ((chunk - j) & 7) + slot, axis=1))
                        if j % 4 == 3:
                            yield w_shuffle
                    v = [moved[-c % 8] for c in range(8)]
                    for bit in (1, 2, 4):
                        v = [jnp.where((chunk & bit) != 0, v[(c - bit) % 8], v[c]) for c in range(8)]
                    for c in range(8):
                        source = slot * 32 + (((head_of >> 2) + c) & 7) * 4 + (head_of & 3)
                        wp[wp_rows(t, i, s, c), :] = pltpu.bitcast(jnp.take_along_axis(v[c], source, axis=1), U32)
                        if c % 4 == 3:
                            yield w_shuffle

        n_shuffle = (WROWS // 16) * NS * 4 * w_shuffle

        weights = ((rq0, rk0, rv0), (rq1, rk1, rv1))
        projected = ((qs0, ks0, vs0), (qs1, ks1, vs1))
        staged = ((sq0, sk0, sv0), (sq1, sk1, sv1))

        def weight_copies(par, grp, w):
            words = (wq_hbm, wuk_hbm, wuv_hbm)[w].bitcast(U32)
            n = words.shape[0]
            return [pltpu.make_async_copy(
                words.at[:, (HB // 2) * parity + grp * (GROUP // 2) + pair],
                staged[par][w].at[pl.ds((2 * pair + parity) * n, n)], sem_w.at[3 * par + w])
                for pair in range(GROUP // 2) for parity in range(2)]

        def group_copies(par, grp):
            return [c for w in range(3) for c in weight_copies(par, grp, w)]

        def c_copies(part):
            return [pltpu.make_async_copy(c_hbm.at[pl.ds(i * MQ + part * PART, PART)],
                                          c_raw.at[pl.ds(i * MQ + part * PART, PART)], sem_c.at[part])
                    for i in range(NS)]

        def wo_copies(grp):
            n = KO // NGROUP
            return [pltpu.make_async_copy(bwo_hbm.at[_ds(i * KO + grp * n, n)],
                                          bwo_raw.at[_ds(i * KO + grp * n, n)], sem_wo) for i in range(NS)]

        x_copy = pltpu.make_async_copy(bx_hbm, bwo_raw.at[pl.ds(0, SEQ)], sem_x)

        def build_weights(par, w, part, hold):
            n = (MB, DC, DC)[w] // 2
            rows = n // NS // GROUP
            src = _shifted(staged[par][w], part, GROUP, rows)
            for s in range(0, rows, 8):
                def load(i, j, hold):
                    return [_split(hold(src[pl.ds((2 * (j // 2) + e) * n + i * (n // NS) + s, 8), :]))[j % 2]
                            for e in range(2)]

                def store(p, words):
                    weights[par][w][p, _ds(part * rows + s, 8), :] = words

                yield from _build_operands(RHS_TERMS, load, store, hold)

        def n_weights(w):
            return (MB, DC, DC)[w] // NS // GROUP // 16 * 7

        def build_group(par, part, hold):
            return _chain(*[build_weights(par, w, part, hold) for w in range(3)])

        n_group = sum(n_weights(w) for w in range(3))

        def build_activations(src, dst, part):
            tiles = src.shape[1] // NS // LANES
            for t in range(tiles):
                for s in range(0, PART, 16):
                    r = part * PART + s

                    def load(i, j, hold):
                        c0 = (j * tiles + t) * LANES
                        return _split(pltpu.bitcast(src[pl.ds(i * MQ + r, 16), c0:c0 + LANES], U32))

                    def store(p, words):
                        dst[p, t, pl.ds(r // 2, 8), :] = words

                    yield from _build_operands(LHS_TERMS, load, store, _same)

        def n_activations(width):
            return width // NS // LANES * (PART // 16) * 7

        def project(par, w, part, mark=_same):
            lhs = lx if w == 0 else lc
            tiles = lhs.shape[1]
            r0 = part * PART
            dst = projected[par][w] if w == 0 else _shifted(projected[par][w], part, GROUP, PART // 2)

            def product(p):
                x = _cat([_matrix(lhs[p, t, _ds(r0 // 2, PART // 2), :]) for t in range(tiles)], 1)
                return mark(jnp.dot(x, _matrix(weights[par][w][p]), preferred_element_type=F32))

            def emit(i, j, v):
                if w == 0:
                    dst[j, _ds(i * MQ + r0, PART), :] = (v * (DB ** -0.5 * LOG2E)).astype(BF16)
                else:
                    dst[pl.ds((j * SEQ + i * MQ) // 2, PART // 2), :] = _join_shuffled(v)

            return _weigh(_multiply(product, emit), tiles)

        n_project = NP * (MB + 2 * DC) // NS // LANES

        def attend(par, h, head_id, pacer, order, qk, pv, lag):
            qs, ks, vs = projected[par]
            hold = pacer.after(lag)
            causal = (lax.broadcasted_iota(I32, (TILE, TILE), 0)
                      >= _unshuffle(lax.broadcasted_iota(I32, (TILE, TILE), 1)))
            keys, values = (r.at[_ds(h * (SEQ // 2), SEQ // 2)] for r in (ks, vs))
            result = ctx.at[_ds(head_id * (SEQ // 2), SEQ // 2)]

            def scores(i):
                q = qs[h, i * TILE:(i + 1) * TILE, :]
                tiles, top = [], None
                for c0 in range(0, i + 1, qk):
                    n = min(qk, i + 1 - c0)
                    k = _matrix(keys[c0 * TILE // 2:(c0 + n) * TILE // 2, :])
                    s = pacer.mark(lax.dot_general(q, k, NT_DIMS, preferred_element_type=F32))
                    for c in range(n):
                        t = s[:, c * TILE:(c + 1) * TILE]
                        if c0 + c == i:
                            t = jnp.where(causal, t, MASKED * LOG2E)
                        tiles.append(t)
                        top = t if top is None else jnp.maximum(top, t)
                    yield n
                return tiles, jnp.max(top, axis=1, keepdims=True)

            def context(i, tiles, top):
                o = total = None
                top = jnp.broadcast_to(top, (TILE, TILE))
                for c0 in range(0, i + 1, pv):
                    n = min(pv, i + 1 - c0)
                    m = hold(top)
                    ps = [jnp.exp2(s - m) for s in tiles[c0:c0 + n]]
                    for p in ps:
                        total = p if total is None else total + p
                    v = _matrix(values[c0 * TILE // 2:(c0 + n) * TILE // 2, :])
                    t = pacer.mark(jnp.dot(_cat(ps, 1).astype(BF16), v, preferred_element_type=F32))
                    o = t if o is None else o + t
                    yield n
                o = o * _reciprocal(jnp.sum(total, axis=1, keepdims=True))
                result[i * TILE // 2:(i + 1) * TILE // 2, :] = _join_shuffled(o)

            pending = {}
            for n in range(NTILE + 2):
                if n < NTILE:
                    pending[n] = yield from scores(order[n])
                if n >= 2:
                    yield from context(order[n - 2], *pending.pop(n - 2))

        n_attend = NTILE * (NTILE + 1)

        def build_wo(head_id, hold):
            n = KO // HB
            src, dst = _shifted(bwo_raw, head_id, HB, n), _shifted(ro, head_id, HB, n // 2)
            for ct in range(TPB):
                for s in range(0, n, 16):
                    def load(i, j, hold):
                        c0 = (j * TPB + ct) * LANES
                        return _split(hold(pltpu.bitcast(src[pl.ds(i * KO + s, 16), c0:c0 + LANES], U32)))

                    def store(p, words):
                        dst[pl.ds(((p * TPB + ct) * KO + s) // 2, 8), :] = words

                    yield from _build_operands(RHS_TERMS, load, store, hold)

        n_wo = TPB * (KO // HB // 16) * 7

        def head_step(par, g, h, more):
            if not dbg:
                @pl.when(h == 0)
                def _():
                    _wait(wo_copies(g))
                    (_start(wo_copies(g + 1)) if more else _wait(a_inputs))

                if more:
                    _when((h == 0) & (g + 2 < NGROUP), lambda: _wait(group_copies(par, g + 2)))
                    _when((h == 0) & (g + 3 < NGROUP), lambda: _start(group_copies(1 - par, g + 3)))
                    if par == 0:
                        _when((h == 0) & (g == NGROUP - 2), lambda: _start(a_inputs))

            pacer = _Pacer(lc[0, 0, 0:8, :])
            hold = pacer.after(lag4)
            head_id = g * GROUP + h
            if more:
                _interleave((attend(par, h, head_id, pacer, **head), n_attend, *sp_att),
                            (_chain(*[project(1 - par, w, h, pacer.mark) for w in (1, 2, 0)]), n_project),
                            (build_wo(head_id, hold), n_wo, *sp_wo),
                            (build_group(par, h, hold), n_group, *sp_w))
            else:
                _interleave((attend(par, h, head_id, pacer, **tail), n_attend),
                            (build_wo(head_id, hold), n_wo, *sp_wo),
                            (_chain(*[shuffle_columns(0, t, hold, [h]) for t in range(3)]),
                             3 * n_shuffle / NS, .1, .8))

        if 'p4' in dbg or 'p5' in dbg:
            touch(lx, lc, rq1, rk1, rv1, ks0, vs0, qs0, sq0, sk0, sv0, bwo_raw, wqkv_raw)
            _loop(16, lambda t: head_step(0, t // GROUP, t % GROUP, 'p4' in dbg))
            touch(wp, ctx, ro, qs1, ks1, vs1, rq0, rk0, rv0)
            return

        def start_up():
            first = c_copies(0) + weight_copies(0, 0, 1)
            _start(first)
            _wait(first)
            _start([c for part in range(1, GROUP) for c in c_copies(part)] + weight_copies(0, 0, 2))
            _run(build_activations(c_raw, lc, 0))
            _loop(GROUP, lambda part: _run(build_weights(0, 1, part, _same)))
            _start([x_copy] + weight_copies(0, 0, 0))
            for part in range(GROUP):
                if part + 1 < GROUP:
                    _wait(c_copies(part + 1))
                    rest = (build_activations(c_raw, lc, part + 1), n_activations(DC))
                else:
                    _wait(weight_copies(0, 0, 2))
                    rest = (_chain(*[build_weights(0, 2, u, _same) for u in range(GROUP)]), GROUP * n_weights(2))
                _interleave((project(0, 1, part), n_project // 4), rest)
            _loop(GROUP - 1 - v_static, lambda part: _run(project(0, 2, part)))
            for part in range(GROUP - 1 - v_static, GROUP - 1):
                _run(project(0, 2, part))
            _wait([x_copy] + weight_copies(0, 0, 0))
            _start(group_copies(1, 1))
            _interleave((project(0, 2, GROUP - 1), n_project // 4),
                        (_chain(*[build_weights(0, 0, u, _same) for u in range(GROUP)],
                                build_activations(bwo_raw, lx, 0)), GROUP * n_weights(0) + n_activations(MB)))
            _interleave((project(0, 0, 0), n_project // 2),
                        (_chain(*[build_activations(bwo_raw, lx, u) for u in range(1, GROUP)]),
                         (GROUP - 1) * n_activations(MB)))
            _wait(group_copies(1, 1))
            _start(group_copies(0, 2) + wo_copies(0))
            _run(build_group(1, 0, _same))

            def first_q(u):
                pacer = _Pacer(rk0[0, 0:8, :])
                _interleave((project(0, 0, u + 1, pacer.mark), n_project // 2),
                            (build_group(1, u + 1, pacer.after(1)), n_group, .05, .95))

            _loop(GROUP - 1, first_q)

        def two_groups(t):
            _loop(GROUP, lambda h: head_step(0, 2 * t, h, True))
            _when(t < NGROUP // 2 - 1, lambda: _loop(GROUP, lambda h: head_step(1, 2 * t + 1, h, True)))

        if not dbg or 'start' in dbg:
            with jax.named_scope('start_up'):
                start_up()
        if 'start' in dbg:
            _wait(group_copies(0, 2) + wo_copies(0))
            touch(qs0, ks0, vs0, rq1, rk1, rv1)
            return
        if not dbg:
            with jax.named_scope('heads'):
                _loop(NGROUP // 2, two_groups)
            with jax.named_scope('last_heads'):
                _loop(GROUP, lambda h: head_step(1, NGROUP - 1, h, False))

        la = lx

        def w_a(t, p, ct, r0, rows):
            if t == 0:
                return (rq0, rq1)[ct], (p, _ds(r0, rows))
            if t == 1:
                return lc, (p, 0, _ds(ct * (KQ // 2) + r0, rows))
            if t == 2:
                buf, tile = divmod(TPB * p + ct, 25)
                assert rows <= 64 or rows == 128
                if rows == 128:
                    return (rk0, rk1, rv0, rv1)[buf], (pl.ds(2 * tile, 2),)
                return (rk0, rk1, rv0, rv1)[buf], (2 * tile + r0 // 64, _ds(r0 % 64, rows))
            buf, tile = divmod(TPB * p, 32)
            return (ks0, ks1, vs0, vs1)[buf], (_ds((tile + ct) * (KQ // 2) + r0, rows),)

        def load_w(t, p):
            tiles = []
            for ct in range(TPB):
                buf, idx = w_a(t, p, ct, 0, KQ // 2)
                tiles.append(_matrix(buf[idx].reshape(KQ // 2, LANES)))
            return _cat(tiles, 1)

        span_a = HALO + SEQ // 2
        group_rows = 16 * NS

        def build_w(blk, t, hold):
            for s in range(0, WROWS, 16):
                for ct in range(TPB):
                    def load(i, j, hold):
                        return _split(hold(wp[wp_rows(t, i, s, j * TPB + ct), :]))

                    def store(p, words):
                        buf, idx = w_a(t, p, ct, (blk * WROWS + s) // 2, 8)
                        buf[idx] = words

                    yield from _build_operands(RHS_TERMS, load, store, hold)

        n_w = (WROWS // 16) * TPB * 7

        def build_x(blk, hold):
            for c in range(ROWS // group_rows):
                for t in range(TPB):
                    def load(i, j, hold):
                        words = ax_raw.at[j * TPB + t].bitcast(U32).at[_ds(blk * (ROWS // 2), ROWS // 2)]
                        w0 = (c * group_rows + 32 * (i // 2)) // 2
                        return [_split(hold(words[pl.ds(w0 + e, 8, stride=2), :]))[i % 2] for e in range(2)]

                    def store(p, words):
                        la[p, t, _ds((blk * (ROWS // NS) + 16 * c) // 2, 8), :] = words

                    yield from _build_operands(LHS_TERMS, load, store, hold)

        n_x = (ROWS // group_rows) * TPB * 7

        def build_awo(blk, hold):
            ct, odd, h0 = blk // 4, (blk // 2) % 2, 16 * (blk % 2)
            pairs = DHA // 2 // NS
            for dp in range(0, pairs, 2):
                src = {}
                for i in range(NS):
                    for j in range(NS):
                        words = awo_raw.at[j * TPB + ct].bitcast(U32).at[pl.ds(pl.multiple_of(h0 * 16, 256), 256)]
                        for e in range(2):
                            w0 = 8 * e * 16 + i * pairs + dp
                            src[i, j, e] = hold(jnp.where(odd == 1, words[pl.ds(w0 + 1, 8, stride=16), :],
                                                          words[pl.ds(w0, 8, stride=16), :]))
                    yield
                for half in range(2):
                    def load(i, j, hold):
                        return [_split(hold(src[i, j, e]))[half] for e in range(2)]

                    def store(p, words):
                        buf, idx = w_a(3, p, ct, ((2 * (dp + odd) + half) * HA + h0) // 2, 8)
                        buf[idx] = words

                    yield from _build_operands(RHS_TERMS, load, store, hold)

        n_awo = (DHA // 2 // NS // 2) * (NS + 2 * 7)

        def output_b(blk):
            slot = blk % 2
            rows = ROWS // NS
            heads = HB // NS
            _when(blk >= 2, lambda: out_copy(slot, 0, DA).wait())
            pacer = _Pacer(ro[0:8, :])
            src = _shifted(ctx, blk, NBLK, ROWS // 2)
            lhs = {}

            def build_lhs(top, hold):
                half = NS // 2
                for h in range(heads):
                    for r in range(0, rows, 16):
                        def quadrant(i, j):
                            return [[_split_shuffled(hold(src[pl.ds(
                                (((j * half + b) * heads + h) * SEQ + (i * half + a) * rows + r) // 2, 8), :]))
                                for b in range(half)] for a in range(half)]

                        for p, v in enumerate(_operands(LHS_TERMS, _operand(LHS_TERMS[top], quadrant))):
                            lhs.setdefault((top * (NP // 7) + p, h), []).append(v)
                        yield

            def product(p):
                x = _cat([_cat(lhs[p, h], 0) for h in range(heads)], 1).astype(BF16)
                w = _cat([_matrix(ro[pl.ds((p * TPB + ct) * KO // 2, KO // 2), :]) for ct in range(TPB)], 1)
                return pacer.mark(jnp.dot(x, w, preferred_element_type=F32))

            def emit(i, j, v):
                stage[slot, i * rows:(i + 1) * rows, j * KQ:(j + 1) * KQ] = v.astype(BF16)

            _run(build_lhs(TOP_ORDER[0], _same))
            hold = pacer.after(lag6)
            _interleave(
                (_multiply(product, emit), NP),
                (_chain(*[build_lhs(t, pacer.after(lagl)) for t in TOP_ORDER[1:]]), 6 * heads * (rows // 16), *sp_lhs),
                *[(_chain(build_w(blk, t, hold), shuffle_columns(blk + 1, t, hold)), n_w + n_shuffle, *sp_a)
                  for t in range(3)],
                (build_x(blk, hold), n_x, *sp_a),
                (build_awo(blk, hold), n_awo, *sp_a))
            out_copy(slot, blk * ROWS, DA).start()

        if 'p6' in dbg:
            touch(ro, ctx, ax_raw, awo_raw, wqkv_raw, wp)
        if not dbg or 'p6' in dbg:
            with jax.named_scope('output_b'):
                _loop(NBLK, output_b)
            _wait([out_copy(0, 0, DA), out_copy(1, 0, DA)])
        if 'p6' in dbg:
            touch(la, rq0, rq1, lc, rk0, rk1, rv0, rv1, ks0, ks1, vs0, vs1, wp)
            return

        def project_a(t, blk, mark):
            rows = ROWS // NS
            dst = _shifted(ro if t == 1 else ctx, blk, NBLK, ROWS // 2)

            def product(p):
                x = _cat([_matrix(la[p, k, _ds(blk * rows // 2, rows // 2), :]) for k in range(TPB)], 1)
                return mark(jnp.dot(x, load_w(t, p), preferred_element_type=F32))

            def emit(i, j, v):
                for ct in range(TPB):
                    for c in range(rows // 16):
                        piece = v[16 * c:16 * (c + 1), ct * LANES:(ct + 1) * LANES]
                        tile = 2 * (j * TPB + ct) + i % 2
                        r = c * (group_rows // 2) + 16 * (i // 2)
                        if t == 0:
                            qa[tile, _ds((blk % 2) * (ROWS // 2) + r, 16), :] = piece
                        else:
                            dst[pl.ds(tile * span_a + HALO + r, 16), :] = pltpu.bitcast(piece, U32)

            return _multiply(product, emit)

        def attend_a(blk, hold):
            row0, slot = blk * (ROWS // 2), blk % 2
            keys, values = (_shifted(buf, blk, NBLK, ROWS // 2) for buf in (ro, ctx))
            o = {}
            for r in range(0, ROWS // 2, 8):
                for par in range(2):
                    def window(buf, j, w):
                        return pltpu.bitcast(buf[pl.ds((2 * j + par) * span_a + HALO + r - w, 8), :], F32)

                    pos = row0 + r + lax.broadcasted_iota(I32, (8, LANES), 0)
                    q = [hold(qa[2 * j + par, _ds(slot * (ROWS // 2) + r, 8), :]) for j in range(8)]
                    logits = []
                    for w in range(WIN):
                        acc = q[0] * hold(window(keys, 0, w))
                        for j in range(1, 8):
                            acc = acc + q[j] * window(keys, j, w)
                        acc = hold(acc)
                        acc = acc + pltpu.roll(acc, 64, 1)
                        acc = acc + pltpu.roll(acc, 32, 1)
                        acc = acc * (DHA ** -0.5 * LOG2E)
                        if r < w:
                            acc = jnp.where(pos >= w, acc, MASKED * LOG2E)
                        logits.append(acc)
                        yield
                    top = functools.reduce(jnp.maximum, logits)
                    e = [jnp.exp2(x - top) for x in logits]
                    scale = _reciprocal(functools.reduce(jnp.add, e))
                    e = [x * scale for x in e]
                    yield w_soft
                    for j in range(8):
                        acc = None
                        for w in range(WIN):
                            v = window(values, j, w)
                            t = e[w] * (hold(v) if w % 4 == 0 else v)
                            acc = t if acc is None else acc + t
                        o[r, par, j] = acc
                        yield
                if (2 * r + 16) % group_rows == 0:
                    c = 2 * r // group_rows
                    for t in range(TPB):
                        def load(i, j, hold):
                            return [hold(o[c * (group_rows // 2) + 8 * i, par, j * TPB + t]) for par in range(2)]

                        def store(p, words):
                            lo[slot * NP + p, t, 8 * c:8 * (c + 1), :] = words

                        yield from _weigh(_build_operands(LHS_TERMS, load, store, hold), w_lo)

        n_attend_a = (16 + w_soft) * (ROWS // 8) + TPB * (ROWS // group_rows) * 7 * w_lo

        def output_a(blk, mark):
            slot = blk % 2

            def product(p):
                x = _cat([_matrix(lo[slot * NP + p, k]) for k in range(TPB)], 1)
                return mark(jnp.dot(x, load_w(3, p), preferred_element_type=F32))

            def emit(i, j, v):
                for c in range(ROWS // group_rows):
                    r = c * group_rows + 16 * i
                    stage[slot, r:r + 16, j * KQ:(j + 1) * KQ] = v[16 * c:16 * (c + 1)].astype(BF16)

            return _multiply(product, emit)

        def step_a(i, pace, project=True, attend=True, output=True):
            if output:
                _when(i >= 3, lambda: out_copy((i - 1) % 2, 0, 0).wait())
            pacer = _Pacer(lc[0, 0, 0:8, :])
            matmuls = [output_a(i - 1, pacer.mark)] if output else []
            matmuls += [project_a(t, i + 1, pacer.mark) for t in a_order] if project else []
            streams = [(_chain(*matmuls), len(matmuls) * NP)]
            if attend:
                streams.append((attend_a(i, pacer.after(pace[0])), n_attend_a, *pace[1]))
            _interleave(*streams)
            if output:
                out_copy((i - 1) % 2, (i - 1) * ROWS, 0).start()

        if dbg:
            touch(la, rq0, rq1, lc, rk0, rk1, rv0, rv1, ks0, ks1, vs0, vs1, lo, qa, ro, ctx)
            if 'pa' in dbg:
                _loop(NBLK - 2, lambda t: step_a(t + 1, a_main))
                _wait([out_copy(0, 0, 0), out_copy(1, 0, 0)])
            elif 'pa3' in dbg:
                _start([out_copy(0, 0, 0), out_copy(1, 0, 0)])
                step_a(NBLK - 1, a_last, project=False)
                step_a(NBLK, None, project=False, attend=False)
                _wait([out_copy(0, 0, 0), out_copy(1, 0, 0)])
            elif 'pa1' in dbg:
                step_a(-1, None, attend=False, output=False)
                step_a(0, a_first, output=False)
            touch(lo, qa, ro, ctx)
            return

        for tile in range(16):
            for buf in (ro, ctx):
                buf[tile * span_a:tile * span_a + HALO, :] = jnp.zeros((HALO, LANES), U32)
        with jax.named_scope('a_first'):
            step_a(-1, None, attend=False, output=False)
            step_a(0, a_first, output=False)
        with jax.named_scope('a_main'):
            _loop(NBLK - 2, lambda t: step_a(t + 1, a_main))
        with jax.named_scope('a_last'):
            step_a(NBLK - 1, a_last, project=False)
            step_a(NBLK, None, project=False, attend=False)
        _wait([out_copy(0, 0, 0), out_copy(1, 0, 0)])

    def words(*shape):
        return pltpu.VMEM(shape + (LANES,), U32)

    scratch = [
        pltpu.VMEM((DA // LANES, SEQ, LANES), BF16),
        pltpu.VMEM((DA, 3 * DA), BF16),
        pltpu.VMEM((DA // LANES, DA, LANES), BF16),
        pltpu.VMEM((SEQ, DC), BF16),
        pltpu.VMEM((HB * DB, MB), BF16),
        words(NP, MB // NS // LANES, MQ // 2),
        words(NP, DC // NS // LANES, MQ // 2),
        *[words(NP, MB // NS // 2)] * 2,
        *[words(NP + 1, DC // NS // 2)] * 4,
        *[pltpu.VMEM((GROUP, SEQ, LANES), BF16)] * 2,
        *[words(GROUP * SEQ // 2)] * 4,
        *[words(GROUP * MB // 2)] * 2,
        *[words(GROUP * DC // 2)] * 4,
        words(HB * SEQ // 2),
        words(NP * TPB * KO // 2),
        words(3 * NS * (WROWS // 16) * 64),
        words(2 * NP, TPB, ROWS // NS // 2),
        pltpu.VMEM((16, ROWS, LANES), F32),
        pltpu.VMEM((2, ROWS, DA), BF16),
        pltpu.SemaphoreType.DMA((GROUP,)),
        pltpu.SemaphoreType.DMA(()),
        pltpu.SemaphoreType.DMA(()),
        pltpu.SemaphoreType.DMA((6,)),
        pltpu.SemaphoreType.DMA(()),
        pltpu.SemaphoreType.DMA((2,)),
    ]

    def run(A_x, A_wqkv, A_wo, B_x, B_c_kv, B_w_q, B_w_uk, B_w_uv, B_w_o):
        hbm = pl.BlockSpec(memory_space=pl.ANY)
        out = pl.pallas_call(
            kernel,
            in_specs=[hbm] * 9,
            out_specs=hbm,
            out_shape=jax.ShapeDtypeStruct((SEQ, DA + MB), BF16),
            scratch_shapes=scratch,
            compiler_params=pltpu.CompilerParams(vmem_limit_bytes=127 * 2 ** 20),
            name=name,
        )(A_x.reshape(SEQ, DA), A_wqkv, A_wo, B_x.reshape(SEQ, MB), B_c_kv.reshape(SEQ, DC),
          B_w_q.reshape(MB // 2, 2 * HB, DB), B_w_uk.reshape(DC // 2, 2 * HB, DB),
          B_w_uv.reshape(DC // 2, 2 * HB, DB), B_w_o.reshape(HB * DB, MB))
        return out.reshape(1, SEQ, DA + MB)

    return run


_fused_call = build()


@jax.jit
def pallas_concat_heads__sliding_local_dilated__compressed_kv_cla__prompt_kernel(A_x, A_wqkv, A_wo, B_x, B_c_kv, B_w_q, B_w_uk, B_w_uv, B_w_o):
    return _fused_call(A_x, A_wqkv, A_wo, B_x, B_c_kv, B_w_q, B_w_uk, B_w_uv, B_w_o)
```

```python
import functools
import math

import jax
import jax.numpy as jnp
from jax import lax
import jax.experimental.pallas as pl
import jax.experimental.pallas.tpu as pltpu

F32 = jnp.float32
BF16 = jnp.bfloat16
U32 = jnp.uint32
I32 = jnp.int32
LANES = 128
NT_DIMS = (((1,), (1,)), ((), ()))
LOG2E = math.log2(math.e)
MASKED = -1e9

SEQ = 2048
DA = 1024
HA, DHA = 32, 32
WIN = 8
HALO = 32
MB = 1024
HB, DB = 32, 128
DC = 512

LEVELS = 2
NS = 2 ** LEVELS
NP = 7 ** LEVELS
GROUP = NS
NGROUP = HB // GROUP
MQ = SEQ // NS
PART = MQ // GROUP
ROWS = 256
NBLK = SEQ // ROWS
KQ = DA // NS
TPB = KQ // LANES
KO = HB * DB // NS
WROWS = KQ // NBLK
TILE = LANES
NTILE = SEQ // TILE
NPAIR = NTILE // 2


LHS_TERMS = (((1, 0, 0), (1, 1, 1)), ((1, 1, 0), (1, 1, 1)), ((1, 0, 0),), ((1, 1, 1),),
             ((1, 0, 0), (1, 0, 1)), ((1, 1, 0), (-1, 0, 0)), ((1, 0, 1), (-1, 1, 1)))
RHS_TERMS = (((1, 0, 0), (1, 1, 1)), ((1, 0, 0),), ((1, 0, 1), (-1, 1, 1)), ((1, 1, 0), (-1, 0, 0)),
             ((1, 1, 1),), ((1, 0, 0), (1, 0, 1)), ((1, 1, 0), (1, 1, 1)))
TOP_ORDER = (1, 3, 0, 6, 4, 2, 5)


def _add(x, y):
    return [[a + b for a, b in zip(rx, ry)] for rx, ry in zip(x, y)]


def _sub(x, y):
    return [[a - b for a, b in zip(rx, ry)] for rx, ry in zip(x, y)]


def _operand(terms, quadrant):
    total = None
    for sign, i, j in terms:
        q = quadrant(i, j)
        total = q if total is None else (_add if sign > 0 else _sub)(total, q)
    return total


def _operands(side, blocks):
    half = len(blocks) // 2
    if half == 0:
        return [blocks[0][0]]

    def quadrant(i, j):
        return [row[j * half:(j + 1) * half] for row in blocks[i * half:(i + 1) * half]]

    return [x for terms in side for x in _operands(side, _operand(terms, quadrant))]


def _multiply(product, emit, level=LEVELS, base=0):
    if level == 0:
        emit(0, 0, product(base))
        yield
        return
    n = 2 ** (level - 1)

    def m(i):
        out = [[None] * n for _ in range(n)]

        def keep(a, b, v):
            out[a][b] = v

        yield from _multiply(product, keep, level - 1, base + (i - 1) * 7 ** (level - 1))
        return out

    def put(x, oi, oj):
        for a in range(n):
            for b in range(n):
                emit(oi * n + a, oj * n + b, x[a][b])

    m2 = yield from m(2)
    m4 = yield from m(4)
    put(_add(m2, m4), 1, 0)
    m1 = yield from m(1)
    c11 = _add(m1, m4)
    c22 = _sub(m1, m2)
    m7 = yield from m(7)
    c11 = _add(c11, m7)
    m5 = yield from m(5)
    put(_sub(c11, m5), 0, 0)
    m3 = yield from m(3)
    put(_add(m3, m5), 0, 1)
    c22 = _add(c22, m3)
    m6 = yield from m(6)
    put(_add(c22, m6), 1, 1)


SPARSE = [0]


def _build_operands(side, load, store, hold, tops=range(7)):
    half = NS // 2
    for top in tops:
        terms = side[top]
        loaded = {(i, j): [[load(i * half + a, j * half + b,
                                 hold if SPARSE[0] == 0 or (a == b and (SPARSE[0] == 1 or n == 0)) else _same)
                            for b in range(half)] for a in range(half)]
                  for n, (_, i, j) in enumerate(terms)}
        lo, hi = (_operands(side, _operand(terms, lambda i, j: [[x[e] for x in row] for row in loaded[i, j]]))
                  for e in range(2))
        for p in range(NP // 7):
            store(top * (NP // 7) + p, _join(lo[p], hi[p]))
        yield


def _split(words):
    return pltpu.bitcast(words << 16, F32), pltpu.bitcast(words & jnp.uint32(0xFFFF0000), F32)


def _join(lo, hi):
    return pltpu.bitcast(pltpu.pack_elementwise([lo, hi], packed_dtype=BF16), U32)


def _join_shuffled(v):
    r, c = v.shape
    v = v.reshape(r // 16, 2, 8, c)
    return _join(v[:, 0].reshape(r // 2, c), v[:, 1].reshape(r // 2, c))


def _split_shuffled(words):
    lo, hi = _split(words)
    r, c = words.shape
    return jnp.stack([lo.reshape(r // 8, 8, c), hi.reshape(r // 8, 8, c)], axis=1).reshape(2 * r, c)


def _unshuffle(pos):
    return (pos & ~15) + ((pos & 15) >> 1) + 8 * (pos & 1)


def _matrix(words):
    return pltpu.bitcast(words, BF16)


def _words(v):
    return pltpu.bitcast(v.astype(BF16), U32)


def _cat(xs, axis):
    return xs[0] if len(xs) == 1 else jnp.concatenate(xs, axis=axis)


def _ds(start, size):
    if isinstance(start, int):
        return pl.ds(start, size)
    return pl.ds(pl.multiple_of(start, min(size, 16)), size)


def _shifted(ref, step, steps, n):
    return ref.at[_ds(step * n, ref.shape[0] - (steps - 1) * n)]


def _when(cond, fn):
    if isinstance(cond, bool):
        if cond:
            fn()
    else:
        pl.when(cond)(fn)


def _loop(n, body):
    lax.fori_loop(0, n, lambda i, carry: body(i), None)


def _start(copies):
    for c in copies:
        c.start()


def _wait(copies):
    for c in copies:
        c.wait()


def _run(steps):
    for _ in steps:
        pass


def _chain(*streams):
    for steps in streams:
        yield from steps


def _weigh(steps, weight):
    for _ in steps:
        yield weight


def _merge(*streams):
    spans = [s[2:] if len(s) > 2 else (0.0, 1.0) for s in streams]
    done = [0.0] * len(streams)
    live = list(range(len(streams)))
    while live:
        i = min(live, key=lambda k: spans[k][0] + (spans[k][1] - spans[k][0]) * done[k] / streams[k][1])
        try:
            weight = next(streams[i][0])
        except StopIteration:
            live.remove(i)
            continue
        weight = 1 if weight is None else weight
        done[i] += weight
        yield weight


def _interleave(*streams):
    _run(_merge(*streams))


class _Pacer:
    def __init__(self, words):
        self.odd = words | 1
        self.marks = []

    def mark(self, v):
        self.marks.append(pltpu.bitcast(v[:, 0:LANES], U32))
        return v

    def after(self, lag):
        def hold(x):
            if len(self.marks) < lag:
                return x
            rows = x.shape[0]
            never = jnp.concatenate([self.odd] * (rows // 8), axis=0) == 0
            return pltpu.bitcast(jnp.where(never, self.marks[-lag][0:rows], pltpu.bitcast(x, U32)), x.dtype)

        return hold


def _same(x):
    return x


def _reciprocal(x):
    r = pltpu.reciprocal(x, approx=True)
    return r * (2.0 - x * r)


S = (.03, .95)


def plan_b(lag=3):
    return (
    ('c0 k', 'c2 c3', 'k0', 'c0 k', '', lag, S),
    ('v c1', 'q x0', 'v0', 'v', 'c1', lag, S),
    ('c2 c3', 'x1 x2 x3', 'k1 v1', '', 'c2 c3', lag, S),
    ('q', 'g1', 'k2 v2', '', 'q', lag, S),
    ('x0', '', 'k3 v3', '', 'x0', lag, S),
    ('x1 x2 x3', 'g2 o', 'q0 q1 q2', '', 'x1 x2 x3', lag, S),
    ('g1', '', 'q3', '', 'g', lag, S),
)


def plan_c(lag=3):
    return (
    ('c0 k', 'c2 c3', 'k0', 'c0 k', '', lag, S),
    ('v c1', 'q x0', 'v0', 'v', 'c1', lag, S),
    ('c2 c3', 'x1 x2 x3', 'k1 v1', '', 'c2 c3', lag, S),
    ('q x0', 'g1', 'k2 v2 k3 v3', '', 'q x0', lag, S),
    ('x1 x2 x3', 'g2 o', 'q0 q1', '', 'x1 x2 x3', lag, S),
    ('g1', '', 'q2 q3', '', 'g', lag, S),
)


def plan_d(lag=3):
    return (
    ('c0 k', 'c2 c3', 'k0', 'c0 k', '', lag, S),
    ('v c1', 'q x0', 'v0', 'v', 'c1', lag, S),
    ('c2 c3 q', 'x1 x2 x3', 'k1 v1', '', 'c2 q0 q1', lag, S),
    ('x0', 'g1', 'k2 v2', '', 'q2 q3 x0', lag, S),
    ('x1 x2', '', 'q0 q1', '', 'x1 x2 c3', lag, S),
    ('x3 g1', 'g2 o', 'q2 k3 v3 q3', '', 'x3 g', lag, S),
)


def build(name="fused_attention", dbg=(),
          head=dict(early_diag=True, lag=9, late='1,4,0,2,5,3,6,', mix=(0, .7, .15, 1), order=(1, 3, 5, 7, 6, 4, 2, 0), w_qk=1),
          tail=dict(early_diag=True, lag=9, late='1,4,0,2,5,3,6,', mix=(0, .7, .15, 1), order=(1, 3, 5, 7, 6, 4, 2, 0), w_qk=1),
          sp_att=(0., .86), sp_wo=(.03, .3), sp_w=(.03, .95), lag4=1, sp_wo5=(.05, .4), sp_sh5=(.1, .8), lag5=1,
          sp_lhs=(0., .84), sp_a=(.02, .95), w_shuffle=.4, lag6=1, lagl=1,
          a_main=(5, (.07, 1.)), a_first=(2, (.06, .98)), a_last=(4, (0., .96)), w_lo=6, w_soft=2,
          a_order=(1, 2, 0), plan='plan_b()', lag_ahead=1, end_ahead=.84, n_ahead=7, first_copies='c0 k v c1', lag_all=0, sparse6=0, p_order=(1, 2, 0), a_holds=(8, 1, 0, 4), sparse=2, span_all=()):

    SPARSE[0] = sparse
    plan = eval(plan) if isinstance(plan, str) else plan

    def kernel(ax_hbm, wqkv_hbm, awo_hbm, bx_hbm, c_hbm, wq_hbm, wuk_hbm, wuv_hbm, bwo_hbm, out_hbm,
               ax_raw, wqkv_raw, awo_raw, c_raw, bwo_raw,
               lx, lc, rq0, rq1, rk0, rk1, rv0, rv1, qs0, qs1, ks0, ks1, vs0, vs1,
               sq0, sq1, sk0, sk1, sv0, sv1, ctx, ro, wp, lo, qa, stage,
               sem_c, sem_x, sem_wo, sem_w, sem_a, sem_out):

        def out_copy(slot, row0, col0):
            return pltpu.make_async_copy(
                stage.at[slot], out_hbm.at[_ds(row0, ROWS), pl.ds(col0, DA)], sem_out.at[slot])

        def touch(*refs):
            for r in refs:
                while len(r.shape) > 2:
                    r = r.at[0]
                if r.dtype == BF16:
                    pltpu.sync_copy(r.at[pl.ds(0, 16), pl.ds(0, LANES)], out_hbm.at[pl.ds(0, 16), pl.ds(0, LANES)])
                    pltpu.sync_copy(out_hbm.at[pl.ds(0, 16), pl.ds(0, LANES)], r.at[pl.ds(0, 16), pl.ds(0, LANES)])
                else:
                    o = out_hbm.bitcast(r.dtype).at[pl.ds(0, 8), pl.ds(0, LANES)]
                    pltpu.sync_copy(r.at[pl.ds(0, 8)], o)
                    pltpu.sync_copy(o, r.at[pl.ds(0, 8)])

        a_inputs = ([pltpu.make_async_copy(ax_hbm.at[:, pl.ds(j * LANES, LANES)], ax_raw.at[j], sem_a)
                     for j in range(DA // LANES)]
                    + [pltpu.make_async_copy(awo_hbm.at[:, pl.ds(j * LANES, LANES)], awo_raw.at[j], sem_a)
                       for j in range(DA // LANES)]
                    + [pltpu.make_async_copy(wqkv_hbm, wqkv_raw, sem_a)])

        def wp_rows(t, i, s, c):
            return _ds((((t * NS + i) * (WROWS // 16) + s // 16) * 8 + c) * 8, 8)

        def shuffle_columns(blk, t, hold, quarters=range(NS)):
            lane = lax.broadcasted_iota(I32, (8, LANES), 1)
            slot, chunk, low = lane >> 5, (lane & 31) >> 2, lane & 3
            head_of = _unshuffle(lane & 31)
            for s in range(0, WROWS, 16):
                for i in quarters:
                    rows = _ds(i * KQ + (blk % NBLK) * WROWS + s, 16)
                    moved = []
                    for j in range(8):
                        c0 = t * DA + j * LANES
                        u = hold(pltpu.bitcast(wqkv_raw[rows, c0:c0 + LANES], I32))
                        moved.append(jnp.take_along_axis(u, low * 32 + 4 * ((chunk - j) & 7) + slot, axis=1))
                        if j % 4 == 3:
                            yield w_shuffle
                    v = [moved[-c % 8] for c in range(8)]
                    for bit in (1, 2, 4):
                        v = [jnp.where((chunk & bit) != 0, v[(c - bit) % 8], v[c]) for c in range(8)]
                    for c in range(8):
                        source = slot * 32 + (((head_of >> 2) + c) & 7) * 4 + (head_of & 3)
                        wp[wp_rows(t, i, s, c), :] = pltpu.bitcast(jnp.take_along_axis(v[c], source, axis=1), U32)
                        if c % 4 == 3:
                            yield w_shuffle

        n_shuffle = (WROWS // 16) * NS * 4 * w_shuffle

        weights = ((rq0, rk0, rv0), (rq1, rk1, rv1))
        projected = ((qs0, ks0, vs0), (qs1, ks1, vs1))
        staged = ((sq0, sk0, sv0), (sq1, sk1, sv1))

        def weight_copies(par, grp, w):
            words = (wq_hbm, wuk_hbm, wuv_hbm)[w].bitcast(U32)
            n = words.shape[0]
            return [pltpu.make_async_copy(
                words.at[:, (HB // 2) * parity + grp * (GROUP // 2) + pair],
                staged[par][w].at[pl.ds((2 * pair + parity) * n, n)], sem_w.at[3 * par + w])
                for pair in range(GROUP // 2) for parity in range(2)]

        def group_copies(par, grp):
            return [c for w in range(3) for c in weight_copies(par, grp, w)]

        def c_copies(part):
            return [pltpu.make_async_copy(c_hbm.at[part], c_raw.at[:, pl.ds(part * PART, PART)], sem_c.at[part])]

        def x_copies(part):
            return [pltpu.make_async_copy(bx_hbm.at[part], bwo_raw.at[:, pl.ds(part * PART, PART)], sem_x.at[part])]

        def wo_copies(grp):
            rows = (slice(None), _ds(grp * (KO // NGROUP), KO // NGROUP))
            return [pltpu.make_async_copy(bwo_hbm.at[rows], bwo_raw.at[rows], sem_wo)]

        def build_weights(par, w, part, hold, tops=range(7)):
            n = (MB, DC, DC)[w] // 2
            rows = n // NS // GROUP
            src = _shifted(staged[par][w], part, GROUP, rows)
            for s in range(0, rows, 8):
                def load(i, j, hold):
                    return [_split(hold(src[pl.ds((2 * (j // 2) + e) * n + i * (n // NS) + s, 8), :]))[j % 2]
                            for e in range(2)]

                def store(p, words):
                    weights[par][w][p, _ds(part * rows + s, 8), :] = words

                yield from _build_operands(RHS_TERMS, load, store, hold, tops)

        def n_weights(w):
            return (MB, DC, DC)[w] // NS // GROUP // 16 * 7

        def build_group(par, part, hold):
            return _chain(*[build_weights(par, w, part, hold) for w in range(3)])

        n_group = sum(n_weights(w) for w in range(3))

        def build_activations(src, dst, part, hold, tops=range(7)):
            tiles = src.shape[2] // NS // LANES
            for t in range(tiles):
                for s in range(0, PART, 16):
                    r = part * PART + s

                    def load(i, j, hold):
                        c0 = (j * tiles + t) * LANES
                        return _split(hold(pltpu.bitcast(src[i, pl.ds(r, 16), c0:c0 + LANES], U32)))

                    def store(p, words):
                        dst[p, t, pl.ds(r // 2, 8), :] = words

                    yield from _build_operands(LHS_TERMS, load, store, hold, tops)

        def n_activations(width):
            return width // NS // LANES * (PART // 16) * 7

        def project(par, w, part, mark):
            lhs = lx if w == 0 else lc
            tiles = lhs.shape[1]
            dst = projected[par][w]
            if w > 0:
                dst = _shifted(dst, part, GROUP, dst.shape[0] // GROUP // GROUP)
            pending = {}

            def product(p):
                x = _cat([_matrix(lhs[p, t, _ds(part * PART // 2, PART // 2), :]) for t in range(tiles)], 1)
                return mark(jnp.dot(x, _matrix(weights[par][w][p]), preferred_element_type=F32))

            def emit(i, j, v):
                if w == 0:
                    dst[j, _ds((part * NS + i) * PART, PART), :] = (v * (DB ** -0.5 * LOG2E)).astype(BF16)
                elif w == 1:
                    dst[pl.ds((j * SEQ + i * PART) // 2, PART // 2), :] = _words(v)
                else:
                    pending[i, j] = v.T
                    if i % 2 == 1:
                        pair = [pending.pop((i - 1 + b, j)) for b in range(2)]
                        blocks = [[t[a * DB // 2:(a + 1) * DB // 2] for t in pair] for a in range(2)]
                        for p, x in enumerate(_operands(LHS_TERMS, blocks)):
                            dst[pl.ds(((j * NPAIR + i // 2) * 7 + p) * DB // 4, DB // 4), :] = _words(x)

            return _weigh(_multiply(product, emit), tiles)

        n_project = NP * (MB + 2 * DC) // NS // LANES

        def attend(par, h, head_id, pacer, order, lag, late, early_diag, w_qk, mix, fast=NPAIR):
            qs, ks, vs = projected[par]
            hold = pacer.after(lag)
            causal = lax.broadcasted_iota(I32, (TILE, TILE), 0) <= lax.broadcasted_iota(I32, (TILE, TILE), 1)
            keys, values = (r.at[_ds(h * (r.shape[0] // GROUP), r.shape[0] // GROUP)] for r in (ks, vs))
            result = ctx.at[_ds(head_id * (SEQ // 2), SEQ // 2)]
            pending = {}

            def fold(op, t):
                return functools.reduce(op, [t[r:r + 8] for r in range(0, TILE, 8)])

            def scores(i):
                q = qs[h, i * TILE:(i + 1) * TILE, :]
                tiles, peaks = [], []
                for j in range(i + 1):
                    k = _matrix(keys[j * TILE // 2:(j + 1) * TILE // 2, :])
                    s = pacer.mark(lax.dot_general(k, q, NT_DIMS, preferred_element_type=F32))
                    if j == i:
                        s = jnp.where(causal, s, MASKED * LOG2E)
                    tiles.append(s)
                    peaks.append(fold(jnp.maximum, s))
                    yield w_qk
                top = jnp.max(functools.reduce(jnp.maximum, peaks), axis=0, keepdims=True)
                if 0 < i // 2 and i // 2 >= NPAIR - fast:
                    mass = functools.reduce(jnp.add, [jnp.exp2(x - top) for x in peaks])
                    top = top + jnp.log2(jnp.sum(mass, axis=0, keepdims=True))
                pending[i] = tiles, jnp.broadcast_to(top, (8, TILE))

            def context(i):
                both = [pending.pop(2 * i + c) for c in range(2)]
                totals = [None, None]
                o = [[None, None], [None, None]]

                def weight(j, c):
                    p = jnp.exp2(both[c][0][j] - _cat([hold(both[c][1])] * (TILE // 8), 0))
                    t = fold(jnp.add, p)
                    totals[c] = t if totals[c] is None else totals[c] + t
                    return p

                def product(j, p, x):
                    v = _matrix(values[(j * 7 + p) * DB // 4:(j * 7 + p + 1) * DB // 4, :])
                    return pacer.mark(jnp.dot(v, x.astype(BF16), preferred_element_type=F32))

                def emit(a, c, v):
                    o[a][c] = v if o[a][c] is None else o[a][c] + v

                def plain(j, c, tiles):
                    for b in range(tiles):
                        p = weight(2 * j + b, c)
                        shared = product(j, 2 + b, p)
                        emit(b, c, shared)
                        emit(1 - b, c, shared + product(j, 5 + b, p))
                        yield 1

                def diagonal():
                    yield from plain(i, 0, 1)
                    yield from plain(i, 1, 2)

                if early_diag:
                    yield from diagonal()
                acc = [None] * 7
                for j in range(i):
                    if i < NPAIR - fast:
                        yield from plain(j, 0, 2)
                        yield from plain(j, 1, 2)
                        continue
                    tiles, n = {}, 0
                    for p in late:
                        if p == ',':
                            yield 4 / 7 * n
                            n = 0
                            continue
                        p = int(p)
                        for _, b, c in RHS_TERMS[p]:
                            if (b, c) not in tiles:
                                tiles[b, c] = weight(2 * j + b, c)
                        t = product(j, p, _operand(RHS_TERMS[p], lambda b, c: [[tiles[b, c]]])[0][0])
                        acc[p] = t if acc[p] is None else acc[p] + t
                        n += 1
                if acc[0] is not None:
                    _run(_multiply(lambda p: acc[p], emit, 1))
                if not early_diag:
                    yield from diagonal()
                for c in range(2):
                    x = _cat([o[0][c], o[1][c]], 0) * _reciprocal(jnp.sum(totals[c], axis=0, keepdims=True))
                    result[(2 * i + c) * TILE // 2:(2 * i + c + 1) * TILE // 2, :] = _join_shuffled(x.T)

            for n in range(NPAIR + 1):
                streams = []
                if n < NPAIR:
                    i = order[n]
                    streams.append((_chain(scores(2 * i), scores(2 * i + 1)), (4 * i + 3) * w_qk, *mix[0:2]))
                if n > 0:
                    streams.append((context(order[n - 1]), 4 * order[n - 1] + 3, *mix[2:4]))
                yield from _merge(*streams)

        def n_attend(w_qk, **_):
            return NTILE * (NTILE + 1) * (1 + w_qk) / 2

        def build_wo(head_id, hold):
            n = KO // HB
            src, dst = bwo_raw.at[:, _ds(head_id * n, n)], _shifted(ro, head_id, HB, n // 2)
            for ct in range(TPB):
                for s in range(0, n, 16):
                    def load(i, j, hold):
                        c0 = (j * TPB + ct) * LANES
                        return _split(hold(pltpu.bitcast(src[i, pl.ds(s, 16), c0:c0 + LANES], U32)))

                    def store(p, words):
                        dst[pl.ds(((p * TPB + ct) * KO + s) // 2, 8), :] = words

                    yield from _build_operands(RHS_TERMS, load, store, hold)

        n_wo = TPB * (KO // HB // 16) * 7

        def head_step(par, g, h, more):
            if not dbg:
                @pl.when(h == 0)
                def _():
                    _wait(wo_copies(g))
                    (_start(wo_copies(g + 1)) if more else _wait(a_inputs))

                if more:
                    _when((h == 0) & (g + 2 < NGROUP), lambda: _wait(group_copies(par, g + 2)))
                    _when((h == 0) & (g + 3 < NGROUP), lambda: _start(group_copies(1 - par, g + 3)))
                    if par == 0:
                        _when((h == 0) & (g == NGROUP - 2), lambda: _start(a_inputs))

            pacer = _Pacer(lc[0, 0, 0:8, :])
            hold = pacer.after(lag4 if more else lag5)
            head_id = g * GROUP + h
            if more:
                _interleave((attend(par, h, head_id, pacer, **head), n_attend(**head), *sp_att),
                            (_chain(*[project(1 - par, w, h, pacer.mark) for w in p_order]), n_project),
                            (build_wo(head_id, hold), n_wo, *sp_wo),
                            (build_group(par, h, hold), n_group, *sp_w))
            else:
                _interleave((attend(par, h, head_id, pacer, **tail), n_attend(**tail)),
                            (build_wo(head_id, hold), n_wo, *sp_wo5),
                            (_chain(*[shuffle_columns(0, t, hold, [h]) for t in range(3)]),
                             3 * n_shuffle / NS, *sp_sh5))

        if 'p4' in dbg or 'p5' in dbg:
            touch(lx, lc, rq1, rk1, rv1, ks0, vs0, qs0, sq0, sk0, sv0, bwo_raw, wqkv_raw)
            _loop(16, lambda t: head_step(0, t // GROUP, t % GROUP, 'p4' in dbg))
            touch(wp, ctx, ro, qs1, ks1, vs1, rq0, rk0, rv0)
            return

        def start_up():
            data = {'k': weight_copies(0, 0, 1), 'v': weight_copies(0, 0, 2), 'q': weight_copies(0, 0, 0),
                    'g1': group_copies(1, 1), 'g2': group_copies(0, 2), 'o': wo_copies(0)}
            for part in range(GROUP):
                data['c%d' % part], data['x%d' % part] = c_copies(part), x_copies(part)

            def operands(job, hold, tops=range(7)):
                kind, part = job[0], int(job[1])
                if kind in 'cx':
                    src, dst = (c_raw, lc) if kind == 'c' else (bwo_raw, lx)
                    return build_activations(src, dst, part, hold, tops), n_activations(src.shape[2])
                if kind == 'g':
                    return build_group(1, part, hold), n_group
                return build_weights(0, 'qkv'.index(kind), part, hold, tops), n_weights('qkv'.index(kind))

            def expand(jobs):
                return [j for job in jobs.split() for j in ([job + str(u) for u in range(GROUP)] if len(job) == 1 else [job])]

            def issue(starts):
                for k in starts.split():
                    if k.isdigit():
                        pl.delay(int(k))
                        continue
                    for c in data[k.rstrip('*')]:
                        c.start(priority=int(k.endswith('*')))

            def step(n, waits, starts, products, ahead, jobs, lag, span):
                with jax.named_scope('s%d_wait' % n):
                    _wait([c for k in waits.split() for c in data[k]])
                    issue(starts)
                with jax.named_scope('s%d_mm' % n):
                    pacer = _Pacer(pltpu.bitcast(c_raw[0, 0:16, 0:LANES], U32))
                    products = [('qkv'.index(p[0]), int(p[1])) for p in products.split()]
                    sizes = [n_project // (4 if w else 2) for w, _ in products]
                    streams = [(_chain(*[project(0, w, part, pacer.mark) for w, part in products]), sum(sizes))]
                    if ahead:
                        def first(tops, hold):
                            return _chain(*[operands(job, hold, [top])[0] for top in tops for job in expand(ahead)])

                        _run(first(TOP_ORDER[:n_ahead], _same))
                        if n_ahead < 7:
                            streams.append((first(TOP_ORDER[n_ahead:], pacer.after(lag_ahead)),
                                            sum(operands(job, None)[1] for job in expand(ahead)) * (7 - n_ahead) / 7,
                                            0., end_ahead * sizes[0] / sum(sizes)))
                    if jobs:
                        jobs = [operands(job, pacer.after(lag_all or lag)) for job in expand(jobs)]
                        streams.append((_chain(*[j[0] for j in jobs]), sum(j[1] for j in jobs), *(span_all or span)))
                    _interleave(*streams)

            def nth(i):
                for n, args in enumerate(plan):
                    pl.when(i == n)(functools.partial(step, n, *args))

            issue(first_copies)
            _loop(len(plan), nth)

        def two_groups(t):
            _loop(GROUP, lambda h: head_step(0, 2 * t, h, True))
            _when(t < NGROUP // 2 - 1, lambda: _loop(GROUP, lambda h: head_step(1, 2 * t + 1, h, True)))

        if not dbg or 'start' in dbg:
            with jax.named_scope('start_up'):
                start_up()
        if 'start' in dbg:
            _wait(group_copies(0, 2) + wo_copies(0))
            touch(qs0, ks0, vs0, rq1, rk1, rv1)
            return
        if not dbg:
            with jax.named_scope('heads'):
                _loop(NGROUP // 2, two_groups)
            with jax.named_scope('last_heads'):
                _loop(GROUP, lambda h: head_step(1, NGROUP - 1, h, False))

        la = lx

        def w_a(t, p, ct, r0, rows):
            if t == 0:
                return (rq0, rq1)[ct], (p, _ds(r0, rows))
            if t == 1:
                return lc, (p, 0, _ds(ct * (KQ // 2) + r0, rows))
            if t == 2:
                buf, tile = divmod(TPB * p + ct, 25)
                assert rows <= 64 or rows == 128
                if rows == 128:
                    return (rk0, rk1, rv0, rv1)[buf], (pl.ds(2 * tile, 2),)
                return (rk0, rk1, rv0, rv1)[buf], (2 * tile + r0 // 64, _ds(r0 % 64, rows))
            buf, tile = divmod(TPB * p, 50)
            return (vs0, vs1)[buf], (_ds((tile + ct) * (KQ // 2) + r0, rows),)

        def load_w(t, p):
            tiles = []
            for ct in range(TPB):
                buf, idx = w_a(t, p, ct, 0, KQ // 2)
                tiles.append(_matrix(buf[idx].reshape(KQ // 2, LANES)))
            return _cat(tiles, 1)

        span_a = HALO + SEQ // 2
        group_rows = 16 * NS

        def build_w(blk, t, hold):
            for s in range(0, WROWS, 16):
                for ct in range(TPB):
                    def load(i, j, hold):
                        return _split(hold(wp[wp_rows(t, i, s, j * TPB + ct), :]))

                    def store(p, words):
                        buf, idx = w_a(t, p, ct, (blk * WROWS + s) // 2, 8)
                        buf[idx] = words

                    yield from _build_operands(RHS_TERMS, load, store, hold)

        n_w = (WROWS // 16) * TPB * 7

        def build_x(blk, hold):
            for c in range(ROWS // group_rows):
                for t in range(TPB):
                    def load(i, j, hold):
                        words = ax_raw.at[j * TPB + t].bitcast(U32).at[_ds(blk * (ROWS // 2), ROWS // 2)]
                        w0 = (c * group_rows + 32 * (i // 2)) // 2
                        return [_split(hold(words[pl.ds(w0 + e, 8, stride=2), :]))[i % 2] for e in range(2)]

                    def store(p, words):
                        la[p, t, _ds((blk * (ROWS // NS) + 16 * c) // 2, 8), :] = words

                    yield from _build_operands(LHS_TERMS, load, store, hold)

        n_x = (ROWS // group_rows) * TPB * 7

        def build_awo(blk, hold):
            ct, odd, h0 = blk // 4, (blk // 2) % 2, 16 * (blk % 2)
            pairs = DHA // 2 // NS
            for dp in range(0, pairs, 2):
                src = {}
                for i in range(NS):
                    for j in range(NS):
                        words = awo_raw.at[j * TPB + ct].bitcast(U32).at[pl.ds(pl.multiple_of(h0 * 16, 256), 256)]
                        for e in range(2):
                            w0 = 8 * e * 16 + i * pairs + dp
                            src[i, j, e] = hold(jnp.where(odd == 1, words[pl.ds(w0 + 1, 8, stride=16), :],
                                                          words[pl.ds(w0, 8, stride=16), :]))
                    yield
                for half in range(2):
                    def load(i, j, hold):
                        return [_split(hold(src[i, j, e]))[half] for e in range(2)]

                    def store(p, words):
                        buf, idx = w_a(3, p, ct, ((2 * (dp + odd) + half) * HA + h0) // 2, 8)
                        buf[idx] = words

                    yield from _build_operands(RHS_TERMS, load, store, hold)

        n_awo = (DHA // 2 // NS // 2) * (NS + 2 * 7)

        def output_b(blk):
            SPARSE[0] = sparse6
            slot = blk % 2
            rows = ROWS // NS
            heads = HB // NS
            _when(blk >= 2, lambda: out_copy(slot, 0, DA).wait())
            pacer = _Pacer(ro[0:8, :])
            src = _shifted(ctx, blk, NBLK, ROWS // 2)
            lhs = {}

            def build_lhs(top, hold):
                half = NS // 2
                for h in range(heads):
                    for r in range(0, rows, 16):
                        def quadrant(i, j):
                            return [[_split_shuffled(hold(src[pl.ds(
                                (((j * half + b) * heads + h) * SEQ + (i * half + a) * rows + r) // 2, 8), :]))
                                for b in range(half)] for a in range(half)]

                        for p, v in enumerate(_operands(LHS_TERMS, _operand(LHS_TERMS[top], quadrant))):
                            lhs.setdefault((top * (NP // 7) + p, h), []).append(v)
                        yield

            def product(p):
                x = _cat([_cat(lhs[p, h], 0) for h in range(heads)], 1).astype(BF16)
                w = _cat([_matrix(ro[pl.ds((p * TPB + ct) * KO // 2, KO // 2), :]) for ct in range(TPB)], 1)
                return pacer.mark(jnp.dot(x, w, preferred_element_type=F32))

            def emit(i, j, v):
                stage[slot, i * rows:(i + 1) * rows, j * KQ:(j + 1) * KQ] = v.astype(BF16)

            _run(build_lhs(TOP_ORDER[0], _same))
            hold = pacer.after(lag6)
            _interleave(
                (_multiply(product, emit), NP),
                (_chain(*[build_lhs(t, pacer.after(lagl)) for t in TOP_ORDER[1:]]), 6 * heads * (rows // 16), *sp_lhs),
                *[(_chain(build_w(blk, t, hold), shuffle_columns(blk + 1, t, hold)), n_w + n_shuffle, *sp_a)
                  for t in range(3)],
                (build_x(blk, hold), n_x, *sp_a),
                (build_awo(blk, hold), n_awo, *sp_a))
            out_copy(slot, blk * ROWS, DA).start()

        if 'p6' in dbg:
            touch(ro, ctx, ax_raw, awo_raw, wqkv_raw, wp)
        if not dbg or 'p6' in dbg:
            with jax.named_scope('output_b'):
                _loop(NBLK, output_b)
            _wait([out_copy(0, 0, DA), out_copy(1, 0, DA)])
        if 'p6' in dbg:
            touch(la, rq0, rq1, lc, rk0, rk1, rv0, rv1, ks0, ks1, vs0, vs1, wp)
            return

        def project_a(t, blk, mark):
            rows = ROWS // NS
            dst = _shifted(ro if t == 1 else ctx, blk, NBLK, ROWS // 2)

            def product(p):
                x = _cat([_matrix(la[p, k, _ds(blk * rows // 2, rows // 2), :]) for k in range(TPB)], 1)
                return mark(jnp.dot(x, load_w(t, p), preferred_element_type=F32))

            def emit(i, j, v):
                for ct in range(TPB):
                    for c in range(rows // 16):
                        piece = v[16 * c:16 * (c + 1), ct * LANES:(ct + 1) * LANES]
                        tile = 2 * (j * TPB + ct) + i % 2
                        r = c * (group_rows // 2) + 16 * (i // 2)
                        if t == 0:
                            qa[tile, _ds((blk % 2) * (ROWS // 2) + r, 16), :] = piece
                        else:
                            dst[pl.ds(tile * span_a + HALO + r, 16), :] = pltpu.bitcast(piece, U32)

            return _multiply(product, emit)

        def attend_a(blk, hold):
            row0, slot = blk * (ROWS // 2), blk % 2
            keys, values = (_shifted(buf, blk, NBLK, ROWS // 2) for buf in (ro, ctx))
            o = {}
            for r in range(0, ROWS // 2, 8):
                for par in range(2):
                    def window(buf, j, w):
                        return pltpu.bitcast(buf[pl.ds((2 * j + par) * span_a + HALO + r - w, 8), :], F32)

                    pos = row0 + r + lax.broadcasted_iota(I32, (8, LANES), 0)
                    q = [(hold if j % a_holds[0] == 0 else _same)(qa[2 * j + par, _ds(slot * (ROWS // 2) + r, 8), :]) for j in range(8)]
                    logits = []
                    for w in range(WIN):
                        acc = q[0] * (hold if a_holds[1] else _same)(window(keys, 0, w))
                        for j in range(1, 8):
                            acc = acc + q[j] * window(keys, j, w)
                        acc = (hold if a_holds[2] else _same)(acc)
                        acc = acc + pltpu.roll(acc, 64, 1)
                        acc = acc + pltpu.roll(acc, 32, 1)
                        acc = acc * (DHA ** -0.5 * LOG2E)
                        if r < w:
                            acc = jnp.where(pos >= w, acc, MASKED * LOG2E)
                        logits.append(acc)
                        yield
                    top = functools.reduce(jnp.maximum, logits)
                    e = [jnp.exp2(x - top) for x in logits]
                    scale = _reciprocal(functools.reduce(jnp.add, e))
                    e = [x * scale for x in e]
                    yield w_soft
                    for j in range(8):
                        acc = None
                        for w in range(WIN):
                            v = window(values, j, w)
                            t = e[w] * (hold(v) if w % a_holds[3] == 0 else v)
                            acc = t if acc is None else acc + t
                        o[r, par, j] = acc
                        yield
                if (2 * r + 16) % group_rows == 0:
                    c = 2 * r // group_rows
                    for t in range(TPB):
                        def load(i, j, hold):
                            return [hold(o[c * (group_rows // 2) + 8 * i, par, j * TPB + t]) for par in range(2)]

                        def store(p, words):
                            lo[slot * NP + p, t, 8 * c:8 * (c + 1), :] = words

                        yield from _weigh(_build_operands(LHS_TERMS, load, store, hold), w_lo)

        n_attend_a = (16 + w_soft) * (ROWS // 8) + TPB * (ROWS // group_rows) * 7 * w_lo

        def output_a(blk, mark):
            slot = blk % 2

            def product(p):
                x = _cat([_matrix(lo[slot * NP + p, k]) for k in range(TPB)], 1)
                return mark(jnp.dot(x, load_w(3, p), preferred_element_type=F32))

            def emit(i, j, v):
                for c in range(ROWS // group_rows):
                    r = c * group_rows + 16 * i
                    stage[slot, r:r + 16, j * KQ:(j + 1) * KQ] = v[16 * c:16 * (c + 1)].astype(BF16)

            return _multiply(product, emit)

        def step_a(i, pace, project=True, attend=True, output=True):
            SPARSE[0] = sparse
            if output:
                _when(i >= 3, lambda: out_copy((i - 1) % 2, 0, 0).wait())
            pacer = _Pacer(lc[0, 0, 0:8, :])
            matmuls = [output_a(i - 1, pacer.mark)] if output else []
            matmuls += [project_a(t, i + 1, pacer.mark) for t in a_order] if project else []
            streams = [(_chain(*matmuls), len(matmuls) * NP)]
            if attend:
                streams.append((attend_a(i, pacer.after(pace[0])), n_attend_a, *pace[1]))
            _interleave(*streams)
            if output:
                out_copy((i - 1) % 2, (i - 1) * ROWS, 0).start()

        if dbg:
            touch(la, rq0, rq1, lc, rk0, rk1, rv0, rv1, ks0, ks1, vs0, vs1, lo, qa, ro, ctx)
            if 'pa' in dbg:
                _loop(NBLK - 2, lambda t: step_a(t + 1, a_main))
                _wait([out_copy(0, 0, 0), out_copy(1, 0, 0)])
            elif 'pa3' in dbg:
                _start([out_copy(0, 0, 0), out_copy(1, 0, 0)])
                step_a(NBLK - 1, a_last, project=False)
                step_a(NBLK, None, project=False, attend=False)
                _wait([out_copy(0, 0, 0), out_copy(1, 0, 0)])
            elif 'pa1' in dbg:
                step_a(-1, None, attend=False, output=False)
                step_a(0, a_first, output=False)
            touch(lo, qa, ro, ctx)
            return

        for tile in range(16):
            for buf in (ro, ctx):
                buf[tile * span_a:tile * span_a + HALO, :] = jnp.zeros((HALO, LANES), U32)
        with jax.named_scope('a_first'):
            step_a(-1, None, attend=False, output=False)
            step_a(0, a_first, output=False)
        with jax.named_scope('a_main'):
            _loop(NBLK - 2, lambda t: step_a(t + 1, a_main))
        with jax.named_scope('a_last'):
            step_a(NBLK - 1, a_last, project=False)
            step_a(NBLK, None, project=False, attend=False)
        _wait([out_copy(0, 0, 0), out_copy(1, 0, 0)])

    def words(*shape):
        return pltpu.VMEM(shape + (LANES,), U32)

    scratch = [
        pltpu.VMEM((DA // LANES, SEQ, LANES), BF16),
        pltpu.VMEM((DA, 3 * DA), BF16),
        pltpu.VMEM((DA // LANES, DA, LANES), BF16),
        pltpu.VMEM((NS, MQ, DC), BF16),
        pltpu.VMEM((NS, KO, MB), BF16),
        words(NP, MB // NS // LANES, MQ // 2),
        words(NP, DC // NS // LANES, MQ // 2),
        *[words(NP, MB // NS // 2)] * 2,
        *[words(NP + 1, DC // NS // 2)] * 4,
        *[pltpu.VMEM((GROUP, SEQ, LANES), BF16)] * 2,
        *[words(GROUP * SEQ // 2)] * 2,
        *[words(GROUP * NPAIR * 7 * DB // 4)] * 2,
        *[words(GROUP * MB // 2)] * 2,
        *[words(GROUP * DC // 2)] * 4,
        words(HB * SEQ // 2),
        words(NP * TPB * KO // 2),
        words(3 * NS * (WROWS // 16) * 64),
        words(2 * NP, TPB, ROWS // NS // 2),
        pltpu.VMEM((16, ROWS, LANES), F32),
        pltpu.VMEM((2, ROWS, DA), BF16),
        pltpu.SemaphoreType.DMA((GROUP,)),
        pltpu.SemaphoreType.DMA((GROUP,)),
        pltpu.SemaphoreType.DMA(()),
        pltpu.SemaphoreType.DMA((6,)),
        pltpu.SemaphoreType.DMA(()),
        pltpu.SemaphoreType.DMA((2,)),
    ]

    def run(A_x, A_wqkv, A_wo, B_x, B_c_kv, B_w_q, B_w_uk, B_w_uv, B_w_o):
        hbm = pl.BlockSpec(memory_space=pl.ANY)
        out = pl.pallas_call(
            kernel,
            in_specs=[hbm] * 9,
            out_specs=hbm,
            out_shape=jax.ShapeDtypeStruct((SEQ, DA + MB), BF16),
            scratch_shapes=scratch,
            compiler_params=pltpu.CompilerParams(vmem_limit_bytes=127 * 2 ** 20),
            name=name,
        )(A_x.reshape(SEQ, DA), A_wqkv, A_wo, B_x.reshape(GROUP, NS, PART, MB), B_c_kv.reshape(GROUP, NS, PART, DC),
          B_w_q.reshape(MB // 2, 2 * HB, DB), B_w_uk.reshape(DC // 2, 2 * HB, DB),
          B_w_uv.reshape(DC // 2, 2 * HB, DB), B_w_o.reshape(NS, KO, MB))
        return out.reshape(1, SEQ, DA + MB)

    return run


_fused_call = build()


@jax.jit
def pallas_concat_heads__sliding_local_dilated__compressed_kv_cla__prompt_kernel(A_x, A_wqkv, A_wo, B_x, B_c_kv, B_w_q, B_w_uk, B_w_uv, B_w_o):
    return _fused_call(A_x, A_wqkv, A_wo, B_x, B_c_kv, B_w_q, B_w_uk, B_w_uv, B_w_o)
```

```python
import functools
import math

import jax
import jax.numpy as jnp
from jax import lax
import jax.experimental.pallas as pl
import jax.experimental.pallas.tpu as pltpu

F32 = jnp.float32
BF16 = jnp.bfloat16
U32 = jnp.uint32
I32 = jnp.int32
LANES = 128
NT_DIMS = (((1,), (1,)), ((), ()))
LOG2E = math.log2(math.e)
MASKED = -1e9

SEQ = 2048
DA = 1024
HA, DHA = 32, 32
WIN = 8
HALO = 32
MB = 1024
HB, DB = 32, 128
DC = 512

LEVELS = 2
NS = 2 ** LEVELS
NP = 7 ** LEVELS
GROUP = NS
NGROUP = HB // GROUP
MQ = SEQ // NS
PART = MQ // GROUP
ROWS = 256
NBLK = SEQ // ROWS
KQ = DA // NS
TPB = KQ // LANES
KO = HB * DB // NS
WROWS = KQ // NBLK
TILE = LANES
NTILE = SEQ // TILE
NPAIR = NTILE // 2


LHS_TERMS = (((1, 0, 0), (1, 1, 1)), ((1, 1, 0), (1, 1, 1)), ((1, 0, 0),), ((1, 1, 1),),
             ((1, 0, 0), (1, 0, 1)), ((1, 1, 0), (-1, 0, 0)), ((1, 0, 1), (-1, 1, 1)))
RHS_TERMS = (((1, 0, 0), (1, 1, 1)), ((1, 0, 0),), ((1, 0, 1), (-1, 1, 1)), ((1, 1, 0), (-1, 0, 0)),
             ((1, 1, 1),), ((1, 0, 0), (1, 0, 1)), ((1, 1, 0), (1, 1, 1)))
TOP_ORDER = (1, 3, 0, 6, 4, 2, 5)


def _add(x, y):
    return [[a + b for a, b in zip(rx, ry)] for rx, ry in zip(x, y)]


def _sub(x, y):
    return [[a - b for a, b in zip(rx, ry)] for rx, ry in zip(x, y)]


def _operand(terms, quadrant):
    total = None
    for sign, i, j in terms:
        q = quadrant(i, j)
        total = q if total is None else (_add if sign > 0 else _sub)(total, q)
    return total


def _operands(side, blocks):
    half = len(blocks) // 2
    if half == 0:
        return [blocks[0][0]]

    def quadrant(i, j):
        return [row[j * half:(j + 1) * half] for row in blocks[i * half:(i + 1) * half]]

    return [x for terms in side for x in _operands(side, _operand(terms, quadrant))]


def _multiply(product, emit, level=LEVELS, base=0):
    if level == 0:
        emit(0, 0, product(base))
        yield
        return
    n = 2 ** (level - 1)

    def m(i):
        out = [[None] * n for _ in range(n)]

        def keep(a, b, v):
            out[a][b] = v

        yield from _multiply(product, keep, level - 1, base + (i - 1) * 7 ** (level - 1))
        return out

    def put(x, oi, oj):
        for a in range(n):
            for b in range(n):
                emit(oi * n + a, oj * n + b, x[a][b])

    m2 = yield from m(2)
    m4 = yield from m(4)
    put(_add(m2, m4), 1, 0)
    m1 = yield from m(1)
    c11 = _add(m1, m4)
    c22 = _sub(m1, m2)
    m7 = yield from m(7)
    c11 = _add(c11, m7)
    m5 = yield from m(5)
    put(_sub(c11, m5), 0, 0)
    m3 = yield from m(3)
    put(_add(m3, m5), 0, 1)
    c22 = _add(c22, m3)
    m6 = yield from m(6)
    put(_add(c22, m6), 1, 1)


SPARSE = [0]


def _build_operands(side, load, store, hold, tops=range(7)):
    half = NS // 2
    for top in tops:
        terms = side[top]
        loaded = {(i, j): [[load(i * half + a, j * half + b,
                                 hold if SPARSE[0] == 0 or (a == b and (SPARSE[0] == 1 or n == 0)) else _same)
                            for b in range(half)] for a in range(half)]
                  for n, (_, i, j) in enumerate(terms)}
        lo, hi = (_operands(side, _operand(terms, lambda i, j: [[x[e] for x in row] for row in loaded[i, j]]))
                  for e in range(2))
        for p in range(NP // 7):
            store(top * (NP // 7) + p, _join(lo[p], hi[p]))
        yield


def _split(words):
    return pltpu.bitcast(words << 16, F32), pltpu.bitcast(words & jnp.uint32(0xFFFF0000), F32)


def _join(lo, hi):
    return pltpu.bitcast(pltpu.pack_elementwise([lo, hi], packed_dtype=BF16), U32)


def _join_shuffled(v):
    r, c = v.shape
    v = v.reshape(r // 16, 2, 8, c)
    return _join(v[:, 0].reshape(r // 2, c), v[:, 1].reshape(r // 2, c))


def _split_shuffled(words):
    lo, hi = _split(words)
    r, c = words.shape
    return jnp.stack([lo.reshape(r // 8, 8, c), hi.reshape(r // 8, 8, c)], axis=1).reshape(2 * r, c)


def _unshuffle(pos):
    return (pos & ~15) + ((pos & 15) >> 1) + 8 * (pos & 1)


def _matrix(words):
    return pltpu.bitcast(words, BF16)


def _cat(xs, axis):
    return xs[0] if len(xs) == 1 else jnp.concatenate(xs, axis=axis)


def _ds(start, size):
    if isinstance(start, int):
        return pl.ds(start, size)
    return pl.ds(pl.multiple_of(start, min(size, 16)), size)


def _shifted(ref, step, steps, n):
    return ref.at[_ds(step * n, ref.shape[0] - (steps - 1) * n)]


def _when(cond, fn):
    if isinstance(cond, bool):
        if cond:
            fn()
    else:
        pl.when(cond)(fn)


def _loop(n, body):
    lax.fori_loop(0, n, lambda i, carry: body(i), None)


def _start(copies):
    for c in copies:
        c.start()


def _wait(copies):
    for c in copies:
        c.wait()


def _run(steps):
    for _ in steps:
        pass


def _chain(*streams):
    for steps in streams:
        yield from steps


def _weigh(steps, weight):
    for _ in steps:
        yield weight


def _merge(*streams):
    spans = [s[2:] if len(s) > 2 else (0.0, 1.0) for s in streams]
    done = [0.0] * len(streams)
    live = list(range(len(streams)))
    while live:
        i = min(live, key=lambda k: spans[k][0] + (spans[k][1] - spans[k][0]) * done[k] / streams[k][1])
        try:
            weight = next(streams[i][0])
        except StopIteration:
            live.remove(i)
            continue
        weight = 1 if weight is None else weight
        done[i] += weight
        yield weight


def _interleave(*streams):
    _run(_merge(*streams))


class _Pacer:
    def __init__(self, words):
        self.odd = words | 1
        self.marks = []

    def mark(self, v):
        self.marks.append(pltpu.bitcast(v[:, 0:LANES], U32))
        return v

    def after(self, lag):
        def hold(x):
            if len(self.marks) < lag:
                return x
            rows = x.shape[0]
            never = jnp.concatenate([self.odd] * (rows // 8), axis=0) == 0
            return pltpu.bitcast(jnp.where(never, self.marks[-lag][0:rows], pltpu.bitcast(x, U32)), x.dtype)

        return hold


def _same(x):
    return x


def _reciprocal(x):
    r = pltpu.reciprocal(x, approx=True)
    return r * (2.0 - x * r)


PLANS = dict(
    e=(('c0 k', 'c2 q', 'k0', 'c0 k', ''),
       ('v c1', 'x0 c3', 'v0', 'v', 'c1'),
       ('c2 q', 'x1 x2 x3', 'k1 v1', '', 'c2 q0 q1'),
       ('x0', 'g1', 'k2 v2', '', 'q2 q3 x0'),
       ('c3 x1 x2', 'g2 o', 'q0 q1', '', 'x1 x2 c3'),
       ('x3 g1', '', 'q2 k3 v3 q3', '', 'x3 g')),
)


def build(name="fused_attention", dbg=(),
          head=dict(early_diag=True, lag=9, late='1,4,0,2,5,3,6,', mix=(0, .7, .15, 1), order=(1, 3, 5, 7, 6, 4, 2, 0), w_qk=1),
          tail=dict(early_diag=True, lag=11, late='14,02,53,6,', mix=(0, .6, .25, 1), order=(1, 3, 5, 7, 6, 4, 2, 0), w_qk=1.1, fast=5),
          sp_att=(0., .86), sp_wo=(.02, .2), sp_w=(.3, .98), lag4=1, sp_wo5=(.03, .3), sp_sh5=(.1, .8), lag5=1,
          sp_lhs=(0., .84), sp_a=(.02, .95), w_shuffle=1., lag6=1, lagl=1,
          a_main=(5, (.07, 1.)), a_first=(2, (.06, .98)), a_last=(4, (0., .96)), w_lo=6, w_soft=2,
          a_order=(1, 2, 0), plan='e', paces={'s0': (5, 0.07, 0.9, 1), 's1': (99, 0.04, 0.93, 2), 's2': (14, 0.0, 0.93, 2), 's3': (14, 0.02, 0.99, 2), 's4': (1, 0.02, 0.99, 1), 's5': (3, 0.02, 0.96, 2)}, lag_ahead=1, end_ahead=.84, n_ahead=7, first_copies='c0 k v c1', sparsel=4, sparse6=0, p_order=(2, 1, 0), a_holds=(8, 1, 0, 4), sparse=2):

    SPARSE[0] = sparse
    plan = PLANS[plan]

    def kernel(ax_hbm, wqkv_hbm, awo_hbm, bx_hbm, c_hbm, wq_hbm, wuk_hbm, wuv_hbm, bwo_hbm, out_hbm,
               ax_raw, wqkv_raw, awo_raw, c_raw, bwo_raw,
               lx, lc, rq0, rq1, rk0, rk1, rv0, rv1, qs0, qs1, ks0, ks1, vs0, vs1,
               sq0, sq1, sk0, sk1, sv0, sv1, ctx, ro, wp, lo, qa, stage,
               sem_c, sem_x, sem_wo, sem_w, sem_a, sem_out):

        def out_copy(slot, row0, col0):
            return pltpu.make_async_copy(
                stage.at[slot], out_hbm.at[_ds(row0, ROWS), pl.ds(col0, DA)], sem_out.at[slot])

        def touch(*refs):
            for r in refs:
                while len(r.shape) > 2:
                    r = r.at[0]
                if r.dtype == BF16:
                    pltpu.sync_copy(r.at[pl.ds(0, 16), pl.ds(0, LANES)], out_hbm.at[pl.ds(0, 16), pl.ds(0, LANES)])
                    pltpu.sync_copy(out_hbm.at[pl.ds(0, 16), pl.ds(0, LANES)], r.at[pl.ds(0, 16), pl.ds(0, LANES)])
                else:
                    o = out_hbm.bitcast(r.dtype).at[pl.ds(0, 8), pl.ds(0, LANES)]
                    pltpu.sync_copy(r.at[pl.ds(0, 8)], o)
                    pltpu.sync_copy(o, r.at[pl.ds(0, 8)])

        a_inputs = ([pltpu.make_async_copy(ax_hbm.at[:, pl.ds(j * LANES, LANES)], ax_raw.at[j], sem_a)
                     for j in range(DA // LANES)]
                    + [pltpu.make_async_copy(awo_hbm.at[:, pl.ds(j * LANES, LANES)], awo_raw.at[j], sem_a)
                       for j in range(DA // LANES)]
                    + [pltpu.make_async_copy(wqkv_hbm, wqkv_raw, sem_a)])

        def wp_rows(t, i, s, c):
            return _ds((((t * NS + i) * (WROWS // 16) + s // 16) * 8 + c) * 8, 8)

        def shuffle_columns(blk, t, hold, quarters=range(NS)):
            lane = lax.broadcasted_iota(I32, (8, LANES), 1)
            slot, chunk, low = lane >> 5, (lane & 31) >> 2, lane & 3
            head_of = _unshuffle(lane & 31)
            for s in range(0, WROWS, 16):
                for i in quarters:
                    rows = _ds(i * KQ + (blk % NBLK) * WROWS + s, 16)
                    moved = []
                    for j in range(8):
                        c0 = t * DA + j * LANES
                        u = hold(pltpu.bitcast(wqkv_raw[rows, c0:c0 + LANES], I32))
                        moved.append(jnp.take_along_axis(u, low * 32 + 4 * ((chunk - j) & 7) + slot, axis=1))
                        if j % 4 == 3:
                            yield w_shuffle
                    v = [moved[-c % 8] for c in range(8)]
                    for bit in (1, 2, 4):
                        v = [jnp.where((chunk & bit) != 0, v[(c - bit) % 8], v[c]) for c in range(8)]
                    for c in range(8):
                        source = slot * 32 + (((head_of >> 2) + c) & 7) * 4 + (head_of & 3)
                        wp[wp_rows(t, i, s, c), :] = pltpu.bitcast(jnp.take_along_axis(v[c], source, axis=1), U32)
                        if c % 4 == 3:
                            yield w_shuffle

        n_shuffle = (WROWS // 16) * NS * 4 * w_shuffle

        weights = ((rq0, rk0, rv0), (rq1, rk1, rv1))
        projected = ((qs0, ks0, vs0), (qs1, ks1, vs1))
        staged = ((sq0, sk0, sv0), (sq1, sk1, sv1))

        def weight_copies(par, grp, w):
            words = (wq_hbm, wuk_hbm, wuv_hbm)[w].bitcast(U32)
            n = words.shape[0]
            return [pltpu.make_async_copy(
                words.at[:, (HB // 2) * parity + grp * (GROUP // 2) + pair],
                staged[par][w].at[pl.ds((2 * pair + parity) * n, n)], sem_w.at[3 * par + w])
                for pair in range(GROUP // 2) for parity in range(2)]

        def group_copies(par, grp):
            return [c for w in range(3) for c in weight_copies(par, grp, w)]

        def c_copies(part):
            return [pltpu.make_async_copy(c_hbm.at[part], c_raw.at[:, pl.ds(part * PART, PART)], sem_c.at[part])]

        def x_copies(part):
            return [pltpu.make_async_copy(bx_hbm.at[part], bwo_raw.at[:, pl.ds(part * PART, PART)], sem_x.at[part])]

        def wo_copies(grp):
            rows = (slice(None), _ds(grp * (KO // NGROUP), KO // NGROUP))
            return [pltpu.make_async_copy(bwo_hbm.at[rows], bwo_raw.at[rows], sem_wo)]

        def build_weights(par, w, part, hold, tops=range(7)):
            n = (MB, DC, DC)[w] // 2
            rows = n // NS // GROUP
            src = _shifted(staged[par][w], part, GROUP, rows)
            for s in range(0, rows, 8):
                def load(i, j, hold):
                    return [_split(hold(src[pl.ds((2 * (j // 2) + e) * n + i * (n // NS) + s, 8), :]))[j % 2]
                            for e in range(2)]

                def store(p, words):
                    weights[par][w][p, _ds(part * rows + s, 8), :] = words

                yield from _build_operands(RHS_TERMS, load, store, hold, tops)

        def n_weights(w):
            return (MB, DC, DC)[w] // NS // GROUP // 16 * 7

        def build_group(par, part, hold):
            return _chain(*[build_weights(par, w, part, hold) for w in range(3)])

        n_group = sum(n_weights(w) for w in range(3))

        def build_activations(src, dst, part, hold, tops=range(7)):
            tiles = src.shape[2] // NS // LANES
            for t in range(tiles):
                for s in range(0, PART, 16):
                    r = part * PART + s

                    def load(i, j, hold):
                        c0 = (j * tiles + t) * LANES
                        return _split(hold(pltpu.bitcast(src[i, pl.ds(r, 16), c0:c0 + LANES], U32)))

                    def store(p, words):
                        dst[p, t, pl.ds(r // 2, 8), :] = words

                    yield from _build_operands(LHS_TERMS, load, store, hold, tops)

        def n_activations(width):
            return width // NS // LANES * (PART // 16) * 7

        def project(par, w, part, mark):
            lhs = lx if w == 0 else lc
            tiles = lhs.shape[1]
            dst = projected[par][w]
            dst = _shifted(dst, part, GROUP, dst.shape[0] // GROUP // GROUP)
            pending = {}

            def product(p):
                x = _cat([_matrix(lhs[p, t, _ds(part * PART // 2, PART // 2), :]) for t in range(tiles)], 1)
                return mark(jnp.dot(x, _matrix(weights[par][w][p]), preferred_element_type=F32))

            def emit(i, j, v):
                if w < 2:
                    dst[pl.ds((j * SEQ + i * PART) // 2, PART // 2), :] = (
                        pltpu.bitcast(v.astype(BF16), U32) if w else _join_shuffled(v * (DB ** -0.5 * LOG2E)))
                else:
                    pending[i, j] = v.T
                    if i % 2 == 1:
                        pair = [pending.pop((i - 1 + b, j)) for b in range(2)]
                        blocks = [[t[a * DB // 2:(a + 1) * DB // 2] for t in pair] for a in range(2)]
                        for p, x in enumerate(_operands(LHS_TERMS, blocks)):
                            dst[pl.ds(((j * NPAIR + i // 2) * 7 + p) * DB // 4, DB // 4), :] = _join_shuffled(x)

            return _weigh(_multiply(product, emit), tiles)

        n_project = NP * (MB + 2 * DC) // NS // LANES

        def attend(par, h, head_id, pacer, order, lag, late, early_diag, w_qk, mix, fast=NPAIR):
            hold = pacer.after(lag)
            causal = (lax.broadcasted_iota(I32, (TILE, TILE), 0)
                      <= _unshuffle(lax.broadcasted_iota(I32, (TILE, TILE), 1)))
            queries, keys, values = (r.at[_ds(h * (r.shape[0] // GROUP), r.shape[0] // GROUP)] for r in projected[par])
            result = ctx.at[_ds(head_id * (SEQ // 2), SEQ // 2)]
            pending = {}

            def fold(op, t):
                return functools.reduce(op, [t[r:r + 8] for r in range(0, TILE, 8)])

            def scores(i):
                q = _matrix(queries[i * TILE // 2:(i + 1) * TILE // 2, :])
                tiles, peaks = [], []
                for j in range(i + 1):
                    k = _matrix(keys[j * TILE // 2:(j + 1) * TILE // 2, :])
                    s = pacer.mark(lax.dot_general(k, q, NT_DIMS, preferred_element_type=F32))
                    if j == i:
                        s = jnp.where(causal, s, MASKED * LOG2E)
                    tiles.append(s)
                    peaks.append(fold(jnp.maximum, s))
                    yield w_qk
                top = jnp.max(functools.reduce(jnp.maximum, peaks), axis=0, keepdims=True)
                if 0 < i // 2 and i // 2 >= NPAIR - fast:
                    mass = functools.reduce(jnp.add, [jnp.exp2(x - top) for x in peaks])
                    top = top + jnp.log2(jnp.sum(mass, axis=0, keepdims=True))
                pending[i] = tiles, jnp.broadcast_to(top, (8, TILE))

            def context(i):
                both = [pending.pop(2 * i + c) for c in range(2)]
                totals = [None, None]
                o = [[None, None], [None, None]]

                def weight(j, c):
                    p = jnp.exp2(both[c][0][j] - _cat([hold(both[c][1])] * (TILE // 8), 0))
                    t = fold(jnp.add, p)
                    totals[c] = t if totals[c] is None else totals[c] + t
                    return p

                def product(j, p, x):
                    v = _matrix(values[(j * 7 + p) * DB // 4:(j * 7 + p + 1) * DB // 4, :])
                    return pacer.mark(jnp.dot(v, x.astype(BF16), preferred_element_type=F32))

                def emit(a, c, v):
                    o[a][c] = v if o[a][c] is None else o[a][c] + v

                def plain(j, c, tiles):
                    for b in range(tiles):
                        p = weight(2 * j + b, c)
                        shared = product(j, 2 + b, p)
                        emit(b, c, shared)
                        emit(1 - b, c, shared + product(j, 5 + b, p))
                        yield 1

                def diagonal():
                    yield from plain(i, 0, 1)
                    yield from plain(i, 1, 2)

                if early_diag:
                    yield from diagonal()
                acc = [None] * 7
                for j in range(i):
                    if i < NPAIR - fast:
                        yield from plain(j, 0, 2)
                        yield from plain(j, 1, 2)
                        continue
                    tiles, n = {}, 0
                    for p in late:
                        if p == ',':
                            yield 4 / 7 * n
                            n = 0
                            continue
                        p = int(p)
                        for _, b, c in RHS_TERMS[p]:
                            if (b, c) not in tiles:
                                tiles[b, c] = weight(2 * j + b, c)
                        t = product(j, p, _operand(RHS_TERMS[p], lambda b, c: [[tiles[b, c]]])[0][0])
                        acc[p] = t if acc[p] is None else acc[p] + t
                        n += 1
                if acc[0] is not None:
                    _run(_multiply(lambda p: acc[p], emit, 1))
                if not early_diag:
                    yield from diagonal()
                for c in range(2):
                    x = _cat([o[0][c], o[1][c]], 0) * _reciprocal(jnp.sum(totals[c], axis=0, keepdims=True))
                    result[(2 * i + c) * TILE // 2:(2 * i + c + 1) * TILE // 2, :] = pltpu.bitcast(x.astype(BF16).T, U32)

            for n in range(NPAIR + 1):
                streams = []
                if n < NPAIR:
                    i = order[n]
                    streams.append((_chain(scores(2 * i), scores(2 * i + 1)), (4 * i + 3) * w_qk, *mix[0:2]))
                if n > 0:
                    streams.append((context(order[n - 1]), 4 * order[n - 1] + 3, *mix[2:4]))
                yield from _merge(*streams)

        def n_attend(w_qk, **_):
            return NTILE * (NTILE + 1) * (1 + w_qk) / 2

        def build_wo(head_id, hold):
            n = KO // HB
            src, dst = bwo_raw.at[:, _ds(head_id * n, n)], _shifted(ro, head_id, HB, n // 2)
            for ct in range(TPB):
                for s in range(0, n, 16):
                    def load(i, j, hold):
                        c0 = (j * TPB + ct) * LANES
                        v = src[i, pl.ds(s, 16), c0:c0 + LANES].astype(F32)
                        return [hold(v[0:8]), hold(v[8:16])]

                    def store(p, words):
                        dst[pl.ds(((p * TPB + ct) * KO + s) // 2, 8), :] = words

                    yield from _build_operands(RHS_TERMS, load, store, hold)

        n_wo = TPB * (KO // HB // 16) * 7

        def head_step(par, g, h, more):
            SPARSE[0] = sparse
            if not dbg:
                @pl.when(h == 0)
                def _():
                    _wait(wo_copies(g))
                    (_start(wo_copies(g + 1)) if more else _wait(a_inputs))

                if more:
                    _when((h == 0) & (g + 2 < NGROUP), lambda: _wait(group_copies(par, g + 2)))
                    _when((h == 0) & (g + 3 < NGROUP), lambda: _start(group_copies(1 - par, g + 3)))
                    if par == 0:
                        _when((h == 0) & (g == NGROUP - 2), lambda: _start(a_inputs))

            pacer = _Pacer(lc[0, 0, 0:8, :])
            hold = pacer.after(lag4 if more else lag5)
            head_id = g * GROUP + h
            if more:
                _interleave((attend(par, h, head_id, pacer, **head), n_attend(**head), *sp_att),
                            (_chain(*[project(1 - par, w, h, pacer.mark) for w in p_order]), n_project),
                            (build_wo(head_id, hold), n_wo, *sp_wo),
                            (build_group(par, h, hold), n_group, *sp_w))
            else:
                _interleave((attend(par, h, head_id, pacer, **tail), n_attend(**tail)),
                            (build_wo(head_id, hold), n_wo, *sp_wo5),
                            (_chain(*[shuffle_columns(0, t, hold, [h]) for t in range(3)]),
                             3 * n_shuffle / NS, *sp_sh5))

        if 'p4' in dbg or 'p5' in dbg:
            touch(lx, lc, rq1, rk1, rv1, ks0, vs0, qs0, sq0, sk0, sv0, bwo_raw, wqkv_raw)
            _loop(16, lambda t: head_step(0, t // GROUP, t % GROUP, 'p4' in dbg))
            touch(wp, ctx, ro, qs1, ks1, vs1, rq0, rk0, rv0)
            return

        def start_up():
            data = {'k': weight_copies(0, 0, 1), 'v': weight_copies(0, 0, 2), 'q': weight_copies(0, 0, 0),
                    'g1': group_copies(1, 1), 'g2': group_copies(0, 2), 'o': wo_copies(0)}
            for part in range(GROUP):
                data['c%d' % part], data['x%d' % part] = c_copies(part), x_copies(part)

            def operands(job, hold, tops=range(7)):
                if job[0] == '!':
                    def await_copies():
                        _wait(data[job[1:]])
                        yield 1e-6

                    return await_copies(), 1e-6
                kind, part = job[0], int(job[1])
                if kind in 'cx':
                    src, dst = (c_raw, lc) if kind == 'c' else (bwo_raw, lx)
                    return build_activations(src, dst, part, hold, tops), n_activations(src.shape[2])
                if kind == 'g':
                    return build_group(1, part, hold), n_group
                return build_weights(0, 'qkv'.index(kind), part, hold, tops), n_weights('qkv'.index(kind))

            def expand(jobs):
                return [j for job in jobs.split() for j in ([job + str(u) for u in range(GROUP)] if len(job) == 1 else [job])]

            def issue(starts):
                for k in starts.split():
                    if k.isdigit():
                        pl.delay(int(k))
                        continue
                    for c in data[k.rstrip('*')]:
                        c.start(priority=int(k.endswith('*')))

            def step(n, waits, starts, products, ahead, jobs):
                lag, *span, SPARSE[0] = paces.get('s%d' % n, (3, .03, .95, 2))
                with jax.named_scope('s%d_wait' % n):
                    _wait([c for k in waits.split() for c in data[k]])
                    issue(starts)
                with jax.named_scope('s%d_mm' % n):
                    pacer = _Pacer(pltpu.bitcast(c_raw[0, 0:16, 0:LANES], U32))
                    products = [('qkv'.index(p[0]), int(p[1])) for p in products.split()]
                    sizes = [n_project // (4 if w else 2) for w, _ in products]
                    streams = [(_chain(*[project(0, w, part, pacer.mark) for w, part in products]), sum(sizes))]
                    if ahead:
                        def first(tops, hold):
                            return _chain(*[operands(job, hold, [top])[0] for top in tops for job in expand(ahead)])

                        _run(first(TOP_ORDER[:n_ahead], _same))
                        if n_ahead < 7:
                            streams.append((first(TOP_ORDER[n_ahead:], pacer.after(lag_ahead)),
                                            sum(operands(job, None)[1] for job in expand(ahead)) * (7 - n_ahead) / 7,
                                            0., end_ahead * sizes[0] / sum(sizes)))
                    if jobs:
                        jobs = [operands(job, pacer.after(lag)) for job in expand(jobs)]
                        streams.append((_chain(*[j[0] for j in jobs]), sum(j[1] for j in jobs), *span))
                    _interleave(*streams)

            def nth(i):
                for n, args in enumerate(plan):
                    pl.when(i == n)(functools.partial(step, n, *args))

            issue(first_copies)
            _loop(len(plan), nth)

        def two_groups(t):
            _loop(GROUP, lambda h: head_step(0, 2 * t, h, True))
            _when(t < NGROUP // 2 - 1, lambda: _loop(GROUP, lambda h: head_step(1, 2 * t + 1, h, True)))

        if not dbg or 'start' in dbg:
            with jax.named_scope('start_up'):
                start_up()
        if 'start' in dbg:
            _wait(group_copies(0, 2) + wo_copies(0))
            touch(qs0, ks0, vs0, rq1, rk1, rv1)
            return
        if not dbg:
            with jax.named_scope('heads'):
                _loop(NGROUP // 2, two_groups)
            with jax.named_scope('last_heads'):
                _loop(GROUP, lambda h: head_step(1, NGROUP - 1, h, False))

        la = lx

        def w_a(t, p, ct, r0, rows):
            if t == 0:
                return (rq0, rq1)[ct], (p, _ds(r0, rows))
            if t == 1:
                return lc, (p, 0, _ds(ct * (KQ // 2) + r0, rows))
            if t == 2:
                buf, tile = divmod(TPB * p + ct, 25)
                assert rows <= 64 or rows == 128
                if rows == 128:
                    return (rk0, rk1, rv0, rv1)[buf], (pl.ds(2 * tile, 2),)
                return (rk0, rk1, rv0, rv1)[buf], (2 * tile + r0 // 64, _ds(r0 % 64, rows))
            buf, tile = divmod(TPB * p, 50)
            return (vs0, vs1)[buf], (_ds((tile + ct) * (KQ // 2) + r0, rows),)

        def load_w(t, p):
            tiles = []
            for ct in range(TPB):
                buf, idx = w_a(t, p, ct, 0, KQ // 2)
                tiles.append(_matrix(buf[idx].reshape(KQ // 2, LANES)))
            return _cat(tiles, 1)

        span_a = HALO + SEQ // 2
        group_rows = 16 * NS

        def build_w(blk, t, hold):
            for s in range(0, WROWS, 16):
                for ct in range(TPB):
                    def load(i, j, hold):
                        return _split(hold(wp[wp_rows(t, i, s, j * TPB + ct), :]))

                    def store(p, words):
                        buf, idx = w_a(t, p, ct, (blk * WROWS + s) // 2, 8)
                        buf[idx] = words

                    yield from _build_operands(RHS_TERMS, load, store, hold)

        n_w = (WROWS // 16) * TPB * 7

        def build_x(blk, hold):
            for c in range(ROWS // group_rows):
                for t in range(TPB):
                    def load(i, j, hold):
                        words = ax_raw.at[j * TPB + t].bitcast(U32).at[_ds(blk * (ROWS // 2), ROWS // 2)]
                        w0 = (c * group_rows + 32 * (i // 2)) // 2
                        return [_split(hold(words[pl.ds(w0 + e, 8, stride=2), :]))[i % 2] for e in range(2)]

                    def store(p, words):
                        la[p, t, _ds((blk * (ROWS // NS) + 16 * c) // 2, 8), :] = words

                    yield from _build_operands(LHS_TERMS, load, store, hold)

        n_x = (ROWS // group_rows) * TPB * 7

        def build_awo(blk, hold):
            ct, odd, h0 = blk // 4, (blk // 2) % 2, 16 * (blk % 2)
            pairs = DHA // 2 // NS
            for dp in range(0, pairs, 2):
                src = {}
                for i in range(NS):
                    for j in range(NS):
                        words = awo_raw.at[j * TPB + ct].bitcast(U32).at[pl.ds(pl.multiple_of(h0 * 16, 256), 256)]
                        for e in range(2):
                            w0 = 8 * e * 16 + i * pairs + dp
                            src[i, j, e] = hold(jnp.where(odd == 1, words[pl.ds(w0 + 1, 8, stride=16), :],
                                                          words[pl.ds(w0, 8, stride=16), :]))
                    yield
                for half in range(2):
                    def load(i, j, hold):
                        return [_split(hold(src[i, j, e]))[half] for e in range(2)]

                    def store(p, words):
                        buf, idx = w_a(3, p, ct, ((2 * (dp + odd) + half) * HA + h0) // 2, 8)
                        buf[idx] = words

                    yield from _build_operands(RHS_TERMS, load, store, hold)

        n_awo = (DHA // 2 // NS // 2) * (NS + 2 * 7)

        def output_b(blk):
            SPARSE[0] = sparse6
            slot = blk % 2
            rows = ROWS // NS
            heads = HB // NS
            _when(blk >= 2, lambda: out_copy(slot, 0, DA).wait())
            pacer = _Pacer(ro[0:8, :])
            src = _shifted(ctx, blk, NBLK, ROWS // 2)
            lhs = {}

            def build_lhs(top, hold):
                half = NS // 2
                for h in range(heads):
                    for r in range(0, rows, 16):
                        def quadrant(i, j):
                            return [[_split_shuffled((hold if (a == b or sparsel == 4) and (sparsel > 1 or (i, j) == LHS_TERMS[top][0][1:]) else _same)(src[pl.ds(
                                (((j * half + b) * heads + h) * SEQ + (i * half + a) * rows + r) // 2, 8), :]))
                                for b in range(half)] for a in range(half)]

                        for p, v in enumerate(_operands(LHS_TERMS, _operand(LHS_TERMS[top], quadrant))):
                            lhs.setdefault((top * (NP // 7) + p, h), []).append(v)
                        yield

            def product(p):
                x = _cat([_cat(lhs[p, h], 0) for h in range(heads)], 1).astype(BF16)
                w = _cat([_matrix(ro[pl.ds((p * TPB + ct) * KO // 2, KO // 2), :]) for ct in range(TPB)], 1)
                return pacer.mark(jnp.dot(x, w, preferred_element_type=F32))

            def emit(i, j, v):
                stage[slot, i * rows:(i + 1) * rows, j * KQ:(j + 1) * KQ] = v.astype(BF16)

            _run(build_lhs(TOP_ORDER[0], _same))
            hold = pacer.after(lag6)
            _interleave(
                (_multiply(product, emit), NP),
                (_chain(*[build_lhs(t, pacer.after(lagl)) for t in TOP_ORDER[1:]]), 6 * heads * (rows // 16), *sp_lhs),
                *[(_chain(build_w(blk, t, hold), shuffle_columns(blk + 1, t, hold)), n_w + n_shuffle, *sp_a)
                  for t in range(3)],
                (build_x(blk, hold), n_x, *sp_a),
                (build_awo(blk, hold), n_awo, *sp_a))
            out_copy(slot, blk * ROWS, DA).start()

        if 'p6' in dbg:
            touch(ro, ctx, ax_raw, awo_raw, wqkv_raw, wp)
        if not dbg or 'p6' in dbg:
            with jax.named_scope('output_b'):
                _loop(NBLK, output_b)
            _wait([out_copy(0, 0, DA), out_copy(1, 0, DA)])
        if 'p6' in dbg:
            touch(la, rq0, rq1, lc, rk0, rk1, rv0, rv1, ks0, ks1, vs0, vs1, wp)
            return

        def project_a(t, blk, mark):
            rows = ROWS // NS
            dst = _shifted(ro if t == 1 else ctx, blk, NBLK, ROWS // 2)

            def product(p):
                x = _cat([_matrix(la[p, k, _ds(blk * rows // 2, rows // 2), :]) for k in range(TPB)], 1)
                return mark(jnp.dot(x, load_w(t, p), preferred_element_type=F32))

            def emit(i, j, v):
                for ct in range(TPB):
                    for c in range(rows // 16):
                        piece = v[16 * c:16 * (c + 1), ct * LANES:(ct + 1) * LANES]
                        tile = 2 * (j * TPB + ct) + i % 2
                        r = c * (group_rows // 2) + 16 * (i // 2)
                        if t == 0:
                            qa[tile, _ds((blk % 2) * (ROWS // 2) + r, 16), :] = piece
                        else:
                            dst[pl.ds(tile * span_a + HALO + r, 16), :] = pltpu.bitcast(piece, U32)

            return _multiply(product, emit)

        def attend_a(blk, hold):
            row0, slot = blk * (ROWS // 2), blk % 2
            keys, values = (_shifted(buf, blk, NBLK, ROWS // 2) for buf in (ro, ctx))
            o = {}
            for r in range(0, ROWS // 2, 8):
                for par in range(2):
                    def window(buf, j, w):
                        return pltpu.bitcast(buf[pl.ds((2 * j + par) * span_a + HALO + r - w, 8), :], F32)

                    pos = row0 + r + lax.broadcasted_iota(I32, (8, LANES), 0)
                    q = [(hold if j % a_holds[0] == 0 else _same)(qa[2 * j + par, _ds(slot * (ROWS // 2) + r, 8), :]) for j in range(8)]
                    logits = []
                    for w in range(WIN):
                        acc = q[0] * (hold if a_holds[1] else _same)(window(keys, 0, w))
                        for j in range(1, 8):
                            acc = acc + q[j] * window(keys, j, w)
                        acc = (hold if a_holds[2] else _same)(acc)
                        acc = acc + pltpu.roll(acc, 64, 1)
                        acc = acc + pltpu.roll(acc, 32, 1)
                        acc = acc * (DHA ** -0.5 * LOG2E)
                        if r < w:
                            acc = jnp.where(pos >= w, acc, MASKED * LOG2E)
                        logits.append(acc)
                        yield
                    top = functools.reduce(jnp.maximum, logits)
                    e = [jnp.exp2(x - top) for x in logits]
                    scale = _reciprocal(functools.reduce(jnp.add, e))
                    e = [x * scale for x in e]
                    yield w_soft
                    for j in range(8):
                        acc = None
                        for w in range(WIN):
                            v = window(values, j, w)
                            t = e[w] * (hold(v) if w % a_holds[3] == 0 else v)
                            acc = t if acc is None else acc + t
                        o[r, par, j] = acc
                        yield
                if (2 * r + 16) % group_rows == 0:
                    c = 2 * r // group_rows
                    for t in range(TPB):
                        def load(i, j, hold):
                            return [hold(o[c * (group_rows // 2) + 8 * i, par, j * TPB + t]) for par in range(2)]

                        def store(p, words):
                            lo[slot * NP + p, t, 8 * c:8 * (c + 1), :] = words

                        yield from _weigh(_build_operands(LHS_TERMS, load, store, hold), w_lo)

        n_attend_a = (16 + w_soft) * (ROWS // 8) + TPB * (ROWS // group_rows) * 7 * w_lo

        def output_a(blk, mark):
            slot = blk % 2

            def product(p):
                x = _cat([_matrix(lo[slot * NP + p, k]) for k in range(TPB)], 1)
                return mark(jnp.dot(x, load_w(3, p), preferred_element_type=F32))

            def emit(i, j, v):
                for c in range(ROWS // group_rows):
                    r = c * group_rows + 16 * i
                    stage[slot, r:r + 16, j * KQ:(j + 1) * KQ] = v[16 * c:16 * (c + 1)].astype(BF16)

            return _multiply(product, emit)

        def step_a(i, pace, project=True, attend=True, output=True):
            SPARSE[0] = sparse
            if output:
                _when(i >= 3, lambda: out_copy((i - 1) % 2, 0, 0).wait())
            pacer = _Pacer(lc[0, 0, 0:8, :])
            matmuls = [output_a(i - 1, pacer.mark)] if output else []
            matmuls += [project_a(t, i + 1, pacer.mark) for t in a_order] if project else []
            streams = [(_chain(*matmuls), len(matmuls) * NP)]
            if attend:
                streams.append((attend_a(i, pacer.after(pace[0])), n_attend_a, *pace[1]))
            _interleave(*streams)
            if output:
                out_copy((i - 1) % 2, (i - 1) * ROWS, 0).start()

        if dbg:
            touch(la, rq0, rq1, lc, rk0, rk1, rv0, rv1, ks0, ks1, vs0, vs1, lo, qa, ro, ctx)
            if 'pa' in dbg:
                _loop(NBLK - 2, lambda t: step_a(t + 1, a_main))
                _wait([out_copy(0, 0, 0), out_copy(1, 0, 0)])
            elif 'pa3' in dbg:
                _start([out_copy(0, 0, 0), out_copy(1, 0, 0)])
                step_a(NBLK - 1, a_last, project=False)
                step_a(NBLK, None, project=False, attend=False)
                _wait([out_copy(0, 0, 0), out_copy(1, 0, 0)])
            elif 'pa1' in dbg:
                step_a(-1, None, attend=False, output=False)
                step_a(0, a_first, output=False)
            touch(lo, qa, ro, ctx)
            return

        for tile in range(16):
            for buf in (ro, ctx):
                buf[tile * span_a:tile * span_a + HALO, :] = jnp.zeros((HALO, LANES), U32)
        with jax.named_scope('a_first'):
            step_a(-1, None, attend=False, output=False)
            step_a(0, a_first, output=False)
        with jax.named_scope('a_main'):
            _loop(NBLK - 2, lambda t: step_a(t + 1, a_main))
        with jax.named_scope('a_last'):
            step_a(NBLK - 1, a_last, project=False)
            step_a(NBLK, None, project=False, attend=False)
        _wait([out_copy(0, 0, 0), out_copy(1, 0, 0)])

    def words(*shape):
        return pltpu.VMEM(shape + (LANES,), U32)

    scratch = [
        pltpu.VMEM((DA // LANES, SEQ, LANES), BF16),
        pltpu.VMEM((DA, 3 * DA), BF16),
        pltpu.VMEM((DA // LANES, DA, LANES), BF16),
        pltpu.VMEM((NS, MQ, DC), BF16),
        pltpu.VMEM((NS, KO, MB), BF16),
        words(NP, MB // NS // LANES, MQ // 2),
        words(NP, DC // NS // LANES, MQ // 2),
        *[words(NP, MB // NS // 2)] * 2,
        *[words(NP + 1, DC // NS // 2)] * 4,
        *[words(GROUP * SEQ // 2)] * 4,
        *[words(GROUP * NPAIR * 7 * DB // 4)] * 2,
        *[words(GROUP * MB // 2)] * 2,
        *[words(GROUP * DC // 2)] * 4,
        words(HB * SEQ // 2),
        words(NP * TPB * KO // 2),
        words(3 * NS * (WROWS // 16) * 64),
        words(2 * NP, TPB, ROWS // NS // 2),
        pltpu.VMEM((16, ROWS, LANES), F32),
        pltpu.VMEM((2, ROWS, DA), BF16),
        pltpu.SemaphoreType.DMA((GROUP,)),
        pltpu.SemaphoreType.DMA((GROUP,)),
        pltpu.SemaphoreType.DMA(()),
        pltpu.SemaphoreType.DMA((6,)),
        pltpu.SemaphoreType.DMA(()),
        pltpu.SemaphoreType.DMA((2,)),
    ]

    def run(A_x, A_wqkv, A_wo, B_x, B_c_kv, B_w_q, B_w_uk, B_w_uv, B_w_o):
        hbm = pl.BlockSpec(memory_space=pl.ANY)
        out = pl.pallas_call(
            kernel,
            in_specs=[hbm] * 9,
            out_specs=hbm,
            out_shape=jax.ShapeDtypeStruct((SEQ, DA + MB), BF16),
            scratch_shapes=scratch,
            compiler_params=pltpu.CompilerParams(vmem_limit_bytes=127 * 2 ** 20),
            name=name,
        )(A_x.reshape(SEQ, DA), A_wqkv, A_wo, B_x.reshape(GROUP, NS, PART, MB), B_c_kv.reshape(GROUP, NS, PART, DC),
          B_w_q.reshape(MB // 2, 2 * HB, DB), B_w_uk.reshape(DC // 2, 2 * HB, DB),
          B_w_uv.reshape(DC // 2, 2 * HB, DB), B_w_o.reshape(NS, KO, MB))
        return out.reshape(1, SEQ, DA + MB)

    return run


_fused_call = build()


@jax.jit
def pallas_concat_heads__sliding_local_dilated__compressed_kv_cla__prompt_kernel(A_x, A_wqkv, A_wo, B_x, B_c_kv, B_w_q, B_w_uk, B_w_uv, B_w_o):
    return _fused_call(A_x, A_wqkv, A_wo, B_x, B_c_kv, B_w_q, B_w_uk, B_w_uv, B_w_o)
```

```python
import functools
import math

import jax
import jax.numpy as jnp
from jax import lax
import jax.experimental.pallas as pl
import jax.experimental.pallas.tpu as pltpu

F32 = jnp.float32
BF16 = jnp.bfloat16
U32 = jnp.uint32
I32 = jnp.int32
LANES = 128
NT_DIMS = (((1,), (1,)), ((), ()))
LOG2E = math.log2(math.e)
MASKED = -1e9

SEQ = 2048
DA = 1024
HA, DHA = 32, 32
WIN = 8
HALO = 32
MB = 1024
HB, DB = 32, 128
DC = 512

LEVELS = 2
NS = 2 ** LEVELS
NP = 7 ** LEVELS
GROUP = NS
NGROUP = HB // GROUP
MQ = SEQ // NS
PART = MQ // GROUP
ROWS = 256
NBLK = SEQ // ROWS
KQ = DA // NS
TPB = KQ // LANES
KO = HB * DB // NS
WROWS = KQ // NBLK
TILE = LANES
NTILE = SEQ // TILE
NPAIR = NTILE // 2


LHS_TERMS = (((1, 0, 0), (1, 1, 1)), ((1, 1, 0), (1, 1, 1)), ((1, 0, 0),), ((1, 1, 1),),
             ((1, 0, 0), (1, 0, 1)), ((1, 1, 0), (-1, 0, 0)), ((1, 0, 1), (-1, 1, 1)))
RHS_TERMS = (((1, 0, 0), (1, 1, 1)), ((1, 0, 0),), ((1, 0, 1), (-1, 1, 1)), ((1, 1, 0), (-1, 0, 0)),
             ((1, 1, 1),), ((1, 0, 0), (1, 0, 1)), ((1, 1, 0), (1, 1, 1)))
TOP_ORDER = (1, 3, 0, 6, 4, 2, 5)


def _add(x, y):
    return [[a + b for a, b in zip(rx, ry)] for rx, ry in zip(x, y)]


def _sub(x, y):
    return [[a - b for a, b in zip(rx, ry)] for rx, ry in zip(x, y)]


def _operand(terms, quadrant):
    total = None
    for sign, i, j in terms:
        q = quadrant(i, j)
        total = q if total is None else (_add if sign > 0 else _sub)(total, q)
    return total


def _operands(side, blocks):
    half = len(blocks) // 2
    if half == 0:
        return [blocks[0][0]]

    def quadrant(i, j):
        return [row[j * half:(j + 1) * half] for row in blocks[i * half:(i + 1) * half]]

    return [x for terms in side for x in _operands(side, _operand(terms, quadrant))]


def _multiply(product, emit, level=LEVELS, base=0):
    if level == 0:
        emit(0, 0, product(base))
        yield
        return
    n = 2 ** (level - 1)

    def m(i):
        out = [[None] * n for _ in range(n)]

        def keep(a, b, v):
            out[a][b] = v

        yield from _multiply(product, keep, level - 1, base + (i - 1) * 7 ** (level - 1))
        return out

    def put(x, oi, oj):
        for a in range(n):
            for b in range(n):
                emit(oi * n + a, oj * n + b, x[a][b])

    m2 = yield from m(2)
    m4 = yield from m(4)
    put(_add(m2, m4), 1, 0)
    m1 = yield from m(1)
    c11 = _add(m1, m4)
    c22 = _sub(m1, m2)
    m7 = yield from m(7)
    c11 = _add(c11, m7)
    m5 = yield from m(5)
    put(_sub(c11, m5), 0, 0)
    m3 = yield from m(3)
    put(_add(m3, m5), 0, 1)
    c22 = _add(c22, m3)
    m6 = yield from m(6)
    put(_add(c22, m6), 1, 1)


SPARSE = [0]


def _build_operands(side, load, store, hold, tops=range(7)):
    half = NS // 2
    for top in tops:
        terms = side[top]
        loaded = {(i, j): [[load(i * half + a, j * half + b,
                                 hold if SPARSE[0] == 0 or (a == b and (SPARSE[0] == 1 or n == 0)) else _same)
                            for b in range(half)] for a in range(half)]
                  for n, (_, i, j) in enumerate(terms)}
        lo, hi = (_operands(side, _operand(terms, lambda i, j: [[x[e] for x in row] for row in loaded[i, j]]))
                  for e in range(2))
        for p in range(NP // 7):
            store(top * (NP // 7) + p, _join(lo[p], hi[p]))
        yield


def _split(words):
    return pltpu.bitcast(words << 16, F32), pltpu.bitcast(words & jnp.uint32(0xFFFF0000), F32)


def _join(lo, hi):
    return pltpu.bitcast(pltpu.pack_elementwise([lo, hi], packed_dtype=BF16), U32)


def _join_shuffled(v):
    r, c = v.shape
    v = v.reshape(r // 16, 2, 8, c)
    return _join(v[:, 0].reshape(r // 2, c), v[:, 1].reshape(r // 2, c))


def _split_shuffled(words):
    lo, hi = _split(words)
    r, c = words.shape
    return jnp.stack([lo.reshape(r // 8, 8, c), hi.reshape(r // 8, 8, c)], axis=1).reshape(2 * r, c)


def _unshuffle(pos):
    return (pos & ~15) + ((pos & 15) >> 1) + 8 * (pos & 1)


def _matrix(words):
    return pltpu.bitcast(words, BF16)


def _cat(xs, axis):
    return xs[0] if len(xs) == 1 else jnp.concatenate(xs, axis=axis)


def _ds(start, size):
    if isinstance(start, int):
        return pl.ds(start, size)
    return pl.ds(pl.multiple_of(start, min(size, 16)), size)


def _shifted(ref, step, steps, n):
    return ref.at[_ds(step * n, ref.shape[0] - (steps - 1) * n)]


def _when(cond, fn):
    if isinstance(cond, bool):
        if cond:
            fn()
    else:
        pl.when(cond)(fn)


def _loop(n, body):
    lax.fori_loop(0, n, lambda i, carry: body(i), None)


def _start(copies):
    for c in copies:
        c.start()


def _wait(copies):
    for c in copies:
        c.wait()


def _run(steps):
    for _ in steps:
        pass


def _chain(*streams):
    for steps in streams:
        yield from steps


def _weigh(steps, weight):
    for _ in steps:
        yield weight


def _merge(*streams):
    spans = [s[2:] if len(s) > 2 else (0.0, 1.0) for s in streams]
    done = [0.0] * len(streams)
    live = list(range(len(streams)))
    while live:
        i = min(live, key=lambda k: spans[k][0] + (spans[k][1] - spans[k][0]) * done[k] / streams[k][1])
        try:
            weight = next(streams[i][0])
        except StopIteration:
            live.remove(i)
            continue
        weight = 1 if weight is None else weight
        done[i] += weight
        yield weight


def _interleave(*streams):
    _run(_merge(*streams))


class _Pacer:
    def __init__(self, words):
        self.odd = words | 1
        self.marks = []

    def mark(self, v):
        self.marks.append(pltpu.bitcast(v[:, 0:LANES], U32))
        return v

    def after(self, lag):
        def hold(x):
            if len(self.marks) < lag:
                return x
            rows = x.shape[0]
            never = jnp.concatenate([self.odd] * (rows // 8), axis=0) == 0
            return pltpu.bitcast(jnp.where(never, self.marks[-lag][0:rows], pltpu.bitcast(x, U32)), x.dtype)

        return hold


def _same(x):
    return x


def _reciprocal(x):
    r = pltpu.reciprocal(x, approx=True)
    return r * (2.0 - x * r)


PLANS = dict(
    e=(('c0 k', 'c2 q', 'k0', 'c0 k', ''),
       ('v c1', 'x0 c3', 'v0', 'v', 'c1'),
       ('c2', 'x1 x2 x3', 'k1 v1', '', 'c2 !q q0 q1'),
       ('x0', 'g1', 'k2 v2', '', 'q2 q3 x0'),
       ('c3 x1 x2', 'g2 o', 'q0 q1', '', 'x1 x2 c3'),
       ('x3 g1', '', 'q2 k3 v3 q3', '', 'x3 g')),
)


def build(name="fused_attention", dbg=(),
          head=dict(early_diag=True, lag=9, late='1,4,0,2,5,3,6,', mix=(0, .7, .15, 1), order=(1, 3, 5, 7, 6, 4, 2, 0), w_qk=1),
          tail=dict(early_diag=True, lag=11, late='14,02,53,6,', mix=(0, .6, .25, 1), order=(1, 3, 5, 7, 6, 4, 2, 0), w_qk=1.1, fast=5),
          sp_att=(0., .86), sp_wo=(.02, .15), sp_w=(.25, .98), lag4=2, sp_wo5=(.03, .3), lag5=1,
          sp_lhs=(0., .84), sp_a=(.02, .95), w_shuffle=1., lag6=1, lagl=1,
          a_main=dict(lag=6, span=(.08, .99), w_lo=4, w_soft=3, holds=(8, 1, 0, 8), sparse=2, order=(1, 2, 0), overlap=1),
          a_first=dict(lag=3, span=(.02, .98), w_lo=7, w_soft=1, holds=(8, 1, 0, 4), sparse=2, order=(1, 2, 0), overlap=1),
          a_last=dict(lag=2, span=(.02, 1.), w_lo=8, w_soft=4, holds=(1, 1, 1, 8), sparse=2, order=(), overlap=1),
          delay=2, sp_sh5=(.1, .8), sp_x=(.02, .95), sp_awo=(.02, .95), sp_proj=(0., 1.), lagw=1, w_order=(0, 1, 2), slots=4, pad=32, plan='e', paces={'s0': (5, 0.07, 0.9, 1), 's1': (99, 0.04, 0.93, 2), 's2': (14, 0.0, 0.93, 2), 's3': (14, 0.02, 0.99, 2), 's4': (1, 0.02, 0.99, 1), 's5': (3, 0.02, 0.96, 2)}, lag_ahead=1, end_ahead=.84, n_ahead=7, first_copies='c0 k v c1', sparsel=4, sparse6=0, p_order=(1, 2, 0), sparse=2):

    SPARSE[0] = sparse
    plan = PLANS[plan]

    def kernel(ax_hbm, wqkv_hbm, awo_hbm, bx_hbm, c_hbm, wq_hbm, wuk_hbm, wuv_hbm, bwo_hbm, out_hbm,
               ax_raw, wqkv_raw, awo_raw, c_raw, bwo_raw,
               lx, lc, rq0, rq1, rk0, rk1, rv0, rv1, qs0, qs1, ks0, ks1, vs0, vs1,
               sq0, sq1, sk0, sk1, sv0, sv1, ctx, ro, lo, stage, spare,
               sem_c, sem_x, sem_wo, sem_w, sem_a, sem_out):

        def out_copy(slot, row0, col0):
            return pltpu.make_async_copy(
                stage.at[slot], out_hbm.at[_ds(row0, ROWS), pl.ds(col0, DA)], sem_out.at[slot])

        def touch(*refs):
            for r in refs:
                while len(r.shape) > 2:
                    r = r.at[0]
                if r.dtype == BF16:
                    pltpu.sync_copy(r.at[pl.ds(0, 16), pl.ds(0, LANES)], out_hbm.at[pl.ds(0, 16), pl.ds(0, LANES)])
                    pltpu.sync_copy(out_hbm.at[pl.ds(0, 16), pl.ds(0, LANES)], r.at[pl.ds(0, 16), pl.ds(0, LANES)])
                else:
                    o = out_hbm.bitcast(r.dtype).at[pl.ds(0, 8), pl.ds(0, LANES)]
                    pltpu.sync_copy(r.at[pl.ds(0, 8)], o)
                    pltpu.sync_copy(o, r.at[pl.ds(0, 8)])

        a_inputs = ([pltpu.make_async_copy(ax_hbm.at[:, pl.ds(j * LANES, LANES)], ax_raw.at[j], sem_a)
                     for j in range(DA // LANES)]
                    + [pltpu.make_async_copy(awo_hbm.at[:, pl.ds(j * LANES, LANES)], awo_raw.at[j], sem_a)
                       for j in range(DA // LANES)]
                    + [pltpu.make_async_copy(wqkv_hbm, wqkv_raw, sem_a)])

        wp = ks0

        def wp_rows(t, i, s, c):
            return _ds((((t * NS + i) * (WROWS // 16) + s // 16) * 8 + c) * 8, 8)

        def shuffle_columns(blk, t, hold, quarters=range(NS)):
            lane = lax.broadcasted_iota(I32, (8, LANES), 1)
            slot, chunk, low = lane >> 5, (lane & 31) >> 2, lane & 3
            head_of = _unshuffle(lane & 31)
            for s in range(0, WROWS, 16):
                for i in quarters:
                    rows = _ds(i * KQ + (blk % NBLK) * WROWS + s, 16)
                    moved = []
                    for j in range(8):
                        c0 = t * DA + j * LANES
                        u = hold(pltpu.bitcast(wqkv_raw[rows, c0:c0 + LANES], I32))
                        moved.append(jnp.take_along_axis(u, low * 32 + 4 * ((chunk - j) & 7) + slot, axis=1))
                        if j % 4 == 3:
                            yield w_shuffle
                    v = [moved[-c % 8] for c in range(8)]
                    for bit in (1, 2, 4):
                        v = [jnp.where((chunk & bit) != 0, v[(c - bit) % 8], v[c]) for c in range(8)]
                    for c in range(8):
                        source = slot * 32 + (((head_of >> 2) + c) & 7) * 4 + (head_of & 3)
                        wp[wp_rows(t, i, s, c), :] = pltpu.bitcast(jnp.take_along_axis(v[c], source, axis=1), U32)
                        if c % 4 == 3:
                            yield w_shuffle

        n_shuffle = (WROWS // 16) * NS * 4 * w_shuffle

        weights = ((rq0, rk0, rv0), (rq1, rk1, rv1))
        projected = ((qs0, ks0, vs0), (qs1, ks1, vs1))
        staged = ((sq0, sk0, sv0), (sq1, sk1, sv1))

        def weight_copies(par, grp, w):
            words = (wq_hbm, wuk_hbm, wuv_hbm)[w].bitcast(U32)
            n = words.shape[0]
            return [pltpu.make_async_copy(
                words.at[:, (HB // 2) * parity + grp * (GROUP // 2) + pair],
                staged[par][w].at[pl.ds((2 * pair + parity) * n, n)], sem_w.at[3 * par + w])
                for pair in range(GROUP // 2) for parity in range(2)]

        def group_copies(par, grp):
            return [c for w in range(3) for c in weight_copies(par, grp, w)]

        def c_copies(part):
            return [pltpu.make_async_copy(c_hbm.at[part], c_raw.at[:, pl.ds(part * PART, PART)], sem_c.at[part])]

        def x_copies(part):
            return [pltpu.make_async_copy(bx_hbm.at[part], bwo_raw.at[:, pl.ds(part * PART, PART)], sem_x.at[part])]

        def wo_copies(grp):
            rows = (slice(None), _ds(grp * (KO // NGROUP), KO // NGROUP))
            return [pltpu.make_async_copy(bwo_hbm.at[rows], bwo_raw.at[rows], sem_wo)]

        def build_weights(par, w, part, hold, tops=range(7)):
            n = (MB, DC, DC)[w] // 2
            rows = n // NS // GROUP
            src = _shifted(staged[par][w], part, GROUP, rows)
            for s in range(0, rows, 8):
                def load(i, j, hold):
                    return [_split(hold(src[pl.ds((2 * (j // 2) + e) * n + i * (n // NS) + s, 8), :]))[j % 2]
                            for e in range(2)]

                def store(p, words):
                    weights[par][w][p, _ds(part * rows + s, 8), :] = words

                yield from _build_operands(RHS_TERMS, load, store, hold, tops)

        def n_weights(w):
            return (MB, DC, DC)[w] // NS // GROUP // 16 * 7

        def build_group(par, part, hold):
            return _chain(*[build_weights(par, w, part, hold) for w in w_order])

        n_group = sum(n_weights(w) for w in range(3))

        def build_activations(src, dst, part, hold, tops=range(7)):
            tiles = src.shape[2] // NS // LANES
            for t in range(tiles):
                for s in range(0, PART, 16):
                    r = part * PART + s

                    def load(i, j, hold):
                        c0 = (j * tiles + t) * LANES
                        return _split(hold(pltpu.bitcast(src[i, pl.ds(r, 16), c0:c0 + LANES], U32)))

                    def store(p, words):
                        dst[p, t, pl.ds(r // 2, 8), :] = words

                    yield from _build_operands(LHS_TERMS, load, store, hold, tops)

        def n_activations(width):
            return width // NS // LANES * (PART // 16) * 7

        def project(par, w, part, mark):
            lhs = lx if w == 0 else lc
            tiles = lhs.shape[1]
            dst = projected[par][w]
            dst = _shifted(dst, part, GROUP, dst.shape[0] // GROUP // GROUP)
            pending = {}

            def product(p):
                x = _cat([_matrix(lhs[p, t, _ds(part * PART // 2, PART // 2), :]) for t in range(tiles)], 1)
                return mark(jnp.dot(x, _matrix(weights[par][w][p]), preferred_element_type=F32))

            def emit(i, j, v):
                if w < 2:
                    dst[pl.ds((j * SEQ + i * PART) // 2, PART // 2), :] = (
                        pltpu.bitcast(v.astype(BF16), U32) if w else _join_shuffled(v * (DB ** -0.5 * LOG2E)))
                else:
                    pending[i, j] = v.T
                    if i % 2 == 1:
                        pair = [pending.pop((i - 1 + b, j)) for b in range(2)]
                        blocks = [[t[a * DB // 2:(a + 1) * DB // 2] for t in pair] for a in range(2)]
                        for p, x in enumerate(_operands(LHS_TERMS, blocks)):
                            dst[pl.ds(((j * NPAIR + i // 2) * 7 + p) * DB // 4, DB // 4), :] = _join_shuffled(x)

            return _weigh(_multiply(product, emit), tiles)

        n_project = NP * (MB + 2 * DC) // NS // LANES

        def attend(par, h, head_id, pacer, order, lag, late, early_diag, w_qk, mix, fast=NPAIR, w_diag=1):
            hold = pacer.after(lag)
            causal = (lax.broadcasted_iota(I32, (TILE, TILE), 0)
                      <= _unshuffle(lax.broadcasted_iota(I32, (TILE, TILE), 1)))
            queries, keys, values = (r.at[_ds(h * (r.shape[0] // GROUP), r.shape[0] // GROUP)] for r in projected[par])
            result = ctx.at[_ds(head_id * (SEQ // 2), SEQ // 2)]
            pending = {}

            def fold(op, t):
                return functools.reduce(op, [t[r:r + 8] for r in range(0, TILE, 8)])

            def scores(i):
                q = _matrix(queries[i * TILE // 2:(i + 1) * TILE // 2, :])
                tiles, peaks = [], []
                for j in range(i + 1):
                    k = _matrix(keys[j * TILE // 2:(j + 1) * TILE // 2, :])
                    s = pacer.mark(lax.dot_general(k, q, NT_DIMS, preferred_element_type=F32))
                    if j == i:
                        s = jnp.where(causal, s, MASKED * LOG2E)
                    tiles.append(s)
                    peaks.append(fold(jnp.maximum, s))
                    yield w_qk
                top = jnp.max(functools.reduce(jnp.maximum, peaks), axis=0, keepdims=True)
                if 0 < i // 2 and i // 2 >= NPAIR - fast:
                    mass = functools.reduce(jnp.add, [jnp.exp2(x - top) for x in peaks])
                    top = top + jnp.log2(jnp.sum(mass, axis=0, keepdims=True))
                pending[i] = tiles, jnp.broadcast_to(top, (8, TILE))

            def context(i):
                both = [pending.pop(2 * i + c) for c in range(2)]
                totals = [None, None]
                o = [[None, None], [None, None]]

                def weight(j, c):
                    p = jnp.exp2(both[c][0][j] - _cat([hold(both[c][1])] * (TILE // 8), 0))
                    t = fold(jnp.add, p)
                    totals[c] = t if totals[c] is None else totals[c] + t
                    return p

                def product(j, p, x):
                    v = _matrix(values[(j * 7 + p) * DB // 4:(j * 7 + p + 1) * DB // 4, :])
                    return pacer.mark(jnp.dot(v, x.astype(BF16), preferred_element_type=F32))

                def emit(a, c, v):
                    o[a][c] = v if o[a][c] is None else o[a][c] + v

                def plain(j, c, tiles):
                    for b in range(tiles):
                        p = weight(2 * j + b, c)
                        shared = product(j, 2 + b, p)
                        emit(b, c, shared)
                        emit(1 - b, c, shared + product(j, 5 + b, p))
                        yield w_diag

                def diagonal():
                    yield from plain(i, 0, 1)
                    yield from plain(i, 1, 2)

                if early_diag:
                    yield from diagonal()
                acc = [None] * 7
                for j in range(i):
                    if i < NPAIR - fast:
                        yield from plain(j, 0, 2)
                        yield from plain(j, 1, 2)
                        continue
                    tiles, n = {}, 0
                    for p in late:
                        if p == ',':
                            yield 4 / 7 * n
                            n = 0
                            continue
                        p = int(p)
                        for _, b, c in RHS_TERMS[p]:
                            if (b, c) not in tiles:
                                tiles[b, c] = weight(2 * j + b, c)
                        t = product(j, p, _operand(RHS_TERMS[p], lambda b, c: [[tiles[b, c]]])[0][0])
                        acc[p] = t if acc[p] is None else acc[p] + t
                        n += 1
                if acc[0] is not None:
                    _run(_multiply(lambda p: acc[p], emit, 1))
                if not early_diag:
                    yield from diagonal()
                for c in range(2):
                    x = _cat([o[0][c], o[1][c]], 0) * _reciprocal(jnp.sum(totals[c], axis=0, keepdims=True))
                    result[(2 * i + c) * TILE // 2:(2 * i + c + 1) * TILE // 2, :] = pltpu.bitcast(x.astype(BF16).T, U32)

            for n in range(NPAIR + 1):
                streams = []
                if n < NPAIR:
                    i = order[n]
                    streams.append((_chain(scores(2 * i), scores(2 * i + 1)), (4 * i + 3) * w_qk, *mix[0:2]))
                if n > 0:
                    streams.append((context(order[n - 1]), 4 * order[n - 1] + 3, *mix[2:4]))
                yield from _merge(*streams)

        def n_attend(w_qk, fast=NPAIR, w_diag=1, **_):
            plain = 3 * NPAIR + 2 * (NPAIR - fast) * (NPAIR - fast - 1)
            return NTILE * (NTILE + 1) * (1 + w_qk) / 2 + plain * (w_diag - 1)

        def build_wo(head_id, hold):
            n = KO // HB
            src, dst = bwo_raw.at[:, _ds(head_id * n, n)], _shifted(ro, head_id, HB, n // 2)
            for ct in range(TPB):
                for s in range(0, n, 16):
                    def load(i, j, hold):
                        c0 = (j * TPB + ct) * LANES
                        v = src[i, pl.ds(s, 16), c0:c0 + LANES].astype(F32)
                        return [hold(v[0:8]), hold(v[8:16])]

                    def store(p, words):
                        dst[pl.ds(((p * TPB + ct) * KO + s) // 2, 8), :] = words

                    yield from _build_operands(RHS_TERMS, load, store, hold)

        n_wo = TPB * (KO // HB // 16) * 7

        def head_step(par, g, h, more):
            SPARSE[0] = sparse
            pacer = _Pacer(lc[0, 0, 0:8, :])
            hold = pacer.after(lag4 if more else lag5)
            head_id = g * GROUP + h
            if more:
                _interleave((attend(par, h, head_id, pacer, **head), n_attend(**head), *sp_att),
                            (_chain(*[project(1 - par, w, h, pacer.mark) for w in p_order]), n_project, *sp_proj),
                            (build_wo(head_id, hold), n_wo, *sp_wo),
                            (build_group(par, h, pacer.after(lagw)), n_group, *sp_w))
            else:
                _interleave((attend(par, h, head_id, pacer, **tail), n_attend(**tail)),
                            (build_wo(head_id, hold), n_wo, *sp_wo5),
                            (_chain(*[shuffle_columns(0, t, hold, [h]) for t in range(3)]),
                             3 * n_shuffle / NS, *sp_sh5))

        if 'p4' in dbg or 'p5' in dbg:
            touch(lx, lc, rq1, rk1, rv1, ks0, vs0, qs0, sq0, sk0, sv0, bwo_raw, wqkv_raw)
            touch(qs1, ks1, vs1, spare, lo, stage)
            with jax.named_scope('dbg'):
                _loop(16, lambda t: head_step(int('p5' in dbg), t // GROUP, t % GROUP, 'p4' in dbg))
            touch(wp, ctx, ro, qs1, ks1, vs1, rq0, rk0, rv0)
            return

        def start_up():
            data = {'k': weight_copies(0, 0, 1), 'v': weight_copies(0, 0, 2), 'q': weight_copies(0, 0, 0),
                    'g1': group_copies(1, 1), 'g2': group_copies(0, 2), 'o': wo_copies(0)}
            for part in range(GROUP):
                data['c%d' % part], data['x%d' % part] = c_copies(part), x_copies(part)

            def operands(job, hold, tops=range(7)):
                if job[0] == '!':
                    def await_copies():
                        _wait(data[job[1:]])
                        yield 1e-6

                    return await_copies(), 1e-6
                kind, part = job[0], int(job[1])
                if kind in 'cx':
                    src, dst = (c_raw, lc) if kind == 'c' else (bwo_raw, lx)
                    return build_activations(src, dst, part, hold, tops), n_activations(src.shape[2])
                if kind == 'g':
                    return build_group(1, part, hold), n_group
                return build_weights(0, 'qkv'.index(kind), part, hold, tops), n_weights('qkv'.index(kind))

            def expand(jobs):
                return [j for job in jobs.split() for j in ([job + str(u) for u in range(GROUP)] if len(job) == 1 else [job])]

            def issue(starts):
                for k in starts.split():
                    if k.isdigit():
                        pl.delay(int(k))
                        continue
                    for c in data[k.rstrip('*')]:
                        c.start(priority=int(k.endswith('*')))

            def step(n, waits, starts, products, ahead, jobs):
                lag, *span, SPARSE[0] = paces.get('s%d' % n, (3, .03, .95, 2))
                with jax.named_scope('s%d_wait' % n):
                    _wait([c for k in waits.split() for c in data[k]])
                    issue(starts)
                with jax.named_scope('s%d_mm' % n):
                    pacer = _Pacer(pltpu.bitcast(c_raw[0, 0:16, 0:LANES], U32))
                    products = [('qkv'.index(p[0]), int(p[1])) for p in products.split()]
                    sizes = [n_project // (4 if w else 2) for w, _ in products]
                    streams = [(_chain(*[project(0, w, part, pacer.mark) for w, part in products]), sum(sizes))]
                    if ahead:
                        def first(tops, hold):
                            return _chain(*[operands(job, hold, [top])[0] for top in tops for job in expand(ahead)])

                        _run(first(TOP_ORDER[:n_ahead], _same))
                        if n_ahead < 7:
                            streams.append((first(TOP_ORDER[n_ahead:], pacer.after(lag_ahead)),
                                            sum(operands(job, None)[1] for job in expand(ahead)) * (7 - n_ahead) / 7,
                                            0., end_ahead * sizes[0] / sum(sizes)))
                    if jobs:
                        jobs = [operands(job, pacer.after(lag)) for job in expand(jobs)]
                        streams.append((_chain(*[j[0] for j in jobs]), sum(j[1] for j in jobs), *span))
                    _interleave(*streams)

            def nth(i):
                for n, args in enumerate(plan):
                    pl.when(i == n)(functools.partial(step, n, *args))

            issue(first_copies)
            _loop(len(plan), nth)

        def group(par, g):
            _wait(wo_copies(g))
            _start(wo_copies(g + 1))
            _when(g + 2 < NGROUP, lambda: _wait(group_copies(par, g + 2)))
            _when(g + 3 < NGROUP, lambda: _start(group_copies(1 - par, g + 3)))
            if par == 0:
                _when(g == NGROUP - 2, lambda: _start(a_inputs))
            _loop(GROUP, lambda h: head_step(par, g, h, True))

        def two_groups(t):
            group(0, 2 * t)
            _when(t < NGROUP // 2 - 1, lambda: group(1, 2 * t + 1))

        if 'p4s' in dbg:
            touch(lx, lc, rq1, rk1, rv1, ks0, vs0, qs0, sq0, sk0, sv0, bwo_raw, wqkv_raw)
            _loop(4, lambda t: group(0, 2 * t))
            touch(wp, ctx, ro, qs1, ks1, vs1, rq0, rk0, rv0)
            return

        if 'p5s' in dbg:
            touch(qs1, ks1, vs1, bwo_raw, wqkv_raw)
            _loop(GROUP, lambda h: head_step(1, NGROUP - 1, h, False))
            touch(wp, ctx, ro)
            return
        if not dbg or 'start' in dbg:
            with jax.named_scope('start_up'):
                start_up()
        if 'start' in dbg:
            _wait(group_copies(0, 2) + wo_copies(0))
            touch(qs0, ks0, vs0, rq1, rk1, rv1)
            return
        if not dbg:
            with jax.named_scope('heads'):
                _loop(NGROUP // 2, two_groups)
            with jax.named_scope('last_heads'):
                _wait(wo_copies(NGROUP - 1) + a_inputs)
                _loop(GROUP, lambda h: head_step(1, NGROUP - 1, h, False))

        la, qa = lx, qs0

        def w_a(t, p, ct, r0, rows):
            if t == 0:
                return (rq0, rq1)[ct], (p, _ds(r0, rows))
            if t == 1:
                return lc, (p, 0, _ds(ct * (KQ // 2) + r0, rows))
            if t == 2:
                buf, tile = divmod(TPB * p + ct, 25)
                assert rows <= 64 or rows == 128
                if rows == 128:
                    return (rk0, rk1, rv0, rv1)[buf], (pl.ds(2 * tile, 2),)
                return (rk0, rk1, rv0, rv1)[buf], (2 * tile + r0 // 64, _ds(r0 % 64, rows))
            buf, tile = divmod(TPB * p, 50)
            return (vs0, vs1)[buf], (_ds((tile + ct) * (KQ // 2) + r0, rows),)

        def load_w(t, p):
            tiles = []
            for ct in range(TPB):
                buf, idx = w_a(t, p, ct, 0, KQ // 2)
                tiles.append(_matrix(buf[idx].reshape(KQ // 2, LANES)))
            return _cat(tiles, 1)

        span_a = HALO + SEQ // 2
        group_rows = 16 * NS

        def build_w(blk, t, hold):
            for s in range(0, WROWS, 16):
                for ct in range(TPB):
                    def load(i, j, hold):
                        return _split(hold(wp[wp_rows(t, i, s, j * TPB + ct), :]))

                    def store(p, words):
                        buf, idx = w_a(t, p, ct, (blk * WROWS + s) // 2, 8)
                        buf[idx] = words

                    yield from _build_operands(RHS_TERMS, load, store, hold)

        n_w = (WROWS // 16) * TPB * 7

        def build_x(blk, hold):
            for c in range(ROWS // group_rows):
                for t in range(TPB):
                    def load(i, j, hold):
                        words = ax_raw.at[j * TPB + t].bitcast(U32).at[_ds(blk * (ROWS // 2), ROWS // 2)]
                        w0 = (c * group_rows + 32 * (i // 2)) // 2
                        return [_split(hold(words[pl.ds(w0 + e, 8, stride=2), :]))[i % 2] for e in range(2)]

                    def store(p, words):
                        la[p, t, _ds((blk * (ROWS // NS) + 16 * c) // 2, 8), :] = words

                    yield from _build_operands(LHS_TERMS, load, store, hold)

        n_x = (ROWS // group_rows) * TPB * 7

        def build_awo(blk, hold):
            ct, odd, h0 = blk // 4, (blk // 2) % 2, 16 * (blk % 2)
            pairs = DHA // 2 // NS
            for dp in range(0, pairs, 2):
                src = {}
                for i in range(NS):
                    for j in range(NS):
                        words = awo_raw.at[j * TPB + ct].bitcast(U32).at[pl.ds(pl.multiple_of(h0 * 16, 256), 256)]
                        for e in range(2):
                            w0 = 8 * e * 16 + i * pairs + dp
                            src[i, j, e] = hold(jnp.where(odd == 1, words[pl.ds(w0 + 1, 8, stride=16), :],
                                                          words[pl.ds(w0, 8, stride=16), :]))
                    yield
                for half in range(2):
                    def load(i, j, hold):
                        return [_split(hold(src[i, j, e]))[half] for e in range(2)]

                    def store(p, words):
                        buf, idx = w_a(3, p, ct, ((2 * (dp + odd) + half) * HA + h0) // 2, 8)
                        buf[idx] = words

                    yield from _build_operands(RHS_TERMS, load, store, hold)

        n_awo = (DHA // 2 // NS // 2) * (NS + 2 * 7)

        def output_b(blk):
            SPARSE[0] = sparse6
            slot = blk % 2
            rows = ROWS // NS
            heads = HB // NS
            _when(blk >= 2, lambda: out_copy(slot, 0, DA).wait())
            pacer = _Pacer(ro[0:8, :])
            src = _shifted(ctx, blk, NBLK, ROWS // 2)
            lhs = {}

            def build_lhs(top, hold):
                half = NS // 2
                for h in range(heads):
                    for r in range(0, rows, 16):
                        def quadrant(i, j):
                            return [[_split_shuffled((hold if (a == b or sparsel == 4) and (sparsel > 1 or (i, j) == LHS_TERMS[top][0][1:]) else _same)(src[pl.ds(
                                (((j * half + b) * heads + h) * SEQ + (i * half + a) * rows + r) // 2, 8), :]))
                                for b in range(half)] for a in range(half)]

                        for p, v in enumerate(_operands(LHS_TERMS, _operand(LHS_TERMS[top], quadrant))):
                            lhs.setdefault((top * (NP // 7) + p, h), []).append(v)
                        yield

            def product(p):
                x = _cat([_cat(lhs[p, h], 0) for h in range(heads)], 1).astype(BF16)
                w = _cat([_matrix(ro[pl.ds((p * TPB + ct) * KO // 2, KO // 2), :]) for ct in range(TPB)], 1)
                return pacer.mark(jnp.dot(x, w, preferred_element_type=F32))

            def emit(i, j, v):
                stage[slot, i * rows:(i + 1) * rows, j * KQ:(j + 1) * KQ] = v.astype(BF16)

            _run(build_lhs(TOP_ORDER[0], _same))
            hold = pacer.after(lag6)
            _interleave(
                (_multiply(product, emit), NP),
                (_chain(*[build_lhs(t, pacer.after(lagl)) for t in TOP_ORDER[1:]]), 6 * heads * (rows // 16), *sp_lhs),
                *[(_chain(build_w(blk, t, hold), shuffle_columns(blk + 1, t, hold)), n_w + n_shuffle, *sp_a)
                  for t in range(3)],
                (build_x(blk, hold), n_x, *sp_x),
                (build_awo(blk, hold), n_awo, *sp_awo))
            out_copy(slot, blk * ROWS, DA).start()

        if 'p6' in dbg:
            touch(ro, ctx, ax_raw, awo_raw, wqkv_raw, wp)
        if not dbg or 'p6' in dbg:
            with jax.named_scope('output_b'):
                _loop(NBLK, output_b)
        if 'p6' in dbg:
            _wait([out_copy(0, 0, DA), out_copy(1, 0, DA)])
            touch(la, rq0, rq1, lc, rk0, rk1, rv0, rv1, ks0, ks1, vs0, vs1, wp)
            return

        def project_a(t, blk, mark):
            rows = ROWS // NS
            dst = _shifted(ro if t == 1 else ctx, blk, NBLK, ROWS // 2)

            def product(p):
                x = _cat([_matrix(la[p, k, _ds(blk * rows // 2, rows // 2), :]) for k in range(TPB)], 1)
                return mark(jnp.dot(x, load_w(t, p), preferred_element_type=F32))

            def emit(i, j, v):
                for ct in range(TPB):
                    for c in range(rows // 16):
                        piece = v[16 * c:16 * (c + 1), ct * LANES:(ct + 1) * LANES]
                        tile = 2 * (j * TPB + ct) + i % 2
                        r = c * (group_rows // 2) + 16 * (i // 2)
                        if t == 0:
                            qa[_ds(tile * ROWS + (blk % 2) * (ROWS // 2) + r, 16), :] = pltpu.bitcast(piece, U32)
                        else:
                            dst[pl.ds(tile * span_a + HALO + r, 16), :] = pltpu.bitcast(piece, U32)

            return _multiply(product, emit)

        def attend_a(blk, hold, w_lo, w_soft, holds, overlap=0, **_):
            row0, slot = blk * (ROWS // 2), blk % 2
            keys, values = (_shifted(buf, blk, NBLK, ROWS // 2) for buf in (ro, ctx))
            logits, o = {}, {}

            def window(buf, j, r, par, w):
                return pltpu.bitcast(buf[pl.ds((2 * j + par) * span_a + HALO + r - w, 8), :], F32)

            def scores(r, par):
                pos = row0 + r + lax.broadcasted_iota(I32, (8, LANES), 0)
                q = [pltpu.bitcast(qa[_ds((2 * j + par) * ROWS + slot * (ROWS // 2) + r, 8), :], F32) for j in range(8)]
                q = [hold(x) if j % holds[0] == 0 else x for j, x in enumerate(q)]
                logits[r, par] = []
                for w in range(WIN):
                    acc = q[0] * (hold if holds[1] else _same)(window(keys, 0, r, par, w))
                    for j in range(1, 8):
                        acc = acc + q[j] * window(keys, j, r, par, w)
                    acc = (hold if holds[2] else _same)(acc)
                    acc = acc + pltpu.roll(acc, 64, 1)
                    acc = acc + pltpu.roll(acc, 32, 1)
                    acc = acc * (DHA ** -0.5 * LOG2E)
                    if r < w:
                        acc = jnp.where(pos >= w, acc, MASKED * LOG2E)
                    logits[r, par].append(acc)
                    yield

            def context(r, par):
                x = logits.pop((r, par))
                top = functools.reduce(jnp.maximum, x)
                e = [jnp.exp2(t - top) for t in x]
                scale = _reciprocal(functools.reduce(jnp.add, e))
                e = [t * scale for t in e]
                yield w_soft
                for j in range(8):
                    acc = None
                    for w in range(WIN):
                        v = window(values, j, r, par, w)
                        t = e[w] * (hold(v) if w % holds[3] == 0 else v)
                        acc = t if acc is None else acc + t
                    o[r, par, j] = acc
                    yield

            def attention(c):
                units = [(r, par) for r in range(c * group_rows // 2, (c + 1) * group_rows // 2, 8) for par in range(2)]
                if overlap & 1:
                    yield from scores(*units[0])
                    for now, after in zip(units, units[1:]):
                        yield from _merge((scores(*after), WIN), (context(*now), 8 + w_soft))
                    yield from context(*units[-1])
                else:
                    for unit in units:
                        yield from _chain(scores(*unit), context(*unit))

            def operands(c):
                for t in range(TPB):
                    def load(i, j, hold):
                        return [hold(o[c * (group_rows // 2) + 8 * i, par, j * TPB + t]) for par in range(2)]

                    def store(p, words):
                        lo[blk % slots * NP + p, t, 8 * c:8 * (c + 1), :] = words

                    yield from _weigh(_build_operands(LHS_TERMS, load, store, hold), w_lo)

            groups = ROWS // group_rows
            if overlap & 2:
                yield from attention(0)
                for c in range(1, groups):
                    yield from _merge((attention(c), (16 + w_soft) * group_rows // 8),
                                      (operands(c - 1), TPB * 7 * w_lo, 0., overlap // 4 / 10 or 1.))
                yield from operands(groups - 1)
            else:
                for c in range(groups):
                    yield from _chain(attention(c), operands(c))

        def output_a(blk, mark):
            slot = blk % 2

            def product(p):
                x = _cat([_matrix(lo[blk % slots * NP + p, k]) for k in range(TPB)], 1)
                return mark(jnp.dot(x, load_w(3, p), preferred_element_type=F32))

            def emit(i, j, v):
                for c in range(ROWS // group_rows):
                    r = c * group_rows + 16 * i
                    stage[slot, r:r + 16, j * KQ:(j + 1) * KQ] = v[16 * c:16 * (c + 1)].astype(BF16)

            return _multiply(product, emit)

        def outputs_a(blocks, mark):
            for n, blk in enumerate(blocks):
                if n > 0:
                    out_copy((blk - 1) % 2, (blk - 1) * ROWS, 0).start()
                    out_copy(blk % 2, 0, 0).wait()
                yield from output_a(blk, mark)

        def step_a(i, pace, outputs, project=True):
            SPARSE[0] = pace['sparse'] if pace else 0
            pacer = _Pacer(lc[0, 0, 0:8, :])
            matmuls = [project_a(t, i + 1, pacer.mark) for t in (pace['order'] if pace else (1, 2, 0))] if project else []
            matmuls.insert(pace.get('o_at', 0) if pace else 0, outputs_a(outputs, pacer.mark))
            streams = [(_chain(*matmuls), (len(outputs) + len(matmuls) - 1) * NP)]
            if pace:
                n = (16 + pace['w_soft']) * (ROWS // 8) + TPB * (ROWS // group_rows) * 7 * pace['w_lo']
                streams.append((attend_a(i, pacer.after(pace['lag']), **pace), n, *pace['span']))
            if outputs:
                out_copy(outputs[0] % 2, 0, 0).wait()
            _interleave(*streams)
            if outputs:
                out_copy(outputs[-1] % 2, outputs[-1] * ROWS, 0).start()

        if dbg:
            touch(la, rq0, rq1, lc, rk0, rk1, rv0, rv1, ks0, ks1, vs0, vs1, lo, qa, ro, ctx)
            if 'pa' in dbg:
                _loop(NBLK - 1 - delay, lambda t: step_a(t + delay, a_main, [t]))
            elif 'pa3' in dbg:
                step_a(NBLK - 1, a_last, range(NBLK - 1 - delay, NBLK - 1), project=False)
                step_a(NBLK, None, [NBLK - 1], project=False)
            elif 'pa1' in dbg:
                _loop(delay, lambda t: step_a(t, a_first, []))
            touch(lo, qa, ro, ctx)
            return

        for tile in range(16):
            for buf in (ro, ctx):
                buf[tile * span_a:tile * span_a + HALO, :] = jnp.zeros((HALO, LANES), U32)
        with jax.named_scope('a_first'):
            step_a(-1, None, [])
            _loop(delay, lambda t: step_a(t, a_first, []))
        with jax.named_scope('a_main'):
            _loop(NBLK - 1 - delay, lambda t: step_a(t + delay, a_main, [t]))
        with jax.named_scope('a_last'):
            step_a(NBLK - 1, a_last, range(NBLK - 1 - delay, NBLK - 1), project=False)
            step_a(NBLK, None, [NBLK - 1], project=False)
        _wait([out_copy(0, 0, 0), out_copy(1, 0, 0)])

    def words(*shape):
        return pltpu.VMEM(shape + (LANES,), U32)

    scratch = [
        pltpu.VMEM((DA // LANES, SEQ, LANES), BF16),
        pltpu.VMEM((DA, 3 * DA), BF16),
        pltpu.VMEM((DA // LANES, DA, LANES), BF16),
        pltpu.VMEM((NS, MQ, DC), BF16),
        pltpu.VMEM((NS, KO, MB), BF16),
        words(NP, MB // NS // LANES, MQ // 2),
        words(NP, DC // NS // LANES, MQ // 2),
        *[words(NP, MB // NS // 2)] * 2,
        *[words(NP + 1, DC // NS // 2)] * 4,
        *[words(GROUP * SEQ // 2)] * 4,
        *[words(GROUP * NPAIR * 7 * DB // 4)] * 2,
        *[words(GROUP * MB // 2)] * 2,
        *[words(GROUP * DC // 2)] * 4,
        words(HB * SEQ // 2),
        words(NP * TPB * KO // 2),
        words(slots * NP, TPB, ROWS // NS // 2),
        pltpu.VMEM((2, ROWS, DA), BF16),
        words(pad),
        pltpu.SemaphoreType.DMA((GROUP,)),
        pltpu.SemaphoreType.DMA((GROUP,)),
        pltpu.SemaphoreType.DMA(()),
        pltpu.SemaphoreType.DMA((6,)),
        pltpu.SemaphoreType.DMA(()),
        pltpu.SemaphoreType.DMA((2,)),
    ]

    def run(A_x, A_wqkv, A_wo, B_x, B_c_kv, B_w_q, B_w_uk, B_w_uv, B_w_o):
        hbm = pl.BlockSpec(memory_space=pl.ANY)
        out = pl.pallas_call(
            kernel,
            in_specs=[hbm] * 9,
            out_specs=hbm,
            out_shape=jax.ShapeDtypeStruct((SEQ, DA + MB), BF16),
            scratch_shapes=scratch,
            compiler_params=pltpu.CompilerParams(vmem_limit_bytes=127 * 2 ** 20),
            name=name,
        )(A_x.reshape(SEQ, DA), A_wqkv, A_wo, B_x.reshape(GROUP, NS, PART, MB), B_c_kv.reshape(GROUP, NS, PART, DC),
          B_w_q.reshape(MB // 2, 2 * HB, DB), B_w_uk.reshape(DC // 2, 2 * HB, DB),
          B_w_uv.reshape(DC // 2, 2 * HB, DB), B_w_o.reshape(NS, KO, MB))
        return out.reshape(1, SEQ, DA + MB)

    return run


_fused_call = build()


@jax.jit
def pallas_concat_heads__sliding_local_dilated__compressed_kv_cla__prompt_kernel(A_x, A_wqkv, A_wo, B_x, B_c_kv, B_w_q, B_w_uk, B_w_uv, B_w_o):
    return _fused_call(A_x, A_wqkv, A_wo, B_x, B_c_kv, B_w_q, B_w_uk, B_w_uv, B_w_o)
```

```python
import functools
import math

import jax
import jax.numpy as jnp
from jax import lax
import jax.experimental.pallas as pl
import jax.experimental.pallas.tpu as pltpu

F32 = jnp.float32
BF16 = jnp.bfloat16
U32 = jnp.uint32
I32 = jnp.int32
LANES = 128
NT_DIMS = (((1,), (1,)), ((), ()))
LOG2E = math.log2(math.e)
MASKED = -1e9

SEQ = 2048
DA = 1024
HA, DHA = 32, 32
WIN = 8
HALO = 32
MB = 1024
HB, DB = 32, 128
DC = 512

LEVELS = 2
NS = 2 ** LEVELS
NP = 7 ** LEVELS
GROUP = NS
NGROUP = HB // GROUP
MQ = SEQ // NS
PART = MQ // GROUP
ROWS = 256
NBLK = SEQ // ROWS
KQ = DA // NS
TPB = KQ // LANES
KO = HB * DB // NS
WROWS = KQ // NBLK
TILE = LANES
NPAIR = SEQ // TILE // 2
DELAY = 2
SLOTS = 4

START_UP = (
    ("c0 k", "c2 c3", "k0", "c0 k", "", 1, (0., 1.)),
    ("v c1", "q x0", "v0", "v", "c1", 40, (.04, .9)),
    ("c2 c3", "x1 x2 x3", "k1 v1 k2 v2 k3", "", "c2 c3 !q +g1 q !x0 x0", 14, (.07, 1.)),
    ("x1 x2", "", "q0 q1", "", "x1 x2", 1, (.02, .96)),
    ("x3 g1", "g2 o", "q2 v3 q3", "", "x3 g", 10, (.07, 1.)),
)
PAIR_ORDER = (1, 3, 5, 7, 6, 4, 2, 0)
HEAD = dict(lag=9, bursts=((1,), (4,), (0,), (2,), (5,), (3,), (6,)), fast=NPAIR,
            score_weight=1, score_span=(0, .7), context_span=(.15, 1))
LAST_HEAD = dict(lag=11, bursts=((1, 4), (0, 2), (5, 3), (6,)), fast=5,
                 score_weight=1.1, score_span=(0, .6), context_span=(.25, 1))
A_FIRST = dict(lag=3, span=(.02, .98), softmax_weight=1, operand_weight=7, hold_q=8, hold_sum=False, hold_v=4)
A_MAIN = dict(lag=6, span=(.08, .99), softmax_weight=3, operand_weight=4, hold_q=8, hold_sum=False, hold_v=8)
A_LAST = dict(lag=2, span=(.02, 1.), softmax_weight=4, operand_weight=8, hold_q=1, hold_sum=True, hold_v=8)


LHS_TERMS = (((1, 0, 0), (1, 1, 1)), ((1, 1, 0), (1, 1, 1)), ((1, 0, 0),), ((1, 1, 1),),
             ((1, 0, 0), (1, 0, 1)), ((1, 1, 0), (-1, 0, 0)), ((1, 0, 1), (-1, 1, 1)))
RHS_TERMS = (((1, 0, 0), (1, 1, 1)), ((1, 0, 0),), ((1, 0, 1), (-1, 1, 1)), ((1, 1, 0), (-1, 0, 0)),
             ((1, 1, 1),), ((1, 0, 0), (1, 0, 1)), ((1, 1, 0), (1, 1, 1)))
TOP_ORDER = (1, 3, 0, 6, 4, 2, 5)


def _add(x, y):
    return [[a + b for a, b in zip(rx, ry)] for rx, ry in zip(x, y)]


def _sub(x, y):
    return [[a - b for a, b in zip(rx, ry)] for rx, ry in zip(x, y)]


def _operand(terms, quadrant):
    total = None
    for sign, i, j in terms:
        q = quadrant(i, j)
        total = q if total is None else (_add if sign > 0 else _sub)(total, q)
    return total


def _operands(side, blocks):
    half = len(blocks) // 2
    if half == 0:
        return [blocks[0][0]]

    def quadrant(i, j):
        return [row[j * half:(j + 1) * half] for row in blocks[i * half:(i + 1) * half]]

    return [x for terms in side for x in _operands(side, _operand(terms, quadrant))]


def _multiply(product, emit, level=LEVELS, base=0):
    if level == 0:
        emit(0, 0, product(base))
        yield
        return
    n = 2 ** (level - 1)

    def m(i):
        out = [[None] * n for _ in range(n)]

        def keep(a, b, v):
            out[a][b] = v

        yield from _multiply(product, keep, level - 1, base + (i - 1) * 7 ** (level - 1))
        return out

    def put(x, oi, oj):
        for a in range(n):
            for b in range(n):
                emit(oi * n + a, oj * n + b, x[a][b])

    m2 = yield from m(2)
    m4 = yield from m(4)
    put(_add(m2, m4), 1, 0)
    m1 = yield from m(1)
    c11 = _add(m1, m4)
    c22 = _sub(m1, m2)
    m7 = yield from m(7)
    c11 = _add(c11, m7)
    m5 = yield from m(5)
    put(_sub(c11, m5), 0, 0)
    m3 = yield from m(3)
    put(_add(m3, m5), 0, 1)
    c22 = _add(c22, m3)
    m6 = yield from m(6)
    put(_add(c22, m6), 1, 1)


def _build_operands(side, load, store, hold, hold_all=False, tops=range(7)):
    half = NS // 2
    for top in tops:
        terms = side[top]
        loaded = {(i, j): [[load(i * half + a, j * half + b, hold if hold_all or (a == b and n == 0) else _same)
                            for b in range(half)] for a in range(half)]
                  for n, (_, i, j) in enumerate(terms)}
        lo, hi = (_operands(side, _operand(terms, lambda i, j: [[x[e] for x in row] for row in loaded[i, j]]))
                  for e in range(2))
        for p in range(NP // 7):
            store(top * (NP // 7) + p, _join(lo[p], hi[p]))
        yield


def _split(words):
    return pltpu.bitcast(words << 16, F32), pltpu.bitcast(words & jnp.uint32(0xFFFF0000), F32)


def _join(lo, hi):
    return pltpu.bitcast(pltpu.pack_elementwise([lo, hi], packed_dtype=BF16), U32)


def _join_shuffled(v):
    r, c = v.shape
    v = v.reshape(r // 16, 2, 8, c)
    return _join(v[:, 0].reshape(r // 2, c), v[:, 1].reshape(r // 2, c))


def _split_shuffled(words):
    lo, hi = _split(words)
    r, c = words.shape
    return jnp.stack([lo.reshape(r // 8, 8, c), hi.reshape(r // 8, 8, c)], axis=1).reshape(2 * r, c)


def _unshuffle(pos):
    return (pos & ~15) + ((pos & 15) >> 1) + 8 * (pos & 1)


def _matrix(words):
    return pltpu.bitcast(words, BF16)


def _cat(xs, axis):
    return xs[0] if len(xs) == 1 else jnp.concatenate(xs, axis=axis)


def _ds(start, size):
    if isinstance(start, int):
        return pl.ds(start, size)
    return pl.ds(pl.multiple_of(start, min(size, 16)), size)


def _shifted(ref, step, steps, n):
    return ref.at[_ds(step * n, ref.shape[0] - (steps - 1) * n)]


def _loop(n, body):
    lax.fori_loop(0, n, lambda i, carry: body(i), None)


def _start(copies):
    for c in copies:
        c.start()


def _wait(copies):
    for c in copies:
        c.wait()


def _run(steps):
    for _ in steps:
        pass


def _chain(*streams):
    for steps in streams:
        yield from steps


def _weigh(steps, weight):
    for _ in steps:
        yield weight


def _merge(*streams):
    spans = [s[2:] if len(s) > 2 else (0.0, 1.0) for s in streams]
    done = [0.0] * len(streams)
    live = list(range(len(streams)))
    while live:
        i = min(live, key=lambda k: spans[k][0] + (spans[k][1] - spans[k][0]) * done[k] / streams[k][1])
        try:
            weight = next(streams[i][0])
        except StopIteration:
            live.remove(i)
            continue
        weight = 1 if weight is None else weight
        done[i] += weight
        yield weight


def _interleave(*streams):
    _run(_merge(*streams))


class _Pacer:
    def __init__(self, words):
        self.odd = words | 1
        self.marks = []

    def mark(self, v):
        self.marks.append(pltpu.bitcast(v[:, 0:LANES], U32))
        return v

    def after(self, lag):
        def hold(x):
            if len(self.marks) < lag:
                return x
            rows = x.shape[0]
            never = jnp.concatenate([self.odd] * (rows // 8), axis=0) == 0
            return pltpu.bitcast(jnp.where(never, self.marks[-lag][0:rows], pltpu.bitcast(x, U32)), x.dtype)

        return hold


def _same(x):
    return x


def _reciprocal(x):
    r = pltpu.reciprocal(x, approx=True)
    return r * (2.0 - x * r)


def _kernel(ax_hbm, wqkv_hbm, awo_hbm, bx_hbm, c_hbm, wq_hbm, wuk_hbm, wuv_hbm, bwo_hbm, out_hbm,
            ax_raw, wqkv_raw, awo_raw, c_raw, bwo_raw,
            lx, lc, rq0, rq1, rk0, rk1, rv0, rv1, qs0, qs1, ks0, ks1, vs0, vs1,
            sq0, sq1, sk0, sk1, sv0, sv1, ctx, ro, lo, stage,
            sem_c, sem_x, sem_wo, sem_w, sem_a, sem_out):

    def out_copy(n):
        return pltpu.make_async_copy(
            stage.at[n % 2], out_hbm.at[_ds(n % NBLK * ROWS, ROWS), _ds((1 - n // NBLK) * DA, DA)], sem_out.at[n % 2])

    a_inputs = ([pltpu.make_async_copy(ax_hbm.at[:, pl.ds(j * LANES, LANES)], ax_raw.at[j], sem_a)
                 for j in range(DA // LANES)]
                + [pltpu.make_async_copy(awo_hbm.at[:, pl.ds(j * LANES, LANES)], awo_raw.at[j], sem_a)
                   for j in range(DA // LANES)]
                + [pltpu.make_async_copy(wqkv_hbm, wqkv_raw, sem_a)])

    wp = ks0

    def wp_rows(t, i, s, c):
        return _ds((((t * NS + i) * (WROWS // 16) + s // 16) * 8 + c) * 8, 8)

    def shuffle_columns(blk, t, hold, quarters=range(NS)):
        lane = lax.broadcasted_iota(I32, (8, LANES), 1)
        slot, chunk, low = lane >> 5, (lane & 31) >> 2, lane & 3
        head_of = _unshuffle(lane & 31)
        for s in range(0, WROWS, 16):
            for i in quarters:
                rows = _ds(i * KQ + (blk % NBLK) * WROWS + s, 16)
                moved = []
                for j in range(8):
                    c0 = t * DA + j * LANES
                    u = hold(pltpu.bitcast(wqkv_raw[rows, c0:c0 + LANES], I32))
                    moved.append(jnp.take_along_axis(u, low * 32 + 4 * ((chunk - j) & 7) + slot, axis=1))
                    if j % 4 == 3:
                        yield
                v = [moved[-c % 8] for c in range(8)]
                for bit in (1, 2, 4):
                    v = [jnp.where((chunk & bit) != 0, v[(c - bit) % 8], v[c]) for c in range(8)]
                for c in range(8):
                    source = slot * 32 + (((head_of >> 2) + c) & 7) * 4 + (head_of & 3)
                    wp[wp_rows(t, i, s, c), :] = pltpu.bitcast(jnp.take_along_axis(v[c], source, axis=1), U32)
                    if c % 4 == 3:
                        yield

    n_shuffle = (WROWS // 16) * NS * 4

    weights = ((rq0, rk0, rv0), (rq1, rk1, rv1))
    projected = ((qs0, ks0, vs0), (qs1, ks1, vs1))
    staged = ((sq0, sk0, sv0), (sq1, sk1, sv1))

    def weight_copies(par, grp, w):
        words = (wq_hbm, wuk_hbm, wuv_hbm)[w].bitcast(U32)
        n = words.shape[0]
        return [pltpu.make_async_copy(
            words.at[:, (HB // 2) * parity + grp * (GROUP // 2) + pair],
            staged[par][w].at[pl.ds((2 * pair + parity) * n, n)], sem_w.at[3 * par + w])
            for pair in range(GROUP // 2) for parity in range(2)]

    def group_copies(par, grp):
        return [c for w in range(3) for c in weight_copies(par, grp, w)]

    def c_copies(part):
        return [pltpu.make_async_copy(c_hbm.at[part], c_raw.at[:, pl.ds(part * PART, PART)], sem_c.at[part])]

    def x_copies(part):
        return [pltpu.make_async_copy(bx_hbm.at[part], bwo_raw.at[:, pl.ds(part * PART, PART)], sem_x.at[part])]

    def wo_copies(grp):
        rows = (slice(None), _ds(grp * (KO // NGROUP), KO // NGROUP))
        return [pltpu.make_async_copy(bwo_hbm.at[rows], bwo_raw.at[rows], sem_wo)]

    def build_weights(par, w, part, hold, tops=range(7)):
        n = (MB, DC, DC)[w] // 2
        rows = n // NS // GROUP
        src = _shifted(staged[par][w], part, GROUP, rows)
        for s in range(0, rows, 8):
            def load(i, j, hold):
                return [_split(hold(src[pl.ds((2 * (j // 2) + e) * n + i * (n // NS) + s, 8), :]))[j % 2]
                        for e in range(2)]

            def store(p, words):
                weights[par][w][p, _ds(part * rows + s, 8), :] = words

            yield from _build_operands(RHS_TERMS, load, store, hold, tops=tops)

    def n_weights(w):
        return (MB, DC, DC)[w] // NS // GROUP // 16 * 7

    def build_group(par, part, hold):
        return _chain(*[build_weights(par, w, part, hold) for w in range(3)])

    n_group = sum(n_weights(w) for w in range(3))

    def build_activations(src, dst, part, hold, tops=range(7)):
        tiles = src.shape[2] // NS // LANES
        for t in range(tiles):
            for s in range(0, PART, 16):
                r = part * PART + s

                def load(i, j, hold):
                    c0 = (j * tiles + t) * LANES
                    return _split(hold(pltpu.bitcast(src[i, pl.ds(r, 16), c0:c0 + LANES], U32)))

                def store(p, words):
                    dst[p, t, pl.ds(r // 2, 8), :] = words

                yield from _build_operands(LHS_TERMS, load, store, hold, tops=tops)

    def n_activations(width):
        return width // NS // LANES * (PART // 16) * 7

    def project(par, w, part, mark):
        lhs = lx if w == 0 else lc
        tiles = lhs.shape[1]
        dst = projected[par][w]
        dst = _shifted(dst, part, GROUP, dst.shape[0] // GROUP // GROUP)
        pending = {}

        def product(p):
            x = _cat([_matrix(lhs[p, t, _ds(part * PART // 2, PART // 2), :]) for t in range(tiles)], 1)
            return mark(jnp.dot(x, _matrix(weights[par][w][p]), preferred_element_type=F32))

        def emit(i, j, v):
            if w < 2:
                dst[pl.ds((j * SEQ + i * PART) // 2, PART // 2), :] = (
                    pltpu.bitcast(v.astype(BF16), U32) if w else _join_shuffled(v * (DB ** -0.5 * LOG2E)))
            else:
                pending[i, j] = v.T
                if i % 2 == 1:
                    pair = [pending.pop((i - 1 + b, j)) for b in range(2)]
                    blocks = [[t[a * DB // 2:(a + 1) * DB // 2] for t in pair] for a in range(2)]
                    for p, x in enumerate(_operands(LHS_TERMS, blocks)):
                        dst[pl.ds(((j * NPAIR + i // 2) * 7 + p) * DB // 4, DB // 4), :] = _join_shuffled(x)

        return _weigh(_multiply(product, emit), tiles)

    n_project = NP * (MB + 2 * DC) // NS // LANES

    def attend(par, h, head_id, pacer, lag, bursts, fast, score_weight, score_span, context_span):
        hold = pacer.after(lag)
        causal = (lax.broadcasted_iota(I32, (TILE, TILE), 0)
                  <= _unshuffle(lax.broadcasted_iota(I32, (TILE, TILE), 1)))
        queries, keys, values = (r.at[_ds(h * (r.shape[0] // GROUP), r.shape[0] // GROUP)] for r in projected[par])
        result = ctx.at[_ds(head_id * (SEQ // 2), SEQ // 2)]
        pending = {}

        def fold(op, t):
            return functools.reduce(op, [t[r:r + 8] for r in range(0, TILE, 8)])

        def scores(i):
            q = _matrix(queries[i * TILE // 2:(i + 1) * TILE // 2, :])
            tiles, peaks = [], []
            for j in range(i + 1):
                k = _matrix(keys[j * TILE // 2:(j + 1) * TILE // 2, :])
                s = pacer.mark(lax.dot_general(k, q, NT_DIMS, preferred_element_type=F32))
                if j == i:
                    s = jnp.where(causal, s, MASKED * LOG2E)
                tiles.append(s)
                peaks.append(fold(jnp.maximum, s))
                yield score_weight
            top = jnp.max(functools.reduce(jnp.maximum, peaks), axis=0, keepdims=True)
            if i // 2 >= max(1, NPAIR - fast):
                mass = functools.reduce(jnp.add, [jnp.exp2(x - top) for x in peaks])
                top = top + jnp.log2(jnp.sum(mass, axis=0, keepdims=True))
            pending[i] = tiles, jnp.broadcast_to(top, (8, TILE))

        def context(i):
            both = [pending.pop(2 * i + c) for c in range(2)]
            totals = [None, None]
            o = [[None, None], [None, None]]

            def weight(j, c):
                p = jnp.exp2(both[c][0][j] - _cat([hold(both[c][1])] * (TILE // 8), 0))
                t = fold(jnp.add, p)
                totals[c] = t if totals[c] is None else totals[c] + t
                return p

            def product(j, p, x):
                v = _matrix(values[(j * 7 + p) * DB // 4:(j * 7 + p + 1) * DB // 4, :])
                return pacer.mark(jnp.dot(v, x.astype(BF16), preferred_element_type=F32))

            def emit(a, c, v):
                o[a][c] = v if o[a][c] is None else o[a][c] + v

            def plain(j, c, tiles):
                for b in range(tiles):
                    p = weight(2 * j + b, c)
                    shared = product(j, 2 + b, p)
                    emit(b, c, shared)
                    emit(1 - b, c, shared + product(j, 5 + b, p))
                    yield 1

            yield from plain(i, 0, 1)
            yield from plain(i, 1, 2)
            acc = [None] * 7
            for j in range(i):
                if i < NPAIR - fast:
                    yield from plain(j, 0, 2)
                    yield from plain(j, 1, 2)
                    continue
                tiles = {}
                for burst in bursts:
                    for p in burst:
                        for _, b, c in RHS_TERMS[p]:
                            if (b, c) not in tiles:
                                tiles[b, c] = weight(2 * j + b, c)
                        t = product(j, p, _operand(RHS_TERMS[p], lambda b, c: [[tiles[b, c]]])[0][0])
                        acc[p] = t if acc[p] is None else acc[p] + t
                    yield 4 / 7 * len(burst)
            if acc[0] is not None:
                _run(_multiply(lambda p: acc[p], emit, 1))
            for c in range(2):
                x = _cat([o[0][c], o[1][c]], 0) * _reciprocal(jnp.sum(totals[c], axis=0, keepdims=True))
                result[(2 * i + c) * TILE // 2:(2 * i + c + 1) * TILE // 2, :] = pltpu.bitcast(x.astype(BF16).T, U32)

        for n in range(NPAIR + 1):
            streams = []
            if n < NPAIR:
                i = PAIR_ORDER[n]
                streams.append((_chain(scores(2 * i), scores(2 * i + 1)), (4 * i + 3) * score_weight, *score_span))
            if n > 0:
                i = PAIR_ORDER[n - 1]
                streams.append((context(i), 4 * i + 3, *context_span))
            yield from _merge(*streams)

    def n_attend(pace):
        return NPAIR * (2 * NPAIR + 1) * (1 + pace["score_weight"])

    def build_wo(head_id, hold):
        n = KO // HB
        src, dst = bwo_raw.at[:, _ds(head_id * n, n)], _shifted(ro, head_id, HB, n // 2)
        for ct in range(TPB):
            for s in range(0, n, 16):
                def load(i, j, hold):
                    c0 = (j * TPB + ct) * LANES
                    v = src[i, pl.ds(s, 16), c0:c0 + LANES].astype(F32)
                    return [hold(v[0:8]), hold(v[8:16])]

                def store(p, words):
                    dst[pl.ds(((p * TPB + ct) * KO + s) // 2, 8), :] = words

                yield from _build_operands(RHS_TERMS, load, store, hold)

    n_wo = TPB * (KO // HB // 16) * 7

    def head_step(par, g, h):
        pacer = _Pacer(lc[0, 0, 0:8, :])
        head_id = g * GROUP + h
        _interleave((attend(par, h, head_id, pacer, **HEAD), n_attend(HEAD), 0., .86),
                    (_chain(*[project(1 - par, w, h, pacer.mark) for w in (1, 2, 0)]), n_project),
                    (build_wo(head_id, pacer.after(2)), n_wo, .02, .15),
                    (build_group(par, h, pacer.after(1)), n_group, .25, .98))

    def last_head_step(h):
        pacer = _Pacer(lc[0, 0, 0:8, :])
        hold = pacer.after(1)
        head_id = (NGROUP - 1) * GROUP + h
        _interleave((attend(1, h, head_id, pacer, **LAST_HEAD), n_attend(LAST_HEAD)),
                    (build_wo(head_id, hold), n_wo, .03, .3),
                    (_chain(*[shuffle_columns(0, t, hold, [h]) for t in range(3)]), 3 * n_shuffle / NS, .1, .8))

    def start_up():
        data = {"k": weight_copies(0, 0, 1), "v": weight_copies(0, 0, 2), "q": weight_copies(0, 0, 0),
                "g1": group_copies(1, 1), "g2": group_copies(0, 2), "o": wo_copies(0)}
        for part in range(GROUP):
            data["c%d" % part], data["x%d" % part] = c_copies(part), x_copies(part)
        built = set()

        def copies(names):
            return [c for name in names.split() for c in data[name]]

        def operands(job, hold, tops=range(7)):
            if job[0] in "!+":
                (_wait if job[0] == "!" else _start)(copies(job[1:]))
            elif job[0] in "cx":
                src, dst = (c_raw, lc) if job[0] == "c" else (bwo_raw, lx)
                yield from build_activations(src, dst, int(job[1]), hold, tops)
            else:
                for part in range(GROUP):
                    yield from (build_group(1, part, hold) if job == "g" else
                                build_weights(0, "qkv".index(job), part, hold, tops))
            built.add(job)

        size = dict(c=n_activations(DC), x=n_activations(MB), g=GROUP * n_group,
                    **{name: GROUP * n_weights(w) for w, name in enumerate("qkv")})

        def projection(name, mark):
            assert {name[0], "xcc"["qkv".index(name[0])] + name[1]} <= built
            yield from project(0, "qkv".index(name[0]), int(name[1]), mark)

        def step(waits, starts, products, ahead, jobs, lag, span):
            _wait(copies(waits))
            _start(copies(starts))
            pacer = _Pacer(pltpu.bitcast(c_raw[0, 0:16, 0:LANES], U32))
            for top in TOP_ORDER:
                for job in ahead.split():
                    _run(operands(job, _same, [top]))
            _interleave((_chain(*[projection(name, pacer.mark) for name in products.split()]),
                         sum(n_project // (2 if name[0] == "q" else 4) for name in products.split())),
                        (_chain(*[operands(job, pacer.after(lag)) for job in jobs.split()]),
                         sum(size.get(job[0], 0) for job in jobs.split()) or 1, *span))

        def steps(i):
            for n, args in enumerate(START_UP):
                pl.when(i == n)(functools.partial(step, *args))

        _start(copies("c0 k v c1"))
        _loop(len(START_UP), steps)

    def group(par, g):
        _wait(wo_copies(g))
        _start(wo_copies(g + 1))
        pl.when(g + 2 < NGROUP)(lambda: _wait(group_copies(par, g + 2)))
        pl.when(g + 3 < NGROUP)(lambda: _start(group_copies(1 - par, g + 3)))
        if par == 0:
            pl.when(g == NGROUP - 2)(lambda: _start(a_inputs))
        _loop(GROUP, lambda h: head_step(par, g, h))

    def two_groups(t):
        group(0, 2 * t)
        pl.when(t < NGROUP // 2 - 1)(lambda: group(1, 2 * t + 1))

    start_up()
    _loop(NGROUP // 2, two_groups)
    _wait(wo_copies(NGROUP - 1) + a_inputs)
    _loop(GROUP, last_head_step)

    la, qa = lx, qs0

    def w_a(t, p, ct, r0, rows):
        if t == 0:
            return (rq0, rq1)[ct], (p, _ds(r0, rows))
        if t == 1:
            return lc, (p, 0, _ds(ct * (KQ // 2) + r0, rows))
        if t == 2:
            buf, tile = divmod(TPB * p + ct, 25)
            assert rows <= 64 or rows == 128
            if rows == 128:
                return (rk0, rk1, rv0, rv1)[buf], (pl.ds(2 * tile, 2),)
            return (rk0, rk1, rv0, rv1)[buf], (2 * tile + r0 // 64, _ds(r0 % 64, rows))
        buf, tile = divmod(TPB * p, 50)
        return (vs0, vs1)[buf], (_ds((tile + ct) * (KQ // 2) + r0, rows),)

    def load_w(t, p):
        tiles = []
        for ct in range(TPB):
            buf, idx = w_a(t, p, ct, 0, KQ // 2)
            tiles.append(_matrix(buf[idx].reshape(KQ // 2, LANES)))
        return _cat(tiles, 1)

    span_a = HALO + SEQ // 2
    group_rows = 16 * NS

    def build_w(blk, t, hold):
        for s in range(0, WROWS, 16):
            for ct in range(TPB):
                def load(i, j, hold):
                    return _split(hold(wp[wp_rows(t, i, s, j * TPB + ct), :]))

                def store(p, words):
                    buf, idx = w_a(t, p, ct, (blk * WROWS + s) // 2, 8)
                    buf[idx] = words

                yield from _build_operands(RHS_TERMS, load, store, hold, True)

    n_w = (WROWS // 16) * TPB * 7

    def build_x(blk, hold):
        for c in range(ROWS // group_rows):
            for t in range(TPB):
                def load(i, j, hold):
                    words = ax_raw.at[j * TPB + t].bitcast(U32).at[_ds(blk * (ROWS // 2), ROWS // 2)]
                    w0 = (c * group_rows + 32 * (i // 2)) // 2
                    return [_split(hold(words[pl.ds(w0 + e, 8, stride=2), :]))[i % 2] for e in range(2)]

                def store(p, words):
                    la[p, t, _ds((blk * (ROWS // NS) + 16 * c) // 2, 8), :] = words

                yield from _build_operands(LHS_TERMS, load, store, hold, True)

    n_x = (ROWS // group_rows) * TPB * 7

    def build_awo(blk, hold):
        ct, odd, h0 = blk // 4, (blk // 2) % 2, 16 * (blk % 2)
        pairs = DHA // 2 // NS
        for dp in range(0, pairs, 2):
            src = {}
            for i in range(NS):
                for j in range(NS):
                    words = awo_raw.at[j * TPB + ct].bitcast(U32).at[pl.ds(pl.multiple_of(h0 * 16, 256), 256)]
                    for e in range(2):
                        w0 = 8 * e * 16 + i * pairs + dp
                        src[i, j, e] = hold(jnp.where(odd == 1, words[pl.ds(w0 + 1, 8, stride=16), :],
                                                      words[pl.ds(w0, 8, stride=16), :]))
                yield
            for half in range(2):
                def load(i, j, hold):
                    return [_split(hold(src[i, j, e]))[half] for e in range(2)]

                def store(p, words):
                    buf, idx = w_a(3, p, ct, ((2 * (dp + odd) + half) * HA + h0) // 2, 8)
                    buf[idx] = words

                yield from _build_operands(RHS_TERMS, load, store, hold, True)

    n_awo = (DHA // 2 // NS // 2) * (NS + 2 * 7)

    def output_b(blk):
        slot = blk % 2
        rows = ROWS // NS
        heads = HB // NS
        pl.when(blk >= 2)(lambda: out_copy(blk - 2).wait())
        pacer = _Pacer(ro[0:8, :])
        src = _shifted(ctx, blk, NBLK, ROWS // 2)
        lhs = {}

        def build_lhs(top, hold):
            half = NS // 2
            for h in range(heads):
                for r in range(0, rows, 16):
                    def quadrant(i, j):
                        return [[_split_shuffled(hold(src[pl.ds(
                            (((j * half + b) * heads + h) * SEQ + (i * half + a) * rows + r) // 2, 8), :]))
                            for b in range(half)] for a in range(half)]

                    for p, v in enumerate(_operands(LHS_TERMS, _operand(LHS_TERMS[top], quadrant))):
                        lhs.setdefault((top * (NP // 7) + p, h), []).append(v)
                    yield

        def product(p):
            x = _cat([_cat(lhs[p, h], 0) for h in range(heads)], 1).astype(BF16)
            w = _cat([_matrix(ro[pl.ds((p * TPB + ct) * KO // 2, KO // 2), :]) for ct in range(TPB)], 1)
            return pacer.mark(jnp.dot(x, w, preferred_element_type=F32))

        def emit(i, j, v):
            stage[slot, i * rows:(i + 1) * rows, j * KQ:(j + 1) * KQ] = v.astype(BF16)

        _run(build_lhs(TOP_ORDER[0], _same))
        hold = pacer.after(1)
        _interleave(
            (_multiply(product, emit), NP),
            (_chain(*[build_lhs(t, hold) for t in TOP_ORDER[1:]]), 6 * heads * (rows // 16), 0., .84),
            *[(_chain(build_w(blk, t, hold), shuffle_columns(blk + 1, t, hold)), n_w + n_shuffle, .02, .95)
              for t in range(3)],
            (build_x(blk, hold), n_x, .02, .95),
            (build_awo(blk, hold), n_awo, .02, .95))
        out_copy(blk).start()

    _loop(NBLK, output_b)

    def project_a(t, blk, mark):
        rows = ROWS // NS
        dst = _shifted(ro if t == 1 else ctx, blk, NBLK, ROWS // 2)

        def product(p):
            x = _cat([_matrix(la[p, k, _ds(blk * rows // 2, rows // 2), :]) for k in range(TPB)], 1)
            return mark(jnp.dot(x, load_w(t, p), preferred_element_type=F32))

        def emit(i, j, v):
            for ct in range(TPB):
                for c in range(rows // 16):
                    piece = v[16 * c:16 * (c + 1), ct * LANES:(ct + 1) * LANES]
                    tile = 2 * (j * TPB + ct) + i % 2
                    r = c * (group_rows // 2) + 16 * (i // 2)
                    if t == 0:
                        qa[_ds(tile * ROWS + (blk % 2) * (ROWS // 2) + r, 16), :] = pltpu.bitcast(piece, U32)
                    else:
                        dst[pl.ds(tile * span_a + HALO + r, 16), :] = pltpu.bitcast(piece, U32)

        return _multiply(product, emit)

    def attend_a(blk, hold, softmax_weight, operand_weight, hold_q, hold_sum, hold_v, **_):
        row0, slot = blk * (ROWS // 2), blk % 2
        keys, values = (_shifted(buf, blk, NBLK, ROWS // 2) for buf in (ro, ctx))
        logits, o = {}, {}

        def window(buf, j, r, par, w):
            return pltpu.bitcast(buf[pl.ds((2 * j + par) * span_a + HALO + r - w, 8), :], F32)

        def scores(r, par):
            pos = row0 + r + lax.broadcasted_iota(I32, (8, LANES), 0)
            q = [pltpu.bitcast(qa[_ds((2 * j + par) * ROWS + slot * (ROWS // 2) + r, 8), :], F32) for j in range(8)]
            q = [hold(x) if j % hold_q == 0 else x for j, x in enumerate(q)]
            logits[r, par] = []
            for w in range(WIN):
                acc = q[0] * hold(window(keys, 0, r, par, w))
                for j in range(1, 8):
                    acc = acc + q[j] * window(keys, j, r, par, w)
                acc = hold(acc) if hold_sum else acc
                acc = acc + pltpu.roll(acc, 64, 1)
                acc = acc + pltpu.roll(acc, 32, 1)
                acc = acc * (DHA ** -0.5 * LOG2E)
                if r < w:
                    acc = jnp.where(pos >= w, acc, MASKED * LOG2E)
                logits[r, par].append(acc)
                yield

        def context(r, par):
            x = logits.pop((r, par))
            top = functools.reduce(jnp.maximum, x)
            e = [jnp.exp2(t - top) for t in x]
            scale = _reciprocal(functools.reduce(jnp.add, e))
            e = [t * scale for t in e]
            yield softmax_weight
            for j in range(8):
                acc = None
                for w in range(WIN):
                    v = window(values, j, r, par, w)
                    t = e[w] * (hold(v) if w % hold_v == 0 else v)
                    acc = t if acc is None else acc + t
                o[r, par, j] = acc
                yield

        def operands(c):
            for t in range(TPB):
                def load(i, j, hold):
                    return [hold(o[c * (group_rows // 2) + 8 * i, par, j * TPB + t]) for par in range(2)]

                def store(p, words):
                    lo[blk % SLOTS * NP + p, t, 8 * c:8 * (c + 1), :] = words

                yield from _weigh(_build_operands(LHS_TERMS, load, store, hold), operand_weight)

        for c in range(ROWS // group_rows):
            units = [(r, par) for r in range(c * group_rows // 2, (c + 1) * group_rows // 2, 8) for par in range(2)]
            yield from scores(*units[0])
            for now, after in zip(units, units[1:]):
                yield from _merge((scores(*after), WIN), (context(*now), 8 + softmax_weight))
            yield from context(*units[-1])
            yield from operands(c)

    def output_a(blk, mark):
        slot = blk % 2

        def product(p):
            x = _cat([_matrix(lo[blk % SLOTS * NP + p, k]) for k in range(TPB)], 1)
            return mark(jnp.dot(x, load_w(3, p), preferred_element_type=F32))

        def emit(i, j, v):
            for c in range(ROWS // group_rows):
                r = c * group_rows + 16 * i
                stage[slot, r:r + 16, j * KQ:(j + 1) * KQ] = v[16 * c:16 * (c + 1)].astype(BF16)

        return _multiply(product, emit)

    def outputs_a(blocks, mark):
        for n, blk in enumerate(blocks):
            if n > 0:
                out_copy(NBLK + blk - 1).start()
                out_copy(NBLK + blk - 2).wait()
            yield from output_a(blk, mark)

    def step_a(project, attend, outputs, pace=None):
        pacer = _Pacer(lc[0, 0, 0:8, :])
        matmuls = [] if project is None else [project_a(t, project, pacer.mark) for t in (1, 2, 0)]
        streams = [(_chain(outputs_a(outputs, pacer.mark), *matmuls), (len(outputs) + len(matmuls)) * NP)]
        if attend is not None:
            total = ((WIN + 8 + pace["softmax_weight"]) * (ROWS // 8)
                     + TPB * (ROWS // group_rows) * 7 * pace["operand_weight"])
            streams.append((attend_a(attend, pacer.after(pace["lag"]), **pace), total, *pace["span"]))
        if outputs:
            out_copy(NBLK + outputs[0] - 2).wait()
        _interleave(*streams)
        if outputs:
            out_copy(NBLK + outputs[-1]).start()

    for tile in range(16):
        for buf in (ro, ctx):
            buf[tile * span_a:tile * span_a + HALO, :] = jnp.zeros((HALO, LANES), U32)
    step_a(0, None, [])
    _loop(DELAY, lambda i: step_a(i + 1, i, [], A_FIRST))
    _loop(NBLK - 1 - DELAY, lambda i: step_a(i + DELAY + 1, i + DELAY, [i], A_MAIN))
    step_a(None, NBLK - 1, range(NBLK - 1 - DELAY, NBLK - 1), A_LAST)
    step_a(None, None, [NBLK - 1])
    _wait([out_copy(2 * NBLK - 2), out_copy(2 * NBLK - 1)])


def _words(*shape):
    return pltpu.VMEM(shape + (LANES,), U32)


SCRATCH = [
    pltpu.VMEM((DA // LANES, SEQ, LANES), BF16),
    pltpu.VMEM((DA, 3 * DA), BF16),
    pltpu.VMEM((DA // LANES, DA, LANES), BF16),
    pltpu.VMEM((NS, MQ, DC), BF16),
    pltpu.VMEM((NS, KO, MB), BF16),
    _words(NP, MB // NS // LANES, MQ // 2),
    _words(NP, DC // NS // LANES, MQ // 2),
    *[_words(NP, MB // NS // 2)] * 2,
    *[_words(NP + 1, DC // NS // 2)] * 4,
    *[_words(GROUP * SEQ // 2)] * 4,
    *[_words(GROUP * NPAIR * 7 * DB // 4)] * 2,
    *[_words(GROUP * MB // 2)] * 2,
    *[_words(GROUP * DC // 2)] * 4,
    _words(HB * SEQ // 2),
    _words(NP * TPB * KO // 2),
    _words(SLOTS * NP, TPB, ROWS // NS // 2),
    pltpu.VMEM((2, ROWS, DA), BF16),
    pltpu.SemaphoreType.DMA((GROUP,)),
    pltpu.SemaphoreType.DMA((GROUP,)),
    pltpu.SemaphoreType.DMA(()),
    pltpu.SemaphoreType.DMA((6,)),
    pltpu.SemaphoreType.DMA(()),
    pltpu.SemaphoreType.DMA((2,)),
]


@jax.jit
def pallas_concat_heads__sliding_local_dilated__compressed_kv_cla__prompt_kernel(A_x, A_wqkv, A_wo, B_x, B_c_kv, B_w_q, B_w_uk, B_w_uv, B_w_o):
    hbm = pl.BlockSpec(memory_space=pl.ANY)
    out = pl.pallas_call(
        _kernel,
        in_specs=[hbm] * 9,
        out_specs=hbm,
        out_shape=jax.ShapeDtypeStruct((SEQ, DA + MB), BF16),
        scratch_shapes=SCRATCH,
        compiler_params=pltpu.CompilerParams(vmem_limit_bytes=127 * 2 ** 20),
        name="fused_attention",
    )(A_x.reshape(SEQ, DA), A_wqkv, A_wo, B_x.reshape(GROUP, NS, PART, MB), B_c_kv.reshape(GROUP, NS, PART, DC),
      B_w_q.reshape(MB // 2, 2 * HB, DB), B_w_uk.reshape(DC // 2, 2 * HB, DB),
      B_w_uv.reshape(DC // 2, 2 * HB, DB), B_w_o.reshape(NS, KO, MB))
    return out.reshape(1, SEQ, DA + MB)
```

```python
import functools
import math

import jax
import jax.numpy as jnp
from jax import lax
import jax.experimental.pallas as pl
import jax.experimental.pallas.tpu as pltpu

F32 = jnp.float32
BF16 = jnp.bfloat16
U32 = jnp.uint32
I32 = jnp.int32
LANES = 128
NT_DIMS = (((1,), (1,)), ((), ()))
LOG2E = math.log2(math.e)
MASKED = -1e9

SEQ = 2048
DA = 1024
HA, DHA = 32, 32
WIN = 8
HALO = 32
MB = 1024
HB, DB = 32, 128
DC = 512

LEVELS = 2
NS = 2 ** LEVELS
NP = 7 ** LEVELS
GROUP = NS
NGROUP = HB // GROUP
MQ = SEQ // NS
PART = MQ // GROUP
ROWS = 256
NBLK = SEQ // ROWS
KQ = DA // NS
TPB = KQ // LANES
KO = HB * DB // NS
WROWS = KQ // NBLK
TILE = LANES
NPAIR = SEQ // TILE // 2
DELAY = 2
SLOTS = 4

START_UP = (
    ("c0 k", "c2 c3", "k0", "c0 k", "", 1, (0., 1.)),
    ("v c1", "q x0", "v0", "v", "c1", 40, (.04, .9)),
    ("c2 c3", "x1 x2 x3", "k1 v1 k2 v2 k3", "", "c2 c3 !q +g1 q !x0 x0", 14, (.07, 1.)),
    ("x1 x2", "", "q0 q1", "", "x1 x2", 1, (.02, .96)),
    ("x3 g1", "g2 o", "q2 v3 q3", "", "x3 g", 10, (.07, 1.)),
)
PAIR_ORDER = (1, 3, 5, 7, 6, 4, 2, 0)
HEAD = dict(lag=9, bursts=((1,), (4,), (0,), (2,), (5,), (3,), (6,)), fast=NPAIR,
            score_weight=1, score_span=(0, .7), context_span=(.15, 1))
LAST_HEAD = dict(lag=11, bursts=((1, 4), (0, 2), (5, 3), (6,)), fast=5,
                 score_weight=1.1, score_span=(0, .6), context_span=(.25, 1))
A_FIRST = dict(lag=3, span=(.02, .98), softmax_weight=1, operand_weight=7, hold_q=8, hold_sum=False, hold_v=4)
A_MAIN = dict(lag=6, span=(.08, .99), softmax_weight=3, operand_weight=4, hold_q=8, hold_sum=False, hold_v=8)
A_LAST = dict(lag=2, span=(.02, 1.), softmax_weight=4, operand_weight=8, hold_q=1, hold_sum=True, hold_v=8)


LHS_TERMS = (((1, 0, 0), (1, 1, 1)), ((1, 1, 0), (1, 1, 1)), ((1, 0, 0),), ((1, 1, 1),),
             ((1, 0, 0), (1, 0, 1)), ((1, 1, 0), (-1, 0, 0)), ((1, 0, 1), (-1, 1, 1)))
RHS_TERMS = (((1, 0, 0), (1, 1, 1)), ((1, 0, 0),), ((1, 0, 1), (-1, 1, 1)), ((1, 1, 0), (-1, 0, 0)),
             ((1, 1, 1),), ((1, 0, 0), (1, 0, 1)), ((1, 1, 0), (1, 1, 1)))
TOP_ORDER = (1, 3, 0, 6, 4, 2, 5)


def _add(x, y):
    return [[a + b for a, b in zip(rx, ry)] for rx, ry in zip(x, y)]


def _sub(x, y):
    return [[a - b for a, b in zip(rx, ry)] for rx, ry in zip(x, y)]


def _operand(terms, quadrant):
    total = None
    for sign, i, j in terms:
        q = quadrant(i, j)
        total = q if total is None else (_add if sign > 0 else _sub)(total, q)
    return total


def _operands(side, blocks):
    half = len(blocks) // 2
    if half == 0:
        return [blocks[0][0]]

    def quadrant(i, j):
        return [row[j * half:(j + 1) * half] for row in blocks[i * half:(i + 1) * half]]

    return [x for terms in side for x in _operands(side, _operand(terms, quadrant))]


def _multiply(product, emit, level=LEVELS, base=0):
    if level == 0:
        emit(0, 0, product(base))
        yield
        return
    n = 2 ** (level - 1)

    def m(i):
        out = [[None] * n for _ in range(n)]

        def keep(a, b, v):
            out[a][b] = v

        yield from _multiply(product, keep, level - 1, base + (i - 1) * 7 ** (level - 1))
        return out

    def put(x, oi, oj):
        for a in range(n):
            for b in range(n):
                emit(oi * n + a, oj * n + b, x[a][b])

    m2 = yield from m(2)
    m4 = yield from m(4)
    put(_add(m2, m4), 1, 0)
    m1 = yield from m(1)
    c11 = _add(m1, m4)
    c22 = _sub(m1, m2)
    m7 = yield from m(7)
    c11 = _add(c11, m7)
    m5 = yield from m(5)
    put(_sub(c11, m5), 0, 0)
    m3 = yield from m(3)
    put(_add(m3, m5), 0, 1)
    c22 = _add(c22, m3)
    m6 = yield from m(6)
    put(_add(c22, m6), 1, 1)


def _build_operands(side, load, store, hold, hold_all=False, tops=range(7)):
    half = NS // 2
    for top in tops:
        terms = side[top]
        loaded = {(i, j): [[load(i * half + a, j * half + b, hold if hold_all or (a == b and n == 0) else _same)
                            for b in range(half)] for a in range(half)]
                  for n, (_, i, j) in enumerate(terms)}
        lo, hi = (_operands(side, _operand(terms, lambda i, j: [[x[e] for x in row] for row in loaded[i, j]]))
                  for e in range(2))
        for p in range(NP // 7):
            store(top * (NP // 7) + p, _join(lo[p], hi[p]))
        yield


def _split(words):
    return pltpu.bitcast(words << 16, F32), pltpu.bitcast(words & jnp.uint32(0xFFFF0000), F32)


def _join(lo, hi):
    return pltpu.bitcast(pltpu.pack_elementwise([lo, hi], packed_dtype=BF16), U32)


def _join_shuffled(v):
    r, c = v.shape
    v = v.reshape(r // 16, 2, 8, c)
    return _join(v[:, 0].reshape(r // 2, c), v[:, 1].reshape(r // 2, c))


def _split_shuffled(words):
    lo, hi = _split(words)
    r, c = words.shape
    return jnp.stack([lo.reshape(r // 8, 8, c), hi.reshape(r // 8, 8, c)], axis=1).reshape(2 * r, c)


def _unshuffle(pos):
    return (pos & ~15) + ((pos & 15) >> 1) + 8 * (pos & 1)


def _matrix(words):
    return pltpu.bitcast(words, BF16)


def _cat(xs, axis):
    return xs[0] if len(xs) == 1 else jnp.concatenate(xs, axis=axis)


def _ds(start, size):
    if isinstance(start, int):
        return pl.ds(start, size)
    return pl.ds(pl.multiple_of(start, min(size, 16)), size)


def _shifted(ref, step, steps, n):
    return ref.at[_ds(step * n, ref.shape[0] - (steps - 1) * n)]


def _loop(n, body):
    lax.fori_loop(0, n, lambda i, carry: body(i), None)


def _start(copies):
    for c in copies:
        c.start()


def _wait(copies):
    for c in copies:
        c.wait()


def _run(steps):
    for _ in steps:
        pass


def _chain(*streams):
    for steps in streams:
        yield from steps


def _weigh(steps, weight):
    for _ in steps:
        yield weight


def _merge(*streams):
    spans = [s[2:] if len(s) > 2 else (0.0, 1.0) for s in streams]
    done = [0.0] * len(streams)
    live = list(range(len(streams)))
    while live:
        i = min(live, key=lambda k: spans[k][0] + (spans[k][1] - spans[k][0]) * done[k] / streams[k][1])
        try:
            weight = next(streams[i][0])
        except StopIteration:
            live.remove(i)
            continue
        weight = 1 if weight is None else weight
        done[i] += weight
        yield weight


def _interleave(*streams):
    _run(_merge(*streams))


class _Pacer:
    def __init__(self, words):
        self.odd = words | 1
        self.marks = []

    def mark(self, v):
        self.marks.append(pltpu.bitcast(v[:, 0:LANES], U32))
        return v

    def after(self, lag):
        def hold(x):
            if len(self.marks) < lag:
                return x
            rows = x.shape[0]
            never = jnp.concatenate([self.odd] * (rows // 8), axis=0) == 0
            return pltpu.bitcast(jnp.where(never, self.marks[-lag][0:rows], pltpu.bitcast(x, U32)), x.dtype)

        return hold


def _same(x):
    return x


def _reciprocal(x):
    r = pltpu.reciprocal(x, approx=True)
    return r * (2.0 - x * r)


def _kernel(ax_hbm, wqkv_hbm, awo_hbm, bx_hbm, c_hbm, wq_hbm, wuk_hbm, wuv_hbm, bwo_hbm, out_hbm,
            ax_raw, wqkv_raw, awo_raw, c_raw, bwo_raw,
            lx, lc, rq0, rq1, rk0, rk1, rv0, rv1, qs0, qs1, ks0, ks1, vs0, vs1,
            sq0, sq1, sk0, sk1, sv0, sv1, ctx, ro, lo, stage,
            sem_c, sem_x, sem_wo, sem_w, sem_a, sem_out):

    def out_copy(n):
        return pltpu.make_async_copy(
            stage.at[n % 2], out_hbm.at[_ds(n % NBLK * ROWS, ROWS), _ds((1 - n // NBLK) * DA, DA)], sem_out.at[n % 2])

    a_inputs = ([pltpu.make_async_copy(ax_hbm.bitcast(U32).at[:, pl.ds(j * LANES, LANES)], ax_raw.at[j], sem_a)
                 for j in range(DA // LANES)]
                + [pltpu.make_async_copy(awo_hbm.bitcast(U32).at[:, pl.ds(j * LANES, LANES)], awo_raw.at[j], sem_a)
                   for j in range(DA // LANES)]
                + [pltpu.make_async_copy(wqkv_hbm.bitcast(U32), wqkv_raw, sem_a)])

    wp = ks0

    def wp_rows(t, i, s, c):
        return _ds((((t * NS + i) * (WROWS // 16) + s // 16) * 8 + c) * 8, 8)

    def shuffle_columns(blk, t, hold, quarters=range(NS)):
        lane = lax.broadcasted_iota(I32, (8, LANES), 1)
        slot, chunk, low = lane >> 5, (lane & 31) >> 2, lane & 3
        head_of = _unshuffle(lane & 31)
        for s in range(0, WROWS, 16):
            for i in quarters:
                rows = _ds((i * KQ + (blk % NBLK) * WROWS + s) // 2, 8)
                moved = []
                for j in range(8):
                    c0 = t * DA + j * LANES
                    u = hold(pltpu.bitcast(wqkv_raw[rows, c0:c0 + LANES], I32))
                    moved.append(jnp.take_along_axis(u, low * 32 + 4 * ((chunk - j) & 7) + slot, axis=1))
                    if j % 4 == 3:
                        yield
                v = [moved[-c % 8] for c in range(8)]
                for bit in (1, 2, 4):
                    v = [jnp.where((chunk & bit) != 0, v[(c - bit) % 8], v[c]) for c in range(8)]
                for c in range(8):
                    source = slot * 32 + (((head_of >> 2) + c) & 7) * 4 + (head_of & 3)
                    wp[wp_rows(t, i, s, c), :] = pltpu.bitcast(jnp.take_along_axis(v[c], source, axis=1), U32)
                    if c % 4 == 3:
                        yield

    n_shuffle = (WROWS // 16) * NS * 4

    weights = ((rq0, rk0, rv0), (rq1, rk1, rv1))
    projected = ((qs0, ks0, vs0), (qs1, ks1, vs1))
    staged = ((sq0, sk0, sv0), (sq1, sk1, sv1))

    def weight_copies(par, grp, w):
        words = (wq_hbm, wuk_hbm, wuv_hbm)[w].bitcast(U32)
        n = words.shape[0]
        return [pltpu.make_async_copy(
            words.at[:, (HB // 2) * parity + grp * (GROUP // 2) + pair],
            staged[par][w].at[pl.ds((2 * pair + parity) * n, n)], sem_w.at[3 * par + w])
            for pair in range(GROUP // 2) for parity in range(2)]

    def group_copies(par, grp):
        return [c for w in range(3) for c in weight_copies(par, grp, w)]

    def c_copies(part):
        return [pltpu.make_async_copy(c_hbm.bitcast(U32).at[part], c_raw.at[:, pl.ds(part * PART // 2, PART // 2)],
                                      sem_c.at[part])]

    def x_copies(part):
        return [pltpu.make_async_copy(bx_hbm.at[part], bwo_raw.at[:, pl.ds(part * PART, PART)], sem_x.at[part])]

    def wo_copies(grp):
        rows = (slice(None), _ds(grp * (KO // NGROUP), KO // NGROUP))
        return [pltpu.make_async_copy(bwo_hbm.at[rows], bwo_raw.at[rows], sem_wo)]

    def build_weights(par, w, part, hold, tops=range(7)):
        n = (MB, DC, DC)[w] // 2
        rows = n // NS // GROUP
        src = _shifted(staged[par][w], part, GROUP, rows)
        for s in range(0, rows, 8):
            def load(i, j, hold):
                return [_split(hold(src[pl.ds((2 * (j // 2) + e) * n + i * (n // NS) + s, 8), :]))[j % 2]
                        for e in range(2)]

            def store(p, words):
                weights[par][w][p, _ds(part * rows + s, 8), :] = words

            yield from _build_operands(RHS_TERMS, load, store, hold, tops=tops)

    def n_weights(w):
        return (MB, DC, DC)[w] // NS // GROUP // 16 * 7

    def build_group(par, part, hold):
        return _chain(*[build_weights(par, w, part, hold) for w in range(3)])

    n_group = sum(n_weights(w) for w in range(3))

    def build_activations(src, dst, part, hold, tops=range(7)):
        tiles = src.shape[2] // NS // LANES
        for t in range(tiles):
            for s in range(0, PART, 16):
                r = part * PART + s

                def load(i, j, hold):
                    c0 = (j * tiles + t) * LANES
                    if src.dtype == U32:
                        return _split(hold(src[i, pl.ds(r // 2, 8), c0:c0 + LANES]))
                    return _split(hold(pltpu.bitcast(src[i, pl.ds(r, 16), c0:c0 + LANES], U32)))

                def store(p, words):
                    dst[p, t, pl.ds(r // 2, 8), :] = words

                yield from _build_operands(LHS_TERMS, load, store, hold, tops=tops)

    def n_activations(width):
        return width // NS // LANES * (PART // 16) * 7

    def project(par, w, part, mark):
        lhs = lx if w == 0 else lc
        tiles = lhs.shape[1]
        dst = projected[par][w]
        dst = _shifted(dst, part, GROUP, dst.shape[0] // GROUP // GROUP)
        pending = {}

        def product(p):
            x = _cat([_matrix(lhs[p, t, _ds(part * PART // 2, PART // 2), :]) for t in range(tiles)], 1)
            return mark(jnp.dot(x, _matrix(weights[par][w][p]), preferred_element_type=F32))

        def emit(i, j, v):
            if w < 2:
                dst[pl.ds((j * SEQ + i * PART) // 2, PART // 2), :] = (
                    pltpu.bitcast(v.astype(BF16), U32) if w else _join_shuffled(v * (DB ** -0.5 * LOG2E)))
            else:
                pending[i, j] = v.T
                if i % 2 == 1:
                    pair = [pending.pop((i - 1 + b, j)) for b in range(2)]
                    blocks = [[t[a * DB // 2:(a + 1) * DB // 2] for t in pair] for a in range(2)]
                    for p, x in enumerate(_operands(LHS_TERMS, blocks)):
                        dst[pl.ds(((j * NPAIR + i // 2) * 7 + p) * DB // 4, DB // 4), :] = _join_shuffled(x)

        return _weigh(_multiply(product, emit), tiles)

    n_project = NP * (MB + 2 * DC) // NS // LANES

    def attend(par, h, head_id, pacer, lag, bursts, fast, score_weight, score_span, context_span):
        hold = pacer.after(lag)
        causal = (lax.broadcasted_iota(I32, (TILE, TILE), 0)
                  <= _unshuffle(lax.broadcasted_iota(I32, (TILE, TILE), 1)))
        queries, keys, values = (r.at[_ds(h * (r.shape[0] // GROUP), r.shape[0] // GROUP)] for r in projected[par])
        result = ctx.at[_ds(head_id * (SEQ // 2), SEQ // 2)]
        pending = {}

        def fold(op, t):
            return functools.reduce(op, [t[r:r + 8] for r in range(0, TILE, 8)])

        def scores(i):
            q = _matrix(queries[i * TILE // 2:(i + 1) * TILE // 2, :])
            tiles, peaks = [], []
            for j in range(i + 1):
                k = _matrix(keys[j * TILE // 2:(j + 1) * TILE // 2, :])
                s = pacer.mark(lax.dot_general(k, q, NT_DIMS, preferred_element_type=F32))
                if j == i:
                    s = jnp.where(causal, s, MASKED * LOG2E)
                tiles.append(s)
                peaks.append(fold(jnp.maximum, s))
                yield score_weight
            top = jnp.max(functools.reduce(jnp.maximum, peaks), axis=0, keepdims=True)
            if i // 2 >= max(1, NPAIR - fast):
                mass = functools.reduce(jnp.add, [jnp.exp2(x - top) for x in peaks])
                top = top + jnp.log2(jnp.sum(mass, axis=0, keepdims=True))
            pending[i] = tiles, jnp.broadcast_to(top, (8, TILE))

        def context(i):
            both = [pending.pop(2 * i + c) for c in range(2)]
            totals = [None, None]
            o = [[None, None], [None, None]]

            def weight(j, c):
                p = jnp.exp2(both[c][0][j] - _cat([hold(both[c][1])] * (TILE // 8), 0))
                t = fold(jnp.add, p)
                totals[c] = t if totals[c] is None else totals[c] + t
                return p

            def product(j, p, x):
                v = _matrix(values[(j * 7 + p) * DB // 4:(j * 7 + p + 1) * DB // 4, :])
                return pacer.mark(jnp.dot(v, x.astype(BF16), preferred_element_type=F32))

            def emit(a, c, v):
                o[a][c] = v if o[a][c] is None else o[a][c] + v

            def plain(j, c, tiles):
                for b in range(tiles):
                    p = weight(2 * j + b, c)
                    shared = product(j, 2 + b, p)
                    emit(b, c, shared)
                    emit(1 - b, c, shared + product(j, 5 + b, p))
                    yield 1

            yield from plain(i, 0, 1)
            yield from plain(i, 1, 2)
            acc = [None] * 7
            for j in range(i):
                if i < NPAIR - fast:
                    yield from plain(j, 0, 2)
                    yield from plain(j, 1, 2)
                    continue
                tiles = {}
                for burst in bursts:
                    for p in burst:
                        for _, b, c in RHS_TERMS[p]:
                            if (b, c) not in tiles:
                                tiles[b, c] = weight(2 * j + b, c)
                        t = product(j, p, _operand(RHS_TERMS[p], lambda b, c: [[tiles[b, c]]])[0][0])
                        acc[p] = t if acc[p] is None else acc[p] + t
                    yield 4 / 7 * len(burst)
            if acc[0] is not None:
                _run(_multiply(lambda p: acc[p], emit, 1))
            for c in range(2):
                x = _cat([o[0][c], o[1][c]], 0) * _reciprocal(jnp.sum(totals[c], axis=0, keepdims=True))
                result[(2 * i + c) * TILE // 2:(2 * i + c + 1) * TILE // 2, :] = pltpu.bitcast(x.astype(BF16).T, U32)

        for n in range(NPAIR + 1):
            streams = []
            if n < NPAIR:
                i = PAIR_ORDER[n]
                streams.append((_chain(scores(2 * i), scores(2 * i + 1)), (4 * i + 3) * score_weight, *score_span))
            if n > 0:
                i = PAIR_ORDER[n - 1]
                streams.append((context(i), 4 * i + 3, *context_span))
            yield from _merge(*streams)

    def n_attend(pace):
        return NPAIR * (2 * NPAIR + 1) * (1 + pace["score_weight"])

    def build_wo(head_id, hold):
        n = KO // HB
        src, dst = bwo_raw.at[:, _ds(head_id * n, n)], _shifted(ro, head_id, HB, n // 2)
        for ct in range(TPB):
            for s in range(0, n, 16):
                def load(i, j, hold):
                    c0 = (j * TPB + ct) * LANES
                    v = src[i, pl.ds(s, 16), c0:c0 + LANES].astype(F32)
                    return [hold(v[0:8]), hold(v[8:16])]

                def store(p, words):
                    dst[pl.ds(((p * TPB + ct) * KO + s) // 2, 8), :] = words

                yield from _build_operands(RHS_TERMS, load, store, hold)

    n_wo = TPB * (KO // HB // 16) * 7

    def head_step(par, g, h):
        pacer = _Pacer(lc[0, 0, 0:8, :])
        head_id = g * GROUP + h
        _interleave((attend(par, h, head_id, pacer, **HEAD), n_attend(HEAD), 0., .86),
                    (_chain(*[project(1 - par, w, h, pacer.mark) for w in (1, 2, 0)]), n_project),
                    (build_wo(head_id, pacer.after(2)), n_wo, .02, .15),
                    (build_group(par, h, pacer.after(1)), n_group, .25, .98))

    def last_head_step(h):
        pacer = _Pacer(lc[0, 0, 0:8, :])
        hold = pacer.after(1)
        head_id = (NGROUP - 1) * GROUP + h
        _interleave((attend(1, h, head_id, pacer, **LAST_HEAD), n_attend(LAST_HEAD)),
                    (build_wo(head_id, hold), n_wo, .03, .3),
                    (_chain(*[shuffle_columns(0, t, hold, [h]) for t in range(3)]), 3 * n_shuffle / NS, .1, .8))

    def start_up():
        data = {"k": weight_copies(0, 0, 1), "v": weight_copies(0, 0, 2), "q": weight_copies(0, 0, 0),
                "g1": group_copies(1, 1), "g2": group_copies(0, 2), "o": wo_copies(0)}
        for part in range(GROUP):
            data["c%d" % part], data["x%d" % part] = c_copies(part), x_copies(part)
        built = set()

        def copies(names):
            return [c for name in names.split() for c in data[name]]

        def operands(job, hold, tops=range(7)):
            if job[0] in "!+":
                (_wait if job[0] == "!" else _start)(copies(job[1:]))
            elif job[0] in "cx":
                src, dst = (c_raw, lc) if job[0] == "c" else (bwo_raw, lx)
                yield from build_activations(src, dst, int(job[1]), hold, tops)
            else:
                for part in range(GROUP):
                    yield from (build_group(1, part, hold) if job == "g" else
                                build_weights(0, "qkv".index(job), part, hold, tops))
            built.add(job)

        size = dict(c=n_activations(DC), x=n_activations(MB), g=GROUP * n_group,
                    **{name: GROUP * n_weights(w) for w, name in enumerate("qkv")})

        def projection(name, mark):
            assert {name[0], "xcc"["qkv".index(name[0])] + name[1]} <= built
            yield from project(0, "qkv".index(name[0]), int(name[1]), mark)

        def step(waits, starts, products, ahead, jobs, lag, span):
            _wait(copies(waits))
            _start(copies(starts))
            pacer = _Pacer(c_raw[0, 0:8, 0:LANES])
            for top in TOP_ORDER:
                for job in ahead.split():
                    _run(operands(job, _same, [top]))
            _interleave((_chain(*[projection(name, pacer.mark) for name in products.split()]),
                         sum(n_project // (2 if name[0] == "q" else 4) for name in products.split())),
                        (_chain(*[operands(job, pacer.after(lag)) for job in jobs.split()]),
                         sum(size.get(job[0], 0) for job in jobs.split()) or 1, *span))

        def steps(i):
            for n, args in enumerate(START_UP):
                pl.when(i == n)(functools.partial(step, *args))

        _start(copies("c0 k v c1"))
        _loop(len(START_UP), steps)

    def group(par, g):
        _wait(wo_copies(g))
        _start(wo_copies(g + 1))
        pl.when(g + 2 < NGROUP)(lambda: _wait(group_copies(par, g + 2)))
        pl.when(g + 3 < NGROUP)(lambda: _start(group_copies(1 - par, g + 3)))
        if par == 0:
            pl.when(g == NGROUP - 2)(lambda: _start(a_inputs))
        _loop(GROUP, lambda h: head_step(par, g, h))

    def two_groups(t):
        group(0, 2 * t)
        pl.when(t < NGROUP // 2 - 1)(lambda: group(1, 2 * t + 1))

    start_up()
    _loop(NGROUP // 2, two_groups)
    _wait(wo_copies(NGROUP - 1) + a_inputs)
    _loop(GROUP, last_head_step)

    la, qa = lx, qs0

    def w_a(t, p, ct, r0, rows):
        if t == 0:
            return (rq0, rq1)[ct], (p, _ds(r0, rows))
        if t == 1:
            return lc, (p, 0, _ds(ct * (KQ // 2) + r0, rows))
        if t == 2:
            buf, tile = divmod(TPB * p + ct, 25)
            assert rows <= 64 or rows == 128
            if rows == 128:
                return (rk0, rk1, rv0, rv1)[buf], (pl.ds(2 * tile, 2),)
            return (rk0, rk1, rv0, rv1)[buf], (2 * tile + r0 // 64, _ds(r0 % 64, rows))
        buf, tile = divmod(TPB * p, 50)
        return (vs0, vs1)[buf], (_ds((tile + ct) * (KQ // 2) + r0, rows),)

    def load_w(t, p):
        tiles = []
        for ct in range(TPB):
            buf, idx = w_a(t, p, ct, 0, KQ // 2)
            tiles.append(_matrix(buf[idx].reshape(KQ // 2, LANES)))
        return _cat(tiles, 1)

    span_a = HALO + SEQ // 2
    group_rows = 16 * NS

    def build_w(blk, t, hold):
        for s in range(0, WROWS, 16):
            for ct in range(TPB):
                def load(i, j, hold):
                    return _split(hold(wp[wp_rows(t, i, s, j * TPB + ct), :]))

                def store(p, words):
                    buf, idx = w_a(t, p, ct, (blk * WROWS + s) // 2, 8)
                    buf[idx] = words

                yield from _build_operands(RHS_TERMS, load, store, hold, True)

    n_w = (WROWS // 16) * TPB * 7

    def build_x(blk, hold):
        for c in range(ROWS // group_rows):
            for t in range(TPB):
                def load(i, j, hold):
                    words = ax_raw.at[j * TPB + t, _ds(blk * (ROWS // 2), ROWS // 2)]
                    w0 = (c * group_rows + 32 * (i // 2)) // 2
                    return [_split(hold(words[pl.ds(w0 + e, 8, stride=2), :]))[i % 2] for e in range(2)]

                def store(p, words):
                    la[p, t, _ds((blk * (ROWS // NS) + 16 * c) // 2, 8), :] = words

                yield from _build_operands(LHS_TERMS, load, store, hold, True)

    n_x = (ROWS // group_rows) * TPB * 7

    def build_awo(blk, hold):
        ct, odd, h0 = blk // 4, (blk // 2) % 2, 16 * (blk % 2)
        pairs = DHA // 2 // NS
        for dp in range(0, pairs, 2):
            src = {}
            for i in range(NS):
                for j in range(NS):
                    words = awo_raw.at[j * TPB + ct, pl.ds(pl.multiple_of(h0 * 16, 256), 256)]
                    for e in range(2):
                        w0 = 8 * e * 16 + i * pairs + dp
                        src[i, j, e] = hold(jnp.where(odd == 1, words[pl.ds(w0 + 1, 8, stride=16), :],
                                                      words[pl.ds(w0, 8, stride=16), :]))
                yield
            for half in range(2):
                def load(i, j, hold):
                    return [_split(hold(src[i, j, e]))[half] for e in range(2)]

                def store(p, words):
                    buf, idx = w_a(3, p, ct, ((2 * (dp + odd) + half) * HA + h0) // 2, 8)
                    buf[idx] = words

                yield from _build_operands(RHS_TERMS, load, store, hold, True)

    n_awo = (DHA // 2 // NS // 2) * (NS + 2 * 7)

    def output_b(blk):
        slot = blk % 2
        rows = ROWS // NS
        heads = HB // NS
        pl.when(blk >= 2)(lambda: out_copy(blk - 2).wait())
        pacer = _Pacer(ro[0:8, :])
        src = _shifted(ctx, blk, NBLK, ROWS // 2)
        lhs = {}

        def build_lhs(top, hold):
            half = NS // 2
            for h in range(heads):
                for r in range(0, rows, 16):
                    def quadrant(i, j):
                        return [[_split_shuffled(hold(src[pl.ds(
                            (((j * half + b) * heads + h) * SEQ + (i * half + a) * rows + r) // 2, 8), :]))
                            for b in range(half)] for a in range(half)]

                    for p, v in enumerate(_operands(LHS_TERMS, _operand(LHS_TERMS[top], quadrant))):
                        lhs.setdefault((top * (NP // 7) + p, h), []).append(v)
                    yield

        def product(p):
            x = _cat([_cat(lhs[p, h], 0) for h in range(heads)], 1).astype(BF16)
            w = _cat([_matrix(ro[pl.ds((p * TPB + ct) * KO // 2, KO // 2), :]) for ct in range(TPB)], 1)
            return pacer.mark(jnp.dot(x, w, preferred_element_type=F32))

        def emit(i, j, v):
            stage[slot, i * rows:(i + 1) * rows, j * KQ:(j + 1) * KQ] = v.astype(BF16)

        _run(build_lhs(TOP_ORDER[0], _same))
        hold = pacer.after(1)
        _interleave(
            (_multiply(product, emit), NP),
            (_chain(*[build_lhs(t, hold) for t in TOP_ORDER[1:]]), 6 * heads * (rows // 16), 0., .84),
            *[(_chain(build_w(blk, t, hold), shuffle_columns(blk + 1, t, hold)), n_w + n_shuffle, .02, .95)
              for t in range(3)],
            (build_x(blk, hold), n_x, .02, .95),
            (build_awo(blk, hold), n_awo, .02, .95))
        out_copy(blk).start()

    _loop(NBLK, output_b)

    def project_a(t, blk, mark):
        rows = ROWS // NS
        dst = _shifted(ro if t == 1 else ctx, blk, NBLK, ROWS // 2)

        def product(p):
            x = _cat([_matrix(la[p, k, _ds(blk * rows // 2, rows // 2), :]) for k in range(TPB)], 1)
            return mark(jnp.dot(x, load_w(t, p), preferred_element_type=F32))

        def emit(i, j, v):
            for ct in range(TPB):
                for c in range(rows // 16):
                    piece = v[16 * c:16 * (c + 1), ct * LANES:(ct + 1) * LANES]
                    tile = 2 * (j * TPB + ct) + i % 2
                    r = c * (group_rows // 2) + 16 * (i // 2)
                    if t == 0:
                        qa[_ds(tile * ROWS + (blk % 2) * (ROWS // 2) + r, 16), :] = pltpu.bitcast(piece, U32)
                    else:
                        dst[pl.ds(tile * span_a + HALO + r, 16), :] = pltpu.bitcast(piece, U32)

        return _multiply(product, emit)

    def attend_a(blk, hold, softmax_weight, operand_weight, hold_q, hold_sum, hold_v, **_):
        row0, slot = blk * (ROWS // 2), blk % 2
        keys, values = (_shifted(buf, blk, NBLK, ROWS // 2) for buf in (ro, ctx))
        logits, o = {}, {}

        def window(buf, j, r, par, w):
            return pltpu.bitcast(buf[pl.ds((2 * j + par) * span_a + HALO + r - w, 8), :], F32)

        def scores(r, par):
            pos = row0 + r + lax.broadcasted_iota(I32, (8, LANES), 0)
            q = [pltpu.bitcast(qa[_ds((2 * j + par) * ROWS + slot * (ROWS // 2) + r, 8), :], F32) for j in range(8)]
            q = [hold(x) if j % hold_q == 0 else x for j, x in enumerate(q)]
            logits[r, par] = []
            for w in range(WIN):
                acc = q[0] * hold(window(keys, 0, r, par, w))
                for j in range(1, 8):
                    acc = acc + q[j] * window(keys, j, r, par, w)
                acc = hold(acc) if hold_sum else acc
                acc = acc + pltpu.roll(acc, 64, 1)
                acc = acc + pltpu.roll(acc, 32, 1)
                acc = acc * (DHA ** -0.5 * LOG2E)
                if r < w:
                    acc = jnp.where(pos >= w, acc, MASKED * LOG2E)
                logits[r, par].append(acc)
                yield

        def context(r, par):
            x = logits.pop((r, par))
            top = functools.reduce(jnp.maximum, x)
            e = [jnp.exp2(t - top) for t in x]
            scale = _reciprocal(functools.reduce(jnp.add, e))
            e = [t * scale for t in e]
            yield softmax_weight
            for j in range(8):
                acc = None
                for w in range(WIN):
                    v = window(values, j, r, par, w)
                    t = e[w] * (hold(v) if w % hold_v == 0 else v)
                    acc = t if acc is None else acc + t
                o[r, par, j] = acc
                yield

        def operands(c):
            for t in range(TPB):
                def load(i, j, hold):
                    return [hold(o[c * (group_rows // 2) + 8 * i, par, j * TPB + t]) for par in range(2)]

                def store(p, words):
                    lo[blk % SLOTS * NP + p, t, 8 * c:8 * (c + 1), :] = words

                yield from _weigh(_build_operands(LHS_TERMS, load, store, hold), operand_weight)

        for c in range(ROWS // group_rows):
            units = [(r, par) for r in range(c * group_rows // 2, (c + 1) * group_rows // 2, 8) for par in range(2)]
            yield from scores(*units[0])
            for now, after in zip(units, units[1:]):
                yield from _merge((scores(*after), WIN), (context(*now), 8 + softmax_weight))
            yield from context(*units[-1])
            yield from operands(c)

    def output_a(blk, mark):
        slot = blk % 2

        def product(p):
            x = _cat([_matrix(lo[blk % SLOTS * NP + p, k]) for k in range(TPB)], 1)
            return mark(jnp.dot(x, load_w(3, p), preferred_element_type=F32))

        def emit(i, j, v):
            for c in range(ROWS // group_rows):
                r = c * group_rows + 16 * i
                stage[slot, r:r + 16, j * KQ:(j + 1) * KQ] = v[16 * c:16 * (c + 1)].astype(BF16)

        return _multiply(product, emit)

    def outputs_a(blocks, mark):
        for n, blk in enumerate(blocks):
            if n > 0:
                out_copy(NBLK + blk - 1).start()
                out_copy(NBLK + blk - 2).wait()
            yield from output_a(blk, mark)

    def step_a(project, attend, outputs, pace=None):
        pacer = _Pacer(lc[0, 0, 0:8, :])
        matmuls = [] if project is None else [project_a(t, project, pacer.mark) for t in (1, 2, 0)]
        streams = [(_chain(outputs_a(outputs, pacer.mark), *matmuls), (len(outputs) + len(matmuls)) * NP)]
        if pace:
            total = ((WIN + 8 + pace["softmax_weight"]) * (ROWS // 8)
                     + TPB * (ROWS // group_rows) * 7 * pace["operand_weight"])
            streams.append((attend_a(attend, pacer.after(pace["lag"]), **pace), total, *pace["span"]))
        if outputs:
            out_copy(NBLK + outputs[0] - 2).wait()
        _interleave(*streams)
        if outputs:
            out_copy(NBLK + outputs[-1]).start()

    for tile in range(16):
        for buf in (ro, ctx):
            buf[tile * span_a:tile * span_a + HALO, :] = jnp.zeros((HALO, LANES), U32)
    step_a(0, None, [])
    _loop(DELAY, lambda i: step_a(i + 1, i, [], A_FIRST))
    _loop(NBLK - 1 - DELAY, lambda i: step_a(i + DELAY + 1, i + DELAY, [i], A_MAIN))
    step_a(None, NBLK - 1, range(NBLK - 1 - DELAY, NBLK - 1), A_LAST)

    halves = [pltpu.make_async_copy(stage.at[1, :, pl.ds(c, DA // 2)],
                                    out_hbm.at[pl.ds(SEQ - ROWS, ROWS), pl.ds(c, DA // 2)], sem_out.at[1])
              for c in (0, DA // 2)]
    out_copy(2 * NBLK - 3).wait()
    for n, _ in enumerate(output_a(NBLK - 1, _same)):
        if n == 5 * NP // 7:
            halves[0].start()
    halves[1].start()
    _wait([out_copy(2 * NBLK - 2)] + halves)


def _words(*shape):
    return pltpu.VMEM(shape + (LANES,), U32)


SCRATCH = [
    _words(DA // LANES, SEQ // 2),
    pltpu.VMEM((DA // 2, 3 * DA), U32),
    _words(DA // LANES, DA // 2),
    pltpu.VMEM((NS, MQ // 2, DC), U32),
    pltpu.VMEM((NS, KO, MB), BF16),
    _words(NP, MB // NS // LANES, MQ // 2),
    _words(NP, DC // NS // LANES, MQ // 2),
    *[_words(NP, MB // NS // 2)] * 2,
    *[_words(NP + 1, DC // NS // 2)] * 4,
    *[_words(GROUP * SEQ // 2)] * 4,
    *[_words(GROUP * NPAIR * 7 * DB // 4)] * 2,
    *[_words(GROUP * MB // 2)] * 2,
    *[_words(GROUP * DC // 2)] * 4,
    _words(HB * SEQ // 2),
    _words(NP * TPB * KO // 2),
    _words(SLOTS * NP, TPB, ROWS // NS // 2),
    pltpu.VMEM((2, ROWS, DA), BF16),
    pltpu.SemaphoreType.DMA((GROUP,)),
    pltpu.SemaphoreType.DMA((GROUP,)),
    pltpu.SemaphoreType.DMA(()),
    pltpu.SemaphoreType.DMA((6,)),
    pltpu.SemaphoreType.DMA(()),
    pltpu.SemaphoreType.DMA((2,)),
]


@jax.jit
def pallas_concat_heads__sliding_local_dilated__compressed_kv_cla__prompt_kernel(A_x, A_wqkv, A_wo, B_x, B_c_kv, B_w_q, B_w_uk, B_w_uv, B_w_o):
    hbm = pl.BlockSpec(memory_space=pl.ANY)
    out = pl.pallas_call(
        _kernel,
        in_specs=[hbm] * 9,
        out_specs=hbm,
        out_shape=jax.ShapeDtypeStruct((SEQ, DA + MB), BF16),
        scratch_shapes=SCRATCH,
        compiler_params=pltpu.CompilerParams(vmem_limit_bytes=127 * 2 ** 20),
        name="fused_attention",
    )(A_x.reshape(SEQ, DA), A_wqkv, A_wo, B_x.reshape(GROUP, NS, PART, MB), B_c_kv.reshape(GROUP, NS, PART, DC),
      B_w_q.reshape(MB // 2, 2 * HB, DB), B_w_uk.reshape(DC // 2, 2 * HB, DB),
      B_w_uv.reshape(DC // 2, 2 * HB, DB), B_w_o.reshape(NS, KO, MB))
    return out.reshape(1, SEQ, DA + MB)
```

```python
import functools
import math

import jax
import jax.numpy as jnp
from jax import lax
import jax.experimental.pallas as pl
import jax.experimental.pallas.tpu as pltpu

F32 = jnp.float32
BF16 = jnp.bfloat16
U32 = jnp.uint32
I32 = jnp.int32
LANES = 128
NT_DIMS = (((1,), (1,)), ((), ()))
LOG2E = math.log2(math.e)
MASKED = -1e9

SEQ = 2048
DA = 1024
HA, DHA = 32, 32
WIN = 8
HALO = 32
MB = 1024
HB, DB = 32, 128
DC = 512

LEVELS = 2
NS = 2 ** LEVELS
NP = 7 ** LEVELS
GROUP = NS
NGROUP = HB // GROUP
MQ = SEQ // NS
PART = MQ // GROUP
ROWS = 256
NBLK = SEQ // ROWS
KQ = DA // NS
TPB = KQ // LANES
KO = HB * DB // NS
WROWS = KQ // NBLK
TILE = LANES
NPAIR = SEQ // TILE // 2
DELAY = 2
SLOTS = 4

START_UP = (
    ("c0 k", "c2 c3", "k0", "c0 k", "", 1, (0., 1.)),
    ("v c1", "q x0", "v0", "v", "c1", 20, (.02, 1.01)),
    ("c2 c3", "x1 x2 x3", "k1 v1 k2 v2 k3", "", "c2 c3 !q +g1 q !x0 x0", 14, (0., .98)),
    ("x1 x2", "", "q0 q1", "", "x1 x2", 6, (.055, .93)),
    ("x3 g1", "g2 o", "q2 v3 q3", "", "x3 g", 2, (0., .98)),
)
PAIR_ORDER = (1, 3, 5, 7, 6, 4, 2, 0)
HEAD = dict(lag=9, bursts=((1,), (4,), (0,), (2,), (5,), (3,), (6,)), fast=NPAIR,
            score_weight=1, score_span=(0, .7), context_span=(.15, 1))
LAST_HEAD = dict(lag=11, bursts=((1, 4), (0, 2), (5, 3), (6,)), fast=5,
                 score_weight=1.1, score_span=(0, .6), context_span=(.25, 1))
A_FIRST = dict(lag=3, span=(.02, .98), softmax_weight=1, operand_weight=7, hold_q=8, hold_sum=False, hold_v=4)
A_MAIN = dict(lag=6, span=(.08, .99), softmax_weight=3, operand_weight=4, hold_q=8, hold_sum=False, hold_v=8)
A_LAST = dict(lag=2, span=(.02, 1.), softmax_weight=4, operand_weight=8, hold_q=1, hold_sum=True, hold_v=8)


LHS_TERMS = (((1, 0, 0), (1, 1, 1)), ((1, 1, 0), (1, 1, 1)), ((1, 0, 0),), ((1, 1, 1),),
             ((1, 0, 0), (1, 0, 1)), ((1, 1, 0), (-1, 0, 0)), ((1, 0, 1), (-1, 1, 1)))
RHS_TERMS = (((1, 0, 0), (1, 1, 1)), ((1, 0, 0),), ((1, 0, 1), (-1, 1, 1)), ((1, 1, 0), (-1, 0, 0)),
             ((1, 1, 1),), ((1, 0, 0), (1, 0, 1)), ((1, 1, 0), (1, 1, 1)))
TOP_ORDER = (1, 3, 0, 6, 4, 2, 5)


def _add(x, y):
    return [[a + b for a, b in zip(rx, ry)] for rx, ry in zip(x, y)]


def _sub(x, y):
    return [[a - b for a, b in zip(rx, ry)] for rx, ry in zip(x, y)]


def _operand(terms, quadrant):
    total = None
    for sign, i, j in terms:
        q = quadrant(i, j)
        total = q if total is None else (_add if sign > 0 else _sub)(total, q)
    return total


def _operands(side, blocks):
    half = len(blocks) // 2
    if half == 0:
        return [blocks[0][0]]

    def quadrant(i, j):
        return [row[j * half:(j + 1) * half] for row in blocks[i * half:(i + 1) * half]]

    return [x for terms in side for x in _operands(side, _operand(terms, quadrant))]


def _multiply(product, emit, level=LEVELS, base=0):
    if level == 0:
        emit(0, 0, product(base))
        yield
        return
    n = 2 ** (level - 1)

    def m(i):
        out = [[None] * n for _ in range(n)]

        def keep(a, b, v):
            out[a][b] = v

        yield from _multiply(product, keep, level - 1, base + (i - 1) * 7 ** (level - 1))
        return out

    def put(x, oi, oj):
        for a in range(n):
            for b in range(n):
                emit(oi * n + a, oj * n + b, x[a][b])

    m2 = yield from m(2)
    m4 = yield from m(4)
    put(_add(m2, m4), 1, 0)
    m1 = yield from m(1)
    c11 = _add(m1, m4)
    c22 = _sub(m1, m2)
    m7 = yield from m(7)
    c11 = _add(c11, m7)
    m5 = yield from m(5)
    put(_sub(c11, m5), 0, 0)
    m3 = yield from m(3)
    put(_add(m3, m5), 0, 1)
    c22 = _add(c22, m3)
    m6 = yield from m(6)
    put(_add(c22, m6), 1, 1)


def _build_operands(side, load, store, hold, hold_all=False, tops=range(7)):
    half = NS // 2
    for top in tops:
        terms = side[top]
        loaded = {(i, j): [[load(i * half + a, j * half + b, hold if hold_all or (a == b and n == 0) else _same)
                            for b in range(half)] for a in range(half)]
                  for n, (_, i, j) in enumerate(terms)}
        lo, hi = (_operands(side, _operand(terms, lambda i, j: [[x[e] for x in row] for row in loaded[i, j]]))
                  for e in range(2))
        for p in range(NP // 7):
            store(top * (NP // 7) + p, _join(lo[p], hi[p]))
        yield


def _split(words):
    return pltpu.bitcast(words << 16, F32), pltpu.bitcast(words & jnp.uint32(0xFFFF0000), F32)


def _join(lo, hi):
    return pltpu.bitcast(pltpu.pack_elementwise([lo, hi], packed_dtype=BF16), U32)


def _join_shuffled(v):
    r, c = v.shape
    v = v.reshape(r // 16, 2, 8, c)
    return _join(v[:, 0].reshape(r // 2, c), v[:, 1].reshape(r // 2, c))


def _split_shuffled(words):
    lo, hi = _split(words)
    r, c = words.shape
    return jnp.stack([lo.reshape(r // 8, 8, c), hi.reshape(r // 8, 8, c)], axis=1).reshape(2 * r, c)


def _unshuffle(pos):
    return (pos & ~15) + ((pos & 15) >> 1) + 8 * (pos & 1)


def _matrix(words):
    return pltpu.bitcast(words, BF16)


def _cat(xs, axis):
    return xs[0] if len(xs) == 1 else jnp.concatenate(xs, axis=axis)


def _ds(start, size):
    if isinstance(start, int):
        return pl.ds(start, size)
    return pl.ds(pl.multiple_of(start, min(size, 16)), size)


def _shifted(ref, step, steps, n):
    return ref.at[_ds(step * n, ref.shape[0] - (steps - 1) * n)]


def _loop(n, body):
    lax.fori_loop(0, n, lambda i, carry: body(i), None)


def _start(copies):
    for c in copies:
        c.start()


def _wait(copies):
    for c in copies:
        c.wait()


def _run(steps):
    for _ in steps:
        pass


def _chain(*streams):
    for steps in streams:
        yield from steps


def _weigh(steps, weight):
    for _ in steps:
        yield weight


def _merge(*streams):
    spans = [s[2:] if len(s) > 2 else (0.0, 1.0) for s in streams]
    done = [0.0] * len(streams)
    live = list(range(len(streams)))
    while live:
        i = min(live, key=lambda k: spans[k][0] + (spans[k][1] - spans[k][0]) * done[k] / streams[k][1])
        try:
            weight = next(streams[i][0])
        except StopIteration:
            live.remove(i)
            continue
        weight = 1 if weight is None else weight
        done[i] += weight
        yield weight


def _interleave(*streams):
    _run(_merge(*streams))


class _Pacer:
    def __init__(self, words):
        self.odd = words | 1
        self.marks = []

    def mark(self, v):
        self.marks.append(pltpu.bitcast(v[:, 0:LANES], U32))
        return v

    def after(self, lag):
        def hold(x):
            if len(self.marks) < lag:
                return x
            rows = x.shape[0]
            never = jnp.concatenate([self.odd] * (rows // 8), axis=0) == 0
            return pltpu.bitcast(jnp.where(never, self.marks[-lag][0:rows], pltpu.bitcast(x, U32)), x.dtype)

        return hold


def _same(x):
    return x


def _reciprocal(x):
    r = pltpu.reciprocal(x, approx=True)
    return r * (2.0 - x * r)


def _kernel(ax_hbm, wqkv_hbm, awo_hbm, bx_hbm, c_hbm, wq_hbm, wuk_hbm, wuv_hbm, bwo_hbm, out_hbm,
            ax_raw, wqkv_raw, awo_raw, c_raw, bwo_raw,
            lx, lc, rq0, rq1, rk0, rk1, rv0, rv1, qs0, qs1, ks0, ks1, vs0, vs1,
            sq0, sq1, sk0, sk1, sv0, sv1, ctx, ro, lo, stage,
            sem_c, sem_x, sem_wo, sem_w, sem_a, sem_out):

    def out_copy(n):
        return pltpu.make_async_copy(
            stage.at[n % 2], out_hbm.at[_ds(n % NBLK * ROWS, ROWS), _ds((1 - n // NBLK) * DA, DA)], sem_out.at[n % 2])

    a_inputs = ([pltpu.make_async_copy(ax_hbm.bitcast(U32).at[:, pl.ds(j * LANES, LANES)], ax_raw.at[j], sem_a)
                 for j in range(DA // LANES)]
                + [pltpu.make_async_copy(awo_hbm.bitcast(U32).at[:, pl.ds(j * LANES, LANES)], awo_raw.at[j], sem_a)
                   for j in range(DA // LANES)]
                + [pltpu.make_async_copy(wqkv_hbm.bitcast(U32), wqkv_raw, sem_a)])

    wp = ks0

    def wp_rows(t, i, s, c):
        return _ds((((t * NS + i) * (WROWS // 16) + s // 16) * 8 + c) * 8, 8)

    def shuffle_columns(blk, t, hold, quarters=range(NS)):
        lane = lax.broadcasted_iota(I32, (8, LANES), 1)
        slot, chunk, low = lane >> 5, (lane & 31) >> 2, lane & 3
        head_of = _unshuffle(lane & 31)
        for s in range(0, WROWS, 16):
            for i in quarters:
                rows = _ds((i * KQ + (blk % NBLK) * WROWS + s) // 2, 8)
                moved = []
                for j in range(8):
                    c0 = t * DA + j * LANES
                    u = hold(pltpu.bitcast(wqkv_raw[rows, c0:c0 + LANES], I32))
                    moved.append(jnp.take_along_axis(u, low * 32 + 4 * ((chunk - j) & 7) + slot, axis=1))
                    if j % 4 == 3:
                        yield
                v = [moved[-c % 8] for c in range(8)]
                for bit in (1, 2, 4):
                    v = [jnp.where((chunk & bit) != 0, v[(c - bit) % 8], v[c]) for c in range(8)]
                for c in range(8):
                    source = slot * 32 + (((head_of >> 2) + c) & 7) * 4 + (head_of & 3)
                    wp[wp_rows(t, i, s, c), :] = pltpu.bitcast(jnp.take_along_axis(v[c], source, axis=1), U32)
                    if c % 4 == 3:
                        yield

    n_shuffle = (WROWS // 16) * NS * 4

    weights = ((rq0, rk0, rv0), (rq1, rk1, rv1))
    projected = ((qs0, ks0, vs0), (qs1, ks1, vs1))
    staged = ((sq0, sk0, sv0), (sq1, sk1, sv1))

    def weight_copies(par, grp, w):
        words = (wq_hbm, wuk_hbm, wuv_hbm)[w].bitcast(U32)
        n = words.shape[0]
        return [pltpu.make_async_copy(
            words.at[:, (HB // 2) * parity + grp * (GROUP // 2) + pair],
            staged[par][w].at[pl.ds((2 * pair + parity) * n, n)], sem_w.at[3 * par + w])
            for pair in range(GROUP // 2) for parity in range(2)]

    def group_copies(par, grp):
        return [c for w in range(3) for c in weight_copies(par, grp, w)]

    def c_copies(part):
        return [pltpu.make_async_copy(c_hbm.bitcast(U32).at[part], c_raw.at[:, pl.ds(part * PART // 2, PART // 2)],
                                      sem_c.at[part])]

    def x_copies(part):
        return [pltpu.make_async_copy(bx_hbm.at[part], bwo_raw.at[:, pl.ds(part * PART, PART)], sem_x.at[part])]

    def wo_copies(grp):
        rows = (slice(None), _ds(grp * (KO // NGROUP), KO // NGROUP))
        return [pltpu.make_async_copy(bwo_hbm.at[rows], bwo_raw.at[rows], sem_wo)]

    def build_weights(par, w, part, hold, tops=range(7)):
        n = (MB, DC, DC)[w] // 2
        rows = n // NS // GROUP
        src = _shifted(staged[par][w], part, GROUP, rows)
        for s in range(0, rows, 8):
            def load(i, j, hold):
                return [_split(hold(src[pl.ds((2 * (j // 2) + e) * n + i * (n // NS) + s, 8), :]))[j % 2]
                        for e in range(2)]

            def store(p, words):
                weights[par][w][p, _ds(part * rows + s, 8), :] = words

            yield from _build_operands(RHS_TERMS, load, store, hold, tops=tops)

    def n_weights(w):
        return (MB, DC, DC)[w] // NS // GROUP // 16 * 7

    def build_group(par, part, hold):
        return _chain(*[build_weights(par, w, part, hold) for w in range(3)])

    n_group = sum(n_weights(w) for w in range(3))

    def build_activations(src, dst, part, hold, tops=range(7)):
        tiles = src.shape[2] // NS // LANES
        for t in range(tiles):
            for s in range(0, PART, 16):
                r = part * PART + s

                def load(i, j, hold):
                    c0 = (j * tiles + t) * LANES
                    if src.dtype == U32:
                        return _split(hold(src[i, pl.ds(r // 2, 8), c0:c0 + LANES]))
                    return _split(hold(pltpu.bitcast(src[i, pl.ds(r, 16), c0:c0 + LANES], U32)))

                def store(p, words):
                    dst[p, t, pl.ds(r // 2, 8), :] = words

                yield from _build_operands(LHS_TERMS, load, store, hold, tops=tops)

    def n_activations(width):
        return width // NS // LANES * (PART // 16) * 7

    def project(par, w, part, mark):
        lhs = lx if w == 0 else lc
        tiles = lhs.shape[1]
        dst = projected[par][w]
        dst = _shifted(dst, part, GROUP, dst.shape[0] // GROUP // GROUP)
        pending = {}

        def product(p):
            x = _cat([_matrix(lhs[p, t, _ds(part * PART // 2, PART // 2), :]) for t in range(tiles)], 1)
            return mark(jnp.dot(x, _matrix(weights[par][w][p]), preferred_element_type=F32))

        def emit(i, j, v):
            if w < 2:
                dst[pl.ds((j * SEQ + i * PART) // 2, PART // 2), :] = (
                    pltpu.bitcast(v.astype(BF16), U32) if w else _join_shuffled(v * (DB ** -0.5 * LOG2E)))
            else:
                pending[i, j] = v.T
                if i % 2 == 1:
                    pair = [pending.pop((i - 1 + b, j)) for b in range(2)]
                    blocks = [[t[a * DB // 2:(a + 1) * DB // 2] for t in pair] for a in range(2)]
                    for p, x in enumerate(_operands(LHS_TERMS, blocks)):
                        dst[pl.ds(((j * NPAIR + i // 2) * 7 + p) * DB // 4, DB // 4), :] = _join_shuffled(x)

        return _weigh(_multiply(product, emit), tiles)

    n_project = NP * (MB + 2 * DC) // NS // LANES

    def attend(par, h, head_id, pacer, lag, bursts, fast, score_weight, score_span, context_span):
        hold = pacer.after(lag)
        causal = (lax.broadcasted_iota(I32, (TILE, TILE), 0)
                  <= _unshuffle(lax.broadcasted_iota(I32, (TILE, TILE), 1)))
        queries, keys, values = (r.at[_ds(h * (r.shape[0] // GROUP), r.shape[0] // GROUP)] for r in projected[par])
        result = ctx.at[_ds(head_id * (SEQ // 2), SEQ // 2)]
        pending = {}

        def fold(op, t):
            return functools.reduce(op, [t[r:r + 8] for r in range(0, TILE, 8)])

        def scores(i):
            q = _matrix(queries[i * TILE // 2:(i + 1) * TILE // 2, :])
            tiles, peaks = [], []
            for j in range(i + 1):
                k = _matrix(keys[j * TILE // 2:(j + 1) * TILE // 2, :])
                s = pacer.mark(lax.dot_general(k, q, NT_DIMS, preferred_element_type=F32))
                if j == i:
                    s = jnp.where(causal, s, MASKED * LOG2E)
                tiles.append(s)
                peaks.append(fold(jnp.maximum, s))
                yield score_weight
            top = jnp.max(functools.reduce(jnp.maximum, peaks), axis=0, keepdims=True)
            if i // 2 >= max(1, NPAIR - fast):
                mass = functools.reduce(jnp.add, [jnp.exp2(x - top) for x in peaks])
                top = top + jnp.log2(jnp.sum(mass, axis=0, keepdims=True))
            pending[i] = tiles, jnp.broadcast_to(top, (8, TILE))

        def context(i):
            both = [pending.pop(2 * i + c) for c in range(2)]
            totals = [None, None]
            o = [[None, None], [None, None]]

            def weight(j, c):
                p = jnp.exp2(both[c][0][j] - _cat([hold(both[c][1])] * (TILE // 8), 0))
                t = fold(jnp.add, p)
                totals[c] = t if totals[c] is None else totals[c] + t
                return p

            def product(j, p, x):
                v = _matrix(values[(j * 7 + p) * DB // 4:(j * 7 + p + 1) * DB // 4, :])
                return pacer.mark(jnp.dot(v, x.astype(BF16), preferred_element_type=F32))

            def emit(a, c, v):
                o[a][c] = v if o[a][c] is None else o[a][c] + v

            def plain(j, c, tiles):
                for b in range(tiles):
                    p = weight(2 * j + b, c)
                    shared = product(j, 2 + b, p)
                    emit(b, c, shared)
                    emit(1 - b, c, shared + product(j, 5 + b, p))
                    yield 1

            yield from plain(i, 0, 1)
            yield from plain(i, 1, 2)
            acc = [None] * 7
            for j in range(i):
                if i < NPAIR - fast:
                    yield from plain(j, 0, 2)
                    yield from plain(j, 1, 2)
                    continue
                tiles = {}
                for burst in bursts:
                    for p in burst:
                        for _, b, c in RHS_TERMS[p]:
                            if (b, c) not in tiles:
                                tiles[b, c] = weight(2 * j + b, c)
                        t = product(j, p, _operand(RHS_TERMS[p], lambda b, c: [[tiles[b, c]]])[0][0])
                        acc[p] = t if acc[p] is None else acc[p] + t
                    yield 4 / 7 * len(burst)
            if acc[0] is not None:
                _run(_multiply(lambda p: acc[p], emit, 1))
            for c in range(2):
                x = _cat([o[0][c], o[1][c]], 0) * _reciprocal(jnp.sum(totals[c], axis=0, keepdims=True))
                result[(2 * i + c) * TILE // 2:(2 * i + c + 1) * TILE // 2, :] = pltpu.bitcast(x.astype(BF16).T, U32)

        for n in range(NPAIR + 1):
            streams = []
            if n < NPAIR:
                i = PAIR_ORDER[n]
                streams.append((_chain(scores(2 * i), scores(2 * i + 1)), (4 * i + 3) * score_weight, *score_span))
            if n > 0:
                i = PAIR_ORDER[n - 1]
                streams.append((context(i), 4 * i + 3, *context_span))
            yield from _merge(*streams)

    def n_attend(pace):
        return NPAIR * (2 * NPAIR + 1) * (1 + pace["score_weight"])

    def build_wo(head_id, hold):
        n = KO // HB
        src, dst = bwo_raw.at[:, _ds(head_id * n, n)], _shifted(ro, head_id, HB, n // 2)
        for ct in range(TPB):
            for s in range(0, n, 16):
                def load(i, j, hold):
                    c0 = (j * TPB + ct) * LANES
                    v = src[i, pl.ds(s, 16), c0:c0 + LANES].astype(F32)
                    return [hold(v[0:8]), hold(v[8:16])]

                def store(p, words):
                    dst[pl.ds(((p * TPB + ct) * KO + s) // 2, 8), :] = words

                yield from _build_operands(RHS_TERMS, load, store, hold)

    n_wo = TPB * (KO // HB // 16) * 7

    def head_step(par, g, h):
        pacer = _Pacer(lc[0, 0, 0:8, :])
        head_id = g * GROUP + h
        _interleave((attend(par, h, head_id, pacer, **HEAD), n_attend(HEAD), 0., .86),
                    (_chain(*[project(1 - par, w, h, pacer.mark) for w in (1, 2, 0)]), n_project),
                    (build_wo(head_id, pacer.after(2)), n_wo, .02, .15),
                    (build_group(par, h, pacer.after(1)), n_group, .25, .98))

    def last_head_step(h):
        pacer = _Pacer(lc[0, 0, 0:8, :])
        hold = pacer.after(1)
        head_id = (NGROUP - 1) * GROUP + h
        _interleave((attend(1, h, head_id, pacer, **LAST_HEAD), n_attend(LAST_HEAD)),
                    (build_wo(head_id, hold), n_wo, .03, .3),
                    (_chain(*[shuffle_columns(0, t, hold, [h]) for t in range(3)]), 3 * n_shuffle / NS, .1, .8))

    def start_up():
        data = {"k": weight_copies(0, 0, 1), "v": weight_copies(0, 0, 2), "q": weight_copies(0, 0, 0),
                "g1": group_copies(1, 1), "g2": group_copies(0, 2), "o": wo_copies(0)}
        for part in range(GROUP):
            data["c%d" % part], data["x%d" % part] = c_copies(part), x_copies(part)
        built = set()

        def copies(names):
            return [c for name in names.split() for c in data[name]]

        def operands(job, hold, tops=range(7)):
            if job[0] in "!+":
                (_wait if job[0] == "!" else _start)(copies(job[1:]))
            elif job[0] in "cx":
                src, dst = (c_raw, lc) if job[0] == "c" else (bwo_raw, lx)
                yield from build_activations(src, dst, int(job[1]), hold, tops)
            else:
                for part in range(GROUP):
                    yield from (build_group(1, part, hold) if job == "g" else
                                build_weights(0, "qkv".index(job), part, hold, tops))
            built.add(job)

        size = dict(c=n_activations(DC), x=n_activations(MB), g=GROUP * n_group,
                    **{name: GROUP * n_weights(w) for w, name in enumerate("qkv")})

        def projection(name, mark):
            assert {name[0], "xcc"["qkv".index(name[0])] + name[1]} <= built
            yield from project(0, "qkv".index(name[0]), int(name[1]), mark)

        def step(waits, starts, products, ahead, jobs, lag, span):
            _wait(copies(waits))
            _start(copies(starts))
            pacer = _Pacer(c_raw[0, 0:8, 0:LANES])
            for top in TOP_ORDER:
                for job in ahead.split():
                    _run(operands(job, _same, [top]))
            _interleave((_chain(*[projection(name, pacer.mark) for name in products.split()]),
                         sum(n_project // (2 if name[0] == "q" else 4) for name in products.split())),
                        (_chain(*[operands(job, pacer.after(lag)) for job in jobs.split()]),
                         sum(size.get(job[0], 0) for job in jobs.split()) or 1, *span))

        def steps(i):
            for n, args in enumerate(START_UP):
                pl.when(i == n)(functools.partial(step, *args))

        _start(copies("c0 k v c1"))
        _loop(len(START_UP), steps)

    def group(par, g):
        _wait(wo_copies(g))
        _start(wo_copies(g + 1))
        pl.when(g + 2 < NGROUP)(lambda: _wait(group_copies(par, g + 2)))
        pl.when(g + 3 < NGROUP)(lambda: _start(group_copies(1 - par, g + 3)))
        if par == 0:
            pl.when(g == NGROUP - 2)(lambda: _start(a_inputs))
        _loop(GROUP, lambda h: head_step(par, g, h))

    def two_groups(t):
        group(0, 2 * t)
        pl.when(t < NGROUP // 2 - 1)(lambda: group(1, 2 * t + 1))

    start_up()
    _loop(NGROUP // 2, two_groups)
    _wait(wo_copies(NGROUP - 1) + a_inputs)
    _loop(GROUP, last_head_step)

    la, qa = lx, qs0

    def w_a(t, p, ct, r0, rows):
        if t == 0:
            return (rq0, rq1)[ct], (p, _ds(r0, rows))
        if t == 1:
            return lc, (p, 0, _ds(ct * (KQ // 2) + r0, rows))
        if t == 2:
            buf, tile = divmod(TPB * p + ct, 25)
            assert rows <= 64 or rows == 128
            if rows == 128:
                return (rk0, rk1, rv0, rv1)[buf], (pl.ds(2 * tile, 2),)
            return (rk0, rk1, rv0, rv1)[buf], (2 * tile + r0 // 64, _ds(r0 % 64, rows))
        buf, tile = divmod(TPB * p, 50)
        return (vs0, vs1)[buf], (_ds((tile + ct) * (KQ // 2) + r0, rows),)

    def load_w(t, p):
        tiles = []
        for ct in range(TPB):
            buf, idx = w_a(t, p, ct, 0, KQ // 2)
            tiles.append(_matrix(buf[idx].reshape(KQ // 2, LANES)))
        return _cat(tiles, 1)

    span_a = HALO + SEQ // 2
    group_rows = 16 * NS

    def build_w(blk, t, hold):
        for s in range(0, WROWS, 16):
            for ct in range(TPB):
                def load(i, j, hold):
                    return _split(hold(wp[wp_rows(t, i, s, j * TPB + ct), :]))

                def store(p, words):
                    buf, idx = w_a(t, p, ct, (blk * WROWS + s) // 2, 8)
                    buf[idx] = words

                yield from _build_operands(RHS_TERMS, load, store, hold, True)

    n_w = (WROWS // 16) * TPB * 7

    def build_x(blk, hold):
        for c in range(ROWS // group_rows):
            for t in range(TPB):
                def load(i, j, hold):
                    words = ax_raw.at[j * TPB + t, _ds(blk * (ROWS // 2), ROWS // 2)]
                    w0 = (c * group_rows + 32 * (i // 2)) // 2
                    return [_split(hold(words[pl.ds(w0 + e, 8, stride=2), :]))[i % 2] for e in range(2)]

                def store(p, words):
                    la[p, t, _ds((blk * (ROWS // NS) + 16 * c) // 2, 8), :] = words

                yield from _build_operands(LHS_TERMS, load, store, hold, True)

    n_x = (ROWS // group_rows) * TPB * 7

    def build_awo(blk, hold):
        ct, odd, h0 = blk // 4, (blk // 2) % 2, 16 * (blk % 2)
        pairs = DHA // 2 // NS
        for dp in range(0, pairs, 2):
            src = {}
            for i in range(NS):
                for j in range(NS):
                    words = awo_raw.at[j * TPB + ct, pl.ds(pl.multiple_of(h0 * 16, 256), 256)]
                    for e in range(2):
                        w0 = 8 * e * 16 + i * pairs + dp
                        src[i, j, e] = hold(jnp.where(odd == 1, words[pl.ds(w0 + 1, 8, stride=16), :],
                                                      words[pl.ds(w0, 8, stride=16), :]))
                yield
            for half in range(2):
                def load(i, j, hold):
                    return [_split(hold(src[i, j, e]))[half] for e in range(2)]

                def store(p, words):
                    buf, idx = w_a(3, p, ct, ((2 * (dp + odd) + half) * HA + h0) // 2, 8)
                    buf[idx] = words

                yield from _build_operands(RHS_TERMS, load, store, hold, True)

    n_awo = (DHA // 2 // NS // 2) * (NS + 2 * 7)

    def output_b(blk):
        slot = blk % 2
        rows = ROWS // NS
        heads = HB // NS
        pl.when(blk >= 2)(lambda: out_copy(blk - 2).wait())
        pacer = _Pacer(ro[0:8, :])
        src = _shifted(ctx, blk, NBLK, ROWS // 2)
        lhs = {}

        def build_lhs(top, hold):
            half = NS // 2
            for h in range(heads):
                for r in range(0, rows, 16):
                    def quadrant(i, j):
                        return [[_split_shuffled(hold(src[pl.ds(
                            (((j * half + b) * heads + h) * SEQ + (i * half + a) * rows + r) // 2, 8), :]))
                            for b in range(half)] for a in range(half)]

                    for p, v in enumerate(_operands(LHS_TERMS, _operand(LHS_TERMS[top], quadrant))):
                        lhs.setdefault((top * (NP // 7) + p, h), []).append(v)
                    yield

        def product(p):
            x = _cat([_cat(lhs[p, h], 0) for h in range(heads)], 1).astype(BF16)
            w = _cat([_matrix(ro[pl.ds((p * TPB + ct) * KO // 2, KO // 2), :]) for ct in range(TPB)], 1)
            return pacer.mark(jnp.dot(x, w, preferred_element_type=F32))

        def emit(i, j, v):
            stage[slot, i * rows:(i + 1) * rows, j * KQ:(j + 1) * KQ] = v.astype(BF16)

        _run(build_lhs(TOP_ORDER[0], _same))
        hold = pacer.after(1)
        _interleave(
            (_multiply(product, emit), NP),
            (_chain(*[build_lhs(t, hold) for t in TOP_ORDER[1:]]), 6 * heads * (rows // 16), 0., .84),
            *[(_chain(build_w(blk, t, hold), shuffle_columns(blk + 1, t, hold)), n_w + n_shuffle, .02, .95)
              for t in range(3)],
            (build_x(blk, hold), n_x, .02, .95),
            (build_awo(blk, hold), n_awo, .02, .95))
        out_copy(blk).start()

    _loop(NBLK, output_b)

    def project_a(t, blk, mark):
        rows = ROWS // NS
        dst = _shifted(ro if t == 1 else ctx, blk, NBLK, ROWS // 2)

        def product(p):
            x = _cat([_matrix(la[p, k, _ds(blk * rows // 2, rows // 2), :]) for k in range(TPB)], 1)
            return mark(jnp.dot(x, load_w(t, p), preferred_element_type=F32))

        def emit(i, j, v):
            for ct in range(TPB):
                for c in range(rows // 16):
                    piece = v[16 * c:16 * (c + 1), ct * LANES:(ct + 1) * LANES]
                    tile = 2 * (j * TPB + ct) + i % 2
                    r = c * (group_rows // 2) + 16 * (i // 2)
                    if t == 0:
                        qa[_ds(tile * ROWS + (blk % 2) * (ROWS // 2) + r, 16), :] = pltpu.bitcast(piece, U32)
                    else:
                        dst[pl.ds(tile * span_a + HALO + r, 16), :] = pltpu.bitcast(piece, U32)

        return _multiply(product, emit)

    def attend_a(blk, hold, softmax_weight, operand_weight, hold_q, hold_sum, hold_v, **_):
        row0, slot = blk * (ROWS // 2), blk % 2
        keys, values = (_shifted(buf, blk, NBLK, ROWS // 2) for buf in (ro, ctx))
        logits, o = {}, {}

        def window(buf, j, r, par, w):
            return pltpu.bitcast(buf[pl.ds((2 * j + par) * span_a + HALO + r - w, 8), :], F32)

        def scores(r, par):
            pos = row0 + r + lax.broadcasted_iota(I32, (8, LANES), 0)
            q = [pltpu.bitcast(qa[_ds((2 * j + par) * ROWS + slot * (ROWS // 2) + r, 8), :], F32) for j in range(8)]
            q = [hold(x) if j % hold_q == 0 else x for j, x in enumerate(q)]
            logits[r, par] = []
            for w in range(WIN):
                acc = q[0] * hold(window(keys, 0, r, par, w))
                for j in range(1, 8):
                    acc = acc + q[j] * window(keys, j, r, par, w)
                acc = hold(acc) if hold_sum else acc
                acc = acc + pltpu.roll(acc, 64, 1)
                acc = acc + pltpu.roll(acc, 32, 1)
                acc = acc * (DHA ** -0.5 * LOG2E)
                if r < w:
                    acc = jnp.where(pos >= w, acc, MASKED * LOG2E)
                logits[r, par].append(acc)
                yield

        def context(r, par):
            x = logits.pop((r, par))
            top = functools.reduce(jnp.maximum, x)
            e = [jnp.exp2(t - top) for t in x]
            scale = _reciprocal(functools.reduce(jnp.add, e))
            e = [t * scale for t in e]
            yield softmax_weight
            for j in range(8):
                acc = None
                for w in range(WIN):
                    v = window(values, j, r, par, w)
                    t = e[w] * (hold(v) if w % hold_v == 0 else v)
                    acc = t if acc is None else acc + t
                o[r, par, j] = acc
                yield

        def operands(c):
            for t in range(TPB):
                def load(i, j, hold):
                    return [hold(o[c * (group_rows // 2) + 8 * i, par, j * TPB + t]) for par in range(2)]

                def store(p, words):
                    lo[blk % SLOTS * NP + p, t, 8 * c:8 * (c + 1), :] = words

                yield from _weigh(_build_operands(LHS_TERMS, load, store, hold), operand_weight)

        for c in range(ROWS // group_rows):
            units = [(r, par) for r in range(c * group_rows // 2, (c + 1) * group_rows // 2, 8) for par in range(2)]
            yield from scores(*units[0])
            for now, after in zip(units, units[1:]):
                yield from _merge((scores(*after), WIN), (context(*now), 8 + softmax_weight))
            yield from context(*units[-1])
            yield from operands(c)

    def output_a(blk, mark):
        slot = blk % 2

        def product(p):
            x = _cat([_matrix(lo[blk % SLOTS * NP + p, k]) for k in range(TPB)], 1)
            return mark(jnp.dot(x, load_w(3, p), preferred_element_type=F32))

        def emit(i, j, v):
            for c in range(ROWS // group_rows):
                r = c * group_rows + 16 * i
                stage[slot, r:r + 16, j * KQ:(j + 1) * KQ] = v[16 * c:16 * (c + 1)].astype(BF16)

        return _multiply(product, emit)

    def outputs_a(blocks, mark):
        for n, blk in enumerate(blocks):
            if n > 0:
                out_copy(NBLK + blk - 1).start()
                out_copy(NBLK + blk - 2).wait()
            yield from output_a(blk, mark)

    def step_a(project, attend, outputs, pace=None):
        pacer = _Pacer(lc[0, 0, 0:8, :])
        matmuls = [] if project is None else [project_a(t, project, pacer.mark) for t in (1, 2, 0)]
        streams = [(_chain(outputs_a(outputs, pacer.mark), *matmuls), (len(outputs) + len(matmuls)) * NP)]
        if pace:
            total = ((WIN + 8 + pace["softmax_weight"]) * (ROWS // 8)
                     + TPB * (ROWS // group_rows) * 7 * pace["operand_weight"])
            streams.append((attend_a(attend, pacer.after(pace["lag"]), **pace), total, *pace["span"]))
        if outputs:
            out_copy(NBLK + outputs[0] - 2).wait()
        _interleave(*streams)
        if outputs:
            out_copy(NBLK + outputs[-1]).start()

    for tile in range(16):
        for buf in (ro, ctx):
            buf[tile * span_a:tile * span_a + HALO, :] = jnp.zeros((HALO, LANES), U32)
    step_a(0, None, [])
    _loop(DELAY, lambda i: step_a(i + 1, i, [], A_FIRST))
    _loop(NBLK - 1 - DELAY, lambda i: step_a(i + DELAY + 1, i + DELAY, [i], A_MAIN))
    step_a(None, NBLK - 1, range(NBLK - 1 - DELAY, NBLK - 1), A_LAST)

    halves = [pltpu.make_async_copy(stage.at[1, :, pl.ds(c, DA // 2)],
                                    out_hbm.at[pl.ds(SEQ - ROWS, ROWS), pl.ds(c, DA // 2)], sem_out.at[1])
              for c in (0, DA // 2)]
    out_copy(2 * NBLK - 3).wait()
    for n, _ in enumerate(output_a(NBLK - 1, _same)):
        if n == 5 * NP // 7:
            halves[0].start()
    halves[1].start()
    _wait([out_copy(2 * NBLK - 2)] + halves)


def _words(*shape):
    return pltpu.VMEM(shape + (LANES,), U32)


SCRATCH = [
    _words(DA // LANES, SEQ // 2),
    pltpu.VMEM((DA // 2, 3 * DA), U32),
    _words(DA // LANES, DA // 2),
    pltpu.VMEM((NS, MQ // 2, DC), U32),
    pltpu.VMEM((NS, KO, MB), BF16),
    _words(NP, MB // NS // LANES, MQ // 2),
    _words(NP, DC // NS // LANES, MQ // 2),
    *[_words(NP, MB // NS // 2)] * 2,
    *[_words(NP + 1, DC // NS // 2)] * 4,
    *[_words(GROUP * SEQ // 2)] * 4,
    *[_words(GROUP * NPAIR * 7 * DB // 4)] * 2,
    *[_words(GROUP * MB // 2)] * 2,
    *[_words(GROUP * DC // 2)] * 4,
    _words(HB * SEQ // 2),
    _words(NP * TPB * KO // 2),
    _words(SLOTS * NP, TPB, ROWS // NS // 2),
    pltpu.VMEM((2, ROWS, DA), BF16),
    pltpu.SemaphoreType.DMA((GROUP,)),
    pltpu.SemaphoreType.DMA((GROUP,)),
    pltpu.SemaphoreType.DMA(()),
    pltpu.SemaphoreType.DMA((6,)),
    pltpu.SemaphoreType.DMA(()),
    pltpu.SemaphoreType.DMA((2,)),
]


@jax.jit
def pallas_concat_heads__sliding_local_dilated__compressed_kv_cla__prompt_kernel(A_x, A_wqkv, A_wo, B_x, B_c_kv, B_w_q, B_w_uk, B_w_uv, B_w_o):
    hbm = pl.BlockSpec(memory_space=pl.ANY)
    out = pl.pallas_call(
        _kernel,
        in_specs=[hbm] * 9,
        out_specs=hbm,
        out_shape=jax.ShapeDtypeStruct((SEQ, DA + MB), BF16),
        scratch_shapes=SCRATCH,
        compiler_params=pltpu.CompilerParams(vmem_limit_bytes=127 * 2 ** 20),
        name="fused_attention",
    )(A_x.reshape(SEQ, DA), A_wqkv, A_wo, B_x.reshape(GROUP, NS, PART, MB), B_c_kv.reshape(GROUP, NS, PART, DC),
      B_w_q.reshape(MB // 2, 2 * HB, DB), B_w_uk.reshape(DC // 2, 2 * HB, DB),
      B_w_uv.reshape(DC // 2, 2 * HB, DB), B_w_o.reshape(NS, KO, MB))
    return out.reshape(1, SEQ, DA + MB)
```

```python
import functools
import math

import jax
import jax.numpy as jnp
import numpy as np
from jax import lax
import jax.experimental.pallas as pl
import jax.experimental.pallas.tpu as pltpu

F32 = jnp.float32
BF16 = jnp.bfloat16
U32 = jnp.uint32
I32 = jnp.int32
LANES = 128
NT_DIMS = (((1,), (1,)), ((), ()))
LOG2E = math.log2(math.e)
MASKED = -1e9

SEQ = 2048
DA = 1024
HA, DHA = 32, 32
WIN = 8
HALO = 32
MB = 1024
HB, DB = 32, 128
DC = 512

LEVELS = 2
NS = 2 ** LEVELS
NP = 7 ** LEVELS
GROUP = NS
NGROUP = HB // GROUP
MQ = SEQ // NS
PART = MQ // GROUP
ROWS = 256
NBLK = SEQ // ROWS
KQ = DA // NS
TPB = KQ // LANES
KO = HB * DB // NS
WROWS = KQ // NBLK
TILE = LANES
NPAIR = SEQ // TILE // 2
DELAY = 2
SLOTS = 4

START_UP = (
    ("c0 k", "c2 c3", "k0", "c0 k", "", 1, (0., 1.)),
    ("v c1", "q x0", "v0", "v", "c1", 20, (.02, 1.01)),
    ("c2 c3", "x1 x2 x3", "k1 v1 k2 v2 k3", "", "c2 c3 !q +g1 q !x0 x0", 14, (0., .98)),
    ("x1 x2", "", "q0 q1", "", "x1 x2", 6, (.055, .93)),
    ("x3 g1", "g2 o", "q2 v3 q3", "", "x3 g", 2, (0., .98)),
)
PAIR_ORDER = (1, 3, 5, 7, 6, 4, 2, 0)
HEAD = dict(lag=9, bursts=((1,), (4,), (0,), (2,), (5,), (3,), (6,)), fast=NPAIR,
            score_weight=1, score_span=(0, .7), context_span=(.15, 1))
LAST_HEAD = dict(lag=11, bursts=((1, 4), (0, 2), (5, 3), (6,)), fast=5,
                 score_weight=1.1, score_span=(0, .6), context_span=(.25, 1))
A_FIRST = dict(lag=3, span=(.02, .98), softmax_weight=1, operand_weight=7, hold_q=8, hold_v=4)
A_MAIN = dict(lag=6, span=(.08, .99), softmax_weight=3, operand_weight=4, hold_q=8, hold_v=8)
A_LAST = dict(lag=2, span=(.02, 1.), softmax_weight=6, operand_weight=12, hold_q=1, hold_v=8)


LHS_TERMS = (((1, 0, 0), (1, 1, 1)), ((1, 1, 0), (1, 1, 1)), ((1, 0, 0),), ((1, 1, 1),),
             ((1, 0, 0), (1, 0, 1)), ((1, 1, 0), (-1, 0, 0)), ((1, 0, 1), (-1, 1, 1)))
RHS_TERMS = (((1, 0, 0), (1, 1, 1)), ((1, 0, 0),), ((1, 0, 1), (-1, 1, 1)), ((1, 1, 0), (-1, 0, 0)),
             ((1, 1, 1),), ((1, 0, 0), (1, 0, 1)), ((1, 1, 0), (1, 1, 1)))
TOP_ORDER = (1, 3, 0, 6, 4, 2, 5)


def _add(x, y):
    return [[lax.add(a, b) for a, b in zip(rx, ry)] for rx, ry in zip(x, y)]


def _sub(x, y):
    return [[lax.sub(a, b) for a, b in zip(rx, ry)] for rx, ry in zip(x, y)]


def _operand(terms, quadrant):
    total = None
    for sign, i, j in terms:
        q = quadrant(i, j)
        total = q if total is None else (_add if sign > 0 else _sub)(total, q)
    return total


def _operands(side, blocks):
    half = len(blocks) // 2
    if half == 0:
        return [blocks[0][0]]

    def quadrant(i, j):
        return [row[j * half:(j + 1) * half] for row in blocks[i * half:(i + 1) * half]]

    return [x for terms in side for x in _operands(side, _operand(terms, quadrant))]


def _multiply(product, emit, level=LEVELS, base=0):
    if level == 0:
        emit(0, 0, product(base))
        yield
        return
    n = 2 ** (level - 1)

    def m(i):
        out = [[None] * n for _ in range(n)]

        def keep(a, b, v):
            out[a][b] = v

        yield from _multiply(product, keep, level - 1, base + (i - 1) * 7 ** (level - 1))
        return out

    def put(x, oi, oj):
        for a in range(n):
            for b in range(n):
                emit(oi * n + a, oj * n + b, x[a][b])

    m2 = yield from m(2)
    m4 = yield from m(4)
    put(_add(m2, m4), 1, 0)
    m1 = yield from m(1)
    c11 = _add(m1, m4)
    c22 = _sub(m1, m2)
    m7 = yield from m(7)
    c11 = _add(c11, m7)
    m5 = yield from m(5)
    put(_sub(c11, m5), 0, 0)
    m3 = yield from m(3)
    put(_add(m3, m5), 0, 1)
    c22 = _add(c22, m3)
    m6 = yield from m(6)
    put(_add(c22, m6), 1, 1)


def _build_operands(side, load, store, hold, hold_all=False, tops=range(7)):
    half = NS // 2
    for top in tops:
        terms = side[top]
        loaded = {(i, j): [[load(i * half + a, j * half + b, hold if hold_all or (a == b and n == 0) else _same)
                            for b in range(half)] for a in range(half)]
                  for n, (_, i, j) in enumerate(terms)}
        lo, hi = (_operands(side, _operand(terms, lambda i, j: [[x[e] for x in row] for row in loaded[i, j]]))
                  for e in range(2))
        for p in range(NP // 7):
            store(top * (NP // 7) + p, _join(lo[p], hi[p]))
        yield


def _low(words):
    return pltpu.bitcast(lax.shift_left(words, np.uint32(16)), F32)


def _high(words):
    return pltpu.bitcast(lax.bitwise_and(words, np.uint32(0xFFFF0000)), F32)


def _split(words):
    return _low(words), _high(words)


def _join(lo, hi):
    return pltpu.bitcast(pltpu.pack_elementwise([lo, hi], packed_dtype=BF16), U32)


def _join_shuffled(v):
    r, c = v.shape
    v = v.reshape(r // 16, 2, 8, c)
    return _join(v[:, 0].reshape(r // 2, c), v[:, 1].reshape(r // 2, c))


def _split_shuffled(words):
    lo, hi = _split(words)
    r, c = words.shape
    return jnp.stack([lo.reshape(r // 8, 8, c), hi.reshape(r // 8, 8, c)], axis=1).reshape(2 * r, c)


def _unshuffle(pos):
    return (pos & ~15) + ((pos & 15) >> 1) + 8 * (pos & 1)


def _matrix(words):
    return pltpu.bitcast(words, BF16)


def _cat(xs, axis):
    return xs[0] if len(xs) == 1 else jnp.concatenate(xs, axis=axis)


def _ds(start, size):
    if isinstance(start, int):
        return pl.ds(start, size)
    return pl.ds(pl.multiple_of(start, min(size, 16)), size)


def _shifted(ref, step, steps, n):
    return ref.at[_ds(step * n, ref.shape[0] - (steps - 1) * n)]


def _loop(n, body):
    lax.fori_loop(0, n, lambda i, carry: body(i), None)


def _start(copies):
    for c in copies:
        c.start()


def _wait(copies):
    for c in copies:
        c.wait()


def _run(steps):
    for _ in steps:
        pass


def _chain(*streams):
    for steps in streams:
        yield from steps


def _weigh(steps, weight):
    for _ in steps:
        yield weight


def _merge(*streams):
    spans = [s[2:] if len(s) > 2 else (0.0, 1.0) for s in streams]
    done = [0.0] * len(streams)
    live = list(range(len(streams)))
    while live:
        i = min(live, key=lambda k: spans[k][0] + (spans[k][1] - spans[k][0]) * done[k] / streams[k][1])
        try:
            weight = next(streams[i][0])
        except StopIteration:
            live.remove(i)
            continue
        weight = 1 if weight is None else weight
        done[i] += weight
        yield weight


def _interleave(*streams):
    _run(_merge(*streams))


class _Pacer:
    def __init__(self, words):
        self.never = (words | 1) == 0
        self.marks = []

    def mark(self, v):
        self.marks.append({None: v})
        return v

    def after(self, lag):
        def hold(x):
            if len(self.marks) < lag:
                return x
            mark = self.marks[-lag]
            if x.dtype not in mark:
                mark[x.dtype] = pltpu.bitcast(mark[None][0:8, 0:LANES], x.dtype)
            return lax.select(self.never, mark[x.dtype], x)

        return hold


def _same(x):
    return x


def _reciprocal(x):
    r = pltpu.reciprocal(x, approx=True)
    return r * (2.0 - x * r)


def _kernel(ax_hbm, wqkv_hbm, awo_hbm, bx_hbm, c_hbm, wq_hbm, wuk_hbm, wuv_hbm, bwo_hbm, out_hbm,
            ax_raw, wqkv_raw, awo_raw, c_raw, bwo_raw,
            lx, lc, rq0, rq1, rk0, rk1, rv0, rv1, qs0, qs1, ks0, ks1, vs0, vs1,
            sq0, sq1, sk0, sk1, sv0, sv1, ctx, ro, lo, stage,
            sem_c, sem_x, sem_wo, sem_w, sem_a, sem_out):

    def out_copy(n):
        return pltpu.make_async_copy(
            stage.at[n % 2], out_hbm.at[_ds(n % NBLK * ROWS, ROWS), _ds((1 - n // NBLK) * DA, DA)], sem_out.at[n % 2])

    a_inputs = ([pltpu.make_async_copy(ax_hbm.bitcast(U32).at[:, pl.ds(j * LANES, LANES)], ax_raw.at[j], sem_a)
                 for j in range(DA // LANES)]
                + [pltpu.make_async_copy(awo_hbm.bitcast(U32).at[:, pl.ds(j * LANES, LANES)], awo_raw.at[j], sem_a)
                   for j in range(DA // LANES)]
                + [pltpu.make_async_copy(wqkv_hbm.bitcast(U32), wqkv_raw, sem_a)])

    wp = ks0

    def wp_rows(t, i, s, c):
        return _ds((((t * NS + i) * (WROWS // 16) + s // 16) * 8 + c) * 8, 8)

    def shuffle_columns(blk, t, hold, quarters=range(NS)):
        lane = lax.broadcasted_iota(I32, (8, LANES), 1)
        slot, chunk, low = lane >> 5, (lane & 31) >> 2, lane & 3
        head_of = _unshuffle(lane & 31)
        for s in range(0, WROWS, 16):
            for i in quarters:
                rows = _ds((i * KQ + (blk % NBLK) * WROWS + s) // 2, 8)
                moved = []
                for j in range(8):
                    c0 = t * DA + j * LANES
                    u = hold(pltpu.bitcast(wqkv_raw[rows, c0:c0 + LANES], I32))
                    moved.append(jnp.take_along_axis(u, low * 32 + 4 * ((chunk - j) & 7) + slot, axis=1))
                    if j % 4 == 3:
                        yield
                v = [moved[-c % 8] for c in range(8)]
                for bit in (1, 2, 4):
                    v = [jnp.where((chunk & bit) != 0, v[(c - bit) % 8], v[c]) for c in range(8)]
                for c in range(8):
                    source = slot * 32 + (((head_of >> 2) + c) & 7) * 4 + (head_of & 3)
                    wp[wp_rows(t, i, s, c), :] = pltpu.bitcast(jnp.take_along_axis(v[c], source, axis=1), U32)
                    if c % 4 == 3:
                        yield

    n_shuffle = (WROWS // 16) * NS * 4

    weights = ((rq0, rk0, rv0), (rq1, rk1, rv1))
    projected = ((qs0, ks0, vs0), (qs1, ks1, vs1))
    staged = ((sq0, sk0, sv0), (sq1, sk1, sv1))

    def weight_copies(par, grp, w):
        words = (wq_hbm, wuk_hbm, wuv_hbm)[w].bitcast(U32)
        n = words.shape[0]
        return [pltpu.make_async_copy(
            words.at[:, (HB // 2) * parity + grp * (GROUP // 2) + pair],
            staged[par][w].at[pl.ds((2 * pair + parity) * n, n)], sem_w.at[3 * par + w])
            for pair in range(GROUP // 2) for parity in range(2)]

    def group_copies(par, grp):
        return [c for w in range(3) for c in weight_copies(par, grp, w)]

    def c_copies(part):
        return [pltpu.make_async_copy(c_hbm.bitcast(U32).at[part], c_raw.at[:, pl.ds(part * PART // 2, PART // 2)],
                                      sem_c.at[part])]

    def x_copies(part):
        return [pltpu.make_async_copy(bx_hbm.at[part], bwo_raw.at[:, pl.ds(part * PART, PART)], sem_x.at[part])]

    def wo_copies(grp):
        rows = (slice(None), _ds(grp * (KO // NGROUP), KO // NGROUP))
        return [pltpu.make_async_copy(bwo_hbm.at[rows], bwo_raw.at[rows], sem_wo)]

    def build_weights(par, w, part, hold, tops=range(7)):
        n = (MB, DC, DC)[w] // 2
        rows = n // NS // GROUP
        src = _shifted(staged[par][w], part, GROUP, rows)
        for s in range(0, rows, 8):
            target = _ds(part * rows + s, 8)

            def load(i, j, hold):
                return [(_low, _high)[j % 2](hold(src[pl.ds((2 * (j // 2) + e) * n + i * (n // NS) + s, 8), :]))
                        for e in range(2)]

            def store(p, words):
                weights[par][w][p, target, :] = words

            yield from _build_operands(RHS_TERMS, load, store, hold, tops=tops)

    def n_weights(w):
        return (MB, DC, DC)[w] // NS // GROUP // 16 * 7

    def build_group(par, part, hold):
        return _chain(*[build_weights(par, w, part, hold) for w in range(3)])

    n_group = sum(n_weights(w) for w in range(3))

    def build_activations(src, dst, part, hold, tops=range(7)):
        tiles = src.shape[2] // NS // LANES
        for t in range(tiles):
            for s in range(0, PART, 16):
                r = part * PART + s

                def load(i, j, hold):
                    c0 = (j * tiles + t) * LANES
                    if src.dtype == U32:
                        return _split(hold(src[i, pl.ds(r // 2, 8), c0:c0 + LANES]))
                    return _split(hold(pltpu.bitcast(src[i, pl.ds(r, 16), c0:c0 + LANES], U32)))

                def store(p, words):
                    dst[p, t, pl.ds(r // 2, 8), :] = words

                yield from _build_operands(LHS_TERMS, load, store, hold, tops=tops)

    def n_activations(width):
        return width // NS // LANES * (PART // 16) * 7

    def project(par, w, part, mark):
        lhs = lx if w == 0 else lc
        tiles = lhs.shape[1]
        dst = projected[par][w]
        dst = _shifted(dst, part, GROUP, dst.shape[0] // GROUP // GROUP)
        source = _ds(part * (PART // 2), PART // 2)
        pending = {}

        def product(p):
            x = _cat([_matrix(lhs[p, t, source, :]) for t in range(tiles)], 1)
            return mark(jnp.dot(x, _matrix(weights[par][w][p]), preferred_element_type=F32))

        def emit(i, j, v):
            if w < 2:
                dst[pl.ds((j * SEQ + i * PART) // 2, PART // 2), :] = (
                    pltpu.bitcast(v.astype(BF16), U32) if w else _join_shuffled(v * (DB ** -0.5 * LOG2E)))
            else:
                pending[i, j] = v.T
                if i % 2 == 1:
                    pair = [pending.pop((i - 1 + b, j)) for b in range(2)]
                    blocks = [[t[a * DB // 2:(a + 1) * DB // 2] for t in pair] for a in range(2)]
                    for p, x in enumerate(_operands(LHS_TERMS, blocks)):
                        dst[pl.ds(((j * NPAIR + i // 2) * 7 + p) * DB // 4, DB // 4), :] = _join_shuffled(x)

        return _weigh(_multiply(product, emit), tiles)

    n_project = NP * (MB + 2 * DC) // NS // LANES

    def attend(par, h, head_id, pacer, lag, bursts, fast, score_weight, score_span, context_span):
        hold = pacer.after(lag)
        causal = (lax.broadcasted_iota(I32, (TILE, TILE), 0)
                  <= _unshuffle(lax.broadcasted_iota(I32, (TILE, TILE), 1)))
        queries, keys, values = (r.at[_ds(h * (r.shape[0] // GROUP), r.shape[0] // GROUP)] for r in projected[par])
        result = ctx.at[_ds(head_id * (SEQ // 2), SEQ // 2)]
        pending = {}

        def fold(op, t):
            return functools.reduce(op, [lax.slice(t, (r, 0), (r + 8, TILE)) for r in range(0, TILE, 8)])

        def scores(i):
            q = _matrix(queries[i * TILE // 2:(i + 1) * TILE // 2, :])
            tiles, peaks = [], []
            for j in range(i + 1):
                k = _matrix(keys[j * TILE // 2:(j + 1) * TILE // 2, :])
                s = pacer.mark(lax.dot_general(k, q, NT_DIMS, preferred_element_type=F32))
                if j == i:
                    s = jnp.where(causal, s, MASKED * LOG2E)
                tiles.append(s)
                peaks.append(fold(lax.max, s))
                yield score_weight
            top = jnp.max(functools.reduce(jnp.maximum, peaks), axis=0, keepdims=True)
            if i // 2 >= max(1, NPAIR - fast):
                mass = functools.reduce(jnp.add, [jnp.exp2(x - top) for x in peaks])
                top = top + jnp.log2(jnp.sum(mass, axis=0, keepdims=True))
            pending[i] = tiles, jnp.broadcast_to(top, (8, TILE))

        def context(i):
            both = [pending.pop(2 * i + c) for c in range(2)]
            totals = [None, None]
            o = [[None, None], [None, None]]

            def weight(j, c):
                p = jnp.exp2(both[c][0][j] - _cat([hold(both[c][1])] * (TILE // 8), 0))
                t = fold(lax.add, p)
                totals[c] = t if totals[c] is None else totals[c] + t
                return p

            def product(j, p, x):
                v = _matrix(values[(j * 7 + p) * DB // 4:(j * 7 + p + 1) * DB // 4, :])
                return pacer.mark(jnp.dot(v, x.astype(BF16), preferred_element_type=F32))

            def emit(a, c, v):
                o[a][c] = v if o[a][c] is None else o[a][c] + v

            def plain(j, c, tiles):
                for b in range(tiles):
                    p = weight(2 * j + b, c)
                    shared = product(j, 2 + b, p)
                    emit(b, c, shared)
                    emit(1 - b, c, shared + product(j, 5 + b, p))
                    yield 1

            yield from plain(i, 0, 1)
            yield from plain(i, 1, 2)
            acc = [None] * 7
            for j in range(i):
                if i < NPAIR - fast:
                    yield from plain(j, 0, 2)
                    yield from plain(j, 1, 2)
                    continue
                tiles = {}
                for burst in bursts:
                    for p in burst:
                        for _, b, c in RHS_TERMS[p]:
                            if (b, c) not in tiles:
                                tiles[b, c] = weight(2 * j + b, c)
                        t = product(j, p, _operand(RHS_TERMS[p], lambda b, c: [[tiles[b, c]]])[0][0])
                        acc[p] = t if acc[p] is None else acc[p] + t
                    yield 4 / 7 * len(burst)
            if acc[0] is not None:
                _run(_multiply(lambda p: acc[p], emit, 1))
            for c in range(2):
                x = _cat([o[0][c], o[1][c]], 0) * _reciprocal(jnp.sum(totals[c], axis=0, keepdims=True))
                result[(2 * i + c) * TILE // 2:(2 * i + c + 1) * TILE // 2, :] = pltpu.bitcast(x.astype(BF16).T, U32)

        for n in range(NPAIR + 1):
            streams = []
            if n < NPAIR:
                i = PAIR_ORDER[n]
                streams.append((_chain(scores(2 * i), scores(2 * i + 1)), (4 * i + 3) * score_weight, *score_span))
            if n > 0:
                i = PAIR_ORDER[n - 1]
                streams.append((context(i), 4 * i + 3, *context_span))
            yield from _merge(*streams)

    def n_attend(pace):
        return NPAIR * (2 * NPAIR + 1) * (1 + pace["score_weight"])

    def build_wo(head_id, hold):
        n = KO // HB
        src, dst = bwo_raw.at[:, _ds(head_id * n, n)], _shifted(ro, head_id, HB, n // 2)
        for ct in range(TPB):
            for s in range(0, n, 16):
                def load(i, j, hold):
                    c0 = (j * TPB + ct) * LANES
                    v = src[i, pl.ds(s, 16), c0:c0 + LANES].astype(F32)
                    return [hold(v[0:8]), hold(v[8:16])]

                def store(p, words):
                    dst[pl.ds(((p * TPB + ct) * KO + s) // 2, 8), :] = words

                yield from _build_operands(RHS_TERMS, load, store, hold)

    n_wo = TPB * (KO // HB // 16) * 7

    def head_step(par, g, h):
        pacer = _Pacer(lc[0, 0, 0:8, :])
        head_id = g * GROUP + h
        _interleave((attend(par, h, head_id, pacer, **HEAD), n_attend(HEAD), 0., .86),
                    (_chain(*[project(1 - par, w, h, pacer.mark) for w in (1, 2, 0)]), n_project),
                    (build_wo(head_id, pacer.after(2)), n_wo, .02, .15),
                    (build_group(par, h, pacer.after(1)), n_group, .25, .98))

    def last_head_step(h):
        pacer = _Pacer(lc[0, 0, 0:8, :])
        hold = pacer.after(1)
        head_id = (NGROUP - 1) * GROUP + h
        _interleave((attend(1, h, head_id, pacer, **LAST_HEAD), n_attend(LAST_HEAD)),
                    (build_wo(head_id, hold), n_wo, .03, .3),
                    (_chain(*[shuffle_columns(0, t, hold, [h]) for t in range(3)]), 3 * n_shuffle / NS, .1, .8))

    def start_up():
        data = {"k": weight_copies(0, 0, 1), "v": weight_copies(0, 0, 2), "q": weight_copies(0, 0, 0),
                "g1": group_copies(1, 1), "g2": group_copies(0, 2), "o": wo_copies(0)}
        for part in range(GROUP):
            data["c%d" % part], data["x%d" % part] = c_copies(part), x_copies(part)
        built = set()

        def copies(names):
            return [c for name in names.split() for c in data[name]]

        def operands(job, hold, tops=range(7)):
            if job[0] in "!+":
                (_wait if job[0] == "!" else _start)(copies(job[1:]))
            elif job[0] in "cx":
                src, dst = (c_raw, lc) if job[0] == "c" else (bwo_raw, lx)
                yield from build_activations(src, dst, int(job[1]), hold, tops)
            else:
                for part in range(GROUP):
                    yield from (build_group(1, part, hold) if job == "g" else
                                build_weights(0, "qkv".index(job), part, hold, tops))
            built.add(job)

        size = dict(c=n_activations(DC), x=n_activations(MB), g=GROUP * n_group,
                    **{name: GROUP * n_weights(w) for w, name in enumerate("qkv")})

        def projection(name, mark):
            assert {name[0], "xcc"["qkv".index(name[0])] + name[1]} <= built
            yield from project(0, "qkv".index(name[0]), int(name[1]), mark)

        def step(waits, starts, products, ahead, jobs, lag, span):
            _wait(copies(waits))
            _start(copies(starts))
            pacer = _Pacer(c_raw[0, 0:8, 0:LANES])
            for top in TOP_ORDER:
                for job in ahead.split():
                    _run(operands(job, _same, [top]))
            _interleave((_chain(*[projection(name, pacer.mark) for name in products.split()]),
                         sum(n_project // (2 if name[0] == "q" else 4) for name in products.split())),
                        (_chain(*[operands(job, pacer.after(lag)) for job in jobs.split()]),
                         sum(size.get(job[0], 0) for job in jobs.split()) or 1, *span))

        def steps(i):
            for n, args in enumerate(START_UP):
                pl.when(i == n)(functools.partial(step, *args))

        _start(copies("c0 k v c1"))
        _loop(len(START_UP), steps)

    def group(par, g):
        _wait(wo_copies(g))
        _start(wo_copies(g + 1))
        pl.when(g + 2 < NGROUP)(lambda: _wait(group_copies(par, g + 2)))
        pl.when(g + 3 < NGROUP)(lambda: _start(group_copies(1 - par, g + 3)))
        if par == 0:
            pl.when(g == NGROUP - 2)(lambda: _start(a_inputs))
        _loop(GROUP, lambda h: head_step(par, g, h))

    def two_groups(t):
        group(0, 2 * t)
        pl.when(t < NGROUP // 2 - 1)(lambda: group(1, 2 * t + 1))

    start_up()
    _loop(NGROUP // 2, two_groups)
    _wait(wo_copies(NGROUP - 1) + a_inputs)
    _loop(GROUP, last_head_step)

    la, qa = lx, qs0

    def w_a(t, p, ct, r0, rows):
        if t == 0:
            return (rq0, rq1)[ct], (p, _ds(r0, rows))
        if t == 1:
            return lc, (p, 0, _ds(ct * (KQ // 2) + r0, rows))
        if t == 2:
            buf, tile = divmod(TPB * p + ct, 25)
            assert rows <= 64 or rows == 128
            if rows == 128:
                return (rk0, rk1, rv0, rv1)[buf], (pl.ds(2 * tile, 2),)
            return (rk0, rk1, rv0, rv1)[buf], (2 * tile + r0 // 64, _ds(r0 % 64, rows))
        buf, tile = divmod(TPB * p, 50)
        return (vs0, vs1)[buf], (_ds((tile + ct) * (KQ // 2) + r0, rows),)

    def load_w(t, p):
        tiles = []
        for ct in range(TPB):
            buf, idx = w_a(t, p, ct, 0, KQ // 2)
            tiles.append(_matrix(buf[idx].reshape(KQ // 2, LANES)))
        return _cat(tiles, 1)

    span_a = HALO + SEQ // 2
    group_rows = 16 * NS

    def build_w(blk, t, hold):
        for s in range(0, WROWS, 16):
            for ct in range(TPB):
                def load(i, j, hold):
                    return _split(hold(wp[wp_rows(t, i, s, j * TPB + ct), :]))

                def store(p, words):
                    buf, idx = w_a(t, p, ct, (blk * WROWS + s) // 2, 8)
                    buf[idx] = words

                yield from _build_operands(RHS_TERMS, load, store, hold, True)

    n_w = (WROWS // 16) * TPB * 7

    def build_x(blk, hold):
        for c in range(ROWS // group_rows):
            for t in range(TPB):
                def load(i, j, hold):
                    words = ax_raw.at[j * TPB + t, _ds(blk * (ROWS // 2), ROWS // 2)]
                    w0 = (c * group_rows + 32 * (i // 2)) // 2
                    return [(_low, _high)[i % 2](hold(words[pl.ds(w0 + e, 8, stride=2), :])) for e in range(2)]

                def store(p, words):
                    la[p, t, _ds((blk * (ROWS // NS) + 16 * c) // 2, 8), :] = words

                yield from _build_operands(LHS_TERMS, load, store, hold, True)

    n_x = (ROWS // group_rows) * TPB * 7

    def build_awo(blk, hold):
        ct, odd, h0 = blk // 4, (blk // 2) % 2, 16 * (blk % 2)
        pairs = DHA // 2 // NS
        for dp in range(0, pairs, 2):
            src = {}
            for i in range(NS):
                for j in range(NS):
                    words = awo_raw.at[j * TPB + ct, pl.ds(pl.multiple_of(h0 * 16, 256), 256)]
                    for e in range(2):
                        w0 = 8 * e * 16 + i * pairs + dp
                        src[i, j, e] = hold(jnp.where(odd == 1, words[pl.ds(w0 + 1, 8, stride=16), :],
                                                      words[pl.ds(w0, 8, stride=16), :]))
                yield
            for half in range(2):
                def load(i, j, hold):
                    return [(_low, _high)[half](hold(src[i, j, e])) for e in range(2)]

                def store(p, words):
                    buf, idx = w_a(3, p, ct, ((2 * (dp + odd) + half) * HA + h0) // 2, 8)
                    buf[idx] = words

                yield from _build_operands(RHS_TERMS, load, store, hold, True)

    n_awo = (DHA // 2 // NS // 2) * (NS + 2 * 7)

    def output_b(blk):
        slot = blk % 2
        rows = ROWS // NS
        heads = HB // NS
        pl.when(blk >= 2)(lambda: out_copy(blk - 2).wait())
        pacer = _Pacer(ro[0:8, :])
        src = _shifted(ctx, blk, NBLK, ROWS // 2)
        lhs = {}

        def build_lhs(top, hold):
            half = NS // 2
            for h in range(heads):
                for r in range(0, rows, 16):
                    def quadrant(i, j):
                        return [[_split_shuffled(hold(src[pl.ds(
                            (((j * half + b) * heads + h) * SEQ + (i * half + a) * rows + r) // 2, 8), :]))
                            for b in range(half)] for a in range(half)]

                    for p, v in enumerate(_operands(LHS_TERMS, _operand(LHS_TERMS[top], quadrant))):
                        lhs.setdefault((top * (NP // 7) + p, h), []).append(v)
                    yield

        def product(p):
            x = _cat([_cat(lhs[p, h], 0) for h in range(heads)], 1).astype(BF16)
            w = _cat([_matrix(ro[pl.ds((p * TPB + ct) * KO // 2, KO // 2), :]) for ct in range(TPB)], 1)
            return pacer.mark(jnp.dot(x, w, preferred_element_type=F32))

        def emit(i, j, v):
            stage[slot, i * rows:(i + 1) * rows, j * KQ:(j + 1) * KQ] = v.astype(BF16)

        _run(build_lhs(TOP_ORDER[0], _same))
        hold = pacer.after(1)
        _interleave(
            (_multiply(product, emit), NP),
            (_chain(*[build_lhs(t, hold) for t in TOP_ORDER[1:]]), 6 * heads * (rows // 16), 0., .84),
            *[(_chain(build_w(blk, t, hold), shuffle_columns(blk + 1, t, hold)), n_w + n_shuffle, .02, .95)
              for t in range(3)],
            (build_x(blk, hold), n_x, .02, .95),
            (build_awo(blk, hold), n_awo, .02, .95))
        out_copy(blk).start()

    _loop(NBLK, output_b)

    def project_a(t, blk, mark):
        rows = ROWS // NS
        dst = _shifted(ro if t == 1 else ctx, blk, NBLK, ROWS // 2)
        source, slot = _ds(blk * (rows // 2), rows // 2), blk % 2

        def product(p):
            x = _cat([_matrix(la[p, k, source, :]) for k in range(TPB)], 1)
            return mark(jnp.dot(x, load_w(t, p), preferred_element_type=F32))

        def emit(i, j, v):
            for ct in range(TPB):
                for c in range(rows // 16):
                    piece = v[16 * c:16 * (c + 1), ct * LANES:(ct + 1) * LANES]
                    tile = 2 * (j * TPB + ct) + i % 2
                    r = c * (group_rows // 2) + 16 * (i // 2)
                    if t == 0:
                        qa[_ds(slot * (ROWS // 2) + (tile * ROWS + r), 16), :] = pltpu.bitcast(piece, U32)
                    else:
                        dst[pl.ds(tile * span_a + HALO + r, 16), :] = pltpu.bitcast(piece, U32)

        return _multiply(product, emit)

    def attend_a(blk, hold, softmax_weight, operand_weight, hold_q, hold_v, **_):
        row0, slot, first = blk * (ROWS // 2), blk % 2, blk % SLOTS * NP
        keys, values = (_shifted(buf, blk, NBLK, ROWS // 2) for buf in (ro, ctx))
        logits, o = {}, {}

        def window(buf, j, r, par, w):
            return pltpu.bitcast(buf[pl.ds((2 * j + par) * span_a + HALO + r - w, 8), :], F32)

        def scores(r, par):
            pos = row0 + r + lax.broadcasted_iota(I32, (8, LANES), 0)
            q = [pltpu.bitcast(qa[_ds(slot * (ROWS // 2) + ((2 * j + par) * ROWS + r), 8), :], F32) for j in range(8)]
            q = [hold(x) if j % hold_q == 0 else x for j, x in enumerate(q)]
            logits[r, par] = []
            for w in range(WIN):
                acc = lax.mul(q[0], hold(window(keys, 0, r, par, w)))
                for j in range(1, 8):
                    acc = lax.add(acc, lax.mul(q[j], window(keys, j, r, par, w)))
                acc = acc + pltpu.roll(acc, 64, 1)
                acc = acc + pltpu.roll(acc, 32, 1)
                acc = acc * (DHA ** -0.5 * LOG2E)
                if r < w:
                    acc = jnp.where(pos >= w, acc, MASKED * LOG2E)
                logits[r, par].append(acc)
                yield

        def context(r, par):
            x = logits.pop((r, par))
            top = functools.reduce(jnp.maximum, x)
            e = [jnp.exp2(t - top) for t in x]
            scale = _reciprocal(functools.reduce(jnp.add, e))
            e = [t * scale for t in e]
            yield softmax_weight
            for j in range(8):
                acc = None
                for w in range(WIN):
                    v = window(values, j, r, par, w)
                    t = lax.mul(e[w], hold(v) if w % hold_v == 0 else v)
                    acc = t if acc is None else lax.add(acc, t)
                o[r, par, j] = acc
                yield

        def operands(c):
            for t in range(TPB):
                def load(i, j, hold):
                    return [hold(o[c * (group_rows // 2) + 8 * i, par, j * TPB + t]) for par in range(2)]

                def store(p, words):
                    lo[first + p, t, 8 * c:8 * (c + 1), :] = words

                yield from _weigh(_build_operands(LHS_TERMS, load, store, hold), operand_weight)

        for c in range(ROWS // group_rows):
            units = [(r, par) for r in range(c * group_rows // 2, (c + 1) * group_rows // 2, 8) for par in range(2)]
            yield from scores(*units[0])
            for now, after in zip(units, units[1:]):
                yield from _merge((scores(*after), WIN), (context(*now), 8 + softmax_weight))
            yield from context(*units[-1])
            yield from operands(c)

    def output_a(blk, mark):
        slot, first = blk % 2, blk % SLOTS * NP

        def product(p):
            x = _cat([_matrix(lo[first + p, k]) for k in range(TPB)], 1)
            return mark(jnp.dot(x, load_w(3, p), preferred_element_type=F32))

        def emit(i, j, v):
            for c in range(ROWS // group_rows):
                r = c * group_rows + 16 * i
                stage[slot, r:r + 16, j * KQ:(j + 1) * KQ] = v[16 * c:16 * (c + 1)].astype(BF16)

        return _multiply(product, emit)

    def outputs_a(blocks, mark):
        for n, blk in enumerate(blocks):
            if n > 0:
                out_copy(NBLK + blk - 1).start()
                out_copy(NBLK + blk - 2).wait()
            yield from output_a(blk, mark)

    def step_a(project, attend, outputs, pace=None):
        pacer = _Pacer(lc[0, 0, 0:8, :])
        matmuls = [] if project is None else [project_a(t, project, pacer.mark) for t in (1, 2, 0)]
        streams = [(_chain(outputs_a(outputs, pacer.mark), *matmuls), (len(outputs) + len(matmuls)) * NP)]
        if pace:
            total = ((WIN + 8 + pace["softmax_weight"]) * (ROWS // 8)
                     + TPB * (ROWS // group_rows) * 7 * pace["operand_weight"])
            streams.append((attend_a(attend, pacer.after(pace["lag"]), **pace), total, *pace["span"]))
        if outputs:
            out_copy(NBLK + outputs[0] - 2).wait()
        _interleave(*streams)
        if outputs:
            out_copy(NBLK + outputs[-1]).start()

    for tile in range(16):
        for buf in (ro, ctx):
            buf[tile * span_a:tile * span_a + HALO, :] = jnp.zeros((HALO, LANES), U32)
    step_a(0, None, [])
    _loop(DELAY, lambda i: step_a(i + 1, i, [], A_FIRST))
    _loop(NBLK - 1 - DELAY, lambda i: step_a(i + DELAY + 1, i + DELAY, [i], A_MAIN))
    step_a(None, NBLK - 1, range(NBLK - 1 - DELAY, NBLK - 1), A_LAST)

    halves = [pltpu.make_async_copy(stage.at[1, :, pl.ds(c, DA // 2)],
                                    out_hbm.at[pl.ds(SEQ - ROWS, ROWS), pl.ds(c, DA // 2)], sem_out.at[1])
              for c in (0, DA // 2)]
    out_copy(2 * NBLK - 3).wait()
    for n, _ in enumerate(output_a(NBLK - 1, _same)):
        if n == 5 * NP // 7:
            halves[0].start()
    halves[1].start()
    _wait([out_copy(2 * NBLK - 2)] + halves)


def _words(*shape):
    return pltpu.VMEM(shape + (LANES,), U32)


SCRATCH = [
    _words(DA // LANES, SEQ // 2),
    pltpu.VMEM((DA // 2, 3 * DA), U32),
    _words(DA // LANES, DA // 2),
    pltpu.VMEM((NS, MQ // 2, DC), U32),
    pltpu.VMEM((NS, KO, MB), BF16),
    _words(NP, MB // NS // LANES, MQ // 2),
    _words(NP, DC // NS // LANES, MQ // 2),
    *[_words(NP, MB // NS // 2)] * 2,
    *[_words(NP + 1, DC // NS // 2)] * 4,
    *[_words(GROUP * SEQ // 2)] * 4,
    *[_words(GROUP * NPAIR * 7 * DB // 4)] * 2,
    *[_words(GROUP * MB // 2)] * 2,
    *[_words(GROUP * DC // 2)] * 4,
    _words(HB * SEQ // 2),
    _words(NP * TPB * KO // 2),
    _words(SLOTS * NP, TPB, ROWS // NS // 2),
    pltpu.VMEM((2, ROWS, DA), BF16),
    pltpu.SemaphoreType.DMA((GROUP,)),
    pltpu.SemaphoreType.DMA((GROUP,)),
    pltpu.SemaphoreType.DMA(()),
    pltpu.SemaphoreType.DMA((6,)),
    pltpu.SemaphoreType.DMA(()),
    pltpu.SemaphoreType.DMA((2,)),
]


@jax.jit
def pallas_concat_heads__sliding_local_dilated__compressed_kv_cla__prompt_kernel(A_x, A_wqkv, A_wo, B_x, B_c_kv, B_w_q, B_w_uk, B_w_uv, B_w_o):
    hbm = pl.BlockSpec(memory_space=pl.ANY)
    out = pl.pallas_call(
        _kernel,
        in_specs=[hbm] * 9,
        out_specs=hbm,
        out_shape=jax.ShapeDtypeStruct((SEQ, DA + MB), BF16),
        scratch_shapes=SCRATCH,
        compiler_params=pltpu.CompilerParams(vmem_limit_bytes=127 * 2 ** 20),
        name="fused_attention",
    )(A_x.reshape(SEQ, DA), A_wqkv, A_wo, B_x.reshape(GROUP, NS, PART, MB), B_c_kv.reshape(GROUP, NS, PART, DC),
      B_w_q.reshape(MB // 2, 2 * HB, DB), B_w_uk.reshape(DC // 2, 2 * HB, DB),
      B_w_uv.reshape(DC // 2, 2 * HB, DB), B_w_o.reshape(NS, KO, MB))
    return out.reshape(1, SEQ, DA + MB)
```

```python
import functools
import math

import jax
import jax.numpy as jnp
import numpy as np
from jax import lax
import jax.experimental.pallas as pl
import jax.experimental.pallas.tpu as pltpu

F32 = jnp.float32
BF16 = jnp.bfloat16
U32 = jnp.uint32
I32 = jnp.int32
LANES = 128
NT_DIMS = (((1,), (1,)), ((), ()))
LOG2E = math.log2(math.e)
MASKED = -1e9

SEQ = 2048
DA = 1024
HA, DHA = 32, 32
WIN = 8
HALO = 32
MB = 1024
HB, DB = 32, 128
DC = 512

LEVELS = 2
NS = 2 ** LEVELS
NP = 7 ** LEVELS
GROUP = NS
NGROUP = HB // GROUP
MQ = SEQ // NS
PART = MQ // GROUP
ROWS = 256
NBLK = SEQ // ROWS
KQ = DA // NS
TPB = KQ // LANES
KO = HB * DB // NS
WROWS = KQ // NBLK
TILE = LANES
NPAIR = SEQ // TILE // 2
DELAY = 2
SLOTS = 4

START_UP = (
    ("c0 k", "c2 c3", "k0", "c0 k", "", 1, (0., 1.)),
    ("v c1", "q x0", "v0", "v", "c1", 20, (.02, .98)),
    ("c2 c3", "x1 x2 x3", "k1 v1 k2 v2 k3", "", "c2 c3 !q +g1 q !x0 x0", 12, (.01, .96)),
    ("x1 x2", "", "q0 q1", "", "x1 x2", 1, (.01, .93)),
    ("x3 g1", "g2 o", "q2 v3 q3", "", "x3 g", 2, (0., 1.01)),
)
PAIR_ORDER = (1, 3, 5, 7, 6, 4, 2, 0)
HEAD = dict(lag=9, bursts=((1,), (4,), (0,), (2,), (5,), (3,), (6,)), fast=NPAIR,
            score_weight=1, score_span=(0, .7), context_span=(.15, 1))
LAST_HEAD = dict(lag=11, bursts=((1, 4), (0, 2), (5, 3), (6,)), fast=5,
                 score_weight=1.1, score_span=(0, .6), context_span=(.25, 1))
A_FIRST = dict(lag=3, span=(.02, .98), softmax_weight=1, operand_weight=7, hold_q=8, hold_v=4)
A_MAIN = dict(lag=6, span=(.08, .99), softmax_weight=3, operand_weight=4, hold_q=8, hold_v=8)
A_LAST = dict(lag=2, span=(.02, 1.), softmax_weight=6, operand_weight=12, hold_q=1, hold_v=8)


LHS_TERMS = (((1, 0, 0), (1, 1, 1)), ((1, 1, 0), (1, 1, 1)), ((1, 0, 0),), ((1, 1, 1),),
             ((1, 0, 0), (1, 0, 1)), ((1, 1, 0), (-1, 0, 0)), ((1, 0, 1), (-1, 1, 1)))
RHS_TERMS = (((1, 0, 0), (1, 1, 1)), ((1, 0, 0),), ((1, 0, 1), (-1, 1, 1)), ((1, 1, 0), (-1, 0, 0)),
             ((1, 1, 1),), ((1, 0, 0), (1, 0, 1)), ((1, 1, 0), (1, 1, 1)))
TOP_ORDER = (1, 3, 0, 6, 4, 2, 5)


def _add(x, y):
    return [[lax.add(a, b) for a, b in zip(rx, ry)] for rx, ry in zip(x, y)]


def _sub(x, y):
    return [[lax.sub(a, b) for a, b in zip(rx, ry)] for rx, ry in zip(x, y)]


def _operand(terms, quadrant):
    total = None
    for sign, i, j in terms:
        q = quadrant(i, j)
        total = q if total is None else (_add if sign > 0 else _sub)(total, q)
    return total


def _operands(side, blocks):
    half = len(blocks) // 2
    if half == 0:
        return [blocks[0][0]]

    def quadrant(i, j):
        return [row[j * half:(j + 1) * half] for row in blocks[i * half:(i + 1) * half]]

    return [x for terms in side for x in _operands(side, _operand(terms, quadrant))]


def _multiply(product, emit, level=LEVELS, base=0):
    if level == 0:
        emit(0, 0, product(base))
        yield
        return
    n = 2 ** (level - 1)

    def m(i):
        out = [[None] * n for _ in range(n)]

        def keep(a, b, v):
            out[a][b] = v

        yield from _multiply(product, keep, level - 1, base + (i - 1) * 7 ** (level - 1))
        return out

    def put(x, oi, oj):
        for a in range(n):
            for b in range(n):
                emit(oi * n + a, oj * n + b, x[a][b])

    m2 = yield from m(2)
    m4 = yield from m(4)
    put(_add(m2, m4), 1, 0)
    m1 = yield from m(1)
    c11 = _add(m1, m4)
    c22 = _sub(m1, m2)
    m7 = yield from m(7)
    c11 = _add(c11, m7)
    m5 = yield from m(5)
    put(_sub(c11, m5), 0, 0)
    m3 = yield from m(3)
    put(_add(m3, m5), 0, 1)
    c22 = _add(c22, m3)
    m6 = yield from m(6)
    put(_add(c22, m6), 1, 1)


def _build_operands(side, load, store, hold, held=lambda n, a, b: (n, a, b) == (0, 1, 1), tops=range(7)):
    half = NS // 2
    for top in tops:
        terms = side[top]
        loaded = {(i, j): [[load(i * half + a, j * half + b, hold if held(n, a, b) else _same)
                            for b in range(half)] for a in range(half)]
                  for n, (_, i, j) in enumerate(terms)}
        lo, hi = (_operands(side, _operand(terms, lambda i, j: [[x[e] for x in row] for row in loaded[i, j]]))
                  for e in range(2))
        for p in range(NP // 7):
            store(top * (NP // 7) + p, _join(lo[p], hi[p]))
        yield


def _low(words):
    return pltpu.bitcast(lax.shift_left(words, np.uint32(16)), F32)


def _high(words):
    return pltpu.bitcast(lax.bitwise_and(words, np.uint32(0xFFFF0000)), F32)


def _split(words):
    return _low(words), _high(words)


def _join(lo, hi):
    return pltpu.bitcast(pltpu.pack_elementwise([lo, hi], packed_dtype=BF16), U32)


def _join_shuffled(v):
    r, c = v.shape
    v = v.reshape(r // 16, 2, 8, c)
    return _join(v[:, 0].reshape(r // 2, c), v[:, 1].reshape(r // 2, c))


def _split_shuffled(words):
    lo, hi = _split(words)
    r, c = words.shape
    return jnp.stack([lo.reshape(r // 8, 8, c), hi.reshape(r // 8, 8, c)], axis=1).reshape(2 * r, c)


def _unshuffle(pos):
    return (pos & ~15) + ((pos & 15) >> 1) + 8 * (pos & 1)


def _matrix(words):
    return pltpu.bitcast(words, BF16)


def _cat(xs, axis):
    return xs[0] if len(xs) == 1 else jnp.concatenate(xs, axis=axis)


def _ds(start, size):
    if isinstance(start, int):
        return pl.ds(start, size)
    return pl.ds(pl.multiple_of(start, min(size, 16)), size)


def _shifted(ref, step, steps, n):
    return ref.at[_ds(step * n, ref.shape[0] - (steps - 1) * n)]


def _loop(n, body):
    lax.fori_loop(0, n, lambda i, carry: body(i), None)


def _start(copies):
    for c in copies:
        c.start()


def _wait(copies):
    for c in copies:
        c.wait()


def _run(steps):
    for _ in steps:
        pass


def _chain(*streams):
    for steps in streams:
        yield from steps


def _weigh(steps, weight):
    for _ in steps:
        yield weight


def _merge(*streams):
    spans = [s[2:] if len(s) > 2 else (0.0, 1.0) for s in streams]
    done = [0.0] * len(streams)
    live = list(range(len(streams)))
    while live:
        i = min(live, key=lambda k: spans[k][0] + (spans[k][1] - spans[k][0]) * done[k] / streams[k][1])
        try:
            weight = next(streams[i][0])
        except StopIteration:
            live.remove(i)
            continue
        weight = 1 if weight is None else weight
        done[i] += weight
        yield weight


def _interleave(*streams):
    _run(_merge(*streams))


class _Pacer:
    def __init__(self, words):
        self.never = (words | 1) == 0
        self.marks = []

    def mark(self, v):
        self.marks.append({None: v})
        return v

    def after(self, lag):
        def hold(x):
            if len(self.marks) < lag:
                return x
            mark = self.marks[-lag]
            if x.dtype not in mark:
                mark[x.dtype] = pltpu.bitcast(mark[None][0:8, 0:LANES], x.dtype)
            return lax.select(self.never, mark[x.dtype], x)

        return hold


def _same(x):
    return x


def _reciprocal(x):
    r = pltpu.reciprocal(x, approx=True)
    return r * (2.0 - x * r)


def _kernel(ax_hbm, wqkv_hbm, awo_hbm, bx_hbm, c_hbm, wq_hbm, wuk_hbm, wuv_hbm, bwo_hbm, out_hbm,
            ax_raw, wqkv_raw, awo_raw, c_raw, bwo_raw,
            lx, lc, rq0, rq1, rk0, rk1, rv0, rv1, qs0, qs1, ks0, ks1, vs0, vs1,
            sq0, sq1, sk0, sk1, sv0, sv1, ctx, ro, lo, stage,
            sem_c, sem_x, sem_wo, sem_w, sem_a, sem_out):

    def out_copy(n):
        return pltpu.make_async_copy(
            stage.at[n % 2], out_hbm.at[_ds(n % NBLK * ROWS, ROWS), _ds((1 - n // NBLK) * DA, DA)], sem_out.at[n % 2])

    a_inputs = ([pltpu.make_async_copy(ax_hbm.bitcast(U32).at[:, pl.ds(j * LANES, LANES)], ax_raw.at[j], sem_a)
                 for j in range(DA // LANES)]
                + [pltpu.make_async_copy(awo_hbm.bitcast(U32).at[:, pl.ds(j * LANES, LANES)], awo_raw.at[j], sem_a)
                   for j in range(DA // LANES)]
                + [pltpu.make_async_copy(wqkv_hbm.bitcast(U32), wqkv_raw, sem_a)])

    wp = ks0

    def wp_rows(t, i, s, c):
        return _ds((((t * NS + i) * (WROWS // 16) + s // 16) * 8 + c) * 8, 8)

    def shuffle_columns(blk, t, hold, quarters=range(NS)):
        lane = lax.broadcasted_iota(I32, (8, LANES), 1)
        slot, chunk, low = lane >> 5, (lane & 31) >> 2, lane & 3
        head_of = _unshuffle(lane & 31)
        for s in range(0, WROWS, 16):
            for i in quarters:
                rows = _ds((i * KQ + (blk % NBLK) * WROWS + s) // 2, 8)
                moved = []
                for j in range(8):
                    c0 = t * DA + j * LANES
                    u = hold(pltpu.bitcast(wqkv_raw[rows, c0:c0 + LANES], I32))
                    moved.append(jnp.take_along_axis(u, low * 32 + 4 * ((chunk - j) & 7) + slot, axis=1))
                    if j % 4 == 3:
                        yield
                v = [moved[-c % 8] for c in range(8)]
                for bit in (1, 2, 4):
                    v = [jnp.where((chunk & bit) != 0, v[(c - bit) % 8], v[c]) for c in range(8)]
                for c in range(8):
                    source = slot * 32 + (((head_of >> 2) + c) & 7) * 4 + (head_of & 3)
                    wp[wp_rows(t, i, s, c), :] = pltpu.bitcast(jnp.take_along_axis(v[c], source, axis=1), U32)
                    if c % 4 == 3:
                        yield

    n_shuffle = (WROWS // 16) * NS * 4

    weights = ((rq0, rk0, rv0), (rq1, rk1, rv1))
    projected = ((qs0, ks0, vs0), (qs1, ks1, vs1))
    staged = ((sq0, sk0, sv0), (sq1, sk1, sv1))

    def weight_copies(par, grp, w):
        words = (wq_hbm, wuk_hbm, wuv_hbm)[w].bitcast(U32)
        n = words.shape[0]
        return [pltpu.make_async_copy(
            words.at[:, (HB // 2) * parity + grp * (GROUP // 2) + pair],
            staged[par][w].at[pl.ds((2 * pair + parity) * n, n)], sem_w.at[3 * par + w])
            for pair in range(GROUP // 2) for parity in range(2)]

    def group_copies(par, grp):
        return [c for w in range(3) for c in weight_copies(par, grp, w)]

    def c_copies(part):
        return [pltpu.make_async_copy(c_hbm.bitcast(U32).at[part], c_raw.at[:, pl.ds(part * PART // 2, PART // 2)],
                                      sem_c.at[part])]

    def x_copies(part):
        return [pltpu.make_async_copy(bx_hbm.at[part], bwo_raw.at[:, pl.ds(part * PART, PART)], sem_x.at[part])]

    def wo_copies(grp):
        rows = (slice(None), _ds(grp * (KO // NGROUP), KO // NGROUP))
        return [pltpu.make_async_copy(bwo_hbm.at[rows], bwo_raw.at[rows], sem_wo)]

    def build_weights(par, w, part, hold, tops=range(7)):
        n = (MB, DC, DC)[w] // 2
        rows = n // NS // GROUP
        src = _shifted(staged[par][w], part, GROUP, rows)
        for s in range(0, rows, 8):
            target = _ds(part * rows + s, 8)

            def load(i, j, hold):
                x, y = (src[pl.ds((2 * (j // 2) + e) * n + i * (n // NS) + s, 8), :] for e in range(2))
                return [(_low, _high)[j % 2](z) for z in (hold(x), y)]

            def store(p, words):
                weights[par][w][p, target, :] = words

            yield from _build_operands(RHS_TERMS, load, store, hold, tops=tops)

    def n_weights(w):
        return (MB, DC, DC)[w] // NS // GROUP // 16 * 7

    def build_group(par, part, hold):
        return _chain(*[build_weights(par, w, part, hold) for w in range(3)])

    n_group = sum(n_weights(w) for w in range(3))

    def build_activations(src, dst, part, hold, tops=range(7)):
        tiles = src.shape[2] // NS // LANES
        for t in range(tiles):
            for s in range(0, PART, 16):
                r = part * PART + s

                def load(i, j, hold):
                    c0 = (j * tiles + t) * LANES
                    if src.dtype == U32:
                        return _split(hold(src[i, pl.ds(r // 2, 8), c0:c0 + LANES]))
                    return _split(hold(pltpu.bitcast(src[i, pl.ds(r, 16), c0:c0 + LANES], U32)))

                def store(p, words):
                    dst[p, t, pl.ds(r // 2, 8), :] = words

                yield from _build_operands(LHS_TERMS, load, store, hold, tops=tops)

    def n_activations(width):
        return width // NS // LANES * (PART // 16) * 7

    def project(par, w, part, mark):
        lhs = lx if w == 0 else lc
        tiles = lhs.shape[1]
        dst = projected[par][w]
        dst = _shifted(dst, part, GROUP, dst.shape[0] // GROUP // GROUP)
        source = _ds(part * (PART // 2), PART // 2)
        pending = {}

        def product(p):
            x = _cat([_matrix(lhs[p, t, source, :]) for t in range(tiles)], 1)
            return mark(jnp.dot(x, _matrix(weights[par][w][p]), preferred_element_type=F32))

        def emit(i, j, v):
            if w < 2:
                dst[pl.ds((j * SEQ + i * PART) // 2, PART // 2), :] = (
                    pltpu.bitcast(v.astype(BF16), U32) if w else _join_shuffled(v * (DB ** -0.5 * LOG2E)))
            else:
                pending[i, j] = v.T
                if i % 2 == 1:
                    pair = [pending.pop((i - 1 + b, j)) for b in range(2)]
                    blocks = [[t[a * DB // 2:(a + 1) * DB // 2] for t in pair] for a in range(2)]
                    for p, x in enumerate(_operands(LHS_TERMS, blocks)):
                        dst[pl.ds(((j * NPAIR + i // 2) * 7 + p) * DB // 4, DB // 4), :] = _join_shuffled(x)

        return _weigh(_multiply(product, emit), tiles)

    n_project = NP * (MB + 2 * DC) // NS // LANES

    def attend(par, h, head_id, pacer, lag, bursts, fast, score_weight, score_span, context_span):
        hold = pacer.after(lag)
        causal = (lax.broadcasted_iota(I32, (TILE, TILE), 0)
                  <= _unshuffle(lax.broadcasted_iota(I32, (TILE, TILE), 1)))
        queries, keys, values = (r.at[_ds(h * (r.shape[0] // GROUP), r.shape[0] // GROUP)] for r in projected[par])
        result = ctx.at[_ds(head_id * (SEQ // 2), SEQ // 2)]
        pending = {}

        def fold(op, t):
            return functools.reduce(op, [lax.slice(t, (r, 0), (r + 8, TILE)) for r in range(0, TILE, 8)])

        def scores(i):
            q = _matrix(queries[i * TILE // 2:(i + 1) * TILE // 2, :])
            tiles, peaks = [], []
            for j in range(i + 1):
                k = _matrix(keys[j * TILE // 2:(j + 1) * TILE // 2, :])
                s = pacer.mark(lax.dot_general(k, q, NT_DIMS, preferred_element_type=F32))
                if j == i:
                    s = jnp.where(causal, s, MASKED * LOG2E)
                tiles.append(s)
                peaks.append(fold(lax.max, s))
                yield score_weight
            top = jnp.max(functools.reduce(jnp.maximum, peaks), axis=0, keepdims=True)
            if i // 2 >= max(1, NPAIR - fast):
                mass = functools.reduce(jnp.add, [jnp.exp2(x - top) for x in peaks])
                top = top + jnp.log2(jnp.sum(mass, axis=0, keepdims=True))
            pending[i] = tiles, jnp.broadcast_to(top, (8, TILE))

        def context(i):
            both = [pending.pop(2 * i + c) for c in range(2)]
            totals = [None, None]
            o = [[None, None], [None, None]]

            def weight(j, c):
                p = jnp.exp2(both[c][0][j] - _cat([hold(both[c][1])] * (TILE // 8), 0))
                t = fold(lax.add, p)
                totals[c] = t if totals[c] is None else totals[c] + t
                return p

            def product(j, p, x):
                v = _matrix(values[(j * 7 + p) * DB // 4:(j * 7 + p + 1) * DB // 4, :])
                return pacer.mark(jnp.dot(v, x.astype(BF16), preferred_element_type=F32))

            def emit(a, c, v):
                o[a][c] = v if o[a][c] is None else o[a][c] + v

            def plain(j, c, tiles):
                for b in range(tiles):
                    p = weight(2 * j + b, c)
                    shared = product(j, 2 + b, p)
                    emit(b, c, shared)
                    emit(1 - b, c, shared + product(j, 5 + b, p))
                    yield 1

            yield from plain(i, 0, 1)
            yield from plain(i, 1, 2)
            acc = [None] * 7
            for j in range(i):
                if i < NPAIR - fast:
                    yield from plain(j, 0, 2)
                    yield from plain(j, 1, 2)
                    continue
                tiles = {}
                for burst in bursts:
                    for p in burst:
                        for _, b, c in RHS_TERMS[p]:
                            if (b, c) not in tiles:
                                tiles[b, c] = weight(2 * j + b, c)
                        t = product(j, p, _operand(RHS_TERMS[p], lambda b, c: [[tiles[b, c]]])[0][0])
                        acc[p] = t if acc[p] is None else acc[p] + t
                    yield 4 / 7 * len(burst)
            if acc[0] is not None:
                _run(_multiply(lambda p: acc[p], emit, 1))
            for c in range(2):
                x = _cat([o[0][c], o[1][c]], 0) * _reciprocal(jnp.sum(totals[c], axis=0, keepdims=True))
                result[(2 * i + c) * TILE // 2:(2 * i + c + 1) * TILE // 2, :] = pltpu.bitcast(x.astype(BF16).T, U32)

        for n in range(NPAIR + 1):
            streams = []
            if n < NPAIR:
                i = PAIR_ORDER[n]
                streams.append((_chain(scores(2 * i), scores(2 * i + 1)), (4 * i + 3) * score_weight, *score_span))
            if n > 0:
                i = PAIR_ORDER[n - 1]
                streams.append((context(i), 4 * i + 3, *context_span))
            yield from _merge(*streams)

    def n_attend(pace):
        return NPAIR * (2 * NPAIR + 1) * (1 + pace["score_weight"])

    def build_wo(head_id, hold):
        n = KO // HB
        src, dst = bwo_raw.at[:, _ds(head_id * n, n)], _shifted(ro, head_id, HB, n // 2)
        for ct in range(TPB):
            for s in range(0, n, 16):
                def load(i, j, hold):
                    c0 = (j * TPB + ct) * LANES
                    v = src[i, pl.ds(s, 16), c0:c0 + LANES].astype(F32)
                    return [hold(v[0:8]), hold(v[8:16])]

                def store(p, words):
                    dst[pl.ds(((p * TPB + ct) * KO + s) // 2, 8), :] = words

                yield from _build_operands(RHS_TERMS, load, store, hold)

    n_wo = TPB * (KO // HB // 16) * 7

    def head_step(par, g, h):
        pacer = _Pacer(lc[0, 0, 0:8, :])
        head_id = g * GROUP + h
        _interleave((attend(par, h, head_id, pacer, **HEAD), n_attend(HEAD), 0., .86),
                    (_chain(*[project(1 - par, w, h, pacer.mark) for w in (1, 2, 0)]), n_project),
                    (build_wo(head_id, pacer.after(1)), n_wo, .02, .15),
                    (build_group(par, h, pacer.after(1)), n_group, .25, .98))

    def last_head_step(h):
        pacer = _Pacer(lc[0, 0, 0:8, :])
        hold = pacer.after(1)
        head_id = (NGROUP - 1) * GROUP + h
        _interleave((attend(1, h, head_id, pacer, **LAST_HEAD), n_attend(LAST_HEAD)),
                    (build_wo(head_id, hold), n_wo, .03, .3),
                    (_chain(*[shuffle_columns(0, t, hold, [h]) for t in range(3)]), 3 * n_shuffle / NS, .1, .8))

    def start_up():
        data = {"k": weight_copies(0, 0, 1), "v": weight_copies(0, 0, 2), "q": weight_copies(0, 0, 0),
                "g1": group_copies(1, 1), "g2": group_copies(0, 2), "o": wo_copies(0)}
        for part in range(GROUP):
            data["c%d" % part], data["x%d" % part] = c_copies(part), x_copies(part)
        built = set()

        def copies(names):
            return [c for name in names.split() for c in data[name]]

        def operands(job, hold, tops=range(7)):
            if job[0] in "!+":
                (_wait if job[0] == "!" else _start)(copies(job[1:]))
            elif job[0] in "cx":
                src, dst = (c_raw, lc) if job[0] == "c" else (bwo_raw, lx)
                yield from build_activations(src, dst, int(job[1]), hold, tops)
            else:
                for part in range(GROUP):
                    yield from (build_group(1, part, hold) if job == "g" else
                                build_weights(0, "qkv".index(job), part, hold, tops))
            built.add(job)

        size = dict(c=n_activations(DC), x=n_activations(MB), g=GROUP * n_group,
                    **{name: GROUP * n_weights(w) for w, name in enumerate("qkv")})

        def projection(name, mark):
            assert {name[0], "xcc"["qkv".index(name[0])] + name[1]} <= built
            yield from project(0, "qkv".index(name[0]), int(name[1]), mark)

        def step(waits, starts, products, ahead, jobs, lag, span):
            _wait(copies(waits))
            _start(copies(starts))
            pacer = _Pacer(c_raw[0, 0:8, 0:LANES])
            for top in TOP_ORDER:
                for job in ahead.split():
                    _run(operands(job, _same, [top]))
            _interleave((_chain(*[projection(name, pacer.mark) for name in products.split()]),
                         sum(n_project // (2 if name[0] == "q" else 4) for name in products.split())),
                        (_chain(*[operands(job, pacer.after(lag)) for job in jobs.split()]),
                         sum(size.get(job[0], 0) for job in jobs.split()) or 1, *span))

        def steps(i):
            for n, args in enumerate(START_UP):
                pl.when(i == n)(functools.partial(step, *args))

        _start(copies("c0 k v c1"))
        _loop(len(START_UP), steps)

    def group(par, g):
        _wait(wo_copies(g))
        _start(wo_copies(g + 1))
        pl.when(g + 2 < NGROUP)(lambda: _wait(group_copies(par, g + 2)))
        pl.when(g + 3 < NGROUP)(lambda: _start(group_copies(1 - par, g + 3)))
        if par == 0:
            pl.when(g == NGROUP - 2)(lambda: _start(a_inputs))
        _loop(GROUP, lambda h: head_step(par, g, h))

    def two_groups(t):
        group(0, 2 * t)
        pl.when(t < NGROUP // 2 - 1)(lambda: group(1, 2 * t + 1))

    start_up()
    _loop(NGROUP // 2, two_groups)
    _wait(wo_copies(NGROUP - 1) + a_inputs)
    _loop(GROUP, last_head_step)

    la, qa = lx, qs0

    def w_a(t, p, ct, r0, rows):
        if t == 0:
            return (rq0, rq1)[ct], (p, _ds(r0, rows))
        if t == 1:
            return lc, (p, 0, _ds(ct * (KQ // 2) + r0, rows))
        if t == 2:
            buf, tile = divmod(TPB * p + ct, 25)
            assert rows <= 64 or rows == 128
            if rows == 128:
                return (rk0, rk1, rv0, rv1)[buf], (pl.ds(2 * tile, 2),)
            return (rk0, rk1, rv0, rv1)[buf], (2 * tile + r0 // 64, _ds(r0 % 64, rows))
        buf, tile = divmod(TPB * p, 50)
        return (vs0, vs1)[buf], (_ds((tile + ct) * (KQ // 2) + r0, rows),)

    def load_w(t, p):
        tiles = []
        for ct in range(TPB):
            buf, idx = w_a(t, p, ct, 0, KQ // 2)
            tiles.append(_matrix(buf[idx].reshape(KQ // 2, LANES)))
        return _cat(tiles, 1)

    span_a = HALO + SEQ // 2
    group_rows = 16 * NS

    def build_w(blk, t, hold):
        for s in range(0, WROWS, 16):
            for ct in range(TPB):
                def load(i, j, hold):
                    return _split(hold(wp[wp_rows(t, i, s, j * TPB + ct), :]))

                def store(p, words):
                    buf, idx = w_a(t, p, ct, (blk * WROWS + s) // 2, 8)
                    buf[idx] = words

                yield from _build_operands(RHS_TERMS, load, store, hold, lambda *_: True)

    n_w = (WROWS // 16) * TPB * 7

    def build_x(blk, hold):
        for c in range(ROWS // group_rows):
            for t in range(TPB):
                def load(i, j, hold):
                    words = ax_raw.at[j * TPB + t, _ds(blk * (ROWS // 2), ROWS // 2)]
                    w0 = (c * group_rows + 32 * (i // 2)) // 2
                    return [(_low, _high)[i % 2](hold(words[pl.ds(w0 + e, 8, stride=2), :])) for e in range(2)]

                def store(p, words):
                    la[p, t, _ds((blk * (ROWS // NS) + 16 * c) // 2, 8), :] = words

                yield from _build_operands(LHS_TERMS, load, store, hold, lambda *_: True)

    n_x = (ROWS // group_rows) * TPB * 7

    def build_awo(blk, hold):
        ct, odd, h0 = blk // 4, (blk // 2) % 2, 16 * (blk % 2)
        pairs = DHA // 2 // NS
        for dp in range(0, pairs, 2):
            src = {}
            for i in range(NS):
                for j in range(NS):
                    words = awo_raw.at[j * TPB + ct, pl.ds(pl.multiple_of(h0 * 16, 256), 256)]
                    for e in range(2):
                        w0 = 8 * e * 16 + i * pairs + dp
                        src[i, j, e] = hold(jnp.where(odd == 1, words[pl.ds(w0 + 1, 8, stride=16), :],
                                                      words[pl.ds(w0, 8, stride=16), :]))
                yield
            for half in range(2):
                def load(i, j, hold):
                    return [(_low, _high)[half](hold(src[i, j, e])) for e in range(2)]

                def store(p, words):
                    buf, idx = w_a(3, p, ct, ((2 * (dp + odd) + half) * HA + h0) // 2, 8)
                    buf[idx] = words

                yield from _build_operands(RHS_TERMS, load, store, hold, lambda *_: True)

    n_awo = (DHA // 2 // NS // 2) * (NS + 2 * 7)

    def output_b(blk):
        slot = blk % 2
        rows = ROWS // NS
        heads = HB // NS
        pl.when(blk >= 2)(lambda: out_copy(blk - 2).wait())
        pacer = _Pacer(ro[0:8, :])
        src = _shifted(ctx, blk, NBLK, ROWS // 2)
        lhs = {}

        def build_lhs(top, hold):
            half = NS // 2
            for h in range(heads):
                for r in range(0, rows, 16):
                    def quadrant(i, j):
                        return [[_split_shuffled(hold(src[pl.ds(
                            (((j * half + b) * heads + h) * SEQ + (i * half + a) * rows + r) // 2, 8), :]))
                            for b in range(half)] for a in range(half)]

                    for p, v in enumerate(_operands(LHS_TERMS, _operand(LHS_TERMS[top], quadrant))):
                        lhs.setdefault((top * (NP // 7) + p, h), []).append(v)
                    yield

        def product(p):
            x = _cat([_cat(lhs[p, h], 0) for h in range(heads)], 1).astype(BF16)
            w = _cat([_matrix(ro[pl.ds((p * TPB + ct) * KO // 2, KO // 2), :]) for ct in range(TPB)], 1)
            return pacer.mark(jnp.dot(x, w, preferred_element_type=F32))

        def emit(i, j, v):
            stage[slot, i * rows:(i + 1) * rows, j * KQ:(j + 1) * KQ] = v.astype(BF16)

        _run(build_lhs(TOP_ORDER[0], _same))
        hold = pacer.after(1)
        _interleave(
            (_multiply(product, emit), NP),
            (_chain(*[build_lhs(t, hold) for t in TOP_ORDER[1:]]), 6 * heads * (rows // 16), 0., .84),
            *[(_chain(build_w(blk, t, hold), shuffle_columns(blk + 1, t, hold)), n_w + n_shuffle, .02, .95)
              for t in range(3)],
            (build_x(blk, hold), n_x, .02, .95),
            (build_awo(blk, hold), n_awo, .02, .95))
        out_copy(blk).start()

    _loop(NBLK, output_b)

    def project_a(t, blk, mark):
        rows = ROWS // NS
        dst = _shifted(ro if t == 1 else ctx, blk, NBLK, ROWS // 2)
        source, slot = _ds(blk * (rows // 2), rows // 2), blk % 2

        def product(p):
            x = _cat([_matrix(la[p, k, source, :]) for k in range(TPB)], 1)
            return mark(jnp.dot(x, load_w(t, p), preferred_element_type=F32))

        def emit(i, j, v):
            for ct in range(TPB):
                for c in range(rows // 16):
                    piece = v[16 * c:16 * (c + 1), ct * LANES:(ct + 1) * LANES]
                    tile = 2 * (j * TPB + ct) + i % 2
                    r = c * (group_rows // 2) + 16 * (i // 2)
                    if t == 0:
                        qa[_ds(slot * (ROWS // 2) + (tile * ROWS + r), 16), :] = pltpu.bitcast(piece, U32)
                    else:
                        dst[pl.ds(tile * span_a + HALO + r, 16), :] = pltpu.bitcast(piece, U32)

        return _multiply(product, emit)

    def attend_a(blk, hold, softmax_weight, operand_weight, hold_q, hold_v, **_):
        row0, slot, first = blk * (ROWS // 2), blk % 2, blk % SLOTS * NP
        keys, values = (_shifted(buf, blk, NBLK, ROWS // 2) for buf in (ro, ctx))
        logits, o = {}, {}

        def window(buf, j, r, par, w):
            return pltpu.bitcast(buf[pl.ds((2 * j + par) * span_a + HALO + r - w, 8), :], F32)

        def scores(r, par):
            pos = row0 + r + lax.broadcasted_iota(I32, (8, LANES), 0)
            q = [pltpu.bitcast(qa[_ds(slot * (ROWS // 2) + ((2 * j + par) * ROWS + r), 8), :], F32) for j in range(8)]
            q = [hold(x) if j % hold_q == 0 else x for j, x in enumerate(q)]
            logits[r, par] = []
            for w in range(WIN):
                acc = lax.mul(q[0], hold(window(keys, 0, r, par, w)))
                for j in range(1, 8):
                    acc = lax.add(acc, lax.mul(q[j], window(keys, j, r, par, w)))
                acc = acc + pltpu.roll(acc, 64, 1)
                acc = acc + pltpu.roll(acc, 32, 1)
                acc = acc * (DHA ** -0.5 * LOG2E)
                if r < w:
                    acc = jnp.where(pos >= w, acc, MASKED * LOG2E)
                logits[r, par].append(acc)
                yield

        def context(r, par):
            x = logits.pop((r, par))
            top = functools.reduce(jnp.maximum, x)
            e = [jnp.exp2(t - top) for t in x]
            scale = _reciprocal(functools.reduce(jnp.add, e))
            e = [t * scale for t in e]
            yield softmax_weight
            for j in range(8):
                acc = None
                for w in range(WIN):
                    v = window(values, j, r, par, w)
                    t = lax.mul(e[w], hold(v) if w % hold_v == 0 else v)
                    acc = t if acc is None else lax.add(acc, t)
                o[r, par, j] = acc
                yield

        def operands(c):
            for t in range(TPB):
                def load(i, j, hold):
                    return [hold(o[c * (group_rows // 2) + 8 * i, par, j * TPB + t]) for par in range(2)]

                def store(p, words):
                    lo[first + p, t, 8 * c:8 * (c + 1), :] = words

                yield from _weigh(_build_operands(LHS_TERMS, load, store, hold, lambda n, a, b: n == 0 and a == b),
                                  operand_weight)

        for c in range(ROWS // group_rows):
            units = [(r, par) for r in range(c * group_rows // 2, (c + 1) * group_rows // 2, 8) for par in range(2)]
            yield from scores(*units[0])
            for now, after in zip(units, units[1:]):
                yield from _merge((scores(*after), WIN), (context(*now), 8 + softmax_weight))
            yield from context(*units[-1])
            yield from operands(c)

    def output_a(blk, mark):
        slot, first = blk % 2, blk % SLOTS * NP

        def product(p):
            x = _cat([_matrix(lo[first + p, k]) for k in range(TPB)], 1)
            return mark(jnp.dot(x, load_w(3, p), preferred_element_type=F32))

        def emit(i, j, v):
            for c in range(ROWS // group_rows):
                r = c * group_rows + 16 * i
                stage[slot, r:r + 16, j * KQ:(j + 1) * KQ] = v[16 * c:16 * (c + 1)].astype(BF16)

        return _multiply(product, emit)

    def outputs_a(blocks, mark):
        for n, blk in enumerate(blocks):
            if n > 0:
                out_copy(NBLK + blk - 1).start()
                out_copy(NBLK + blk - 2).wait()
            yield from output_a(blk, mark)

    def step_a(project, attend, outputs, pace=None):
        pacer = _Pacer(lc[0, 0, 0:8, :])
        matmuls = [] if project is None else [project_a(t, project, pacer.mark) for t in (1, 2, 0)]
        streams = [(_chain(outputs_a(outputs, pacer.mark), *matmuls), (len(outputs) + len(matmuls)) * NP)]
        if pace:
            total = ((WIN + 8 + pace["softmax_weight"]) * (ROWS // 8)
                     + TPB * (ROWS // group_rows) * 7 * pace["operand_weight"])
            streams.append((attend_a(attend, pacer.after(pace["lag"]), **pace), total, *pace["span"]))
        if outputs:
            out_copy(NBLK + outputs[0] - 2).wait()
        _interleave(*streams)
        if outputs:
            out_copy(NBLK + outputs[-1]).start()

    for tile in range(16):
        for buf in (ro, ctx):
            buf[tile * span_a:tile * span_a + HALO, :] = jnp.zeros((HALO, LANES), U32)
    step_a(0, None, [])
    _loop(DELAY, lambda i: step_a(i + 1, i, [], A_FIRST))
    _loop(NBLK - 1 - DELAY, lambda i: step_a(i + DELAY + 1, i + DELAY, [i], A_MAIN))
    step_a(None, NBLK - 1, range(NBLK - 1 - DELAY, NBLK - 1), A_LAST)

    halves = [pltpu.make_async_copy(stage.at[1, :, pl.ds(c, DA // 2)],
                                    out_hbm.at[pl.ds(SEQ - ROWS, ROWS), pl.ds(c, DA // 2)], sem_out.at[1])
              for c in (0, DA // 2)]
    out_copy(2 * NBLK - 3).wait()
    for n, _ in enumerate(output_a(NBLK - 1, _same)):
        if n == 5 * NP // 7:
            halves[0].start()
    halves[1].start()
    _wait([out_copy(2 * NBLK - 2)] + halves)


def _words(*shape):
    return pltpu.VMEM(shape + (LANES,), U32)


SCRATCH = [
    _words(DA // LANES, SEQ // 2),
    pltpu.VMEM((DA // 2, 3 * DA), U32),
    _words(DA // LANES, DA // 2),
    pltpu.VMEM((NS, MQ // 2, DC), U32),
    pltpu.VMEM((NS, KO, MB), BF16),
    _words(NP, MB // NS // LANES, MQ // 2),
    _words(NP, DC // NS // LANES, MQ // 2),
    *[_words(NP, MB // NS // 2)] * 2,
    *[_words(NP + 1, DC // NS // 2)] * 4,
    *[_words(GROUP * SEQ // 2)] * 4,
    *[_words(GROUP * NPAIR * 7 * DB // 4)] * 2,
    *[_words(GROUP * MB // 2)] * 2,
    *[_words(GROUP * DC // 2)] * 4,
    _words(HB * SEQ // 2),
    _words(NP * TPB * KO // 2),
    _words(SLOTS * NP, TPB, ROWS // NS // 2),
    pltpu.VMEM((2, ROWS, DA), BF16),
    pltpu.SemaphoreType.DMA((GROUP,)),
    pltpu.SemaphoreType.DMA((GROUP,)),
    pltpu.SemaphoreType.DMA(()),
    pltpu.SemaphoreType.DMA((6,)),
    pltpu.SemaphoreType.DMA(()),
    pltpu.SemaphoreType.DMA((2,)),
]


@jax.jit
def pallas_concat_heads__sliding_local_dilated__compressed_kv_cla__prompt_kernel(A_x, A_wqkv, A_wo, B_x, B_c_kv, B_w_q, B_w_uk, B_w_uv, B_w_o):
    hbm = pl.BlockSpec(memory_space=pl.ANY)
    out = pl.pallas_call(
        _kernel,
        in_specs=[hbm] * 9,
        out_specs=hbm,
        out_shape=jax.ShapeDtypeStruct((SEQ, DA + MB), BF16),
        scratch_shapes=SCRATCH,
        compiler_params=pltpu.CompilerParams(vmem_limit_bytes=127 * 2 ** 20),
        name="fused_attention",
    )(A_x.reshape(SEQ, DA), A_wqkv, A_wo, B_x.reshape(GROUP, NS, PART, MB), B_c_kv.reshape(GROUP, NS, PART, DC),
      B_w_q.reshape(MB // 2, 2 * HB, DB), B_w_uk.reshape(DC // 2, 2 * HB, DB),
      B_w_uv.reshape(DC // 2, 2 * HB, DB), B_w_o.reshape(NS, KO, MB))
    return out.reshape(1, SEQ, DA + MB)
```

```python
import functools
import math

import jax
import jax.numpy as jnp
import numpy as np
from jax import lax
import jax.experimental.pallas as pl
import jax.experimental.pallas.tpu as pltpu

F32 = jnp.float32
BF16 = jnp.bfloat16
U32 = jnp.uint32
I32 = jnp.int32
LANES = 128
NT_DIMS = (((1,), (1,)), ((), ()))
LOG2E = math.log2(math.e)
MASKED = -1e9

SEQ = 2048
DA = 1024
HA, DHA = 32, 32
WIN = 8
HALO = 32
MB = 1024
HB, DB = 32, 128
DC = 512

LEVELS = 2
NS = 2 ** LEVELS
NP = 7 ** LEVELS
GROUP = NS
NGROUP = HB // GROUP
MQ = SEQ // NS
PART = MQ // GROUP
ROWS = 256
NBLK = SEQ // ROWS
KQ = DA // NS
TPB = KQ // LANES
KO = HB * DB // NS
WROWS = KQ // NBLK
TILE = LANES
NPAIR = SEQ // TILE // 2
DELAY = 2
SLOTS = 4

START_UP = (
    ("c0 k", "c2 c3", "k0", "c0 k", "", 1, (0., 1.)),
    ("v c1", "q x0", "v0", "v", "c1", 20, (.02, .98)),
    ("c2 c3", "x1 x2 x3", "k1 v1 k2 v2 k3", "", "c2 c3 !q +g1 q !x0 x0", 12, (.01, .96)),
    ("x1 x2", "", "q0 q1", "", "x1 x2", 1, (.01, .93)),
    ("x3 g1", "g2 o", "q2 v3 q3", "", "x3 g", 2, (0., 1.01)),
)
HEAD = dict(order=(7, 6, 4, 3, 5, 2, 1, 0), reach=2, fast=NPAIR, lag=10,
            bursts=((1,), (4,), (0,), (2,), (5,), (3,), (6,)),
            score_weight=.9, score_span=(0, .68), context_span=(.15, 1))
LAST_HEAD = dict(order=(1, 3, 5, 7, 6, 4, 2, 0), reach=1, fast=5, lag=11,
                 bursts=((1, 4), (0, 2), (5, 3), (6,)),
                 score_weight=1.1, score_span=(0, .6), context_span=(.25, 1))
A_FIRST = dict(lag=3, span=(.02, .98), softmax_weight=1, operand_weight=7, hold_q=8, hold_v=4)
A_MAIN = dict(lag=6, span=(.08, .985), softmax_weight=3, operand_weight=4, hold_q=2, hold_v=4)
A_LAST = dict(lag=2, span=(.02, 1.), softmax_weight=6, operand_weight=12, hold_q=1, hold_v=8)


LHS_TERMS = (((1, 0, 0), (1, 1, 1)), ((1, 1, 0), (1, 1, 1)), ((1, 0, 0),), ((1, 1, 1),),
             ((1, 0, 0), (1, 0, 1)), ((1, 1, 0), (-1, 0, 0)), ((1, 0, 1), (-1, 1, 1)))
RHS_TERMS = (((1, 0, 0), (1, 1, 1)), ((1, 0, 0),), ((1, 0, 1), (-1, 1, 1)), ((1, 1, 0), (-1, 0, 0)),
             ((1, 1, 1),), ((1, 0, 0), (1, 0, 1)), ((1, 1, 0), (1, 1, 1)))
TOP_ORDER = (1, 3, 0, 6, 4, 2, 5)


def _add(x, y):
    return [[lax.add(a, b) for a, b in zip(rx, ry)] for rx, ry in zip(x, y)]


def _sub(x, y):
    return [[lax.sub(a, b) for a, b in zip(rx, ry)] for rx, ry in zip(x, y)]


def _operand(terms, quadrant):
    total = None
    for sign, i, j in terms:
        q = quadrant(i, j)
        total = q if total is None else (_add if sign > 0 else _sub)(total, q)
    return total


def _operands(side, blocks):
    half = len(blocks) // 2
    if half == 0:
        return [blocks[0][0]]

    def quadrant(i, j):
        return [row[j * half:(j + 1) * half] for row in blocks[i * half:(i + 1) * half]]

    return [x for terms in side for x in _operands(side, _operand(terms, quadrant))]


def _multiply(product, emit, level=LEVELS, base=0):
    if level == 0:
        emit(0, 0, product(base))
        yield
        return
    n = 2 ** (level - 1)

    def m(i):
        out = [[None] * n for _ in range(n)]

        def keep(a, b, v):
            out[a][b] = v

        yield from _multiply(product, keep, level - 1, base + (i - 1) * 7 ** (level - 1))
        return out

    def put(x, oi, oj):
        for a in range(n):
            for b in range(n):
                emit(oi * n + a, oj * n + b, x[a][b])

    m2 = yield from m(2)
    m4 = yield from m(4)
    put(_add(m2, m4), 1, 0)
    m1 = yield from m(1)
    c11 = _add(m1, m4)
    c22 = _sub(m1, m2)
    m7 = yield from m(7)
    c11 = _add(c11, m7)
    m5 = yield from m(5)
    put(_sub(c11, m5), 0, 0)
    m3 = yield from m(3)
    put(_add(m3, m5), 0, 1)
    c22 = _add(c22, m3)
    m6 = yield from m(6)
    put(_add(c22, m6), 1, 1)


def _build_operands(side, load, store, hold, held=lambda n, a, b: (n, a, b) == (0, 1, 1), tops=range(7)):
    half = NS // 2
    for top in tops:
        terms = side[top]
        loaded = {(i, j): [[load(i * half + a, j * half + b, hold if held(n, a, b) else _same)
                            for b in range(half)] for a in range(half)]
                  for n, (_, i, j) in enumerate(terms)}
        lo, hi = (_operands(side, _operand(terms, lambda i, j: [[x[e] for x in row] for row in loaded[i, j]]))
                  for e in range(2))
        for p in range(NP // 7):
            store(top * (NP // 7) + p, _join(lo[p], hi[p]))
        yield


def _low(words):
    return pltpu.bitcast(lax.shift_left(words, np.uint32(16)), F32)


def _high(words):
    return pltpu.bitcast(lax.bitwise_and(words, np.uint32(0xFFFF0000)), F32)


def _split(words):
    return _low(words), _high(words)


def _join(lo, hi):
    return pltpu.bitcast(pltpu.pack_elementwise([lo, hi], packed_dtype=BF16), U32)


def _join_shuffled(v):
    r, c = v.shape
    v = v.reshape(r // 16, 2, 8, c)
    return _join(v[:, 0].reshape(r // 2, c), v[:, 1].reshape(r // 2, c))


def _split_shuffled(words):
    lo, hi = _split(words)
    r, c = words.shape
    return jnp.stack([lo.reshape(r // 8, 8, c), hi.reshape(r // 8, 8, c)], axis=1).reshape(2 * r, c)


def _unshuffle(pos):
    return (pos & ~15) + ((pos & 15) >> 1) + 8 * (pos & 1)


def _matrix(words):
    return pltpu.bitcast(words, BF16)


def _cat(xs, axis):
    return xs[0] if len(xs) == 1 else jnp.concatenate(xs, axis=axis)


def _ds(start, size):
    if isinstance(start, int):
        return pl.ds(start, size)
    return pl.ds(pl.multiple_of(start, min(size, 16)), size)


def _shifted(ref, step, steps, n):
    return ref.at[_ds(step * n, ref.shape[0] - (steps - 1) * n)]


def _loop(n, body):
    lax.fori_loop(0, n, lambda i, carry: body(i), None)


def _start(copies):
    for c in copies:
        c.start()


def _wait(copies):
    for c in copies:
        c.wait()


def _run(steps):
    for _ in steps:
        pass


def _chain(*streams):
    for steps in streams:
        yield from steps


def _weigh(steps, weight):
    for _ in steps:
        yield weight


def _merge(*streams):
    spans = [s[2:] if len(s) > 2 else (0.0, 1.0) for s in streams]
    done = [0.0] * len(streams)
    live = list(range(len(streams)))
    while live:
        i = min(live, key=lambda k: spans[k][0] + (spans[k][1] - spans[k][0]) * done[k] / streams[k][1])
        try:
            weight = next(streams[i][0])
        except StopIteration:
            live.remove(i)
            continue
        weight = 1 if weight is None else weight
        done[i] += weight
        yield weight


def _interleave(*streams):
    _run(_merge(*streams))


class _Pacer:
    def __init__(self, words):
        self.never = (words | 1) == 0
        self.marks = []

    def mark(self, v):
        self.marks.append({None: v})
        return v

    def after(self, lag):
        def hold(x):
            if len(self.marks) < lag:
                return x
            mark = self.marks[-lag]
            if x.dtype not in mark:
                mark[x.dtype] = pltpu.bitcast(mark[None][0:8, 0:LANES], x.dtype)
            return lax.select(self.never, mark[x.dtype], x)

        return hold


def _same(x):
    return x


def _reciprocal(x):
    r = pltpu.reciprocal(x, approx=True)
    return r * (2.0 - x * r)


def _kernel(ax_hbm, wqkv_hbm, awo_hbm, bx_hbm, c_hbm, wq_hbm, wuk_hbm, wuv_hbm, bwo_hbm, out_hbm,
            ax_raw, wqkv_raw, awo_raw, c_raw, bwo_raw,
            lx, lc, rq0, rq1, rk0, rk1, rv0, rv1, qs0, qs1, ks0, ks1, vs0, vs1,
            sq0, sq1, sk0, sk1, sv0, sv1, ctx, ro, lo, stage,
            sem_c, sem_x, sem_wo, sem_w, sem_a, sem_out):

    def out_copy(n):
        return pltpu.make_async_copy(
            stage.at[n % 2], out_hbm.at[_ds(n % NBLK * ROWS, ROWS), _ds((1 - n // NBLK) * DA, DA)], sem_out.at[n % 2])

    a_inputs = ([pltpu.make_async_copy(ax_hbm.bitcast(U32).at[:, pl.ds(j * LANES, LANES)], ax_raw.at[j], sem_a)
                 for j in range(DA // LANES)]
                + [pltpu.make_async_copy(awo_hbm.bitcast(U32).at[:, pl.ds(j * LANES, LANES)], awo_raw.at[j], sem_a)
                   for j in range(DA // LANES)]
                + [pltpu.make_async_copy(wqkv_hbm.bitcast(U32), wqkv_raw, sem_a)])

    wp = ks0

    def wp_rows(t, i, s, c):
        return _ds((((t * NS + i) * (WROWS // 16) + s // 16) * 8 + c) * 8, 8)

    def shuffle_columns(blk, t, hold, quarters=range(NS)):
        lane = lax.broadcasted_iota(I32, (8, LANES), 1)
        slot, chunk, low = lane >> 5, (lane & 31) >> 2, lane & 3
        head_of = _unshuffle(lane & 31)
        for s in range(0, WROWS, 16):
            for i in quarters:
                rows = _ds((i * KQ + (blk % NBLK) * WROWS + s) // 2, 8)
                moved = []
                for j in range(8):
                    c0 = t * DA + j * LANES
                    u = hold(pltpu.bitcast(wqkv_raw[rows, c0:c0 + LANES], I32))
                    moved.append(jnp.take_along_axis(u, low * 32 + 4 * ((chunk - j) & 7) + slot, axis=1))
                    if j % 4 == 3:
                        yield
                v = [moved[-c % 8] for c in range(8)]
                for bit in (1, 2, 4):
                    v = [jnp.where((chunk & bit) != 0, v[(c - bit) % 8], v[c]) for c in range(8)]
                for c in range(8):
                    source = slot * 32 + (((head_of >> 2) + c) & 7) * 4 + (head_of & 3)
                    wp[wp_rows(t, i, s, c), :] = pltpu.bitcast(jnp.take_along_axis(v[c], source, axis=1), U32)
                    if c % 4 == 3:
                        yield

    n_shuffle = (WROWS // 16) * NS * 4

    weights = ((rq0, rk0, rv0), (rq1, rk1, rv1))
    projected = ((qs0, ks0, vs0), (qs1, ks1, vs1))
    staged = ((sq0, sk0, sv0), (sq1, sk1, sv1))

    def weight_copies(par, grp, w):
        words = (wq_hbm, wuk_hbm, wuv_hbm)[w].bitcast(U32)
        n = words.shape[0]
        return [pltpu.make_async_copy(
            words.at[:, (HB // 2) * parity + grp * (GROUP // 2) + pair],
            staged[par][w].at[pl.ds((2 * pair + parity) * n, n)], sem_w.at[3 * par + w])
            for pair in range(GROUP // 2) for parity in range(2)]

    def group_copies(par, grp):
        return [c for w in range(3) for c in weight_copies(par, grp, w)]

    def c_copies(part):
        return [pltpu.make_async_copy(c_hbm.bitcast(U32).at[part], c_raw.at[:, pl.ds(part * PART // 2, PART // 2)],
                                      sem_c.at[part])]

    def x_copies(part):
        return [pltpu.make_async_copy(bx_hbm.at[part], bwo_raw.at[:, pl.ds(part * PART, PART)], sem_x.at[part])]

    def wo_copies(grp):
        rows = (slice(None), _ds(grp * (KO // NGROUP), KO // NGROUP))
        return [pltpu.make_async_copy(bwo_hbm.at[rows], bwo_raw.at[rows], sem_wo)]

    def build_weights(par, w, part, hold, tops=range(7)):
        n = (MB, DC, DC)[w] // 2
        rows = n // NS // GROUP
        src = _shifted(staged[par][w], part, GROUP, rows)
        for s in range(0, rows, 8):
            target = _ds(part * rows + s, 8)

            def load(i, j, hold):
                x, y = (src[pl.ds((2 * (j // 2) + e) * n + i * (n // NS) + s, 8), :] for e in range(2))
                return [(_low, _high)[j % 2](z) for z in (hold(x), y)]

            def store(p, words):
                weights[par][w][p, target, :] = words

            yield from _build_operands(RHS_TERMS, load, store, hold, tops=tops)

    def n_weights(w):
        return (MB, DC, DC)[w] // NS // GROUP // 16 * 7

    def build_group(par, part, hold, order=range(3)):
        return _chain(*[build_weights(par, w, part, hold) for w in order])

    n_group = sum(n_weights(w) for w in range(3))

    def build_activations(src, dst, part, hold, tops=range(7)):
        tiles = src.shape[2] // NS // LANES
        for t in range(tiles):
            for s in range(0, PART, 16):
                r = part * PART + s

                def load(i, j, hold):
                    c0 = (j * tiles + t) * LANES
                    if src.dtype == U32:
                        return _split(hold(src[i, pl.ds(r // 2, 8), c0:c0 + LANES]))
                    return _split(hold(pltpu.bitcast(src[i, pl.ds(r, 16), c0:c0 + LANES], U32)))

                def store(p, words):
                    dst[p, t, pl.ds(r // 2, 8), :] = words

                yield from _build_operands(LHS_TERMS, load, store, hold, tops=tops)

    def n_activations(width):
        return width // NS // LANES * (PART // 16) * 7

    def project(par, w, part, mark):
        lhs = lx if w == 0 else lc
        tiles = lhs.shape[1]
        dst = projected[par][w]
        dst = _shifted(dst, part, GROUP, dst.shape[0] // GROUP // GROUP)
        source = _ds(part * (PART // 2), PART // 2)
        pending = {}

        def product(p):
            x = _cat([_matrix(lhs[p, t, source, :]) for t in range(tiles)], 1)
            return mark(jnp.dot(x, _matrix(weights[par][w][p]), preferred_element_type=F32))

        def emit(i, j, v):
            if w < 2:
                dst[pl.ds((j * SEQ + i * PART) // 2, PART // 2), :] = (
                    pltpu.bitcast(v.astype(BF16), U32) if w else _join_shuffled(v * (DB ** -0.5 * LOG2E)))
            else:
                pending[i, j] = v.T
                if i % 2 == 1:
                    pair = [pending.pop((i - 1 + b, j)) for b in range(2)]
                    blocks = [[t[a * DB // 2:(a + 1) * DB // 2] for t in pair] for a in range(2)]
                    for p, x in enumerate(_operands(LHS_TERMS, blocks)):
                        dst[pl.ds(((j * NPAIR + i // 2) * 7 + p) * DB // 4, DB // 4), :] = _join_shuffled(x)

        return _weigh(_multiply(product, emit), tiles)

    n_project = NP * (MB + 2 * DC) // NS // LANES

    def attend(par, h, head_id, pacer, order, reach, fast, lag, bursts, score_weight, score_span, context_span):
        hold = pacer.after(lag)
        causal = (lax.broadcasted_iota(I32, (TILE, TILE), 0)
                  <= _unshuffle(lax.broadcasted_iota(I32, (TILE, TILE), 1)))
        queries, keys, values = (r.at[_ds(h * (r.shape[0] // GROUP), r.shape[0] // GROUP)] for r in projected[par])
        result = ctx.at[_ds(head_id * (SEQ // 2), SEQ // 2)]
        pending = {}

        def fold(op, t):
            return functools.reduce(op, [lax.slice(t, (r, 0), (r + 8, TILE)) for r in range(0, TILE, 8)])

        def scores(i):
            q = _matrix(queries[i * TILE // 2:(i + 1) * TILE // 2, :])
            tiles, peaks = [], []
            for j in range(i + 1):
                if j % reach == 0:
                    k = _matrix(keys[j * TILE // 2:min(j + reach, i + 1) * TILE // 2, :])
                    several = lax.dot_general(k, q, NT_DIMS, preferred_element_type=F32)
                s = pacer.mark(several[j % reach * TILE:(j % reach + 1) * TILE])
                if j == i:
                    s = jnp.where(causal, s, MASKED * LOG2E)
                tiles.append(s)
                peaks.append(fold(lax.max, s))
                yield score_weight
            top = jnp.max(functools.reduce(jnp.maximum, peaks), axis=0, keepdims=True)
            if i // 2 >= max(1, NPAIR - fast):
                mass = functools.reduce(jnp.add, [jnp.exp2(x - top) for x in peaks])
                top = top + jnp.log2(jnp.sum(mass, axis=0, keepdims=True))
            pending[i] = tiles, jnp.broadcast_to(top, (8, TILE))

        def context(i):
            both = [pending.pop(2 * i + c) for c in range(2)]
            totals = [None, None]
            o = [[None, None], [None, None]]

            def weight(j, c):
                p = jnp.exp2(both[c][0][j] - _cat([hold(both[c][1])] * (TILE // 8), 0))
                t = fold(lax.add, p)
                totals[c] = t if totals[c] is None else totals[c] + t
                return p

            def product(j, p, x):
                v = _matrix(values[(j * 7 + p) * DB // 4:(j * 7 + p + 1) * DB // 4, :])
                return pacer.mark(jnp.dot(v, x.astype(BF16), preferred_element_type=F32))

            def emit(a, c, v):
                o[a][c] = v if o[a][c] is None else o[a][c] + v

            def plain(j, c, tiles):
                for b in range(tiles):
                    p = weight(2 * j + b, c)
                    shared = product(j, 2 + b, p)
                    emit(b, c, shared)
                    emit(1 - b, c, shared + product(j, 5 + b, p))
                    yield 1

            yield from plain(i, 0, 1)
            yield from plain(i, 1, 2)
            acc = [None] * 7
            for j in range(i):
                if i < NPAIR - fast:
                    yield from plain(j, 0, 2)
                    yield from plain(j, 1, 2)
                    continue
                tiles = {}
                for burst in bursts:
                    for p in burst:
                        for _, b, c in RHS_TERMS[p]:
                            if (b, c) not in tiles:
                                tiles[b, c] = weight(2 * j + b, c)
                        t = product(j, p, _operand(RHS_TERMS[p], lambda b, c: [[tiles[b, c]]])[0][0])
                        acc[p] = t if acc[p] is None else acc[p] + t
                    yield 4 / 7 * len(burst)
            if acc[0] is not None:
                _run(_multiply(lambda p: acc[p], emit, 1))
            for c in range(2):
                x = _cat([o[0][c], o[1][c]], 0) * _reciprocal(jnp.sum(totals[c], axis=0, keepdims=True))
                result[(2 * i + c) * TILE // 2:(2 * i + c + 1) * TILE // 2, :] = pltpu.bitcast(x.astype(BF16).T, U32)

        for n in range(NPAIR + 1):
            streams = []
            if n < NPAIR:
                i = order[n]
                streams.append((_chain(scores(2 * i), scores(2 * i + 1)), (4 * i + 3) * score_weight, *score_span))
            if n > 0:
                i = order[n - 1]
                streams.append((context(i), 4 * i + 3, *context_span))
            yield from _merge(*streams)

    def n_attend(pace):
        return NPAIR * (2 * NPAIR + 1) * (1 + pace["score_weight"])

    def build_wo(head_id, hold):
        n = KO // HB
        src, dst = bwo_raw.at[:, _ds(head_id * n, n)], _shifted(ro, head_id, HB, n // 2)
        for ct in range(TPB):
            for s in range(0, n, 16):
                def load(i, j, hold):
                    c0 = (j * TPB + ct) * LANES
                    v = src[i, pl.ds(s, 16), c0:c0 + LANES].astype(F32)
                    return [hold(v[0:8]), hold(v[8:16])]

                def store(p, words):
                    dst[pl.ds(((p * TPB + ct) * KO + s) // 2, 8), :] = words

                yield from _build_operands(RHS_TERMS, load, store, hold)

    n_wo = TPB * (KO // HB // 16) * 7

    def head_step(par, g, h):
        pacer = _Pacer(lc[0, 0, 0:8, :])
        head_id = g * GROUP + h
        _interleave((attend(par, h, head_id, pacer, **HEAD), n_attend(HEAD), 0., .96),
                    (_chain(*[project(1 - par, w, h, pacer.mark) for w in (2, 1, 0)]), n_project),
                    (build_wo(head_id, pacer.after(2)), n_wo, .01, .1),
                    (build_group(par, h, pacer.after(5), (1, 2, 0)), n_group, .25, .98))

    def last_head_step(h):
        pacer = _Pacer(lc[0, 0, 0:8, :])
        hold = pacer.after(1)
        head_id = (NGROUP - 1) * GROUP + h
        _interleave((attend(1, h, head_id, pacer, **LAST_HEAD), n_attend(LAST_HEAD)),
                    (build_wo(head_id, hold), n_wo, .03, .3),
                    (_chain(*[shuffle_columns(0, t, hold, [h]) for t in range(3)]), 3 * n_shuffle / NS, .1, .8))

    def start_up():
        data = {"k": weight_copies(0, 0, 1), "v": weight_copies(0, 0, 2), "q": weight_copies(0, 0, 0),
                "g1": group_copies(1, 1), "g2": group_copies(0, 2), "o": wo_copies(0)}
        for part in range(GROUP):
            data["c%d" % part], data["x%d" % part] = c_copies(part), x_copies(part)
        built = set()

        def copies(names):
            return [c for name in names.split() for c in data[name]]

        def operands(job, hold, tops=range(7)):
            if job[0] in "!+":
                (_wait if job[0] == "!" else _start)(copies(job[1:]))
            elif job[0] in "cx":
                src, dst = (c_raw, lc) if job[0] == "c" else (bwo_raw, lx)
                yield from build_activations(src, dst, int(job[1]), hold, tops)
            else:
                for part in range(GROUP):
                    yield from (build_group(1, part, hold) if job == "g" else
                                build_weights(0, "qkv".index(job), part, hold, tops))
            built.add(job)

        size = dict(c=n_activations(DC), x=n_activations(MB), g=GROUP * n_group,
                    **{name: GROUP * n_weights(w) for w, name in enumerate("qkv")})

        def projection(name, mark):
            assert {name[0], "xcc"["qkv".index(name[0])] + name[1]} <= built
            yield from project(0, "qkv".index(name[0]), int(name[1]), mark)

        def step(waits, starts, products, ahead, jobs, lag, span):
            _wait(copies(waits))
            _start(copies(starts))
            pacer = _Pacer(c_raw[0, 0:8, 0:LANES])
            for top in TOP_ORDER:
                for job in ahead.split():
                    _run(operands(job, _same, [top]))
            _interleave((_chain(*[projection(name, pacer.mark) for name in products.split()]),
                         sum(n_project // (2 if name[0] == "q" else 4) for name in products.split())),
                        (_chain(*[operands(job, pacer.after(lag)) for job in jobs.split()]),
                         sum(size.get(job[0], 0) for job in jobs.split()) or 1, *span))

        def steps(i):
            for n, args in enumerate(START_UP):
                pl.when(i == n)(functools.partial(step, *args))

        _start(copies("c0 k v c1"))
        _loop(len(START_UP), steps)

    def group(par, g):
        _wait(wo_copies(g))
        _start(wo_copies(g + 1))
        pl.when(g + 2 < NGROUP)(lambda: _wait(group_copies(par, g + 2)))
        pl.when(g + 3 < NGROUP)(lambda: _start(group_copies(1 - par, g + 3)))
        if par == 0:
            pl.when(g == NGROUP - 2)(lambda: _start(a_inputs))
        _loop(GROUP, lambda h: head_step(par, g, h))

    def two_groups(t):
        group(0, 2 * t)
        pl.when(t < NGROUP // 2 - 1)(lambda: group(1, 2 * t + 1))

    start_up()
    _loop(NGROUP // 2, two_groups)
    _wait(wo_copies(NGROUP - 1) + a_inputs)
    _loop(GROUP, last_head_step)

    la, qa = lx, qs0

    def w_a(t, p, ct, r0, rows):
        if t == 0:
            return (rq0, rq1)[ct], (p, _ds(r0, rows))
        if t == 1:
            return lc, (p, 0, _ds(ct * (KQ // 2) + r0, rows))
        if t == 2:
            buf, tile = divmod(TPB * p + ct, 25)
            assert rows <= 64 or rows == 128
            if rows == 128:
                return (rk0, rk1, rv0, rv1)[buf], (pl.ds(2 * tile, 2),)
            return (rk0, rk1, rv0, rv1)[buf], (2 * tile + r0 // 64, _ds(r0 % 64, rows))
        buf, tile = divmod(TPB * p, 50)
        return (vs0, vs1)[buf], (_ds((tile + ct) * (KQ // 2) + r0, rows),)

    def load_w(t, p):
        tiles = []
        for ct in range(TPB):
            buf, idx = w_a(t, p, ct, 0, KQ // 2)
            tiles.append(_matrix(buf[idx].reshape(KQ // 2, LANES)))
        return _cat(tiles, 1)

    span_a = HALO + SEQ // 2
    group_rows = 16 * NS

    def build_w(blk, t, hold):
        for s in range(0, WROWS, 16):
            for ct in range(TPB):
                def load(i, j, hold):
                    return _split(hold(wp[wp_rows(t, i, s, j * TPB + ct), :]))

                def store(p, words):
                    buf, idx = w_a(t, p, ct, (blk * WROWS + s) // 2, 8)
                    buf[idx] = words

                yield from _build_operands(RHS_TERMS, load, store, hold, lambda *_: True)

    n_w = (WROWS // 16) * TPB * 7

    def build_x(blk, hold):
        for c in range(ROWS // group_rows):
            for t in range(TPB):
                def load(i, j, hold):
                    words = ax_raw.at[j * TPB + t, _ds(blk * (ROWS // 2), ROWS // 2)]
                    w0 = (c * group_rows + 32 * (i // 2)) // 2
                    return [(_low, _high)[i % 2](hold(words[pl.ds(w0 + e, 8, stride=2), :])) for e in range(2)]

                def store(p, words):
                    la[p, t, _ds((blk * (ROWS // NS) + 16 * c) // 2, 8), :] = words

                yield from _build_operands(LHS_TERMS, load, store, hold, lambda *_: True)

    n_x = (ROWS // group_rows) * TPB * 7

    def build_awo(blk, hold):
        ct, odd, h0 = blk // 4, (blk // 2) % 2, 16 * (blk % 2)
        pairs = DHA // 2 // NS
        for dp in range(0, pairs, 2):
            src = {}
            for i in range(NS):
                for j in range(NS):
                    words = awo_raw.at[j * TPB + ct, pl.ds(pl.multiple_of(h0 * 16, 256), 256)]
                    for e in range(2):
                        w0 = 8 * e * 16 + i * pairs + dp
                        src[i, j, e] = hold(jnp.where(odd == 1, words[pl.ds(w0 + 1, 8, stride=16), :],
                                                      words[pl.ds(w0, 8, stride=16), :]))
                yield
            for half in range(2):
                def load(i, j, hold):
                    return [(_low, _high)[half](hold(src[i, j, e])) for e in range(2)]

                def store(p, words):
                    buf, idx = w_a(3, p, ct, ((2 * (dp + odd) + half) * HA + h0) // 2, 8)
                    buf[idx] = words

                yield from _build_operands(RHS_TERMS, load, store, hold, lambda *_: True)

    n_awo = (DHA // 2 // NS // 2) * (NS + 2 * 7)

    def output_b(blk):
        slot = blk % 2
        rows = ROWS // NS
        heads = HB // NS
        pl.when(blk >= 2)(lambda: out_copy(blk - 2).wait())
        pacer = _Pacer(ro[0:8, :])
        src = _shifted(ctx, blk, NBLK, ROWS // 2)
        lhs = {}

        def build_lhs(top, hold):
            half = NS // 2
            for h in range(heads):
                for r in range(0, rows, 16):
                    def quadrant(i, j):
                        return [[_split_shuffled(hold(src[pl.ds(
                            (((j * half + b) * heads + h) * SEQ + (i * half + a) * rows + r) // 2, 8), :]))
                            for b in range(half)] for a in range(half)]

                    for p, v in enumerate(_operands(LHS_TERMS, _operand(LHS_TERMS[top], quadrant))):
                        lhs.setdefault((top * (NP // 7) + p, h), []).append(v)
                    yield

        def product(p):
            x = _cat([_cat(lhs[p, h], 0) for h in range(heads)], 1).astype(BF16)
            w = _cat([_matrix(ro[pl.ds((p * TPB + ct) * KO // 2, KO // 2), :]) for ct in range(TPB)], 1)
            return pacer.mark(jnp.dot(x, w, preferred_element_type=F32))

        def emit(i, j, v):
            stage[slot, i * rows:(i + 1) * rows, j * KQ:(j + 1) * KQ] = v.astype(BF16)

        _run(build_lhs(TOP_ORDER[0], _same))
        hold = pacer.after(1)
        _interleave(
            (_multiply(product, emit), NP),
            (_chain(*[build_lhs(t, hold) for t in TOP_ORDER[1:]]), 6 * heads * (rows // 16), 0., .84),
            *[(_chain(build_w(blk, t, hold), shuffle_columns(blk + 1, t, hold)), n_w + n_shuffle, .02, .95)
              for t in range(3)],
            (build_x(blk, hold), n_x, .02, .95),
            (build_awo(blk, hold), n_awo, .02, .95))
        out_copy(blk).start()

    _loop(NBLK, output_b)

    def project_a(t, blk, mark):
        rows = ROWS // NS
        dst = _shifted(ro if t == 1 else ctx, blk, NBLK, ROWS // 2)
        source, slot = _ds(blk * (rows // 2), rows // 2), blk % 2

        def product(p):
            x = _cat([_matrix(la[p, k, source, :]) for k in range(TPB)], 1)
            return mark(jnp.dot(x, load_w(t, p), preferred_element_type=F32))

        def emit(i, j, v):
            for ct in range(TPB):
                for c in range(rows // 16):
                    piece = v[16 * c:16 * (c + 1), ct * LANES:(ct + 1) * LANES]
                    tile = 2 * (j * TPB + ct) + i % 2
                    r = c * (group_rows // 2) + 16 * (i // 2)
                    if t == 0:
                        qa[_ds(slot * (ROWS // 2) + (tile * ROWS + r), 16), :] = pltpu.bitcast(piece, U32)
                    else:
                        dst[pl.ds(tile * span_a + HALO + r, 16), :] = pltpu.bitcast(piece, U32)

        return _multiply(product, emit)

    def attend_a(blk, hold, softmax_weight, operand_weight, hold_q, hold_v, **_):
        row0, slot, first = blk * (ROWS // 2), blk % 2, blk % SLOTS * NP
        keys, values = (_shifted(buf, blk, NBLK, ROWS // 2) for buf in (ro, ctx))
        logits, o = {}, {}

        def window(buf, j, r, par, w):
            return pltpu.bitcast(buf[pl.ds((2 * j + par) * span_a + HALO + r - w, 8), :], F32)

        def scores(r, par):
            pos = row0 + r + lax.broadcasted_iota(I32, (8, LANES), 0)
            q = [pltpu.bitcast(qa[_ds(slot * (ROWS // 2) + ((2 * j + par) * ROWS + r), 8), :], F32) for j in range(8)]
            q = [hold(x) if j % hold_q == 0 else x for j, x in enumerate(q)]
            logits[r, par] = []
            for w in range(WIN):
                acc = lax.mul(q[0], hold(window(keys, 0, r, par, w)))
                for j in range(1, 8):
                    acc = lax.add(acc, lax.mul(q[j], window(keys, j, r, par, w)))
                acc = acc + pltpu.roll(acc, 64, 1)
                acc = acc + pltpu.roll(acc, 32, 1)
                acc = acc * (DHA ** -0.5 * LOG2E)
                if r < w:
                    acc = jnp.where(pos >= w, acc, MASKED * LOG2E)
                logits[r, par].append(acc)
                yield

        def context(r, par):
            x = logits.pop((r, par))
            top = functools.reduce(jnp.maximum, x)
            e = [jnp.exp2(t - top) for t in x]
            scale = _reciprocal(functools.reduce(jnp.add, e))
            e = [t * scale for t in e]
            yield softmax_weight
            for j in range(8):
                acc = None
                for w in range(WIN):
                    v = window(values, j, r, par, w)
                    t = lax.mul(e[w], hold(v) if w % hold_v == 0 else v)
                    acc = t if acc is None else lax.add(acc, t)
                o[r, par, j] = acc
                yield

        def operands(c):
            for t in range(TPB):
                def load(i, j, hold):
                    return [hold(o[c * (group_rows // 2) + 8 * i, par, j * TPB + t]) for par in range(2)]

                def store(p, words):
                    lo[first + p, t, 8 * c:8 * (c + 1), :] = words

                yield from _weigh(_build_operands(LHS_TERMS, load, store, hold, lambda n, a, b: n == 0 and a == b),
                                  operand_weight)

        for c in range(ROWS // group_rows):
            units = [(r, par) for r in range(c * group_rows // 2, (c + 1) * group_rows // 2, 8) for par in range(2)]
            yield from scores(*units[0])
            for now, after in zip(units, units[1:]):
                yield from _merge((scores(*after), WIN), (context(*now), 8 + softmax_weight))
            yield from context(*units[-1])
            yield from operands(c)

    def output_a(blk, mark):
        slot, first = blk % 2, blk % SLOTS * NP

        def product(p):
            x = _cat([_matrix(lo[first + p, k]) for k in range(TPB)], 1)
            return mark(jnp.dot(x, load_w(3, p), preferred_element_type=F32))

        def emit(i, j, v):
            for c in range(ROWS // group_rows):
                r = c * group_rows + 16 * i
                stage[slot, r:r + 16, j * KQ:(j + 1) * KQ] = v[16 * c:16 * (c + 1)].astype(BF16)

        return _multiply(product, emit)

    def outputs_a(blocks, mark):
        for n, blk in enumerate(blocks):
            if n > 0:
                out_copy(NBLK + blk - 1).start()
                out_copy(NBLK + blk - 2).wait()
            yield from output_a(blk, mark)

    def step_a(project, attend, outputs, pace=None):
        pacer = _Pacer(lc[0, 0, 0:8, :])
        matmuls = [] if project is None else [project_a(t, project, pacer.mark) for t in (1, 2, 0)]
        streams = [(_chain(outputs_a(outputs, pacer.mark), *matmuls), (len(outputs) + len(matmuls)) * NP)]
        if pace:
            total = ((WIN + 8 + pace["softmax_weight"]) * (ROWS // 8)
                     + TPB * (ROWS // group_rows) * 7 * pace["operand_weight"])
            streams.append((attend_a(attend, pacer.after(pace["lag"]), **pace), total, *pace["span"]))
        if outputs:
            out_copy(NBLK + outputs[0] - 2).wait()
        _interleave(*streams)
        if outputs:
            out_copy(NBLK + outputs[-1]).start()

    for tile in range(16):
        for buf in (ro, ctx):
            buf[tile * span_a:tile * span_a + HALO, :] = jnp.zeros((HALO, LANES), U32)
    step_a(0, None, [])
    _loop(DELAY, lambda i: step_a(i + 1, i, [], A_FIRST))
    _loop(NBLK - 1 - DELAY, lambda i: step_a(i + DELAY + 1, i + DELAY, [i], A_MAIN))
    step_a(None, NBLK - 1, range(NBLK - 1 - DELAY, NBLK - 1), A_LAST)

    halves = [pltpu.make_async_copy(stage.at[1, :, pl.ds(c, DA // 2)],
                                    out_hbm.at[pl.ds(SEQ - ROWS, ROWS), pl.ds(c, DA // 2)], sem_out.at[1])
              for c in (0, DA // 2)]
    out_copy(2 * NBLK - 3).wait()
    for n, _ in enumerate(output_a(NBLK - 1, _same)):
        if n == 5 * NP // 7:
            halves[0].start()
    halves[1].start()
    _wait([out_copy(2 * NBLK - 2)] + halves)


def _words(*shape):
    return pltpu.VMEM(shape + (LANES,), U32)


SCRATCH = [
    _words(DA // LANES, SEQ // 2),
    pltpu.VMEM((DA // 2, 3 * DA), U32),
    _words(DA // LANES, DA // 2),
    pltpu.VMEM((NS, MQ // 2, DC), U32),
    pltpu.VMEM((NS, KO, MB), BF16),
    _words(NP, MB // NS // LANES, MQ // 2),
    _words(NP, DC // NS // LANES, MQ // 2),
    *[_words(NP, MB // NS // 2)] * 2,
    *[_words(NP + 1, DC // NS // 2)] * 4,
    *[_words(GROUP * SEQ // 2)] * 4,
    *[_words(GROUP * NPAIR * 7 * DB // 4)] * 2,
    *[_words(GROUP * MB // 2)] * 2,
    *[_words(GROUP * DC // 2)] * 4,
    _words(HB * SEQ // 2),
    _words(NP * TPB * KO // 2),
    _words(SLOTS * NP, TPB, ROWS // NS // 2),
    pltpu.VMEM((2, ROWS, DA), BF16),
    pltpu.SemaphoreType.DMA((GROUP,)),
    pltpu.SemaphoreType.DMA((GROUP,)),
    pltpu.SemaphoreType.DMA(()),
    pltpu.SemaphoreType.DMA((6,)),
    pltpu.SemaphoreType.DMA(()),
    pltpu.SemaphoreType.DMA((2,)),
]


@jax.jit
def pallas_concat_heads__sliding_local_dilated__compressed_kv_cla__prompt_kernel(A_x, A_wqkv, A_wo, B_x, B_c_kv, B_w_q, B_w_uk, B_w_uv, B_w_o):
    hbm = pl.BlockSpec(memory_space=pl.ANY)
    out = pl.pallas_call(
        _kernel,
        in_specs=[hbm] * 9,
        out_specs=hbm,
        out_shape=jax.ShapeDtypeStruct((SEQ, DA + MB), BF16),
        scratch_shapes=SCRATCH,
        compiler_params=pltpu.CompilerParams(vmem_limit_bytes=127 * 2 ** 20),
        name="fused_attention",
    )(A_x.reshape(SEQ, DA), A_wqkv, A_wo, B_x.reshape(GROUP, NS, PART, MB), B_c_kv.reshape(GROUP, NS, PART, DC),
      B_w_q.reshape(MB // 2, 2 * HB, DB), B_w_uk.reshape(DC // 2, 2 * HB, DB),
      B_w_uv.reshape(DC // 2, 2 * HB, DB), B_w_o.reshape(NS, KO, MB))
    return out.reshape(1, SEQ, DA + MB)
```

```python
import functools
import math

import jax
import jax.numpy as jnp
import numpy as np
from jax import lax
import jax.experimental.pallas as pl
import jax.experimental.pallas.tpu as pltpu

F32 = jnp.float32
BF16 = jnp.bfloat16
U32 = jnp.uint32
I32 = jnp.int32
LANES = 128
NT_DIMS = (((1,), (1,)), ((), ()))
LOG2E = math.log2(math.e)
MASKED = -1e9

SEQ = 2048
DA = 1024
HA, DHA = 32, 32
WIN = 8
HALO = 32
MB = 1024
HB, DB = 32, 128
DC = 512

LEVELS = 2
NS = 2 ** LEVELS
NP = 7 ** LEVELS
GROUP = NS
NGROUP = HB // GROUP
MQ = SEQ // NS
PART = MQ // GROUP
ROWS = 256
NBLK = SEQ // ROWS
KQ = DA // NS
TPB = KQ // LANES
KO = HB * DB // NS
WROWS = KQ // NBLK
TILE = LANES
NPAIR = SEQ // TILE // 2
DELAY = 2
SLOTS = 4

START_UP = (
    ("c0 k", "c2 c3", "k0", "c0 k", "", 1, (0., 1.)),
    ("v c1", "q x0", "v0", "v", "c1", 20, (.02, .98)),
    ("c2 c3", "x1 x2 x3", "k1 v1 k2 v2 k3", "", "c2 c3 !q +g1 q !x0 x0", 12, (.01, .96)),
    ("x1 x2", "", "q0 q1", "", "x1 x2", 1, (.01, .93)),
    ("x3 g1", "g2 o", "q2 v3 q3", "", "x3 g", 2, (0., 1.01)),
)
HEAD = dict(order=(7, 6, 4, 3, 5, 2, 1, 0), reach=2, fast=NPAIR, lag=10,
            bursts=((1,), (4,), (0,), (2,), (5,), (3,), (6,)),
            score_weight=.9, score_span=(0, .68), context_span=(.15, 1))
LAST_HEAD = dict(order=(1, 3, 5, 7, 6, 4, 2, 0), reach=1, fast=5, lag=11,
                 bursts=((1, 4), (0, 2), (5, 3), (6,)),
                 score_weight=1.1, score_span=(0, .6), context_span=(.25, 1))
A_FIRST = dict(lag=3, span=(.02, .98), softmax_weight=1, operand_weight=7, hold_q=8, hold_v=4)
A_MAIN = dict(lag=6, span=(.08, .985), softmax_weight=3, operand_weight=4, hold_q=2, hold_v=4)
A_LAST = dict(lag=2, span=(.02, 1.), softmax_weight=6, operand_weight=12, hold_q=1, hold_v=8)


LHS_TERMS = (((1, 0, 0), (1, 1, 1)), ((1, 1, 0), (1, 1, 1)), ((1, 0, 0),), ((1, 1, 1),),
             ((1, 0, 0), (1, 0, 1)), ((1, 1, 0), (-1, 0, 0)), ((1, 0, 1), (-1, 1, 1)))
RHS_TERMS = (((1, 0, 0), (1, 1, 1)), ((1, 0, 0),), ((1, 0, 1), (-1, 1, 1)), ((1, 1, 0), (-1, 0, 0)),
             ((1, 1, 1),), ((1, 0, 0), (1, 0, 1)), ((1, 1, 0), (1, 1, 1)))
TOP_ORDER = (1, 3, 0, 6, 4, 2, 5)


def _add(x, y):
    return [[lax.add(a, b) for a, b in zip(rx, ry)] for rx, ry in zip(x, y)]


def _sub(x, y):
    return [[lax.sub(a, b) for a, b in zip(rx, ry)] for rx, ry in zip(x, y)]


def _operand(terms, quadrant):
    total = None
    for sign, i, j in terms:
        q = quadrant(i, j)
        total = q if total is None else (_add if sign > 0 else _sub)(total, q)
    return total


def _operands(side, blocks):
    half = len(blocks) // 2
    if half == 0:
        return [blocks[0][0]]

    def quadrant(i, j):
        return [row[j * half:(j + 1) * half] for row in blocks[i * half:(i + 1) * half]]

    return [x for terms in side for x in _operands(side, _operand(terms, quadrant))]


def _multiply(product, emit, level=LEVELS, base=0):
    if level == 0:
        emit(0, 0, product(base))
        yield
        return
    n = 2 ** (level - 1)

    def m(i):
        out = [[None] * n for _ in range(n)]

        def keep(a, b, v):
            out[a][b] = v

        yield from _multiply(product, keep, level - 1, base + (i - 1) * 7 ** (level - 1))
        return out

    def put(x, oi, oj):
        for a in range(n):
            for b in range(n):
                emit(oi * n + a, oj * n + b, x[a][b])

    m2 = yield from m(2)
    m4 = yield from m(4)
    put(_add(m2, m4), 1, 0)
    m1 = yield from m(1)
    c11 = _add(m1, m4)
    c22 = _sub(m1, m2)
    m7 = yield from m(7)
    c11 = _add(c11, m7)
    m5 = yield from m(5)
    put(_sub(c11, m5), 0, 0)
    m3 = yield from m(3)
    put(_add(m3, m5), 0, 1)
    c22 = _add(c22, m3)
    m6 = yield from m(6)
    put(_add(c22, m6), 1, 1)


def _build_operands(side, load, store, hold, held=lambda n, a, b: (n, a, b) == (0, 1, 1), tops=range(7)):
    half = NS // 2
    for top in tops:
        terms = side[top]
        loaded = {(i, j): [[load(i * half + a, j * half + b, hold if held(n, a, b) else _same)
                            for b in range(half)] for a in range(half)]
                  for n, (_, i, j) in enumerate(terms)}
        lo, hi = (_operands(side, _operand(terms, lambda i, j: [[x[e] for x in row] for row in loaded[i, j]]))
                  for e in range(2))
        for p in range(NP // 7):
            store(top * (NP // 7) + p, _join(lo[p], hi[p]))
        yield


def _low(words):
    return pltpu.bitcast(lax.shift_left(words, np.uint32(16)), F32)


def _high(words):
    return pltpu.bitcast(lax.bitwise_and(words, np.uint32(0xFFFF0000)), F32)


def _split(words):
    return _low(words), _high(words)


def _join(lo, hi):
    return pltpu.bitcast(pltpu.pack_elementwise([lo, hi], packed_dtype=BF16), U32)


def _join_shuffled(v):
    r, c = v.shape
    v = v.reshape(r // 16, 2, 8, c)
    return _join(v[:, 0].reshape(r // 2, c), v[:, 1].reshape(r // 2, c))


def _split_shuffled(words):
    lo, hi = _split(words)
    r, c = words.shape
    return jnp.stack([lo.reshape(r // 8, 8, c), hi.reshape(r // 8, 8, c)], axis=1).reshape(2 * r, c)


def _unshuffle(pos):
    return (pos & ~15) + ((pos & 15) >> 1) + 8 * (pos & 1)


def _matrix(words):
    return pltpu.bitcast(words, BF16)


def _cat(xs, axis):
    return xs[0] if len(xs) == 1 else jnp.concatenate(xs, axis=axis)


def _ds(start, size):
    if isinstance(start, int):
        return pl.ds(start, size)
    return pl.ds(pl.multiple_of(start, min(size, 16)), size)


def _shifted(ref, step, steps, n):
    return ref.at[_ds(step * n, ref.shape[0] - (steps - 1) * n)]


def _loop(n, body):
    lax.fori_loop(0, n, lambda i, carry: body(i), None)


def _start(copies):
    for c in copies:
        c.start()


def _wait(copies):
    for c in copies:
        c.wait()


def _run(steps):
    for _ in steps:
        pass


def _chain(*streams):
    for steps in streams:
        yield from steps


def _weigh(steps, weight):
    for _ in steps:
        yield weight


def _merge(*streams):
    spans = [s[2:] if len(s) > 2 else (0.0, 1.0) for s in streams]
    done = [0.0] * len(streams)
    live = list(range(len(streams)))
    while live:
        i = min(live, key=lambda k: spans[k][0] + (spans[k][1] - spans[k][0]) * done[k] / streams[k][1])
        try:
            weight = next(streams[i][0])
        except StopIteration:
            live.remove(i)
            continue
        weight = 1 if weight is None else weight
        done[i] += weight
        yield weight


def _interleave(*streams):
    _run(_merge(*streams))


class _Pacer:
    def __init__(self, words):
        self.never = (words | 1) == 0
        self.marks = []

    def mark(self, v):
        self.marks.append({None: v})
        return v

    def after(self, lag):
        def hold(x):
            if len(self.marks) < lag:
                return x
            mark = self.marks[-lag]
            if x.dtype not in mark:
                mark[x.dtype] = pltpu.bitcast(mark[None][0:8, 0:LANES], x.dtype)
            return lax.select(self.never, mark[x.dtype], x)

        return hold


def _same(x):
    return x


def _reciprocal(x):
    r = pltpu.reciprocal(x, approx=True)
    return r * (2.0 - x * r)


def _kernel(ax_hbm, wqkv_hbm, awo_hbm, bx_hbm, c_hbm, wq_hbm, wuk_hbm, wuv_hbm, bwo_hbm, out_hbm,
            ax_raw, wqkv_raw, awo_raw, c_raw, bwo_raw,
            lx, lc, rq0, rq1, rk0, rk1, rv0, rv1, qs0, qs1, ks0, ks1, vs0, vs1,
            sq0, sq1, sk0, sk1, sv0, sv1, ctx, ro, lo, stage,
            sem_c, sem_x, sem_wo, sem_w, sem_a, sem_out):

    def out_copy(n):
        return pltpu.make_async_copy(
            stage.at[n % 2], out_hbm.at[_ds(n % NBLK * ROWS, ROWS), _ds((1 - n // NBLK) * DA, DA)], sem_out.at[n % 2])

    a_inputs = ([pltpu.make_async_copy(ax_hbm.bitcast(U32).at[:, pl.ds(j * LANES, LANES)], ax_raw.at[j], sem_a)
                 for j in range(DA // LANES)]
                + [pltpu.make_async_copy(awo_hbm.bitcast(U32).at[:, pl.ds(j * LANES, LANES)], awo_raw.at[j], sem_a)
                   for j in range(DA // LANES)]
                + [pltpu.make_async_copy(wqkv_hbm.bitcast(U32), wqkv_raw, sem_a)])

    wp = ks0

    def wp_rows(t, i, s, c):
        return _ds((((t * NS + i) * (WROWS // 16) + s // 16) * 8 + c) * 8, 8)

    def shuffle_columns(blk, t, hold, quarters=range(NS)):
        lane = lax.broadcasted_iota(I32, (8, LANES), 1)
        slot, chunk, low = lane >> 5, (lane & 31) >> 2, lane & 3
        head_of = _unshuffle(lane & 31)
        for s in range(0, WROWS, 16):
            for i in quarters:
                rows = _ds((i * KQ + (blk % NBLK) * WROWS + s) // 2, 8)
                moved = []
                for j in range(8):
                    c0 = t * DA + j * LANES
                    u = hold(pltpu.bitcast(wqkv_raw[rows, c0:c0 + LANES], I32))
                    moved.append(jnp.take_along_axis(u, low * 32 + 4 * ((chunk - j) & 7) + slot, axis=1))
                    if j % 4 == 3:
                        yield
                v = [moved[-c % 8] for c in range(8)]
                for bit in (1, 2, 4):
                    v = [jnp.where((chunk & bit) != 0, v[(c - bit) % 8], v[c]) for c in range(8)]
                for c in range(8):
                    source = slot * 32 + (((head_of >> 2) + c) & 7) * 4 + (head_of & 3)
                    wp[wp_rows(t, i, s, c), :] = pltpu.bitcast(jnp.take_along_axis(v[c], source, axis=1), U32)
                    if c % 4 == 3:
                        yield

    n_shuffle = (WROWS // 16) * NS * 4

    weights = ((rq0, rk0, rv0), (rq1, rk1, rv1))
    projected = ((qs0, ks0, vs0), (qs1, ks1, vs1))
    staged = ((sq0, sk0, sv0), (sq1, sk1, sv1))

    def weight_copies(par, grp, w):
        words = (wq_hbm, wuk_hbm, wuv_hbm)[w].bitcast(U32)
        n = words.shape[0]
        return [pltpu.make_async_copy(
            words.at[:, (HB // 2) * parity + grp * (GROUP // 2) + pair],
            staged[par][w].at[pl.ds((2 * pair + parity) * n, n)], sem_w.at[3 * par + w])
            for pair in range(GROUP // 2) for parity in range(2)]

    def group_copies(par, grp):
        return [c for w in range(3) for c in weight_copies(par, grp, w)]

    def c_copies(part):
        return [pltpu.make_async_copy(c_hbm.bitcast(U32).at[part], c_raw.at[:, pl.ds(part * PART // 2, PART // 2)],
                                      sem_c.at[part])]

    def x_copies(part):
        return [pltpu.make_async_copy(bx_hbm.at[part], bwo_raw.at[:, pl.ds(part * PART, PART)], sem_x.at[part])]

    def wo_copies(grp):
        rows = (slice(None), _ds(grp * (KO // NGROUP), KO // NGROUP))
        return [pltpu.make_async_copy(bwo_hbm.at[rows], bwo_raw.at[rows], sem_wo)]

    def build_weights(par, w, part, hold, tops=range(7)):
        n = (MB, DC, DC)[w] // 2
        rows = n // NS // GROUP
        src = _shifted(staged[par][w], part, GROUP, rows)
        for s in range(0, rows, 8):
            target = _ds(part * rows + s, 8)

            def load(i, j, hold):
                x, y = (src[pl.ds((2 * (j // 2) + e) * n + i * (n // NS) + s, 8), :] for e in range(2))
                return [(_low, _high)[j % 2](z) for z in (hold(x), y)]

            def store(p, words):
                weights[par][w][p, target, :] = words

            yield from _build_operands(RHS_TERMS, load, store, hold, tops=tops)

    def n_weights(w):
        return (MB, DC, DC)[w] // NS // GROUP // 16 * 7

    def build_group(par, part, hold, order=range(3)):
        return _chain(*[build_weights(par, w, part, hold) for w in order])

    n_group = sum(n_weights(w) for w in range(3))

    def build_activations(src, dst, part, hold, tops=range(7)):
        tiles = src.shape[2] // NS // LANES
        for t in range(tiles):
            for s in range(0, PART, 16):
                r = part * PART + s

                def load(i, j, hold):
                    c0 = (j * tiles + t) * LANES
                    if src.dtype == U32:
                        return _split(hold(src[i, pl.ds(r // 2, 8), c0:c0 + LANES]))
                    return _split(hold(pltpu.bitcast(src[i, pl.ds(r, 16), c0:c0 + LANES], U32)))

                def store(p, words):
                    dst[p, t, pl.ds(r // 2, 8), :] = words

                yield from _build_operands(LHS_TERMS, load, store, hold, tops=tops)

    def n_activations(width):
        return width // NS // LANES * (PART // 16) * 7

    def project(par, w, part, mark):
        lhs = lx if w == 0 else lc
        tiles = lhs.shape[1]
        dst = projected[par][w]
        dst = _shifted(dst, part, GROUP, dst.shape[0] // GROUP // GROUP)
        source = _ds(part * (PART // 2), PART // 2)
        pending = {}

        def product(p):
            x = _cat([_matrix(lhs[p, t, source, :]) for t in range(tiles)], 1)
            return mark(jnp.dot(x, _matrix(weights[par][w][p]), preferred_element_type=F32))

        def emit(i, j, v):
            if w < 2:
                dst[pl.ds((j * SEQ + i * PART) // 2, PART // 2), :] = (
                    pltpu.bitcast(v.astype(BF16), U32) if w else _join_shuffled(v * (DB ** -0.5 * LOG2E)))
            else:
                pending[i, j] = v.T
                if i % 2 == 1:
                    pair = [pending.pop((i - 1 + b, j)) for b in range(2)]
                    blocks = [[t[a * DB // 2:(a + 1) * DB // 2] for t in pair] for a in range(2)]
                    for p, x in enumerate(_operands(LHS_TERMS, blocks)):
                        dst[pl.ds(((j * NPAIR + i // 2) * 7 + p) * DB // 4, DB // 4), :] = _join_shuffled(x)

        return _weigh(_multiply(product, emit), tiles)

    n_project = NP * (MB + 2 * DC) // NS // LANES

    def attend(par, h, head_id, pacer, order, reach, fast, lag, bursts, score_weight, score_span, context_span):
        hold = pacer.after(lag)
        causal = (lax.broadcasted_iota(I32, (TILE, TILE), 0)
                  <= _unshuffle(lax.broadcasted_iota(I32, (TILE, TILE), 1)))
        queries, keys, values = (r.at[_ds(h * (r.shape[0] // GROUP), r.shape[0] // GROUP)] for r in projected[par])
        result = ctx.at[_ds(head_id * (SEQ // 2), SEQ // 2)]
        pending = {}

        def fold(op, t):
            return functools.reduce(op, [lax.slice(t, (r, 0), (r + 8, TILE)) for r in range(0, TILE, 8)])

        def scores(i):
            q = _matrix(queries[i * TILE // 2:(i + 1) * TILE // 2, :])
            tiles, peaks = [], []
            for j in range(i + 1):
                if j % reach == 0:
                    k = _matrix(keys[j * TILE // 2:min(j + reach, i + 1) * TILE // 2, :])
                    several = lax.dot_general(k, q, NT_DIMS, preferred_element_type=F32)
                s = pacer.mark(several[j % reach * TILE:(j % reach + 1) * TILE])
                if j == i:
                    s = jnp.where(causal, s, MASKED * LOG2E)
                tiles.append(s)
                peaks.append(fold(lax.max, s))
                yield score_weight
            top = jnp.max(functools.reduce(jnp.maximum, peaks), axis=0, keepdims=True)
            if i // 2 >= max(1, NPAIR - fast):
                mass = functools.reduce(jnp.add, [jnp.exp2(x - top) for x in peaks])
                top = top + jnp.log2(jnp.sum(mass, axis=0, keepdims=True))
            pending[i] = tiles, jnp.broadcast_to(top, (8, TILE))

        def context(i):
            both = [pending.pop(2 * i + c) for c in range(2)]
            totals = [None, None]
            o = [[None, None], [None, None]]

            def weight(j, c):
                p = jnp.exp2(both[c][0][j] - _cat([hold(both[c][1])] * (TILE // 8), 0))
                t = fold(lax.add, p)
                totals[c] = t if totals[c] is None else totals[c] + t
                return p

            def product(j, p, x):
                v = _matrix(values[(j * 7 + p) * DB // 4:(j * 7 + p + 1) * DB // 4, :])
                return pacer.mark(jnp.dot(v, x.astype(BF16), preferred_element_type=F32))

            def emit(a, c, v):
                o[a][c] = v if o[a][c] is None else o[a][c] + v

            def plain(j, c, tiles):
                for b in range(tiles):
                    p = weight(2 * j + b, c)
                    shared = product(j, 2 + b, p)
                    emit(b, c, shared)
                    emit(1 - b, c, shared + product(j, 5 + b, p))
                    yield 1

            yield from plain(i, 0, 1)
            yield from plain(i, 1, 2)
            acc = [None] * 7
            for j in range(i):
                if i < NPAIR - fast:
                    yield from plain(j, 0, 2)
                    yield from plain(j, 1, 2)
                    continue
                tiles = {}
                for burst in bursts:
                    for p in burst:
                        for _, b, c in RHS_TERMS[p]:
                            if (b, c) not in tiles:
                                tiles[b, c] = weight(2 * j + b, c)
                        t = product(j, p, _operand(RHS_TERMS[p], lambda b, c: [[tiles[b, c]]])[0][0])
                        acc[p] = t if acc[p] is None else acc[p] + t
                    yield 4 / 7 * len(burst)
            if acc[0] is not None:
                _run(_multiply(lambda p: acc[p], emit, 1))
            for c in range(2):
                x = _cat([o[0][c], o[1][c]], 0) * _reciprocal(jnp.sum(totals[c], axis=0, keepdims=True))
                result[(2 * i + c) * TILE // 2:(2 * i + c + 1) * TILE // 2, :] = pltpu.bitcast(x.astype(BF16).T, U32)

        for n in range(NPAIR + 1):
            streams = []
            if n < NPAIR:
                i = order[n]
                streams.append((_chain(scores(2 * i), scores(2 * i + 1)), (4 * i + 3) * score_weight, *score_span))
            if n > 0:
                i = order[n - 1]
                streams.append((context(i), 4 * i + 3, *context_span))
            yield from _merge(*streams)

    def n_attend(pace):
        return NPAIR * (2 * NPAIR + 1) * (1 + pace["score_weight"])

    def build_wo(head_id, hold):
        n = KO // HB
        src, dst = bwo_raw.at[:, _ds(head_id * n, n)], _shifted(ro, head_id, HB, n // 2)
        for ct in range(TPB):
            for s in range(0, n, 16):
                def load(i, j, hold):
                    c0 = (j * TPB + ct) * LANES
                    v = src[i, pl.ds(s, 16), c0:c0 + LANES].astype(F32)
                    return [hold(v[0:8]), hold(v[8:16])]

                def store(p, words):
                    dst[pl.ds(((p * TPB + ct) * KO + s) // 2, 8), :] = words

                yield from _build_operands(RHS_TERMS, load, store, hold)

    n_wo = TPB * (KO // HB // 16) * 7

    def head_step(par, g, h):
        pacer = _Pacer(lc[0, 0, 0:8, :])
        head_id = g * GROUP + h
        _interleave((attend(par, h, head_id, pacer, **HEAD), n_attend(HEAD), 0., .96),
                    (_chain(*[project(1 - par, w, h, pacer.mark) for w in (2, 1, 0)]), n_project),
                    (build_wo(head_id, pacer.after(2)), n_wo, .01, .1),
                    (build_group(par, h, pacer.after(5), (1, 2, 0)), n_group, .25, .98))

    def last_head_step(h):
        pacer = _Pacer(lc[0, 0, 0:8, :])
        hold = pacer.after(1)
        head_id = (NGROUP - 1) * GROUP + h
        _interleave((attend(1, h, head_id, pacer, **LAST_HEAD), n_attend(LAST_HEAD)),
                    (build_wo(head_id, hold), n_wo, .03, .3),
                    (_chain(*[shuffle_columns(0, t, hold, [h]) for t in range(3)]), 3 * n_shuffle / NS, .1, .8))

    def start_up():
        data = {"k": weight_copies(0, 0, 1), "v": weight_copies(0, 0, 2), "q": weight_copies(0, 0, 0),
                "g1": group_copies(1, 1), "g2": group_copies(0, 2), "o": wo_copies(0)}
        for part in range(GROUP):
            data["c%d" % part], data["x%d" % part] = c_copies(part), x_copies(part)
        built = set()

        def copies(names):
            return [c for name in names.split() for c in data[name]]

        def operands(job, hold, tops=range(7)):
            if job[0] in "!+":
                (_wait if job[0] == "!" else _start)(copies(job[1:]))
            elif job[0] in "cx":
                src, dst = (c_raw, lc) if job[0] == "c" else (bwo_raw, lx)
                yield from build_activations(src, dst, int(job[1]), hold, tops)
            else:
                for part in range(GROUP):
                    yield from (build_group(1, part, hold) if job == "g" else
                                build_weights(0, "qkv".index(job), part, hold, tops))
            built.add(job)

        size = dict(c=n_activations(DC), x=n_activations(MB), g=GROUP * n_group,
                    **{name: GROUP * n_weights(w) for w, name in enumerate("qkv")})

        def projection(name, mark):
            assert {name[0], "xcc"["qkv".index(name[0])] + name[1]} <= built
            yield from project(0, "qkv".index(name[0]), int(name[1]), mark)

        def step(waits, starts, products, ahead, jobs, lag, span):
            _wait(copies(waits))
            _start(copies(starts))
            pacer = _Pacer(c_raw[0, 0:8, 0:LANES])
            for top in TOP_ORDER:
                for job in ahead.split():
                    _run(operands(job, _same, [top]))
            _interleave((_chain(*[projection(name, pacer.mark) for name in products.split()]),
                         sum(n_project // (2 if name[0] == "q" else 4) for name in products.split())),
                        (_chain(*[operands(job, pacer.after(lag)) for job in jobs.split()]),
                         sum(size.get(job[0], 0) for job in jobs.split()) or 1, *span))

        def steps(i):
            for n, args in enumerate(START_UP):
                pl.when(i == n)(functools.partial(step, *args))

        _start(copies("c0 k v c1"))
        _loop(len(START_UP), steps)

    def group(par, g):
        _wait(wo_copies(g))
        _start(wo_copies(g + 1))
        pl.when(g + 2 < NGROUP)(lambda: _wait(group_copies(par, g + 2)))
        pl.when(g + 3 < NGROUP)(lambda: _start(group_copies(1 - par, g + 3)))
        if par == 0:
            pl.when(g == NGROUP - 2)(lambda: _start(a_inputs))
        _loop(GROUP, lambda h: head_step(par, g, h))

    def two_groups(t):
        group(0, 2 * t)
        pl.when(t < NGROUP // 2 - 1)(lambda: group(1, 2 * t + 1))

    start_up()
    _loop(NGROUP // 2, two_groups)
    _wait(wo_copies(NGROUP - 1) + a_inputs)
    _loop(GROUP, last_head_step)

    la, qa = lx, qs0

    def w_a(t, p, ct, r0, rows):
        if t == 0:
            return (rq0, rq1)[ct], (p, _ds(r0, rows))
        if t == 1:
            return lc, (p, 0, _ds(ct * (KQ // 2) + r0, rows))
        if t == 2:
            buf, tile = divmod(TPB * p + ct, 25)
            assert rows <= 64 or rows == 128
            if rows == 128:
                return (rk0, rk1, rv0, rv1)[buf], (pl.ds(2 * tile, 2),)
            return (rk0, rk1, rv0, rv1)[buf], (2 * tile + r0 // 64, _ds(r0 % 64, rows))
        buf, tile = divmod(TPB * p, 50)
        return (vs0, vs1)[buf], (_ds((tile + ct) * (KQ // 2) + r0, rows),)

    def load_w(t, p):
        tiles = []
        for ct in range(TPB):
            buf, idx = w_a(t, p, ct, 0, KQ // 2)
            tiles.append(_matrix(buf[idx].reshape(KQ // 2, LANES)))
        return _cat(tiles, 1)

    span_a = HALO + SEQ // 2
    group_rows = 16 * NS

    def build_w(blk, t, hold):
        for s in range(0, WROWS, 16):
            for ct in range(TPB):
                def load(i, j, hold):
                    return _split(hold(wp[wp_rows(t, i, s, j * TPB + ct), :]))

                def store(p, words):
                    buf, idx = w_a(t, p, ct, (blk * WROWS + s) // 2, 8)
                    buf[idx] = words

                yield from _build_operands(RHS_TERMS, load, store, hold, lambda *_: True)

    n_w = (WROWS // 16) * TPB * 7

    def build_x(blk, hold):
        for c in range(ROWS // group_rows):
            for t in range(TPB):
                def load(i, j, hold):
                    words = ax_raw.at[j * TPB + t, _ds(blk * (ROWS // 2), ROWS // 2)]
                    w0 = (c * group_rows + 32 * (i // 2)) // 2
                    return [(_low, _high)[i % 2](hold(words[pl.ds(w0 + e, 8, stride=2), :])) for e in range(2)]

                def store(p, words):
                    la[p, t, _ds((blk * (ROWS // NS) + 16 * c) // 2, 8), :] = words

                yield from _build_operands(LHS_TERMS, load, store, hold, lambda *_: True)

    n_x = (ROWS // group_rows) * TPB * 7

    def build_awo(blk, hold):
        ct, odd, h0 = blk // 4, (blk // 2) % 2, 16 * (blk % 2)
        pairs = DHA // 2 // NS
        for dp in range(0, pairs, 2):
            src = {}
            for i in range(NS):
                for j in range(NS):
                    words = awo_raw.at[j * TPB + ct, pl.ds(pl.multiple_of(h0 * 16, 256), 256)]
                    for e in range(2):
                        w0 = 8 * e * 16 + i * pairs + dp
                        src[i, j, e] = hold(jnp.where(odd == 1, words[pl.ds(w0 + 1, 8, stride=16), :],
                                                      words[pl.ds(w0, 8, stride=16), :]))
                yield
            for half in range(2):
                def load(i, j, hold):
                    return [(_low, _high)[half](hold(src[i, j, e])) for e in range(2)]

                def store(p, words):
                    buf, idx = w_a(3, p, ct, ((2 * (dp + odd) + half) * HA + h0) // 2, 8)
                    buf[idx] = words

                yield from _build_operands(RHS_TERMS, load, store, hold, lambda *_: True)

    n_awo = (DHA // 2 // NS // 2) * (NS + 2 * 7)

    def output_b(blk):
        slot = blk % 2
        rows = ROWS // NS
        heads = HB // NS
        pl.when(blk >= 2)(lambda: out_copy(blk - 2).wait())
        pacer = _Pacer(ro[0:8, :])
        src = _shifted(ctx, blk, NBLK, ROWS // 2)
        lhs = {}

        def build_lhs(top, hold):
            half = NS // 2
            for h in range(heads):
                for r in range(0, rows, 16):
                    def quadrant(i, j):
                        return [[_split_shuffled(hold(src[pl.ds(
                            (((j * half + b) * heads + h) * SEQ + (i * half + a) * rows + r) // 2, 8), :]))
                            for b in range(half)] for a in range(half)]

                    for p, v in enumerate(_operands(LHS_TERMS, _operand(LHS_TERMS[top], quadrant))):
                        lhs.setdefault((top * (NP // 7) + p, h), []).append(v)
                    yield

        def product(p):
            x = _cat([_cat(lhs[p, h], 0) for h in range(heads)], 1).astype(BF16)
            w = _cat([_matrix(ro[pl.ds((p * TPB + ct) * KO // 2, KO // 2), :]) for ct in range(TPB)], 1)
            return pacer.mark(jnp.dot(x, w, preferred_element_type=F32))

        def emit(i, j, v):
            stage[slot, i * rows:(i + 1) * rows, j * KQ:(j + 1) * KQ] = v.astype(BF16)

        _run(build_lhs(TOP_ORDER[0], _same))
        hold = pacer.after(1)
        _interleave(
            (_multiply(product, emit), NP),
            (_chain(*[build_lhs(t, hold) for t in TOP_ORDER[1:]]), 6 * heads * (rows // 16), 0., .84),
            *[(_chain(build_w(blk, t, hold), shuffle_columns(blk + 1, t, hold)), n_w + n_shuffle, .02, .95)
              for t in range(3)],
            (build_x(blk, hold), n_x, .02, .95),
            (build_awo(blk, hold), n_awo, .02, .95))
        out_copy(blk).start()

    _loop(NBLK, output_b)

    def project_a(t, blk, mark):
        rows = ROWS // NS
        dst = _shifted(ro if t == 1 else ctx, blk, NBLK, ROWS // 2)
        source, slot = _ds(blk * (rows // 2), rows // 2), blk % 2

        def product(p):
            x = _cat([_matrix(la[p, k, source, :]) for k in range(TPB)], 1)
            return mark(jnp.dot(x, load_w(t, p), preferred_element_type=F32))

        def emit(i, j, v):
            for ct in range(TPB):
                for c in range(rows // 16):
                    piece = v[16 * c:16 * (c + 1), ct * LANES:(ct + 1) * LANES]
                    tile = 2 * (j * TPB + ct) + i % 2
                    r = c * (group_rows // 2) + 16 * (i // 2)
                    if t == 0:
                        qa[_ds(slot * (ROWS // 2) + (tile * ROWS + r), 16), :] = pltpu.bitcast(piece, U32)
                    else:
                        dst[pl.ds(tile * span_a + HALO + r, 16), :] = pltpu.bitcast(piece, U32)

        return _multiply(product, emit)

    def attend_a(blk, hold, softmax_weight, operand_weight, hold_q, hold_v, **_):
        row0, slot, first = blk * (ROWS // 2), blk % 2, blk % SLOTS * NP
        keys, values = (_shifted(buf, blk, NBLK, ROWS // 2) for buf in (ro, ctx))
        logits, o = {}, {}

        def window(buf, j, r, par, w):
            return pltpu.bitcast(buf[pl.ds((2 * j + par) * span_a + HALO + r - w, 8), :], F32)

        def scores(r, par):
            pos = row0 + r + lax.broadcasted_iota(I32, (8, LANES), 0)
            q = [pltpu.bitcast(qa[_ds(slot * (ROWS // 2) + ((2 * j + par) * ROWS + r), 8), :], F32) for j in range(8)]
            q = [hold(x) if j % hold_q == 0 else x for j, x in enumerate(q)]
            logits[r, par] = []
            for w in range(WIN):
                acc = lax.mul(q[0], hold(window(keys, 0, r, par, w)))
                for j in range(1, 8):
                    acc = lax.add(acc, lax.mul(q[j], window(keys, j, r, par, w)))
                acc = acc + pltpu.roll(acc, 64, 1)
                acc = acc + pltpu.roll(acc, 32, 1)
                acc = acc * (DHA ** -0.5 * LOG2E)
                if r < w:
                    acc = jnp.where(pos >= w, acc, MASKED * LOG2E)
                logits[r, par].append(acc)
                yield

        def context(r, par):
            x = logits.pop((r, par))
            top = functools.reduce(jnp.maximum, x)
            e = [jnp.exp2(t - top) for t in x]
            scale = _reciprocal(functools.reduce(jnp.add, e))
            e = [t * scale for t in e]
            yield softmax_weight
            for j in range(8):
                acc = None
                for w in range(WIN):
                    v = window(values, j, r, par, w)
                    t = lax.mul(e[w], hold(v) if w % hold_v == 0 else v)
                    acc = t if acc is None else lax.add(acc, t)
                o[r, par, j] = acc
                yield

        def operands(c):
            for t in range(TPB):
                def load(i, j, hold):
                    return [hold(o[c * (group_rows // 2) + 8 * i, par, j * TPB + t]) for par in range(2)]

                def store(p, words):
                    lo[first + p, t, 8 * c:8 * (c + 1), :] = words

                yield from _weigh(_build_operands(LHS_TERMS, load, store, hold, lambda n, a, b: n == 0 and a == b),
                                  operand_weight)

        for c in range(ROWS // group_rows):
            units = [(r, par) for r in range(c * group_rows // 2, (c + 1) * group_rows // 2, 8) for par in range(2)]
            yield from scores(*units[0])
            for now, after in zip(units, units[1:]):
                yield from _merge((scores(*after), WIN), (context(*now), 8 + softmax_weight))
            yield from context(*units[-1])
            yield from operands(c)

    def output_a(blk, mark):
        slot, first = blk % 2, blk % SLOTS * NP

        def product(p):
            x = _cat([_matrix(lo[first + p, k]) for k in range(TPB)], 1)
            return mark(jnp.dot(x, load_w(3, p), preferred_element_type=F32))

        def emit(i, j, v):
            for c in range(ROWS // group_rows):
                r = c * group_rows + 16 * i
                stage[slot, r:r + 16, j * KQ:(j + 1) * KQ] = v[16 * c:16 * (c + 1)].astype(BF16)

        return _multiply(product, emit)

    def outputs_a(blocks, mark):
        for n, blk in enumerate(blocks):
            if n > 0:
                out_copy(NBLK + blk - 1).start()
                out_copy(NBLK + blk - 2).wait()
            yield from output_a(blk, mark)

    def step_a(project, attend, outputs, pace=None):
        pacer = _Pacer(lc[0, 0, 0:8, :])
        matmuls = [] if project is None else [project_a(t, project, pacer.mark) for t in (1, 2, 0)]
        streams = [(_chain(outputs_a(outputs, pacer.mark), *matmuls), (len(outputs) + len(matmuls)) * NP)]
        if pace:
            total = ((WIN + 8 + pace["softmax_weight"]) * (ROWS // 8)
                     + TPB * (ROWS // group_rows) * 7 * pace["operand_weight"])
            streams.append((attend_a(attend, pacer.after(pace["lag"]), **pace), total, *pace["span"]))
        if outputs:
            out_copy(NBLK + outputs[0] - 2).wait()
        _interleave(*streams)
        if outputs:
            out_copy(NBLK + outputs[-1]).start()

    for tile in range(16):
        for buf in (ro, ctx):
            buf[tile * span_a:tile * span_a + HALO, :] = jnp.zeros((HALO, LANES), U32)
    step_a(0, None, [])
    _loop(DELAY, lambda i: step_a(i + 1, i, [], A_FIRST))
    _loop(NBLK - 1 - DELAY, lambda i: step_a(i + DELAY + 1, i + DELAY, [i], A_MAIN))
    step_a(None, NBLK - 1, range(NBLK - 1 - DELAY, NBLK - 1), A_LAST)

    def part_copy(row, rows, col):
        return pltpu.make_async_copy(stage.at[1, pl.ds(row, rows), pl.ds(col, DA // 2)],
                                     out_hbm.at[pl.ds(SEQ - ROWS + row, rows), pl.ds(col, DA // 2)], sem_out.at[1])

    parts = {5 * NP // 7: [part_copy(0, ROWS, 0)]}
    for n in range(2):
        parts[(6 + n) * NP // 7] = [part_copy(r + n * group_rows // 2, group_rows // 2, DA // 2)
                                    for r in range(0, ROWS, group_rows)]
    out_copy(2 * NBLK - 3).wait()
    for n, _ in enumerate(output_a(NBLK - 1, _same)):
        _start(parts.get(n, []))
    _start(parts[NP])
    _wait([out_copy(2 * NBLK - 2)] + [c for copies in parts.values() for c in copies])


def _words(*shape):
    return pltpu.VMEM(shape + (LANES,), U32)


SCRATCH = [
    _words(DA // LANES, SEQ // 2),
    pltpu.VMEM((DA // 2, 3 * DA), U32),
    _words(DA // LANES, DA // 2),
    pltpu.VMEM((NS, MQ // 2, DC), U32),
    pltpu.VMEM((NS, KO, MB), BF16),
    _words(NP, MB // NS // LANES, MQ // 2),
    _words(NP, DC // NS // LANES, MQ // 2),
    *[_words(NP, MB // NS // 2)] * 2,
    *[_words(NP + 1, DC // NS // 2)] * 4,
    *[_words(GROUP * SEQ // 2)] * 4,
    *[_words(GROUP * NPAIR * 7 * DB // 4)] * 2,
    *[_words(GROUP * MB // 2)] * 2,
    *[_words(GROUP * DC // 2)] * 4,
    _words(HB * SEQ // 2),
    _words(NP * TPB * KO // 2),
    _words(SLOTS * NP, TPB, ROWS // NS // 2),
    pltpu.VMEM((2, ROWS, DA), BF16),
    pltpu.SemaphoreType.DMA((GROUP,)),
    pltpu.SemaphoreType.DMA((GROUP,)),
    pltpu.SemaphoreType.DMA(()),
    pltpu.SemaphoreType.DMA((6,)),
    pltpu.SemaphoreType.DMA(()),
    pltpu.SemaphoreType.DMA((2,)),
]


@jax.jit
def pallas_concat_heads__sliding_local_dilated__compressed_kv_cla__prompt_kernel(A_x, A_wqkv, A_wo, B_x, B_c_kv, B_w_q, B_w_uk, B_w_uv, B_w_o):
    hbm = pl.BlockSpec(memory_space=pl.ANY)
    out = pl.pallas_call(
        _kernel,
        in_specs=[hbm] * 9,
        out_specs=hbm,
        out_shape=jax.ShapeDtypeStruct((SEQ, DA + MB), BF16),
        scratch_shapes=SCRATCH,
        compiler_params=pltpu.CompilerParams(vmem_limit_bytes=127 * 2 ** 20),
        name="fused_attention",
    )(A_x.reshape(SEQ, DA), A_wqkv, A_wo, B_x.reshape(GROUP, NS, PART, MB), B_c_kv.reshape(GROUP, NS, PART, DC),
      B_w_q.reshape(MB // 2, 2 * HB, DB), B_w_uk.reshape(DC // 2, 2 * HB, DB),
      B_w_uv.reshape(DC // 2, 2 * HB, DB), B_w_o.reshape(NS, KO, MB))
    return out.reshape(1, SEQ, DA + MB)
```
